```python
import jax
import jax.numpy as jnp

def _softmax(x, axis=-1):
    return jax.nn.softmax(x, axis=axis)

def _gelu(x):
    return jax.nn.gelu(x, approximate=True)

def _silu(x):
    return jax.nn.silu(x)

def _sigmoid(x):
    return jax.nn.sigmoid(x)

def _layernorm(x, axis=-1, eps=1e-05):
    m = jnp.mean(x, axis=axis, keepdims=True)
    v = jnp.var(x, axis=axis, keepdims=True)
    return (x - m) / jnp.sqrt(v + eps)

def _scatter_add(tgt, idx, src, axis=0):
    return tgt.at[idx].add(src)

def _segment_sum(src, seg, n):
    return jax.ops.segment_sum(src, seg, n)

class _Rng:

    def __init__(self, key):
        self._k = key

    def _next(self):
        self._k, sub = jax.random.split(self._k)
        return sub

    def normal(self, shape):
        return jax.random.normal(self._next(), shape, dtype=jnp.bfloat16)

    def randint(self, lo, hi, shape):
        return jax.random.randint(self._next(), shape, lo, hi, dtype=jnp.int32)

    def uniform(self, shape, lo=0.0, hi=1.0):
        return jax.random.uniform(self._next(), shape, jnp.bfloat16, lo, hi)

    def permutation(self, n):
        return jax.random.permutation(self._next(), n)
kernel_name = 'adaLN_cond__ssm_conv_h3__glu_gated_bilinear__prompt'

def setup_inputs():
    _rng = _Rng(jax.random.key(int.from_bytes(__import__("os").urandom(4), "little")))
    _w = lambda a: (lambda t: t.astype(jnp.bfloat16) if jnp.issubdtype(t.dtype, jnp.floating) else t)(jnp.asarray(a))

    def _A_setup():
        B, S, D = (1, 2048, 640)
        ks = 4
        return {'q': _w((lambda *s: _rng.normal(s) * 0.05)(B, S, D)), 'k': _w((lambda *s: _rng.normal(s) * 0.05)(B, S, D)), 'v': _w((lambda *s: _rng.normal(s) * 0.05)(B, S, D)), 'shift_k': _w((lambda *s: _rng.normal(s) * 0.05)(D, ks) * 0.5), 'ssm_k': _w((lambda *s: _rng.normal(s) * 0.05)(D, S) * (1.0 / S ** 0.5)), 'ssm_D': _w((lambda *s: _rng.normal(s) * 0.05)(D))}
    _A_in = _A_setup()

    def _B_setup():
        B, S, D, F = (1, 2048, 640, 1536)
        return {'x': _w((lambda *s: _rng.normal(s) * 0.05)(B, S, D)), 'w_gate': _w((lambda *s: _rng.normal(s) * 0.05)(D, F) * D ** (-0.5)), 'w_up': _w((lambda *s: _rng.normal(s) * 0.05)(D, F) * D ** (-0.5)), 'w_down': _w((lambda *s: _rng.normal(s) * 0.05)(F, D) * F ** (-0.5))}
    _B_in = _B_setup()
    return {'A_q': _A_in['q'], 'A_k': _A_in['k'], 'A_v': _A_in['v'], 'A_shift_k': _A_in['shift_k'], 'A_ssm_k': _A_in['ssm_k'], 'A_ssm_D': _A_in['ssm_D'], 'B_x': _B_in['x'], 'B_w_gate': _B_in['w_gate'], 'B_w_up': _B_in['w_up'], 'B_w_down': _B_in['w_down'], 'c': _w((lambda *s: _rng.normal(s) * 0.05)(1, 640)), 'w_mod': _w((lambda *s: _rng.normal(s) * 0.05)(640, 6 * 640) * 640 ** (-0.5))}

def reference(A_q, A_k, A_v, A_shift_k, A_ssm_k, A_ssm_D, B_x, B_w_gate, B_w_up, B_w_down, c, w_mod):

    def _A_ref(q, k, v, shift_k, ssm_k, ssm_D):
        B, S, D = q.shape
        ks = shift_k.shape[-1]
        k_pad = jnp.pad(k, ((0, 0), (ks - 1, 0), (0, 0)))
        k_shift = jnp.zeros_like(k)
        for t in range(ks):
            k_shift = k_shift + k_pad[:, t:t + S, :] * shift_k[:, ks - 1 - t][None, None, :]
        kv = k_shift * v
        L = 2 * S
        kv_pad = jnp.pad(kv, ((0, 0), (0, S), (0, 0)))
        kf_pad = jnp.pad(ssm_k, ((0, 0), (0, S)))
        kv_f = (lambda x, axes=(-2, -1): jnp.fft.rfft2(x.astype(jnp.float32), axes=axes))(kv_pad[:, None, :, :], axes=(1, 2))
        kf_f = (lambda x, axes=(-2, -1): jnp.fft.rfft2(x.astype(jnp.float32), axes=axes))(kf_pad[:, None, :], axes=(1, 2))
        kf_f = (lambda x, *d: x.transpose(*d))(kf_f, 1, 2, 0)
        y_f = kv_f * kf_f[None, :, :, :]
        y = (lambda x, s, axes=(-2, -1): jnp.fft.irfft2(x, s=s, axes=axes).astype(jnp.bfloat16))(y_f, (1, L), axes=(1, 2))[:, 0, :S, :]
        y = y + kv * ssm_D[None, None, :]
        return q * y

    def _B_ref(x, w_gate, w_up, w_down):
        g = jnp.einsum('bsd,df->bsf', x, w_gate)
        u = jnp.einsum('bsd,df->bsf', x, w_up)
        h = g * u
        return jnp.einsum('bsf,fd->bsd', h, w_down)
    x = A_q
    mod = (_silu(c) @ w_mod).reshape(c.shape[0], 6, 1, -1)
    sa, ca, ga, sb, cb, gb = (mod[:, 0].copy(), mod[:, 1].copy(), mod[:, 2].copy(), mod[:, 3].copy(), mod[:, 4].copy(), mod[:, 5].copy())
    h = _layernorm(x, axis=-1) * (1 + ca) + sa
    x = x + ga * _A_ref(h, A_k, A_v, A_shift_k, A_ssm_k, A_ssm_D)
    h = _layernorm(x, axis=-1) * (1 + cb) + sb
    x = x + gb * _B_ref(h, B_w_gate, B_w_up, B_w_down)
    return x
```

```python
import functools

import numpy as np
import jax
import jax.numpy as jnp
from jax import lax
import jax.experimental.pallas as pl
import jax.experimental.pallas.tpu as pltpu

S = 2048
D = 640
F = 1536
KS = 4
LANES = 128
NT = D // LANES
C = 256
NC = S // C
H = C // 2
EPS = 1e-5
TM = 256
PAD = 8

f32 = jnp.float32
bf16 = jnp.bfloat16


def _dft_tables():
    n2 = 4 * C
    f = np.concatenate([np.arange(0, H, 2), np.arange(1, H, 2)])
    n = np.arange(C)
    ang = 2.0 * np.pi * (((2 * f[:, None] + 1) * n[None, :]) % n2) / n2
    fa = np.concatenate([np.cos(ang), -np.sin(ang)], 0)
    fb = fa * ((-1.0) ** n)[None, :]
    fk = np.concatenate([fa, fb], 0)
    fu = np.concatenate([fa[:, 0::2], fa[:, 1::2]], 1)
    g = fa.T / C
    gi = np.concatenate([g[0::2], g[1::2]], 0)
    return np.concatenate([fk, fu, gi], 0).astype(np.float32)


def _layernorm(x):
    m = jnp.mean(x, axis=-1, keepdims=True)
    xc = x - m
    v = jnp.mean(xc * xc, axis=-1, keepdims=True)
    return xc * lax.rsqrt(v + EPS)


def _kernel(q_hbm, k_hbm, v_hbm, sk_hbm, ssm_hbm, sd_hbm, wg_hbm, wu_hbm, wd_hbm,
            c_hbm, wm_hbm, tab_hbm, o_hbm,
            qb, kb, vb, skb, ssmb, sdb, wgb, wub, wdb, cb_, wmb, tab,
            kf, kvf, ub, kpb, yb, prm, ob, sem, osem):
    def cp(src, dst, i):
        return pltpu.make_async_copy(src, dst, sem.at[i])

    c_tab = cp(tab_hbm, tab, 0)
    c_sk = cp(sk_hbm, skb, 1)
    c_sd = cp(sd_hbm, sdb, 2)
    c_c = cp(c_hbm, cb_, 3)

    def c_ssm(j):
        return cp(ssm_hbm.at[pl.ds(j * LANES, LANES), :], ssmb.at[j], 4 + j)

    def c_k(j):
        return cp(k_hbm.at[0, :, pl.ds(j * LANES, LANES)], kb.at[j], 9 + j)

    def c_v(j):
        return cp(v_hbm.at[0, :, pl.ds(j * LANES, LANES)], vb.at[j], 14 + j)

    c_wm = cp(wm_hbm, wmb, 19)
    c_q = cp(q_hbm.at[0], qb, 20)
    c_wg = cp(wg_hbm, wgb, 21)
    c_wu = cp(wu_hbm, wub, 22)
    c_wd = cp(wd_hbm, wdb, 23)

    for x in (c_tab, c_sk, c_sd, c_c):
        x.start()
    for j in range(NT):
        c_ssm(j).start()
        c_k(j).start()
        c_v(j).start()
    for x in (c_wm, c_q, c_wg, c_wu, c_wd):
        x.start()

    for x in (c_tab, c_sk, c_sd, c_c):
        x.wait()

    sel = (lax.broadcasted_iota(jnp.int32, (16, KS), 0)
           == lax.broadcasted_iota(jnp.int32, (16, KS), 1)).astype(bf16)
    skt = lax.dot_general(sel, skb[...], (((1,), (1,)), ((), ())),
                          preferred_element_type=f32)
    sdv = sdb[...].astype(f32).reshape(1, D)
    for j in range(NT):
        prm[j, 0:KS, :] = skt[0:KS, j * LANES:(j + 1) * LANES]
        prm[j, KS:KS + 1, :] = sdv[:, j * LANES:(j + 1) * LANES]
    kf[0:PAD, :] = jnp.zeros((PAD, LANES), f32)

    def conv_tile(j, carry):
        c_ssm(j).wait()
        c_k(j).wait()
        c_v(j).wait()
        w = [prm[j, t:t + 1, :] for t in range(KS)]
        dvec = prm[j, KS:KS + 1, :]
        kprev = None
        for a in range(NC):
            r0 = a * C
            kf[PAD + r0:PAD + r0 + C, :] = kb[j, r0:r0 + C, :].astype(f32)
            ks = kf[PAD + r0:PAD + r0 + C, :] * w[0]
            for t in range(1, KS):
                ks = ks + kf[PAD + r0 - t:PAD + r0 - t + C, :] * w[t]
            kvf[r0:r0 + C, :] = ks * vb[j, r0:r0 + C, :].astype(f32)
            e = kvf[pl.ds(r0, H, stride=2), :].astype(bf16)
            o = kvf[pl.ds(r0 + 1, H, stride=2), :].astype(bf16)
            ee = jnp.dot(tab[2 * C:3 * C, 0:H], e, preferred_element_type=f32)
            oo = jnp.dot(tab[2 * C:3 * C, H:C], o, preferred_element_type=f32)
            ub[a, 0:C, :] = ee + oo
            ub[a, C:2 * C, :] = ee - oo
            kr = lax.dot_general(tab[0:2 * C, :], ssmb[j, :, r0:r0 + C],
                                 (((1,), (1,)), ((), ())), preferred_element_type=f32)
            hh = H // 2
            for b in range(2):
                re = kr[b * C:b * C + H]
                im = kr[b * C + H:(b + 1) * C]
                if kprev is None:
                    kpb[a, b * C:b * C + H, :] = re + dvec
                    kpb[a, b * C + H:(b + 1) * C, :] = im
                else:
                    pre = kprev[b * C:b * C + H]
                    pim = kprev[b * C + H:(b + 1) * C]
                    kpb[a, b * C:b * C + hh, :] = re[:hh] - pim[:hh]
                    kpb[a, b * C + hh:b * C + H, :] = re[hh:] + pim[hh:]
                    kpb[a, b * C + H:b * C + H + hh, :] = im[:hh] + pre[:hh]
                    kpb[a, b * C + H + hh:(b + 1) * C, :] = im[hh:] - pre[hh:]
            kprev = kr
            R = 16
            pre_l, pim_l, qre_l, qim_l = [], [], [], []
            for r in range(0, H, R):
                acc = []
                for b in range(2):
                    yre = yim = None
                    for m in range(a + 1):
                        ure = ub[a - m, b * C + r:b * C + r + R, :]
                        uim = ub[a - m, b * C + H + r:b * C + H + r + R, :]
                        kre = kpb[m, b * C + r:b * C + r + R, :]
                        kim = kpb[m, b * C + H + r:b * C + H + r + R, :]
                        tre = kre * ure - kim * uim
                        tim = kre * uim + kim * ure
                        yre = tre if yre is None else yre + tre
                        yim = tim if yim is None else yim + tim
                    acc.append((yre, yim))
                (are, aim), (bre, bim) = acc
                pre_l.append((are + bre).astype(bf16))
                pim_l.append((aim + bim).astype(bf16))
                qre_l.append((are - bre).astype(bf16))
                qim_l.append((aim - bim).astype(bf16))
            p = jnp.concatenate(pre_l + pim_l, axis=0)
            qq = jnp.concatenate(qre_l + qim_l, axis=0)
            ye = jnp.dot(tab[3 * C:3 * C + H, :], p, preferred_element_type=f32)
            yo = jnp.dot(tab[3 * C + H:4 * C, :], qq, preferred_element_type=f32)
            yb[j, pl.ds(r0, H, stride=2), :] = ye
            yb[j, pl.ds(r0 + 1, H, stride=2), :] = yo
        return carry

    lax.fori_loop(0, NT, conv_tile, 0)

    c_wm.wait()
    cv = cb_[...].astype(f32)
    cs = (cv * jax.nn.sigmoid(cv)).astype(bf16)
    mod = jnp.dot(jnp.broadcast_to(cs, (16, D)), wmb[...], preferred_element_type=f32)[0:1]
    sa, ca, ga, sb, cb, gb = [mod[:, i * D:(i + 1) * D] for i in range(6)]
    a1 = ga * (1.0 + ca)
    b1 = ga * sa
    a2 = 1.0 + cb

    c_q.wait()
    c_wg.wait()
    c_wu.wait()
    c_wd.wait()

    def o_cp(i):
        return pltpu.make_async_copy(ob.at[pl.ds(i * TM, TM), :],
                                     o_hbm.at[0, pl.ds(i * TM, TM), :], osem.at[i])

    def ffn_block(i, carry):
        r0 = pl.multiple_of(i * TM, TM)
        x = qb[pl.ds(r0, TM), :].astype(f32)
        y = jnp.concatenate([yb[j, pl.ds(r0, TM), :] for j in range(NT)], axis=1)
        x1 = x + (_layernorm(x) * a1 + b1) * y
        h2 = (_layernorm(x1) * a2 + sb).astype(bf16)
        g = jnp.dot(h2, wgb[...], preferred_element_type=f32)
        u = jnp.dot(h2, wub[...], preferred_element_type=f32)
        hh = (g * u).astype(bf16)
        o = jnp.dot(hh, wdb[...], preferred_element_type=f32)
        ob[pl.ds(r0, TM), :] = (x1 + gb * o).astype(bf16)
        o_cp(i).start()
        return carry

    lax.fori_loop(0, S // TM, ffn_block, 0)
    for i in range(S // TM):
        o_cp(i).wait()


@jax.jit
def pallas_adaLN_cond__ssm_conv_h3__glu_gated_bilinear__prompt_kernel(
    A_q: jax.Array,
    A_k: jax.Array,
    A_v: jax.Array,
    A_shift_k: jax.Array,
    A_ssm_k: jax.Array,
    A_ssm_D: jax.Array,
    B_x: jax.Array,
    B_w_gate: jax.Array,
    B_w_up: jax.Array,
    B_w_down: jax.Array,
    c: jax.Array,
    w_mod: jax.Array,
):
    del B_x
    tab = jnp.asarray(_dft_tables(), dtype=bf16)
    any_spec = pl.BlockSpec(memory_space=pl.ANY)
    return pl.pallas_call(
        _kernel,
        in_specs=[any_spec] * 12,
        out_specs=any_spec,
        out_shape=jax.ShapeDtypeStruct((1, S, D), bf16),
        scratch_shapes=[
            pltpu.VMEM((S, D), bf16),
            pltpu.VMEM((NT, S, LANES), bf16),
            pltpu.VMEM((NT, S, LANES), bf16),
            pltpu.VMEM((D, KS), bf16),
            pltpu.VMEM((NT, LANES, S), bf16),
            pltpu.VMEM((D,), bf16),
            pltpu.VMEM((D, F), bf16),
            pltpu.VMEM((D, F), bf16),
            pltpu.VMEM((F, D), bf16),
            pltpu.VMEM((1, D), bf16),
            pltpu.VMEM((D, 6 * D), bf16),
            pltpu.VMEM((4 * C, C), bf16),
            pltpu.VMEM((PAD + S, LANES), f32),
            pltpu.VMEM((S, LANES), f32),
            pltpu.VMEM((NC, 2 * C, LANES), f32),
            pltpu.VMEM((NC, 2 * C, LANES), f32),
            pltpu.VMEM((NT, S, LANES), f32),
            pltpu.VMEM((NT, 8, LANES), f32),
            pltpu.VMEM((S, D), bf16),
            pltpu.SemaphoreType.DMA((24,)),
            pltpu.SemaphoreType.DMA((S // TM,)),
        ],
        compiler_params=pltpu.CompilerParams(vmem_limit_bytes=100 * 1024 * 1024),
        name="adaln_h3_glu",
    )(A_q, A_k, A_v, A_shift_k, A_ssm_k, A_ssm_D, B_w_gate, B_w_up, B_w_down, c, w_mod, tab)
```

```python
import numpy as np
import jax
import jax.numpy as jnp
from jax import lax
import jax.experimental.pallas as pl
import jax.experimental.pallas.tpu as pltpu

S = 2048
D = 640
F = 1536
KS = 4
L = 128
NT = D // L
R = 4
C = R * L
NC = S // C
EPS = 1e-5
PAD = 8
KVR = 64
PR = 32
TM0 = 512
TM = 256
NB = (S - TM0) // TM
TF = 256
WP = (0, 256, 768, 1536)

f32 = jnp.float32
bf16 = jnp.bfloat16


def _dft_tables():
    n2 = 4 * C
    g = np.arange(L)
    j = np.arange(L)
    ts, gs = [], []
    for r in range(R):
        ang = 2.0 * np.pi * (((4 * g[:, None] + 1) * (R * j[None, :] + r)) % n2) / n2
        t = np.stack([np.cos(ang).reshape(16, 8, L), -np.sin(ang).reshape(16, 8, L)], 1)
        t = t.reshape(2 * L, L)
        ts.append(t)
        gt = t.T / C
        gs += [gt[:, :L], gt[:, L:]]
    return np.concatenate(ts + gs, 0).astype(np.float32)


def _layernorm(x):
    m = jnp.mean(x, axis=-1, keepdims=True)
    xc = x - m
    v = jnp.mean(xc * xc, axis=-1, keepdims=True)
    return xc * lax.rsqrt(v + EPS)


def _split(t):
    t = t.reshape(16, 16, L)
    return t[:, :8, :], t[:, 8:, :]


def _radix4(x, sgn):
    (ar, ai), (br, bi), (cr, ci), (dr, di) = x
    s0r, s0i, d0r, d0i = ar + cr, ai + ci, ar - cr, ai - ci
    s1r, s1i, d1r, d1i = br + dr, bi + di, br - dr, bi - di
    o0 = (s0r + s1r, s0i + s1i)
    o2 = (s0r - s1r, s0i - s1i)
    pl_ = (d0r - d1i, d0i + d1r)
    mi_ = (d0r + d1i, d0i - d1r)
    return [o0, pl_, o2, mi_] if sgn > 0 else [o0, mi_, o2, pl_]


def _schedule():
    z = lambda j: [("z", j, a) for a in range(NC)]
    k = lambda j: [("k", j, a) for a in range(NC)]
    u = lambda j: [("u", j, a) for a in range(NC)]
    iv = lambda j: [("i", j, a) for a in range(NC)]
    kv = lambda j: [("kv", j, p) for p in range(S // KVR)]
    m = lambda j: [("mac", j, i, q) for i in range(16) for q in range(R)]
    bl = [(["ssm0", "tabT"], z(0) + k(0), []),
          (["k0", "v0"], u(0), kv(0))]
    for j in range(NT):
        n = j + 1
        if n < NT:
            bl.append(([f"ssm{n}"], z(n) + k(n), m(j)))
            bl.append(([f"k{n}", f"v{n}"] + (["tabG"] if j == 0 else []), iv(j) + u(n), kv(n)))
        else:
            bl.append((["wmA"], [("modA",)], m(j)))
            bl.append((["wmB"], iv(j) + [("modB",)], []))
    return bl


DMA_ORDER = (["sk", "sd", "c", "ssm0", "tabT", "k0", "v0", "ssm1", "k1", "v1", "tabG",
              "ssm2", "k2", "v2", "ssm3", "k3", "v3", "ssm4", "k4", "v4", "wmA", "wmB", "q0",
              "wg0", "wu0", "wg1", "wu1", "wg2", "wu2", "wd", "wmC", "q1", "q2"])


def _kernel(q_hbm, k_hbm, v_hbm, sk_hbm, ssm_hbm, sd_hbm, wg_hbm, wu_hbm, wd_hbm,
            c_hbm, wm_hbm, tab_hbm, o_hbm,
            qb, kb, vb, skb, ssmb, sdb, wgb, wub, wdb, cb_, wmb, tab,
            kf, kvf, ub0, ub1, kpb0, kpb1, pb0, pb1, yb, x1b, h2b, ob, sem, osem):
    cps = {"sk": (sk_hbm, skb), "sd": (sd_hbm, sdb), "c": (c_hbm, cb_), "wd": (wd_hbm, wdb),
           "tabT": (tab_hbm.at[pl.ds(0, 8 * L), :], tab.at[pl.ds(0, 8 * L), :]),
           "tabG": (tab_hbm.at[pl.ds(8 * L, 8 * L), :], tab.at[pl.ds(8 * L, 8 * L), :])}
    for j in range(NT):
        cps[f"ssm{j}"] = (ssm_hbm.at[pl.ds(j * L, L), :], ssmb.at[j])
        cps[f"k{j}"] = (k_hbm.at[0, :, pl.ds(j * L, L)], kb.at[j])
        cps[f"v{j}"] = (v_hbm.at[0, :, pl.ds(j * L, L)], vb.at[j])
    for n, (c0, c1) in (("wmA", (0, 3 * D)), ("wmB", (3 * D, 5 * D)), ("wmC", (5 * D, 6 * D))):
        cps[n] = (wm_hbm.at[:, pl.ds(c0, c1 - c0)], wmb.at[:, pl.ds(c0, c1 - c0)])
    for n, (r0, r1) in (("q0", (0, TM0)), ("q1", (TM0, TM0 + TM)), ("q2", (TM0 + TM, S))):
        cps[n] = (q_hbm.at[0, pl.ds(r0, r1 - r0), :], qb.at[pl.ds(r0, r1 - r0), :])
    for p in range(len(WP) - 1):
        cols = pl.ds(WP[p], WP[p + 1] - WP[p])
        cps[f"wg{p}"] = (wg_hbm.at[:, cols], wgb.at[:, cols])
        cps[f"wu{p}"] = (wu_hbm.at[:, cols], wub.at[:, cols])
    assert sorted(cps) == sorted(DMA_ORDER)

    def cp(name):
        src, dst = cps[name]
        return pltpu.make_async_copy(src, dst, sem.at[DMA_ORDER.index(name)])

    def wait(*names):
        for n in names:
            cp(n).wait()

    for n in DMA_ORDER:
        cp(n).start()

    kf[0:PAD, :] = jnp.zeros((PAD, L), f32)
    ri = lax.broadcasted_iota(jnp.int32, (L, L), 0)
    ci = lax.broadcasted_iota(jnp.int32, (L, L), 1)
    sel = jnp.where(ci == R * (ri % 32) + ri // 32, 1.0, 0.0).astype(bf16)

    wait("sk", "sd", "c")
    skt = skb[...].astype(f32)
    sdv = sdb[...].astype(f32).reshape(1, D)
    cv = cb_[...].astype(f32)
    sig = jax.nn.sigmoid(cv)
    cs = jnp.broadcast_to((cv * sig).astype(bf16), (16, D))
    never = jnp.broadcast_to(sig[:, 0:L], (8, L)) > 2.0

    def gate(x, dep):
        if dep is None:
            return x
        return jnp.where(never, dep, jnp.broadcast_to(x, (8, L)))

    def put(dst, a, xs):
        for qi in range(R):
            dst[a, qi, :, 0:8, :] = xs[qi][0]
            dst[a, qi, :, 8:16, :] = xs[qi][1]

    ubs, kpbs, pbs = (ub0, ub1), (kpb0, kpb1), (pb0, pb1)
    zs = {}
    mod = {}

    def grp_z(j, a):
        z = [lax.dot_general(sel, ssmb[j, :, t * L:(t + 1) * L], (((1,), (1,)), ((), ())),
                             preferred_element_type=f32) for t in range(R * a, R * a + R)]
        zs[j, a] = [jnp.concatenate([z[p][32 * r:32 * (r + 1)] for p in range(R)],
                                    axis=0).astype(bf16) for r in range(R)]
        return [z[0][16 * t:16 * t + 8] for t in range(8)]

    def grp_fwd(ws, dst, a, dvec=None):
        t = [jnp.dot(tab[2 * L * r:2 * L * (r + 1), :], ws[r], preferred_element_type=f32)
             for r in range(R)]
        x = [_split(v) for v in t]
        if dvec is not None:
            x[0] = (x[0][0] + dvec[None], x[0][1])
        put(dst, a, _radix4(x, -1))
        return [t[0][16 * s:16 * s + 8] for s in range(16)]

    def grp_k(j, a):
        return grp_fwd(zs.pop((j, a)), kpbs[j % 2], a,
                       sdv[:, j * L:(j + 1) * L] if a == 0 else None)

    def grp_u(j, a):
        uw = [kvf[pl.ds(a * C + r, L, stride=R), :].astype(bf16) for r in range(R)]
        return grp_fwd(uw, ubs[j % 2], a)

    def grp_i(j, a):
        ys = []
        for r in range(R):
            base = 8 * L + 2 * L * r
            g = jnp.concatenate([tab[base:base + L, :], tab[base + L:base + 2 * L, :]], axis=1)
            y = jnp.dot(g, pbs[j % 2][a, r].reshape(2 * L, L), preferred_element_type=f32)
            yb[j, pl.ds(a * C + r, L, stride=R), :] = y
            ys.append(y)
        return ([ys[0][16 * s:16 * s + 8] for s in range(8)]
                + [ys[2][16 * s:16 * s + 8] for s in range(8)])

    def grp_mod(i0, i1):
        m = jnp.dot(cs, wmb[:, i0 * D:i1 * D], preferred_element_type=f32)
        for i in range(i0, i1):
            mod[i] = m[0:1, (i - i0) * D:(i - i0 + 1) * D]
        return [m[0:8, n * L:(n + 1) * L] for n in range((i1 - i0) * NT)]

    def kv_piece(j, p, dep):
        r0 = p * KVR
        w = [skt[t:t + 1, j * L:(j + 1) * L] for t in range(KS)]
        w0 = gate(w[0], dep)
        if dep is not None:
            w0 = jnp.concatenate([w0] * (KVR // 8), axis=0)
        kf[PAD + r0:PAD + r0 + KVR, :] = kb[j, r0:r0 + KVR, :].astype(f32)
        ks = kf[PAD + r0:PAD + r0 + KVR, :] * w0
        for t in range(1, KS):
            ks = ks + kf[PAD + r0 - t:PAD + r0 - t + KVR, :] * w[t]
        kvf[r0:r0 + KVR, :] = ks * vb[j, r0:r0 + KVR, :].astype(f32)

    st = {}

    def mac_piece(j, i, qi, dep):
        ub, kpb, pb = ubs[j % 2], kpbs[j % 2], pbs[j % 2]
        u = [(ub[a, qi, i, 0:8, :], ub[a, qi, i, 8:16, :]) for a in range(NC)]
        k = [(kpb[a, qi, i, 0:8, :], kpb[a, qi, i, 8:16, :]) for a in range(NC)]
        k[0] = (gate(k[0][0], dep), k[0][1])
        y = []
        for a in range(NC):
            yr = yi = None
            for m in range(a + 1):
                (kr, ki), (ur, ui) = k[m], u[a - m]
                tr = kr * ur - ki * ui
                ti = kr * ui + ki * ur
                yr = tr if yr is None else yr + tr
                yi = ti if yi is None else yi + ti
            y.append((yr, yi))
        st[qi] = [y[0]] + [(y[a][0] - y[a - 1][1], y[a][1] + y[a - 1][0]) for a in range(1, NC)]
        if qi == R - 1:
            for a in range(NC):
                ps = _radix4([st[n][a] for n in range(R)], +1)
                for r in range(R):
                    pb[a, r, i] = jnp.concatenate(ps[r], axis=0).astype(bf16)

    grp_fn = {"z": grp_z, "k": grp_k, "u": grp_u, "i": grp_i,
              "modA": lambda: grp_mod(0, 3), "modB": lambda: grp_mod(3, 5)}
    free = {"i": 52, "z": 56, "k": 44, "u": 44, "modA": 100, "modB": 100}
    nanch = {"i": 16, "z": 8, "k": 16, "u": 16, "modA": 15, "modB": 10}

    def cost(pc):
        return 85 if pc[0] == "kv" else (159 if pc[3] == R - 1 else 79)

    def emit(pc, dep):
        (kv_piece if pc[0] == "kv" else mac_piece)(*pc[1:], dep)

    for waits, groups, pieces in _schedule():
        wait(*waits)
        cap = sum(nanch[g[0]] * free[g[0]] for g in groups)
        rate = max(1.03 * sum(cost(pc) for pc in pieces) / cap, 0.9)
        credit, done = 0.0, 0
        for g in groups:
            if g[0] == "u":
                need = ("kv", g[1], (g[2] + 1) * (C // KVR) - 1)
                while need in pieces[done:]:
                    emit(pieces[done], None)
                    done += 1
            for dep in grp_fn[g[0]](*g[1:]):
                credit += free[g[0]] * rate
                while done < len(pieces) and credit > 0:
                    credit -= cost(pieces[done])
                    emit(pieces[done], dep)
                    done += 1
        for pc in pieces[done:]:
            emit(pc, None)

    sa, ca, ga, sb, cb = [mod[i] for i in range(5)]
    a1 = ga * (1.0 + ca)
    b1 = ga * sa
    a2 = 1.0 + cb

    def o_cp(r0, n, i):
        return pltpu.make_async_copy(ob.at[pl.ds(r0, n), :], o_hbm.at[0, pl.ds(r0, n), :],
                                     osem.at[i])

    def prep(r0, dep=None):
        x = qb[pl.ds(r0, PR), :].astype(f32)
        if dep is not None:
            x0 = jnp.concatenate([gate(x[s:s + 8, 0:L], dep[s:s + 8]) for s in range(0, PR, 8)],
                                 axis=0)
            x = jnp.concatenate([x0, x[:, L:]], axis=1)
        y = jnp.concatenate([yb[j, pl.ds(r0, PR), :] for j in range(NT)], axis=1)
        x1 = x + (_layernorm(x) * a1 + b1) * y
        x1b[pl.ds(r0, PR), :] = x1
        h2 = _layernorm(x1) * a2 + sb
        h2b[pl.ds(r0, PR), :] = h2.astype(bf16)
        return h2[:, 0:L]

    def prep_chain(r0, n):
        dep = None
        for p in range(n // PR):
            dep = prep(r0 + p * PR, dep)

    def gate_up(h2, f0, f1):
        hs = []
        for f in range(f0, f1, TF):
            g = jnp.dot(h2, wgb[:, f:f + TF], preferred_element_type=f32)
            u = jnp.dot(h2, wub[:, f:f + TF], preferred_element_type=f32)
            hs.append(g * u)
        return jnp.concatenate(hs, axis=1).astype(bf16)

    def down(hh, r0, n, gb):
        o = jnp.dot(hh, wdb[...], preferred_element_type=f32)
        ob[pl.ds(r0, n), :] = (x1b[pl.ds(r0, n), :] + gb * o).astype(bf16)

    wait("q0")
    SUB = 128
    for p in range(SUB // PR):
        prep(p * PR)
    wait("wg0", "wu0")
    hs0 = []
    for s in range(0, TM0, SUB):
        if s > 0:
            for p in range(SUB // PR):
                prep(s + p * PR)
        hs0.append(gate_up(h2b[s:s + SUB, :], WP[0], WP[1]))
    hs = [jnp.concatenate(hs0, axis=0)]
    for p in range(1, len(WP) - 1):
        wait(f"wg{p}", f"wu{p}")
        hs.append(gate_up(h2b[0:TM0, :], WP[p], WP[p + 1]))
    wait("wd", "wmC", "q1")
    grp_mod(5, 6)
    gb = mod[5]
    prep_chain(TM0, TM)
    down(jnp.concatenate(hs, axis=1), 0, TM0, gb)
    o_cp(0, TM0, NB).start()
    wait("q2")

    def ffn(i, carry):
        r0 = pl.multiple_of(TM0 + i * TM, TM)
        rn = pl.multiple_of(TM0 + jnp.minimum(i + 1, NB - 1) * TM, TM)
        h2 = h2b[pl.ds(r0, TM), :]
        prep_chain(rn, TM)
        down(gate_up(h2, 0, F), r0, TM, gb)
        o_cp(r0, TM, i).start()
        return carry

    lax.fori_loop(0, NB, ffn, 0)
    o_cp(0, TM0, NB).wait()
    for i in range(NB):
        o_cp(TM0 + i * TM, TM, i).wait()


@jax.jit
def pallas_adaLN_cond__ssm_conv_h3__glu_gated_bilinear__prompt_kernel(
    A_q: jax.Array,
    A_k: jax.Array,
    A_v: jax.Array,
    A_shift_k: jax.Array,
    A_ssm_k: jax.Array,
    A_ssm_D: jax.Array,
    B_x: jax.Array,
    B_w_gate: jax.Array,
    B_w_up: jax.Array,
    B_w_down: jax.Array,
    c: jax.Array,
    w_mod: jax.Array,
):
    del B_x
    tab = jnp.asarray(_dft_tables(), dtype=bf16)
    any_spec = pl.BlockSpec(memory_space=pl.ANY)
    return pl.pallas_call(
        _kernel,
        in_specs=[any_spec] * 12,
        out_specs=any_spec,
        out_shape=jax.ShapeDtypeStruct((1, S, D), bf16),
        scratch_shapes=[
            pltpu.VMEM((S, D), bf16),
            pltpu.VMEM((NT, S, L), bf16),
            pltpu.VMEM((NT, S, L), bf16),
            pltpu.VMEM((KS, D), bf16),
            pltpu.VMEM((NT, L, S), bf16),
            pltpu.VMEM((D,), bf16),
            pltpu.VMEM((D, F), bf16),
            pltpu.VMEM((D, F), bf16),
            pltpu.VMEM((F, D), bf16),
            pltpu.VMEM((1, D), bf16),
            pltpu.VMEM((D, 6 * D), bf16),
            pltpu.VMEM((16 * L, L), bf16),
            pltpu.VMEM((PAD + S, L), f32),
            pltpu.VMEM((S, L), f32),
            pltpu.VMEM((NC, R, 16, 16, L), f32),
            pltpu.VMEM((NC, R, 16, 16, L), f32),
            pltpu.VMEM((NC, R, 16, 16, L), f32),
            pltpu.VMEM((NC, R, 16, 16, L), f32),
            pltpu.VMEM((NC, R, 16, 16, L), bf16),
            pltpu.VMEM((NC, R, 16, 16, L), bf16),
            pltpu.VMEM((NT, S, L), f32),
            pltpu.VMEM((S, D), f32),
            pltpu.VMEM((S, D), bf16),
            pltpu.VMEM((S, D), bf16),
            pltpu.SemaphoreType.DMA((len(DMA_ORDER),)),
            pltpu.SemaphoreType.DMA((NB + 1,)),
        ],
        compiler_params=pltpu.CompilerParams(vmem_limit_bytes=100 * 1024 * 1024),
        name="adaln_h3_glu",
    )(A_q, A_k, A_v, A_shift_k.T, A_ssm_k, A_ssm_D, B_w_gate, B_w_up, B_w_down, c, w_mod, tab)
```

```python
import jax
import jax.numpy as jnp
from jax import lax
import jax.experimental.pallas as pl
import jax.experimental.pallas.tpu as pltpu

S = 2048
D = 640
F = 1536
KS = 4
L = 128
NT = D // L
R = 4
C = R * L
NC = S // C
EPS = 1e-5
PAD = 8
KVR = 64
PR = 32
TM0 = 512
TM = 384
NB = (S - TM0) // TM
TF = 256
WP = (0, 256, 768, 1536)

N3 = 5
N3_0 = 2
WM = {"wmA": (0, 16 * L), "wmB": (16 * L, 26 * L), "wmC": (26 * L, 30 * L)}
SCOPES = False

f32 = jnp.float32
bf16 = jnp.bfloat16


def _cos_turns(t):
    big = 12582912.0
    x = 0.25 - jnp.abs(t - ((t + big) - big))
    x2 = x * x
    return x * (6.283164024 + x2 * (-41.33713150 + x2 * (81.34038544 + x2 * -70.98993683)))


def _make_tables(tab):
    w = lax.broadcasted_iota(jnp.int32, (L, L), 0)
    c = lax.broadcasted_iota(jnp.int32, (L, L), 1)
    inv = 1.0 / (4 * C)
    g_lo = 8 * (w >> 3) + 2 * (w & 3)
    a_lo = (4 * g_lo + 1).astype(f32) * inv
    a_hi = (4 * g_lo + 5).astype(f32) * inv
    off = ((w >> 2) & 1).astype(f32) * 0.25
    for r in range(R):
        n = (R * c + r).astype(f32)
        tab[L * r:L * (r + 1), :] = pltpu.pack_elementwise(
            [_cos_turns(a_lo * n + off), _cos_turns(a_hi * n + off)], packed_dtype=bf16)
    a = (4 * ((w >> 6) * (L // 2) + (c >> 1)) + 1).astype(f32) * inv
    off = (c & 1).astype(f32) * 0.25
    for r in range(R):
        n = (2 * R * (w & (L // 2 - 1)) + r).astype(f32)
        tab[L * (R + r):L * (R + r + 1), :] = pltpu.pack_elementwise(
            [_cos_turns(a * n + off) * (1.0 / C), _cos_turns(a * (n + R) + off) * (1.0 / C)],
            packed_dtype=bf16)


def _layernorm(x):
    m = jnp.mean(x, axis=-1, keepdims=True)
    xc = x - m
    v = jnp.mean(xc * xc, axis=-1, keepdims=True)
    return xc * lax.rsqrt(v + EPS)


def _split(t):
    t = t.reshape(16, 16, L)
    return t[:, :8, :], t[:, 8:, :]


def _radix4(x, sgn):
    (ar, ai), (br, bi), (cr, ci), (dr, di) = x
    s0r, s0i, d0r, d0i = ar + cr, ai + ci, ar - cr, ai - ci
    s1r, s1i, d1r, d1i = br + dr, bi + di, br - dr, bi - di
    o0 = (s0r + s1r, s0i + s1i)
    o2 = (s0r - s1r, s0i - s1i)
    pl_ = (d0r - d1i, d0i + d1r)
    mi_ = (d0r + d1i, d0i - d1r)
    return [o0, pl_, o2, mi_] if sgn > 0 else [o0, mi_, o2, pl_]


def _schedule():
    z = lambda j: [("z", j, a) for a in range(NC)]
    k = lambda j: [("k", j, a) for a in range(NC)]
    u = lambda j: [("u", j, a) for a in range(NC)]
    iv = lambda j, al: [("i", j, a) for a in al]
    kv = lambda j: [("kv", j, p) for p in range(S // KVR)]
    m = lambda j, il, al: [("mac", j, i, q, al) for i in il for q in range(R)]
    bl = [(["ssm0"], z(0) + k(0), []),
          (["k0", "v0"], u(0), kv(0))]
    for j in range(NT - 1):
        n = j + 1
        n3 = N3 if j > 0 else N3_0
        bl.append(([f"ssm{n}"], (iv(j - 1, [3]) if j > 0 else []) + z(n) + k(n),
                   m(j, range(n3), (0, 1, 2, 3)) + m(j, range(n3, 16), (0, 1, 2))))
        bl.append(([f"k{n}", f"v{n}"],
                   iv(j, [0, 1, 2]) + u(n), kv(n) + m(j, range(n3, 16), (3,))))
    j = NT - 1
    bl.append((["wmA"], [("modA",)] + iv(j, [0]), m(j, range(16), (0, 1))))
    return bl, iv(j - 1, [3]) + iv(j, [1]), m(j, range(16), (2, 3)), iv(j, [2, 3])


DMA_ORDER = (["sk", "sd", "c", "ssm0", "k0", "v0", "ssm1", "k1", "v1",
              "ssm2", "k2", "v2", "ssm3", "k3", "v3", "ssm4", "k4", "v4", "wmA", "q0", "wmB",
              ]
             + [f"w{n}{p}" for p in range(len(WP) - 1) for n in "gu"] + ["wmC", "wd", "q1", "q2"])


def _kernel(q_hbm, k_hbm, v_hbm, sk_hbm, ssm_hbm, sd_hbm, wg_hbm, wu_hbm, wd_hbm,
            c_hbm, wm_hbm, o_hbm,
            qb, kb, vb, skb, ssmb, sdb, wgb, wub, wdb, cb_, wmb, tab,
            kf, kvf, ub0, ub1, kpb0, kpb1, pb0, pb1, yb, x1b, h2b, ob, sem, osem):
    cps = {"sk": (sk_hbm, skb), "sd": (sd_hbm, sdb), "c": (c_hbm, cb_), "wd": (wd_hbm, wdb),
           }
    for j in range(NT):
        cps[f"ssm{j}"] = (ssm_hbm.at[pl.ds(j * L, L), :], ssmb.at[j])
        cps[f"k{j}"] = (k_hbm.at[0, :, pl.ds(j * L, L)], kb.at[j])
        cps[f"v{j}"] = (v_hbm.at[0, :, pl.ds(j * L, L)], vb.at[j])
    for n, (c0, c1) in WM.items():
        cps[n] = (wm_hbm.at[:, pl.ds(c0, c1 - c0)], wmb.at[:, pl.ds(c0, c1 - c0)])
    for n, (r0, r1) in (("q0", (0, TM0)), ("q1", (TM0, TM0 + TM)), ("q2", (TM0 + TM, S))):
        cps[n] = (q_hbm.at[0, pl.ds(r0, r1 - r0), :], qb.at[pl.ds(r0, r1 - r0), :])
    for p in range(len(WP) - 1):
        cols = pl.ds(WP[p], WP[p + 1] - WP[p])
        cps[f"wg{p}"] = (wg_hbm.at[:, cols], wgb.at[:, cols])
        cps[f"wu{p}"] = (wu_hbm.at[:, cols], wub.at[:, cols])
    assert sorted(cps) == sorted(DMA_ORDER)

    def cp(name):
        src, dst = cps[name]
        return pltpu.make_async_copy(src, dst, sem.at[DMA_ORDER.index(name)])

    def wait(*names):
        if SCOPES:
            with jax.named_scope("w_" + names[0]):
                for n in names:
                    cp(n).wait()
        else:
            for n in names:
                cp(n).wait()

    for n in DMA_ORDER:
        cp(n).start()

    _make_tables(tab)
    kf[0:PAD, :] = jnp.zeros((PAD, L), f32)
    ri = lax.broadcasted_iota(jnp.int32, (L, L), 0)
    ci = lax.broadcasted_iota(jnp.int32, (L, L), 1)
    sel = jnp.where(ci == R * (ri % 32) + ri // 32, 1.0, 0.0).astype(bf16)

    wait("sk", "sd", "c")
    skt = skb[...].astype(f32)
    sdv = sdb[...].astype(f32).reshape(1, D)
    cv = cb_[...].astype(f32)
    sig = jax.nn.sigmoid(cv)
    cs = jnp.broadcast_to((cv * sig).astype(bf16), (16, D))
    never = jnp.broadcast_to(sig[:, 0:L], (8, L)) > 2.0

    def gate(x, dep):
        if dep is None:
            return x
        return jnp.where(never, dep, jnp.broadcast_to(x, (8, L)))

    def put(dst, a, xs):
        for qi in range(R):
            dst[a, qi, :, 0:8, :] = xs[qi][0]
            dst[a, qi, :, 8:16, :] = xs[qi][1]

    ubs, kpbs, pbs = (ub0, ub1), (kpb0, kpb1), (pb0, pb1)
    zs = {}
    mod = {}

    def grp_z(j, a):
        z = [lax.dot_general(sel, ssmb[j, :, t * L:(t + 1) * L], (((1,), (1,)), ((), ())),
                             preferred_element_type=f32) for t in range(R * a, R * a + R)]
        zs[j, a] = [jnp.concatenate([z[p][32 * r:32 * (r + 1)] for p in range(R)],
                                    axis=0).astype(bf16) for r in range(R)]
        return [z[0][16 * t:16 * t + 8] for t in range(8)]

    def grp_fwd(ws, dst, a, dvec=None):
        t = [jnp.dot(pltpu.bitcast(tab[L * r:L * (r + 1), :], bf16), ws[r],
                     preferred_element_type=f32) for r in range(R)]
        x = [_split(v) for v in t]
        if dvec is not None:
            x[0] = (x[0][0] + dvec[None], x[0][1])
        put(dst, a, _radix4(x, -1))
        return [t[0][16 * s:16 * s + 8] for s in range(16)]

    def grp_k(j, a):
        return grp_fwd(zs.pop((j, a)), kpbs[j % 2], a,
                       sdv[:, j * L:(j + 1) * L] if a == 0 else None)

    def grp_u(j, a):
        uw = [kvf[pl.ds(a * C + r, L, stride=R), :].astype(bf16) for r in range(R)]
        return grp_fwd(uw, ubs[j % 2], a)

    def grp_i(j, a):
        ys = []
        for r in range(R):
            base = 4 * L + L * r
            g = jnp.concatenate([tab[base:base + L // 2, :], tab[base + L // 2:base + L, :]], axis=1)
            y = jnp.dot(pltpu.bitcast(g, bf16), pltpu.bitcast(pbs[j % 2][a, r], bf16),
                        preferred_element_type=f32)
            yb[j, pl.ds(a * C + r, L, stride=R), :] = y
            ys.append(y)
        return ([ys[0][16 * s:16 * s + 8] for s in range(8)]
                + [ys[2][16 * s:16 * s + 8] for s in range(8)])

    def grp_mod(name):
        c0, c1 = WM[name]
        m = jnp.dot(cs, wmb[:, c0:c1], preferred_element_type=f32)
        for c in range(c0, c1, L):
            mod[c // L] = m[0:1, c - c0:c - c0 + L]
        return [m[0:8, c:c + L] for c in range(0, c1 - c0, L)]

    def modv(i):
        return jnp.concatenate([mod[i * NT + n] for n in range(NT)], axis=1)

    def kv_piece(j, p, dep):
        r0 = p * KVR
        w = [skt[t:t + 1, j * L:(j + 1) * L] for t in range(KS)]
        w0 = gate(w[0], dep)
        if dep is not None:
            w0 = jnp.concatenate([w0] * (KVR // 8), axis=0)
        kf[PAD + r0:PAD + r0 + KVR, :] = kb[j, r0:r0 + KVR, :].astype(f32)
        ks = kf[PAD + r0:PAD + r0 + KVR, :] * w0
        for t in range(1, KS):
            ks = ks + kf[PAD + r0 - t:PAD + r0 - t + KVR, :] * w[t]
        kvf[r0:r0 + KVR, :] = ks * vb[j, r0:r0 + KVR, :].astype(f32)

    st = {}

    def mac_piece(j, i, qi, al, dep):
        ub, kpb, pb = ubs[j % 2], kpbs[j % 2], pbs[j % 2]
        top = max(al) + 1
        u = [(ub[a, qi, i, 0:8, :], ub[a, qi, i, 8:16, :]) for a in range(top)]
        k = [(kpb[a, qi, i, 0:8, :], kpb[a, qi, i, 8:16, :]) for a in range(top)]
        k[0] = (gate(k[0][0], dep), k[0][1])
        kp = [k[0]] + [(k[m][0] - k[m - 1][1], k[m][1] + k[m - 1][0]) for m in range(1, top)]
        for a in al:
            yr = yi = None
            for m in range(a + 1):
                (kr, ki), (ur, ui) = kp[m], u[a - m]
                tr = kr * ur - ki * ui
                ti = kr * ui + ki * ur
                yr = tr if yr is None else yr + tr
                yi = ti if yi is None else yi + ti
            st[qi, a] = (yr, yi)
        if qi == R - 1:
            for a in al:
                ps = _radix4([st.pop((n, a)) for n in range(R)], +1)
                for r in range(R):
                    pb[a, r, 8 * i:8 * i + 8, :] = pltpu.pack_elementwise(
                        ps[r], packed_dtype=bf16)

    grp_fn = {"z": grp_z, "k": grp_k, "u": grp_u, "i": grp_i,
              "modA": lambda: grp_mod("wmA")}
    free = {"i": 60, "z": 56, "k": 48, "u": 48, "modA": 140, "modB": 100}
    nanch = {"i": 16, "z": 8, "k": 16, "u": 16, "modA": 16}

    def cost(pc):
        if pc[0] == "kv":
            return 85
        al = pc[4]
        return (1 + 2 * max(al) + sum(8 * a + 6 for a in al)
                + (20 * len(al) if pc[3] == R - 1 else 0))

    def emit(pc, dep):
        (kv_piece if pc[0] == "kv" else mac_piece)(*pc[1:], dep)

    blocks, prep_groups, late_pieces, late_groups = _schedule()
    for waits, groups, pieces in blocks:
        wait(*waits)
        cap = sum(nanch[g[0]] * free[g[0]] for g in groups)
        rate = max(1.03 * sum(cost(pc) for pc in pieces) / cap, 0.9)
        credit, done = 0.0, 0
        for g in groups:
            if g[0] == "u":
                need = ("kv", g[1], (g[2] + 1) * (C // KVR) - 1)
                while need in pieces[done:]:
                    emit(pieces[done], None)
                    done += 1
            if g[0] == "i":
                while any(pc[0] == "mac" and pc[1] == g[1] and g[2] in pc[4]
                          for pc in pieces[done:]):
                    emit(pieces[done], None)
                    done += 1
            for dep in grp_fn[g[0]](*g[1:]):
                credit += free[g[0]] * rate
                while done < len(pieces) and credit > 0:
                    credit -= cost(pieces[done])
                    emit(pieces[done], dep)
                    done += 1
        for pc in pieces[done:]:
            emit(pc, None)

    sa, ca, ga = [modv(i) for i in range(3)]
    a1 = ga * (1.0 + ca)
    b1 = ga * sa

    def o_cp(r0, n, c0, c1, i):
        cols = pl.ds(c0, c1 - c0)
        return pltpu.make_async_copy(ob.at[pl.ds(r0, n), cols], o_hbm.at[0, pl.ds(r0, n), cols],
                                     osem.at[i])

    def prep_norm(r0, dep=None):
        x = qb[pl.ds(r0, PR), :].astype(f32)
        if dep is not None:
            x0 = jnp.concatenate([gate(x[s:s + 8, 0:L], dep[s:s + 8]) for s in range(0, PR, 8)],
                                 axis=0)
            x = jnp.concatenate([x0, x[:, L:]], axis=1)
        y = jnp.concatenate([yb[j, pl.ds(r0, PR), :] for j in range(NT)], axis=1)
        x1 = x + (_layernorm(x) * a1 + b1) * y
        x1b[pl.ds(r0, PR), :] = x1
        return _layernorm(x1)

    wait("q0")
    for g in prep_groups:
        grp_fn[g[0]](*g[1:])
    n2 = jnp.concatenate([prep_norm(p * PR) for p in range(TM0 // PR)], axis=0)
    wait("wmB")
    grp_mod("wmB")
    sb = modv(3)
    a2 = 1.0 + modv(4)

    def prep(r0, dep=None):
        h2 = prep_norm(r0, dep) * a2 + sb
        h2b[pl.ds(r0, PR), :] = h2.astype(bf16)
        return h2[:, 0:L]

    def prep_chain(r0, n):
        dep = None
        for p in range(n // PR):
            dep = prep(r0 + p * PR, dep)

    def gate_up(h2, f0, f1, anchors=None):
        hs = []
        for f in range(f0, f1, TF):
            TF_ = min(TF, f1 - f)
            g = jnp.dot(h2, wgb[:, f:f + TF_], preferred_element_type=f32)
            u = jnp.dot(h2, wub[:, f:f + TF_], preferred_element_type=f32)
            hs.append(g * u)
            if anchors is not None:
                anchors += [t[s:s + 8, n:n + L] for t in (g, u) for n in range(0, TF_, L)
                            for s in range(0, h2.shape[0], 64)]
        return jnp.concatenate(hs, axis=1).astype(bf16)

    OC = (0, D - L, D)

    def down(hh, r0, n, gb, i):
        for c0, c1 in zip(OC[:-1], OC[1:]):
            o = jnp.dot(hh, wdb[:, c0:c1], preferred_element_type=f32)
            ob[pl.ds(r0, n), c0:c1] = (x1b[pl.ds(r0, n), c0:c1] + gb[:, c0:c1] * o).astype(bf16)
            o_cp(r0, n, c0, c1, i).start()

    hs = []
    for p in range(len(WP) - 1):
        wait(f"wg{p}", f"wu{p}", *(["wmC"] if p == len(WP) - 2 else []))
        anchors = []
        if p == 0:
            h2 = (n2 * a2 + sb).astype(bf16)
            half = TM0 // 2
            hs.append(jnp.concatenate([gate_up(h2[:half], WP[0], WP[1]),
                                       gate_up(h2[half:], WP[0], WP[1])], axis=0))
        else:
            hs.append(gate_up(h2, WP[p], WP[p + 1], anchors))
        if p == len(WP) - 3:
            for n, pc in enumerate(late_pieces):
                emit(pc, anchors[n * len(anchors) // len(late_pieces)])
        if p == len(WP) - 2:
            for g in late_groups:
                grp_fn[g[0]](*g[1:])
    grp_mod("wmC")
    gb = modv(5)
    wait("wd", "q1")
    prep_chain(TM0, TM)
    down(jnp.concatenate(hs, axis=1), 0, TM0, gb, NB)
    wait("q2")

    def ffn(i, carry):
        r0 = pl.multiple_of(TM0 + i * TM, PR)
        rn = pl.multiple_of(TM0 + jnp.minimum(i + 1, NB - 1) * TM, PR)
        h2 = h2b[pl.ds(r0, TM), :]
        prep_chain(rn, TM)
        down(gate_up(h2, 0, F), r0, TM, gb, i)
        return carry

    lax.fori_loop(0, NB, ffn, 0)
    for c0, c1 in zip(OC[:-1], OC[1:]):
        o_cp(0, TM0, c0, c1, NB).wait()
    for i in range(NB):
        for c0, c1 in zip(OC[:-1], OC[1:]):
            o_cp(TM0 + i * TM, TM, c0, c1, i).wait()


@jax.jit
def pallas_adaLN_cond__ssm_conv_h3__glu_gated_bilinear__prompt_kernel(
    A_q: jax.Array,
    A_k: jax.Array,
    A_v: jax.Array,
    A_shift_k: jax.Array,
    A_ssm_k: jax.Array,
    A_ssm_D: jax.Array,
    B_x: jax.Array,
    B_w_gate: jax.Array,
    B_w_up: jax.Array,
    B_w_down: jax.Array,
    c: jax.Array,
    w_mod: jax.Array,
):
    del B_x
    any_spec = pl.BlockSpec(memory_space=pl.ANY)
    return pl.pallas_call(
        _kernel,
        in_specs=[any_spec] * 11,
        out_specs=any_spec,
        out_shape=jax.ShapeDtypeStruct((1, S, D), bf16),
        scratch_shapes=[
            pltpu.VMEM((S, D), bf16),
            pltpu.VMEM((NT, S, L), bf16),
            pltpu.VMEM((NT, S, L), bf16),
            pltpu.VMEM((KS, D), bf16),
            pltpu.VMEM((NT, L, S), bf16),
            pltpu.VMEM((D,), bf16),
            pltpu.VMEM((D, F), bf16),
            pltpu.VMEM((D, F), bf16),
            pltpu.VMEM((F, D), bf16),
            pltpu.VMEM((1, D), bf16),
            pltpu.VMEM((D, 6 * D), bf16),
            pltpu.VMEM((8 * L, L), jnp.uint32),
            pltpu.VMEM((PAD + S, L), f32),
            pltpu.VMEM((S, L), f32),
            pltpu.VMEM((NC, R, 16, 16, L), f32),
            pltpu.VMEM((NC, R, 16, 16, L), f32),
            pltpu.VMEM((NC, R, 16, 16, L), f32),
            pltpu.VMEM((NC, R, 16, 16, L), f32),
            pltpu.VMEM((NC, R, L, L), jnp.uint32),
            pltpu.VMEM((NC, R, L, L), jnp.uint32),
            pltpu.VMEM((NT, S, L), f32),
            pltpu.VMEM((S, D), f32),
            pltpu.VMEM((S, D), bf16),
            pltpu.VMEM((S, D), bf16),
            pltpu.SemaphoreType.DMA((len(DMA_ORDER),)),
            pltpu.SemaphoreType.DMA((NB + 1,)),
        ],
        compiler_params=pltpu.CompilerParams(
            vmem_limit_bytes=100 * 1024 * 1024,
            disable_bounds_checks=True, disable_semaphore_checks=True),
        name="adaln_h3_glu",
    )(A_q, A_k, A_v, A_shift_k.T, A_ssm_k, A_ssm_D, B_w_gate, B_w_up, B_w_down, c, w_mod)
```

```python
import jax
import jax.numpy as jnp
from jax import lax
import jax.experimental.pallas as pl
import jax.experimental.pallas.tpu as pltpu

S = 2048
D = 640
F = 1536
KS = 4
L = 128
NT = D // L
R = 4
C = R * L
NC = S // C
EPS = 1e-5
WPT = 4 * NT
PAD = 24
KVR = 64
PR = 32
TM0 = 512
TM = 384
NB = (S - TM0) // TM
TF = 256
WP = (0, 256, 768, 1536)

WM = {"wmA": (0, 16 * L), "wmB": (16 * L, 26 * L), "wmC": (26 * L, 30 * L)}
MIN_RATE = 1.0
SCOPES = False

f32 = jnp.float32
bf16 = jnp.bfloat16
u32 = jnp.uint32


def _cos_turns(t):
    big = 12582912.0
    x = 0.25 - jnp.abs(t - ((t + big) - big))
    x2 = x * x
    return x * (6.283164024 + x2 * (-41.33713150 + x2 * (81.34038544 + x2 * -70.98993683)))


def _make_tables(tab):
    w = lax.broadcasted_iota(jnp.int32, (L, L), 0)
    c = lax.broadcasted_iota(jnp.int32, (L, L), 1)
    inv = 1.0 / (4 * C)
    g_lo = 8 * (w >> 3) + 2 * (w & 3)
    a_lo = (4 * g_lo + 1).astype(f32) * inv
    a_hi = (4 * g_lo + 5).astype(f32) * inv
    off = ((w >> 2) & 1).astype(f32) * 0.25
    for r in range(R):
        n = (R * c + r).astype(f32)
        tab[L * r:L * (r + 1), :] = pltpu.pack_elementwise(
            [_cos_turns(a_lo * n + off), _cos_turns(a_hi * n + off)], packed_dtype=bf16)
    a = (4 * ((w >> 6) * (L // 2) + (c >> 1)) + 1).astype(f32) * inv
    off = (c & 1).astype(f32) * 0.25
    for r in range(R):
        n = (2 * R * (w & (L // 2 - 1)) + r).astype(f32)
        tab[L * (R + r):L * (R + r + 1), :] = pltpu.pack_elementwise(
            [_cos_turns(a * n + off) * (1.0 / C), _cos_turns(a * (n + R) + off) * (1.0 / C)],
            packed_dtype=bf16)


def _layernorm(x):
    m = jnp.mean(x, axis=-1, keepdims=True)
    xc = x - m
    v = jnp.mean(xc * xc, axis=-1, keepdims=True)
    return xc * lax.rsqrt(v + EPS)


def _split(t):
    t = t.reshape(16, 16, L)
    return t[:, :8, :], t[:, 8:, :]


def _radix4(x, sgn):
    (ar, ai), (br, bi), (cr, ci), (dr, di) = x
    s0r, s0i, d0r, d0i = ar + cr, ai + ci, ar - cr, ai - ci
    s1r, s1i, d1r, d1i = br + dr, bi + di, br - dr, bi - di
    o0 = (s0r + s1r, s0i + s1i)
    o2 = (s0r - s1r, s0i - s1i)
    pl_ = (d0r - d1i, d0i + d1r)
    mi_ = (d0r + d1i, d0i - d1r)
    return [o0, pl_, o2, mi_] if sgn > 0 else [o0, mi_, o2, pl_]


T = range(NT)
_z = lambda j: [("z", j, a) for a in range(NC)]
_k = lambda j, al: [("k", j, a) for a in al]
_u = lambda a: [("u", j, a) for j in T]
_iv = lambda jl, al: [("i", j, a) for j in jl for a in al]
_kv = lambda a: [("kv", j, p) for j in T for p in range(a * C // KVR, (a + 1) * C // KVR)]
_m = lambda jl, us, outs: [("mac", j, i, q, us, outs)
                           for j in jl for i in range(16) for q in range(R)]
A3 = (0, 1, 2)

SCHEDULE = [
    (["ssm0"], _z(0) + _k(0, range(NC)), []),
    (["ssm1"], _z(1) + _k(1, [0, 1]), []),
    (["k0", "v0"], _k(1, [2, 3]) + _u(0), _kv(0)),
    (["ssm2"], _z(2) + _k(2, [0, 1]), _m([0, 1], (0,), A3)),
    (["k1", "v1"], _k(2, [2, 3]) + _u(1), _kv(1)),
    (["ssm3"], _z(3) + _k(3, [0, 1]), _m([2], (0, 1), A3)),
    (["k2", "v2"], _k(3, [2, 3]) + _u(2), _kv(2)),
    (["ssm4"], _iv([0, 1], [0]) + _iv([2], [0, 1]) + _z(4) + _k(4, range(NC)),
     _m([0, 1], (1, 2), (1, 2)) + _m([2], (2,), (2,)) + _m([3], A3, A3)),
    (["q0"], _iv([3], [0]) + _iv([0, 1], [1, 2]) + _iv([4], [0]), _m([4], A3, A3)),
]
PREP_GROUPS = _iv([2], [2]) + _iv([3, 4], [1, 2])

DMA_ORDER = (["sk", "sd", "c", "ssm0", "ssm1", "k0", "v0", "ssm2", "k1", "v1", "ssm3", "k2", "v2",
              "ssm4", "q0", "wmA", "wmB"]
             + [f"w{n}{p}" for p in range(len(WP) - 1) for n in "gu"]
             + ["wmC", "wd", "k3", "v3", "q1", "q2"])


def _kernel(q_hbm, k_hbm, v_hbm, sk_hbm, ssm_hbm, sd_hbm, wg_hbm, wu_hbm, wd_hbm,
            c_hbm, wm_hbm, o_hbm,
            qb, kb, vb, skb, ssmb, sdb, wgb, wub, wdb, cb_, wmb, tab,
            uwb, ub, kpb, yp, pb, yb, x1b, h2b, ob, sem, osem):
    cps = {"sk": (sk_hbm, skb), "sd": (sd_hbm, sdb), "c": (c_hbm, cb_), "wd": (wd_hbm, wdb),
           }
    for j in range(NT):
        cps[f"ssm{j}"] = (ssm_hbm.at[pl.ds(j * L, L), :], ssmb.at[j])
    for a in range(NC):
        n = C // 8 * WPT
        cps[f"k{a}"] = (k_hbm.bitcast(u32).at[pl.ds(a * n, n), :], kb.at[pl.ds(PAD + a * n, n), :])
        cps[f"v{a}"] = (v_hbm.bitcast(u32).at[pl.ds(a * n, n), :], vb.at[pl.ds(a * n, n), :])
    for n, (c0, c1) in WM.items():
        cps[n] = (wm_hbm.at[:, pl.ds(c0, c1 - c0)], wmb.at[:, pl.ds(c0, c1 - c0)])
    for n, (r0, r1) in (("q0", (0, TM0)), ("q1", (TM0, TM0 + TM)), ("q2", (TM0 + TM, S))):
        cps[n] = (q_hbm.at[0, pl.ds(r0, r1 - r0), :], qb.at[pl.ds(r0, r1 - r0), :])
    for p in range(len(WP) - 1):
        cols = pl.ds(WP[p], WP[p + 1] - WP[p])
        cps[f"wg{p}"] = (wg_hbm.at[:, cols], wgb.at[:, cols])
        cps[f"wu{p}"] = (wu_hbm.at[:, cols], wub.at[:, cols])
    assert sorted(cps) == sorted(DMA_ORDER)

    def cp(name):
        src, dst = cps[name]
        return pltpu.make_async_copy(src, dst, sem.at[DMA_ORDER.index(name)])

    def wait(*names):
        if SCOPES:
            with jax.named_scope("w_" + names[0]):
                for n in names:
                    cp(n).wait()
        else:
            for n in names:
                cp(n).wait()

    for n in DMA_ORDER:
        cp(n).start()

    _make_tables(tab)
    kb[0:PAD, :] = jnp.zeros((PAD, L), u32)
    for ref in (uwb, pb):
        ref[0, 0, 0, pl.ds(0, 8, stride=2), :] = jnp.zeros((8, L), u32)
    ub[0, 0, 0, 0, pl.ds(0, 8, stride=2), :] = jnp.zeros((8, L), f32)
    ri = lax.broadcasted_iota(jnp.int32, (L, L), 0)
    ci = lax.broadcasted_iota(jnp.int32, (L, L), 1)
    sel = jnp.where(ci == R * (ri % 32) + ri // 32, 1.0, 0.0).astype(bf16)

    wait("sk", "sd", "c")
    skt = skb[...].astype(f32)
    sdv = sdb[...].astype(f32).reshape(1, D)
    cv = cb_[...].astype(f32)
    sig = jax.nn.sigmoid(cv)
    cs = jnp.broadcast_to((cv * sig).astype(bf16), (16, D))
    never = jnp.broadcast_to(sig[:, 0:L], (8, L)) > 2.0

    def gate(x, dep):
        if dep is None:
            return x
        return jnp.where(never, dep, jnp.broadcast_to(x, (8, L)))

    def put(dst, j, a, xs):
        for qi in range(R):
            dst[j, a, qi, :, 0:8, :] = xs[qi][0]
            dst[j, a, qi, :, 8:16, :] = xs[qi][1]

    zs = {}
    mod = {}

    def grp_z(j, a):
        z = [lax.dot_general(sel, ssmb[j, :, t * L:(t + 1) * L], (((1,), (1,)), ((), ())),
                             preferred_element_type=f32) for t in range(R * a, R * a + R)]
        zs[j, a] = [jnp.concatenate([z[p][32 * r:32 * (r + 1)] for p in range(R)],
                                    axis=0).astype(bf16) for r in range(R)]
        return [z[0][16 * t:16 * t + 8] for t in range(8)]

    def grp_fwd(ws, dst, j, a, dvec=None):
        t = [jnp.dot(pltpu.bitcast(tab[L * r:L * (r + 1), :], bf16), ws[r],
                     preferred_element_type=f32) for r in range(R)]
        x = [_split(v) for v in t]
        if dvec is not None:
            x[0] = (x[0][0] + dvec[None], x[0][1])
        put(dst, j, a, _radix4(x, -1))
        return [t[0][16 * s:16 * s + 8] for s in range(16)]

    def grp_k(j, a):
        return grp_fwd(zs.pop((j, a)), kpb, j, a,
                       sdv[:, j * L:(j + 1) * L] if a == 0 else None)

    def grp_u(j, a):
        uw = [pltpu.bitcast(uwb[j, a, r], bf16) for r in range(R)]
        return grp_fwd(uw, ub, j, a)

    def grp_i(j, a):
        ys = []
        for r in range(R):
            base = 4 * L + L * r
            g = jnp.concatenate([tab[base:base + L // 2, :], tab[base + L // 2:base + L, :]], axis=1)
            y = jnp.dot(pltpu.bitcast(g, bf16), pltpu.bitcast(pb[j, a, r], bf16),
                        preferred_element_type=f32)
            yb[j, pl.ds(a * C + r, L, stride=R), :] = y
            ys.append(y)
        return ([ys[0][16 * s:16 * s + 8] for s in range(8)]
                + [ys[2][16 * s:16 * s + 8] for s in range(8)])

    def grp_mod(name):
        c0, c1 = WM[name]
        m = jnp.dot(cs, wmb[:, c0:c1], preferred_element_type=f32)
        for c in range(c0, c1, L):
            mod[c // L] = m[0:1, c - c0:c - c0 + L]
        return [m[0:8, c:c + L] for c in range(0, c1 - c0, L)]

    def modv(i):
        return jnp.concatenate([mod[i * NT + n] for n in range(NT)], axis=1)

    def kv_piece(j, p, dep):
        lo = lambda x: lax.bitcast_convert_type(x << 16, f32)
        hi = lambda x: lax.bitcast_convert_type(x & jnp.uint32(0xFFFF0000), f32)
        base = 8 * p * WPT + 4 * j
        ld = lambda ref, o: ref[pl.ds(base + o, 8, stride=WPT), :]
        k = {}
        for n in range(4):
            x = ld(kb, PAD + n)
            k[2 * n], k[2 * n + 1] = lo(x), hi(x)
        k[-3] = hi(ld(kb, PAD - WPT + 2))
        x = ld(kb, PAD - WPT + 3)
        k[-2], k[-1] = lo(x), hi(x)
        w = [skt[t:t + 1, j * L:(j + 1) * L] for t in range(KS)]
        w[0] = gate(w[0], dep)
        kv = {}
        for n in range(4):
            x = ld(vb, n)
            for ph, v in ((2 * n, lo(x)), (2 * n + 1, hi(x))):
                ks = k[ph] * w[0]
                for t in range(1, KS):
                    ks = ks + k[ph - t] * w[t]
                kv[ph] = ks * v
        a, s = divmod(p, C // KVR)
        for r in range(R):
            uwb[j, a, r, 8 * s:8 * s + 8, :] = pltpu.pack_elementwise(
                [kv[r], kv[r + R]], packed_dtype=bf16)

    st = {}

    def mac_piece(j, i, qi, us, outs, dep):
        def ld(ref, a):
            return ref[j, a, qi, i, 0:8, :], ref[j, a, qi, i, 8:16, :]

        lo, hi = us[0], us[-1]
        u = {a: ld(ub, a) for a in us}
        u[lo] = (gate(u[lo][0], dep), u[lo][1])
        ms = sorted({a - n for a in outs for n in us if n <= a})
        k = {m: ld(kpb, m) for m in sorted(set(ms) | {m - 1 for m in ms if m > 0})}
        kp = {m: k[m] if m == 0 else (k[m][0] - k[m - 1][1], k[m][1] + k[m - 1][0]) for m in ms}
        for a in outs:
            yr, yi = ld(yp, a) if lo > 0 else (None, None)
            for n in us:
                if n > a:
                    continue
                (kr, ki), (ur, ui) = kp[a - n], u[n]
                tr = kr * ur - ki * ui
                ti = kr * ui + ki * ur
                yr = tr if yr is None else yr + tr
                yi = ti if yi is None else yi + ti
            if a <= hi:
                st[qi, a] = (yr, yi)
            else:
                yp[j, a, qi, i, 0:8, :] = yr
                yp[j, a, qi, i, 8:16, :] = yi
        if qi == R - 1:
            for a in outs:
                if a > hi:
                    continue
                ps = _radix4([st.pop((n, a)) for n in range(R)], +1)
                for r in range(R):
                    pb[j, a, r, 8 * i:8 * i + 8, :] = pltpu.pack_elementwise(
                        ps[r], packed_dtype=bf16)

    grp_fn = {"z": grp_z, "k": grp_k, "u": grp_u, "i": grp_i,
              "modA": lambda: grp_mod("wmA")}
    free = {"i": 60, "z": 56, "k": 48, "u": 48, "modA": 140, "modB": 100}
    nanch = {"i": 16, "z": 8, "k": 16, "u": 16, "modA": 16}

    def cost(pc):
        if pc[0] == "kv":
            return 88
        us, outs = pc[4], pc[5]
        pairs = [(a, n) for a in outs for n in us if n <= a]
        fin = sum(a <= us[-1] for a in outs)
        return (1 + 2 * len({a - n for a, n in pairs if a > n}) + 8 * len(pairs)
                - (2 * len(outs) if us[0] == 0 else 0) + (20 * fin if pc[3] == R - 1 else 0))

    def emit(pc, dep):
        (kv_piece if pc[0] == "kv" else mac_piece)(*pc[1:], dep)

    for waits, groups, pieces in SCHEDULE:
        wait(*waits)
        cap = sum(nanch[g[0]] * free[g[0]] for g in groups)
        rate = max(1.03 * sum(cost(pc) for pc in pieces) / cap, MIN_RATE)
        credit, done = 0.0, 0
        for g in groups:
            if g[0] == "u":
                need = ("kv", g[1], (g[2] + 1) * (C // KVR) - 1)
                while need in pieces[done:]:
                    emit(pieces[done], None)
                    done += 1
            if g[0] == "i":
                while any(pc[0] == "mac" and pc[1] == g[1] and g[2] in pc[5]
                          for pc in pieces[done:]):
                    emit(pieces[done], None)
                    done += 1
            for dep in grp_fn[g[0]](*g[1:]):
                credit += free[g[0]] * rate
                while done < len(pieces) and credit > 0:
                    credit -= cost(pieces[done])
                    emit(pieces[done], dep)
                    done += 1
        for pc in pieces[done:]:
            emit(pc, None)

    wait("wmA")
    grp_mod("wmA")
    for g in PREP_GROUPS:
        grp_fn[g[0]](*g[1:])
    sa, ca, ga = [modv(i) for i in range(3)]
    a1 = ga * (1.0 + ca)
    b1 = ga * sa

    def o_cp(r0, n, c0, c1, i):
        cols = pl.ds(c0, c1 - c0)
        return pltpu.make_async_copy(ob.at[pl.ds(r0, n), cols], o_hbm.at[0, pl.ds(r0, n), cols],
                                     osem.at[i])

    def prep_norm(r0, dep=None):
        x = qb[pl.ds(r0, PR), :].astype(f32)
        if dep is not None:
            x0 = jnp.concatenate([gate(x[s:s + 8, 0:L], dep[s:s + 8]) for s in range(0, PR, 8)],
                                 axis=0)
            x = jnp.concatenate([x0, x[:, L:]], axis=1)
        y = jnp.concatenate([yb[j, pl.ds(r0, PR), :] for j in range(NT)], axis=1)
        x1 = x + (_layernorm(x) * a1 + b1) * y
        x1b[pl.ds(r0, PR), :] = x1
        return _layernorm(x1)

    n2 = jnp.concatenate([prep_norm(p * PR) for p in range(TM0 // PR)], axis=0)
    wait("wmB")
    grp_mod("wmB")
    sb = modv(3)
    a2 = 1.0 + modv(4)

    def prep(r0, dep=None):
        h2 = prep_norm(r0, dep) * a2 + sb
        h2b[pl.ds(r0, PR), :] = h2.astype(bf16)
        return h2[:, 0:L]

    def prep_chain(r0, n):
        dep = None
        for p in range(n // PR):
            dep = prep(r0 + p * PR, dep)

    def gate_up(h2, f0, f1, anchors=None):
        hs = []
        for f in range(f0, f1, TF):
            TF_ = min(TF, f1 - f)
            g = jnp.dot(h2, wgb[:, f:f + TF_], preferred_element_type=f32)
            u = jnp.dot(h2, wub[:, f:f + TF_], preferred_element_type=f32)
            hs.append(g * u)
            if anchors is not None:
                anchors += [t[s:s + 8, n:n + L] for t in (g, u) for n in range(0, TF_, L)
                            for s in range(0, h2.shape[0], 16)]
        return jnp.concatenate(hs, axis=1).astype(bf16)

    OC = (0, D - L, D)

    def down(hh, r0, n, gb, i, hook=None):
        for c0, c1 in zip(OC[:-1], OC[1:]):
            os = []
            for c in range(c0, c1, L):
                if hook is None:
                    os.append(jnp.dot(hh, wdb[:, c:c + L], preferred_element_type=f32))
                else:
                    ps = [jnp.dot(hh[:, f:f + 4 * L], wdb[f:f + 4 * L, c:c + L],
                                  preferred_element_type=f32) for f in range(0, F, 4 * L)]
                    os.append(ps[0] + ps[1] + ps[2])
                    hook(c // L, [x[s:s + 8] for x in ps for s in range(0, n, 16)])
            o = jnp.concatenate(os, axis=1)
            ob[pl.ds(r0, n), c0:c1] = (x1b[pl.ds(r0, n), c0:c1] + gb[:, c0:c1] * o).astype(bf16)
            o_cp(r0, n, c0, c1, i).start()

    def spread(pieces, anchors):
        for n, pc in enumerate(pieces):
            emit(pc, anchors[n * len(anchors) // len(pieces)])

    last = NC - 1
    hs = []
    for p in range(len(WP) - 1):
        wait(f"wg{p}", f"wu{p}", *(["wmC"] if p == len(WP) - 2 else []))
        anchors = []
        if p == 0:
            h2 = (n2 * a2 + sb).astype(bf16)
            half = TM0 // 2
            hs.append(jnp.concatenate([gate_up(h2[:half], WP[0], WP[1]),
                                       gate_up(h2[half:], WP[0], WP[1])], axis=0))
        else:
            hs.append(gate_up(h2, WP[p], WP[p + 1], anchors))
        if p == len(WP) - 2:
            spread(_m(T, A3, (last,)), anchors)
    grp_mod("wmC")
    gb = modv(5)
    wait("wd", f"k{last}", f"v{last}", "q1")

    def hook(n, anchors):
        if n == 0:
            spread(_kv(last), anchors)
        if n == 1:
            for g in _u(last):
                grp_u(*g[1:])
        if n == 2:
            spread(_m(T, (last,), (last,)), anchors)
        if n == 3:
            for g in _iv(T, [last]):
                grp_i(*g[1:])

    prep_chain(TM0, TM)
    down(jnp.concatenate(hs, axis=1), 0, TM0, gb, NB, hook)
    wait("q2")

    def ffn(i, carry):
        r0 = pl.multiple_of(TM0 + i * TM, PR)
        rn = pl.multiple_of(TM0 + jnp.minimum(i + 1, NB - 1) * TM, PR)
        h2 = h2b[pl.ds(r0, TM), :]
        prep_chain(rn, TM)
        down(gate_up(h2, 0, F), r0, TM, gb, i)
        return carry

    lax.fori_loop(0, NB, ffn, 0)
    for c0, c1 in zip(OC[:-1], OC[1:]):
        o_cp(0, TM0, c0, c1, NB).wait()
    for i in range(NB):
        for c0, c1 in zip(OC[:-1], OC[1:]):
            o_cp(TM0 + i * TM, TM, c0, c1, i).wait()


@jax.jit
def pallas_adaLN_cond__ssm_conv_h3__glu_gated_bilinear__prompt_kernel(
    A_q: jax.Array,
    A_k: jax.Array,
    A_v: jax.Array,
    A_shift_k: jax.Array,
    A_ssm_k: jax.Array,
    A_ssm_D: jax.Array,
    B_x: jax.Array,
    B_w_gate: jax.Array,
    B_w_up: jax.Array,
    B_w_down: jax.Array,
    c: jax.Array,
    w_mod: jax.Array,
):
    del B_x
    tiles = lambda x: x.reshape(S // 8, 8, NT, L).transpose(0, 2, 1, 3).reshape(S * NT, L)
    any_spec = pl.BlockSpec(memory_space=pl.ANY)
    return pl.pallas_call(
        _kernel,
        in_specs=[any_spec] * 11,
        out_specs=any_spec,
        out_shape=jax.ShapeDtypeStruct((1, S, D), bf16),
        scratch_shapes=[
            pltpu.VMEM((S, D), bf16),
            pltpu.VMEM((PAD + S // 8 * WPT, L), u32),
            pltpu.VMEM((S // 8 * WPT, L), u32),
            pltpu.VMEM((KS, D), bf16),
            pltpu.VMEM((NT, L, S), bf16),
            pltpu.VMEM((D,), bf16),
            pltpu.VMEM((D, F), bf16),
            pltpu.VMEM((D, F), bf16),
            pltpu.VMEM((F, D), bf16),
            pltpu.VMEM((1, D), bf16),
            pltpu.VMEM((D, 6 * D), bf16),
            pltpu.VMEM((8 * L, L), jnp.uint32),
            pltpu.VMEM((NT, NC, R, L // 2, L), u32),
            pltpu.VMEM((NT, NC, R, 16, 16, L), f32),
            pltpu.VMEM((NT, NC, R, 16, 16, L), f32),
            pltpu.VMEM((NT, NC, R, 16, 16, L), f32),
            pltpu.VMEM((NT, NC, R, L, L), jnp.uint32),
            pltpu.VMEM((NT, S, L), f32),
            pltpu.VMEM((S, D), f32),
            pltpu.VMEM((S, D), bf16),
            pltpu.VMEM((S, D), bf16),
            pltpu.SemaphoreType.DMA((len(DMA_ORDER),)),
            pltpu.SemaphoreType.DMA((NB + 1,)),
        ],
        compiler_params=pltpu.CompilerParams(
            vmem_limit_bytes=120 * 1024 * 1024,
            disable_bounds_checks=True, disable_semaphore_checks=True),
        name="adaln_h3_glu",
    )(A_q, tiles(A_k), tiles(A_v), A_shift_k.T, A_ssm_k, A_ssm_D, B_w_gate, B_w_up, B_w_down, c, w_mod)
```

```python
import jax
import jax.numpy as jnp
from jax import lax
import jax.experimental.pallas as pl
import jax.experimental.pallas.tpu as pltpu

S = 2048
D = 640
F = 1536
KS = 4
L = 128
NT = D // L
R = 4
C = R * L
NC = S // C
EPS = 1e-5
WPT = 4 * NT
PAD = 32
KVR = 64
PR = 24
TM0 = 512
TM = 384
NB = (S - TM0) // TM
TF = 256
WP = (0, 128, 384, 896, 1536)

WM = {"wmA": (0, 15 * L), "wmB": (15 * L, 25 * L), "wmC": (25 * L, 30 * L)}
MIN_RATE = 1.0
SCOPES = False

f32 = jnp.float32
bf16 = jnp.bfloat16
u32 = jnp.uint32


def _cos_turns(t):
    big = 12582912.0
    x = 0.25 - jnp.abs(t - ((t + big) - big))
    x2 = x * x
    return x * (6.283164024 + x2 * (-41.33713150 + x2 * (81.34038544 + x2 * -70.98993683)))


def _make_tables(tab):
    w = lax.broadcasted_iota(jnp.int32, (L, L), 0)
    c = lax.broadcasted_iota(jnp.int32, (L, L), 1)
    inv = 1.0 / (4 * C)
    g_lo = 8 * (w >> 3) + 2 * (w & 3)
    a_lo = (4 * g_lo + 1).astype(f32) * inv
    a_hi = (4 * g_lo + 5).astype(f32) * inv
    off = ((w >> 2) & 1).astype(f32) * 0.25
    for r in range(R):
        n = (R * c + r).astype(f32)
        tab[L * r:L * (r + 1), :] = pltpu.pack_elementwise(
            [_cos_turns(a_lo * n + off), _cos_turns(a_hi * n + off)], packed_dtype=bf16)
    a = (4 * ((w >> 6) * (L // 2) + (c >> 1)) + 1).astype(f32) * inv
    off = (c & 1).astype(f32) * 0.25
    for r in range(R):
        n = (2 * R * (w & (L // 2 - 1)) + r).astype(f32)
        tab[L * (R + r):L * (R + r + 1), :] = pltpu.pack_elementwise(
            [_cos_turns(a * n + off) * (1.0 / C), _cos_turns(a * (n + R) + off) * (1.0 / C)],
            packed_dtype=bf16)


def _layernorm(x):
    m = jnp.mean(x, axis=-1, keepdims=True)
    xc = x - m
    v = jnp.mean(xc * xc, axis=-1, keepdims=True)
    return xc * lax.rsqrt(v + EPS)


def _split(t):
    t = t.reshape(16, 16, L)
    return t[:, :8, :], t[:, 8:, :]


def _radix4(x, sgn):
    (ar, ai), (br, bi), (cr, ci), (dr, di) = x
    s0r, s0i, d0r, d0i = ar + cr, ai + ci, ar - cr, ai - ci
    s1r, s1i, d1r, d1i = br + dr, bi + di, br - dr, bi - di
    o0 = (s0r + s1r, s0i + s1i)
    o2 = (s0r - s1r, s0i - s1i)
    pl_ = (d0r - d1i, d0i + d1r)
    mi_ = (d0r + d1i, d0i - d1r)
    return [o0, pl_, o2, mi_] if sgn > 0 else [o0, mi_, o2, pl_]


T = range(NT)
_z = lambda j: [("z", j, a) for a in range(NC)]
_k = lambda j, al: [("k", j, a) for a in al]
_u = lambda a: [("u", j, a) for j in T]
_iv = lambda jl, al: [("i", j, a) for j in jl for a in al]
_kv = lambda a: [("kv", j, p) for j in T for p in range(a * C // KVR, (a + 1) * C // KVR)]
_m = lambda jl, us, outs: [("mac", j, i, q, us, outs)
                           for j in jl for i in range(16) for q in range(R)]
A3 = (0, 1, 2)

SCHEDULE = [
    (["ssm0"], _z(0) + _k(0, range(NC)), []),
    (["ssm1"], _z(1) + _k(1, [0, 1]), []),
    (["k0", "v0"], _k(1, [2, 3]) + _u(0), _kv(0)),
    (["ssm2"], _z(2) + _k(2, [0, 1]), _m([0, 1], (0,), (0,))),
    (["k1", "v1"], _k(2, [2, 3]) + _u(1), _kv(1)),
    (["ssm3"], _z(3) + _k(3, [0, 1]), _m([2], (0, 1), A3)),
    (["k2", "v2"], _k(3, [2, 3]) + _u(2), _kv(2)),
    (["ssm4"], _iv([0, 1], [0]) + _iv([2], [0, 1]) + _z(4) + _k(4, range(NC)),
     _m([0, 1], A3, (1, 2)) + _m([2], (2,), (2,)) + _m([3], A3, A3)),
    (["q0"], _iv([3], [0]) + _iv([0, 1], [1, 2]) + _iv([4], [0]), _m([4], A3, A3)),
]
PREP_GROUPS = _iv([2], [2]) + _iv([3, 4], [1, 2])

DMA_ORDER = (["sk", "sd", "c", "ssm0", "ssm1", "k0", "v0", "ssm2", "k1", "v1", "ssm3", "k2", "v2",
              "ssm4", "q0", "wmA", "wmB"]
             + [f"w{n}{p}" for p in range(len(WP) - 1) for n in "gu"]
             + ["q1", "wd", "wmC", "k3", "v3"] + [f"q{i + 1}" for i in range(1, NB)])


def _kernel(q_hbm, k_hbm, v_hbm, sk_hbm, ssm_hbm, sd_hbm, wg_hbm, wu_hbm, wd_hbm,
            c_hbm, wm_hbm, o_hbm,
            qb0, qb, kb, vb, ssmb, wgb, wub, wdb, wmb, tab, uwb, ub, kpb, yp, pb, yb, x1b0, x1b, h2b, hb, ob0, ob, skb, sdb, cb_, sem, osem):
    cps = {"sk": (sk_hbm, skb), "sd": (sd_hbm, sdb), "c": (c_hbm, cb_), "wd": (wd_hbm, wdb),
           }
    for j in range(NT):
        cps[f"ssm{j}"] = (ssm_hbm.at[pl.ds(j * L, L), :], ssmb.at[j])
    for a in range(NC):
        n = C // 8 * WPT
        cps[f"k{a}"] = (k_hbm.bitcast(u32).at[pl.ds(a * n, n), :], kb.at[pl.ds(PAD + a * n, n), :])
        cps[f"v{a}"] = (v_hbm.bitcast(u32).at[pl.ds(a * n, n), :], vb.at[pl.ds(a * n, n), :])
    for n, (c0, c1) in WM.items():
        cps[n] = (wm_hbm.at[:, pl.ds(c0, c1 - c0)], wmb.at[:, pl.ds(c0, c1 - c0)])
    cps["q0"] = (q_hbm.at[0, pl.ds(0, TM0), :], qb0)
    for i in range(NB):
        cps[f"q{i + 1}"] = (q_hbm.at[0, pl.ds(TM0 + i * TM, TM), :], qb.at[i])
    for p in range(len(WP) - 1):
        cols = pl.ds(WP[p], WP[p + 1] - WP[p])
        cps[f"wg{p}"] = (wg_hbm.at[:, cols], wgb.at[:, cols])
        cps[f"wu{p}"] = (wu_hbm.at[:, cols], wub.at[:, cols])
    assert sorted(cps) == sorted(DMA_ORDER)

    def cp(name):
        src, dst = cps[name]
        return pltpu.make_async_copy(src, dst, sem.at[DMA_ORDER.index(name)])

    def wait(*names):
        if SCOPES:
            with jax.named_scope("w_" + names[0]):
                for n in names:
                    cp(n).wait()
        else:
            for n in names:
                cp(n).wait()

    for n in DMA_ORDER:
        cp(n).start()

    _make_tables(tab)
    kb[0:PAD, :] = jnp.zeros((PAD, L), u32)
    for ref in (uwb, pb):
        ref[0, 0, 0, pl.ds(0, 8, stride=2), :] = jnp.zeros((8, L), u32)
    ub[0, 0, 0, 0, pl.ds(0, 8, stride=2), :] = jnp.zeros((8, L), f32)
    ri = lax.broadcasted_iota(jnp.int32, (L, L), 0)
    ci = lax.broadcasted_iota(jnp.int32, (L, L), 1)
    sel = jnp.where(ci == R * (ri % 32) + ri // 32, 1.0, 0.0).astype(bf16)

    wait("sk", "sd", "c")
    skt = skb[...].astype(f32)
    sdv = sdb[...].astype(f32).reshape(1, D)
    cv = cb_[...].astype(f32)
    sig = jax.nn.sigmoid(cv)
    cs = jnp.broadcast_to((cv * sig).astype(bf16), (16, D))
    never = jnp.broadcast_to(sig[:, 0:L], (8, L)) > 2.0

    def gate(x, dep):
        if dep is None:
            return x
        return jnp.where(never, dep, jnp.broadcast_to(x, (8, L)))

    def put(dst, j, a, xs):
        for qi in range(R):
            dst[j, a, qi, :, 0:8, :] = xs[qi][0]
            dst[j, a, qi, :, 8:16, :] = xs[qi][1]

    zs = {}
    mod = {}

    def grp_z(j, a):
        z = [lax.dot_general(sel, ssmb[j, :, t * L:(t + 1) * L], (((1,), (1,)), ((), ())),
                             preferred_element_type=f32) for t in range(R * a, R * a + R)]
        zs[j, a] = [jnp.concatenate([z[p][32 * r:32 * (r + 1)] for p in range(R)],
                                    axis=0).astype(bf16) for r in range(R)]
        return [z[0][16 * t:16 * t + 8] for t in range(8)]

    def grp_fwd(ws, dst, j, a, dvec=None):
        t = [jnp.dot(pltpu.bitcast(tab[L * r:L * (r + 1), :], bf16), ws[r],
                     preferred_element_type=f32) for r in range(R)]
        x = [_split(v) for v in t]
        if dvec is not None:
            x[0] = (x[0][0] + dvec[None], x[0][1])
        put(dst, j, a, _radix4(x, -1))
        return [t[0][16 * s:16 * s + 8] for s in range(16)]

    def grp_k(j, a):
        return grp_fwd(zs.pop((j, a)), kpb, j, a,
                       sdv[:, j * L:(j + 1) * L] if a == 0 else None)

    def grp_u(j, a):
        uw = [pltpu.bitcast(uwb[j, a, r], bf16) for r in range(R)]
        return grp_fwd(uw, ub, j, a)

    def grp_i(j, a):
        ys = []
        for r in range(R):
            base = 4 * L + L * r
            g = jnp.concatenate([tab[base:base + L // 2, :], tab[base + L // 2:base + L, :]], axis=1)
            y = jnp.dot(pltpu.bitcast(g, bf16), pltpu.bitcast(pb[j, a, r], bf16),
                        preferred_element_type=f32)
            yb[j, pl.ds(a * C + r, L, stride=R), :] = y
            ys.append(y)
        return ([ys[0][16 * s:16 * s + 8] for s in range(8)]
                + [ys[2][16 * s:16 * s + 8] for s in range(8)])

    def grp_mod(name):
        c0, c1 = WM[name]
        m = jnp.dot(cs, wmb[:, c0:c1], preferred_element_type=f32)
        for c in range(c0, c1, L):
            mod[c // L] = m[0:1, c - c0:c - c0 + L]
        return [m[0:8, c:c + L] for c in range(0, c1 - c0, L)]

    def modv(i):
        return jnp.concatenate([mod[i * NT + n] for n in range(NT)], axis=1)

    def kv_piece(j, p, dep):
        lo = lambda x: lax.bitcast_convert_type(x << 16, f32)
        hi = lambda x: lax.bitcast_convert_type(x & jnp.uint32(0xFFFF0000), f32)
        base = 8 * p * WPT + 4 * j
        ld = lambda ref, o: ref[pl.ds(base + o, 8, stride=WPT), :]
        k = {}
        for n in range(4):
            x = ld(kb, PAD + n)
            k[2 * n], k[2 * n + 1] = lo(x), hi(x)
        k[-3] = hi(ld(kb, PAD - WPT + 2))
        x = ld(kb, PAD - WPT + 3)
        k[-2], k[-1] = lo(x), hi(x)
        w = [skt[t:t + 1, j * L:(j + 1) * L] for t in range(KS)]
        w[0] = gate(w[0], dep)
        kv = {}
        for n in range(4):
            x = ld(vb, n)
            for ph, v in ((2 * n, lo(x)), (2 * n + 1, hi(x))):
                ks = k[ph] * w[0]
                for t in range(1, KS):
                    ks = ks + k[ph - t] * w[t]
                kv[ph] = ks * v
        a, s = divmod(p, C // KVR)
        for r in range(R):
            uwb[j, a, r, 8 * s:8 * s + 8, :] = pltpu.pack_elementwise(
                [kv[r], kv[r + R]], packed_dtype=bf16)

    st = {}

    def mac_piece(j, i, qi, us, outs, dep):
        def ld(ref, a):
            return ref[j, a, qi, i, 0:8, :], ref[j, a, qi, i, 8:16, :]

        lo, hi = us[0], us[-1]
        u = {a: ld(ub, a) for a in us}
        u[lo] = (gate(u[lo][0], dep), u[lo][1])
        ms = sorted({a - n for a in outs for n in us if n <= a})
        k = {m: ld(kpb, m) for m in sorted(set(ms) | {m - 1 for m in ms if m > 0})}
        kp = {m: k[m] if m == 0 else (k[m][0] - k[m - 1][1], k[m][1] + k[m - 1][0]) for m in ms}
        for a in outs:
            yr, yi = ld(yp, a) if lo > 0 else (None, None)
            for n in us:
                if n > a:
                    continue
                (kr, ki), (ur, ui) = kp[a - n], u[n]
                tr = kr * ur - ki * ui
                ti = kr * ui + ki * ur
                yr = tr if yr is None else yr + tr
                yi = ti if yi is None else yi + ti
            if a <= hi:
                st[qi, a] = (yr, yi)
            else:
                yp[j, a, qi, i, 0:8, :] = yr
                yp[j, a, qi, i, 8:16, :] = yi
        if qi == R - 1:
            for a in outs:
                if a > hi:
                    continue
                ps = _radix4([st.pop((n, a)) for n in range(R)], +1)
                for r in range(R):
                    pb[j, a, r, 8 * i:8 * i + 8, :] = pltpu.pack_elementwise(
                        ps[r], packed_dtype=bf16)

    grp_fn = {"z": grp_z, "k": grp_k, "u": grp_u, "i": grp_i,
              "modA": lambda: grp_mod("wmA")}
    free = {"i": 60, "z": 56, "k": 48, "u": 48, "modA": 140, "modB": 100}
    nanch = {"i": 16, "z": 8, "k": 16, "u": 16, "modA": 16}

    def cost(pc):
        if pc[0] == "kv":
            return 88
        us, outs = pc[4], pc[5]
        pairs = [(a, n) for a in outs for n in us if n <= a]
        fin = sum(a <= us[-1] for a in outs)
        return (1 + 2 * len({a - n for a, n in pairs if a > n}) + 8 * len(pairs)
                - (2 * len(outs) if us[0] == 0 else 0) + (20 * fin if pc[3] == R - 1 else 0))

    def emit(pc, dep):
        (kv_piece if pc[0] == "kv" else mac_piece)(*pc[1:], dep)

    for waits, groups, pieces in SCHEDULE:
        wait(*waits)
        cap = sum(nanch[g[0]] * free[g[0]] for g in groups)
        rate = max(1.03 * sum(cost(pc) for pc in pieces) / cap, MIN_RATE)
        credit, done = 0.0, 0
        for g in groups:
            if g[0] == "u":
                need = ("kv", g[1], (g[2] + 1) * (C // KVR) - 1)
                while need in pieces[done:]:
                    emit(pieces[done], None)
                    done += 1
            if g[0] == "i":
                while any(pc[0] == "mac" and pc[1] == g[1] and g[2] in pc[5]
                          for pc in pieces[done:]):
                    emit(pieces[done], None)
                    done += 1
            for dep in grp_fn[g[0]](*g[1:]):
                credit += free[g[0]] * rate
                while done < len(pieces) and credit > 0:
                    credit -= cost(pieces[done])
                    emit(pieces[done], dep)
                    done += 1
        for pc in pieces[done:]:
            emit(pc, None)

    wait("wmA")
    grp_mod("wmA")
    for g in PREP_GROUPS:
        grp_fn[g[0]](*g[1:])
    sa, ca, ga = [modv(i) for i in range(3)]
    a1 = ga * (1.0 + ca)
    b1 = ga * sa

    def o_cp(i, c0, c1):
        cols = pl.ds(c0, c1 - c0)
        if i is None:
            return pltpu.make_async_copy(ob0.at[:, cols], o_hbm.at[0, pl.ds(0, TM0), cols],
                                         osem.at[NB])
        r0 = TM0 + i * TM
        if not isinstance(i, int):
            r0 = pl.multiple_of(r0, L)
        return pltpu.make_async_copy(ob.at[i, :, cols], o_hbm.at[0, pl.ds(r0, TM), cols],
                                     osem.at[i])

    def prep_norm(q_ref, x1_ref, y0, r0, n, dep=None):
        x = q_ref[r0:r0 + n, :].astype(f32)
        if dep is not None:
            x0 = jnp.concatenate([gate(x[s:s + 8, 0:L], dep[s:s + 8]) for s in range(0, n, 8)],
                                 axis=0)
            x = jnp.concatenate([x0, x[:, L:]], axis=1)
        y = jnp.concatenate([yb[j, pl.ds(y0 + r0, n), :] for j in range(NT)], axis=1)
        x1 = x + (_layernorm(x) * a1 + b1) * y
        x1_ref[r0:r0 + n, :] = x1
        return _layernorm(x1)

    n2 = prep_norm(qb0, x1b0, 0, 0, TM0)
    wait("wmB")
    grp_mod("wmB")
    sb = modv(3)
    a2 = 1.0 + modv(4)

    def prep_chain(i, r0, r1):
        y0 = TM0 + i * TM
        if not isinstance(i, int):
            y0 = pl.multiple_of(y0, L)
        dep = None
        for r in range(r0, r1, PR):
            h2 = prep_norm(qb.at[i], x1b.at[i], y0, r, PR, dep) * a2 + sb
            h2b[i, r:r + PR, :] = h2.astype(bf16)
            dep = h2[:, 0:L]

    def gate_up(h2, f0, f1, anchors=None):
        hs = []
        for f in range(f0, f1, TF):
            n = min(TF, f1 - f)
            parts = [h2] if n == TF else [h2[:h2.shape[0] // 2], h2[h2.shape[0] // 2:]]
            prod = []
            for x in parts:
                g = jnp.dot(x, wgb[:, f:f + n], preferred_element_type=f32)
                u = jnp.dot(x, wub[:, f:f + n], preferred_element_type=f32)
                prod.append(g * u)
                if anchors is not None:
                    anchors += [t[s:s + 8, c:c + L] for t in (g, u) for c in range(0, n, L)
                                for s in range(0, x.shape[0], 16)]
            hs.append(jnp.concatenate(prod, axis=0))
        return jnp.concatenate(hs, axis=1).astype(bf16)

    OC = (0, D - L, D)

    def down(hh, gb, i, hook=None):
        n = hh.shape[0]
        x1_ref, o_ref = (x1b0, ob0) if i is None else (x1b.at[i], ob.at[i])
        for c0, c1 in zip(OC[:-1], OC[1:]):
            os = []
            for c in range(c0, c1, L):
                if hook is None:
                    os.append(jnp.dot(hh, wdb[:, c:c + L], preferred_element_type=f32))
                else:
                    ps = [jnp.dot(hh[:, f:f + 4 * L], wdb[f:f + 4 * L, c:c + L],
                                  preferred_element_type=f32) for f in range(0, F, 4 * L)]
                    os.append(ps[0] + ps[1] + ps[2])
                    hook(c // L, [x[s:s + 8] for x in ps for s in range(0, n, 16)])
            o = jnp.concatenate(os, axis=1)
            o_ref[:, c0:c1] = (x1_ref[:, c0:c1] + gb[:, c0:c1] * o).astype(bf16)
            o_cp(i, c0, c1).start()

    def spread(pieces, anchors, first_only=False):
        for n, pc in enumerate(pieces):
            skip = first_only and pc[3] != 0
            emit(pc, None if skip else anchors[n * len(anchors) // len(pieces)])

    last = NC - 1
    for p in range(len(WP) - 1):
        wait(f"wg{p}", f"wu{p}", *(["q1"] if p == len(WP) - 2 else []))
        anchors = []
        if p == 0:
            h2 = (n2 * a2 + sb).astype(bf16)
        hb[:, WP[p]:WP[p + 1]] = gate_up(h2, WP[p], WP[p + 1], anchors)
        if p == len(WP) - 3:
            spread(_m(T, A3, (last,)), anchors)
    prep_chain(0, 0, 10 * PR)
    wait("wd", "wmC", f"k{last}", f"v{last}")
    grp_mod("wmC")
    gb = modv(5)

    prep_chain(0, 10 * PR, TM)
    held = []

    def hook(n, anchors):
        if n in (0, 2):
            held[:] = anchors
        if n == 1:
            spread(_kv(last), held + anchors[:len(anchors) // 2])
            for g in _u(last):
                grp_u(*g[1:])
        if n == 3:
            spread(_m(T, (last,), (last,)), held + anchors[:len(anchors) // 2], True)
            for g in _iv(T, [last]):
                grp_i(*g[1:])

    down(hb[...], gb, None, hook)
    wait(*[f"q{i + 1}" for i in range(1, NB)])

    def ffn(i, carry):
        h2 = h2b[i]
        prep_chain(jnp.minimum(i + 1, NB - 1), 0, TM)
        down(gate_up(h2, 0, F), gb, i)
        return carry

    lax.fori_loop(0, NB, ffn, 0)

    def final_waits():
        for i in [None] + list(range(NB)):
            for c0, c1 in zip(OC[:-1], OC[1:]):
                o_cp(i, c0, c1).wait()

    if SCOPES:
        with jax.named_scope("w_out"):
            final_waits()
    else:
        final_waits()


@jax.jit
def pallas_adaLN_cond__ssm_conv_h3__glu_gated_bilinear__prompt_kernel(
    A_q: jax.Array,
    A_k: jax.Array,
    A_v: jax.Array,
    A_shift_k: jax.Array,
    A_ssm_k: jax.Array,
    A_ssm_D: jax.Array,
    B_x: jax.Array,
    B_w_gate: jax.Array,
    B_w_up: jax.Array,
    B_w_down: jax.Array,
    c: jax.Array,
    w_mod: jax.Array,
):
    del B_x
    tiles = lambda x: x.reshape(S // 8, 8, NT, L).transpose(0, 2, 1, 3).reshape(S * NT, L)
    any_spec = pl.BlockSpec(memory_space=pl.ANY)
    return pl.pallas_call(
        _kernel,
        in_specs=[any_spec] * 11,
        out_specs=any_spec,
        out_shape=jax.ShapeDtypeStruct((1, S, D), bf16),
        scratch_shapes=[
            pltpu.VMEM((TM0, D), bf16),
            pltpu.VMEM((NB, TM, D), bf16),
            pltpu.VMEM((PAD + S // 8 * WPT, L), u32),
            pltpu.VMEM((S // 8 * WPT, L), u32),
            pltpu.VMEM((NT, L, S), bf16),
            pltpu.VMEM((D, F), bf16),
            pltpu.VMEM((D, F), bf16),
            pltpu.VMEM((F, D), bf16),
            pltpu.VMEM((D, 6 * D), bf16),
            pltpu.VMEM((8 * L, L), jnp.uint32),
            pltpu.VMEM((NT, NC, R, L // 2, L), u32),
            pltpu.VMEM((NT, NC, R, 16, 16, L), f32),
            pltpu.VMEM((NT, NC, R, 16, 16, L), f32),
            pltpu.VMEM((NT, NC, R, 16, 16, L), f32),
            pltpu.VMEM((NT, NC, R, L, L), jnp.uint32),
            pltpu.VMEM((NT, S, L), f32),
            pltpu.VMEM((TM0, D), f32),
            pltpu.VMEM((NB, TM, D), f32),
            pltpu.VMEM((NB, TM, D), bf16),
            pltpu.VMEM((TM0, F), bf16),
            pltpu.VMEM((TM0, D), bf16),
            pltpu.VMEM((NB, TM, D), bf16),
            pltpu.VMEM((KS, D), bf16),
            pltpu.VMEM((D,), bf16),
            pltpu.VMEM((1, D), bf16),
            pltpu.SemaphoreType.DMA((len(DMA_ORDER),)),
            pltpu.SemaphoreType.DMA((NB + 1,)),
        ],
        compiler_params=pltpu.CompilerParams(
            vmem_limit_bytes=120 * 1024 * 1024,
            disable_bounds_checks=True, disable_semaphore_checks=True),
        name="adaln_h3_glu",
    )(A_q, tiles(A_k), tiles(A_v), A_shift_k.T, A_ssm_k, A_ssm_D, B_w_gate, B_w_up, B_w_down, c, w_mod)
```

```python
import jax
import jax.numpy as jnp
from jax import lax
import jax.experimental.pallas as pl
import jax.experimental.pallas.tpu as pltpu

S = 2048
D = 640
F = 1536
KS = 4
L = 128
NT = D // L
R = 4
C = R * L
NC = S // C
EPS = 1e-5
WPT = 4 * NT
PAD = 32
PR = 24
TM0 = 512
TM = 384
NB = (S - TM0) // TM
TF = 256
WP = (0, 128, 384, 896, 1536)

WM = {"wmA": (0, 15 * L), "wmB": (15 * L, 25 * L), "wmC": (25 * L, 30 * L)}
WF = 1
PR1 = 128
SCOPES = False

f32 = jnp.float32
bf16 = jnp.bfloat16
u32 = jnp.uint32


def _cos_turns(t):
    x = jnp.abs(t - jnp.floor(t) - 0.5) - 0.25
    x2 = x * x
    return x * (6.283164024 + x2 * (-41.33713150 + x2 * (81.34038544 + x2 * -70.98993683)))


def _tables(inverse):
    shape = (L, 2 * L) if inverse else (2 * L, L)
    rho = lax.broadcasted_iota(jnp.int32, shape, 1 if inverse else 0)
    j = lax.broadcasted_iota(jnp.int32, shape, 0 if inverse else 1)
    if not inverse:
        j = _perm(j)
    a = (4 * (8 * (rho >> 4) + (rho & 7)) + 1).astype(f32) * (1.0 / (4 * C))
    off = ((rho >> 3) & 1).astype(f32) * 0.25
    ts = [_cos_turns(a * (R * j + r).astype(f32) + off) for r in range(R)]
    return [(t * (1.0 / C) if inverse else t).astype(bf16) for t in ts]


def _perm(c):
    return 16 * (c >> 4) + 2 * (c & 7) + ((c >> 3) & 1)


def _layernorm(x):
    m = jnp.mean(x, axis=-1, keepdims=True)
    xc = x - m
    v = jnp.mean(xc * xc, axis=-1, keepdims=True)
    return xc * lax.rsqrt(v + EPS)


def _split(t):
    t = t.reshape(16, 16, L)
    return t[:, :8, :], t[:, 8:, :]


def _radix4(x, sgn):
    (ar, ai), (br, bi), (cr, ci), (dr, di) = x
    s0r, s0i, d0r, d0i = ar + cr, ai + ci, ar - cr, ai - ci
    s1r, s1i, d1r, d1i = br + dr, bi + di, br - dr, bi - di
    o0 = (s0r + s1r, s0i + s1i)
    o2 = (s0r - s1r, s0i - s1i)
    pl_ = (d0r - d1i, d0i + d1r)
    mi_ = (d0r + d1i, d0i - d1r)
    return [o0, pl_, o2, mi_] if sgn > 0 else [o0, mi_, o2, pl_]


T = range(NT)
_z = lambda j: [("z", j, a) for a in range(NC)]
_k = lambda j, al: [("k", j, a) for a in al]
_u = lambda a: [("u", j, a) for j in T]
_iv = lambda jl, al: [("i", j, a) for j in jl for a in al]
_kv = lambda a: [("kv", j, a) for j in T]
_m = lambda jl, us, outs: [("mac", j, us, outs) for j in jl]
A3 = (0, 1, 2)

SCHEDULE = [
    (["ssm0"], _z(0) + _k(0, range(NC)), []),
    (["ssm1"], _z(1) + _k(1, [0, 1]), []),
    (["k0", "v0"], _k(1, [2, 3]) + _u(0), _kv(0)),
    (["ssm2"], _z(2) + _k(2, [0, 1]), _m([0, 1], (0,), (0,))),
    (["k1", "v1"], _k(2, [2, 3]) + _u(1), _kv(1) + _m([2], (0,), (0,))),
    (["ssm3"], _iv([0], [0]) + _z(3) + _k(3, [0, 1]), _m([0, 1, 2], (0, 1), (1,))),
    (["k2", "v2"], _k(3, [2, 3]) + _u(2), _kv(2) + _m([3], (0,), (0,))),
    (["ssm4"], _iv([1, 2, 3], [0]) + _iv([0], [1]) + _z(4) + _k(4, range(NC)),
     _m([0, 1, 2], A3, (2,)) + _m([3], A3, (1, 2))),
    (["q0"], _iv([1, 2, 3], [1]) + _iv([0, 1, 2], [2]) + _iv([4], [0]), _m([4], A3, A3)),
]
PREP_GROUPS = _iv([3], [2]) + _iv([4], [1, 2])

DMA_ORDER = (["sk", "sd", "c", "ssm0", "ssm1", "k0", "v0", "ssm2", "k1", "v1", "ssm3", "k2", "v2",
              "ssm4", "q0", "wmA", "wmB"]
             + [f"w{n}{p}" for p in range(len(WP) - 1) for n in "gu"]
             + ["q1", "wd", "wmC", "k3", "v3"] + [f"q{i + 1}" for i in range(1, NB)])


def _costs(job):
    if job[0] == "kv":
        return [88] * (C // 64)
    us, outs = job[2], job[3]
    pairs = [(a, n) for a in outs for n in us if n <= a]
    mac = (2 * len({a - n for a, n in pairs if a > n}) + 8 * len(pairs)
           - (2 * len(outs) if us[0] == 0 else 0))
    fin = 20 * sum(a <= us[-1] for a in outs)
    if mac < 12 and outs[-1] <= us[-1]:
        return [1 + R * mac + fin] * 16
    return [1 + mac, 1 + mac, 1 + mac, 1 + mac + fin] * 16


def _plan(groups, jobs):
    free = {"i": 56, "z": 56, "k": 47, "u": 46}
    steps = {"i": 16, "z": 8, "k": 16, "u": 16}
    slots = [free[g[0]] for g in groups for _ in range(steps[g[0]])]
    rate = max(1.03 * sum(sum(_costs(j)) for j in jobs) / sum(slots), 1.0)
    plan, credit, n = [], slots[0] * rate, 0
    for job in jobs:
        limit, first = len(slots), 0
        for g in groups:
            if g[1] == job[1] and ((g[0], job[0]) == ("u", "kv") and g[2] == job[2]
                                   or (g[0], job[0]) == ("i", "mac") and g[2] in job[3]):
                limit = min(limit, first)
            first += steps[g[0]]
        idx = []
        for c in _costs(job):
            while credit <= 0 and n + 1 < limit:
                n += 1
                credit += slots[n] * rate
            credit -= c
            idx.append(n)
        plan.append(idx)
    return plan


def _kernel(q_hbm, k_hbm, v_hbm, sk_hbm, ssm_hbm, sd_hbm, wg_hbm, wu_hbm, wd_hbm,
            c_hbm, wm_hbm, o_hbm,
            qb0, qb, kb, vb, ssmb, wgb, wub, wdb, wmb, uwb, ub, kpb, yp, pb, yb, x1b0, x1b, h2b, hb, ob0, ob, skb, sdb, cb_, sem, osem):
    cps = {"sk": (sk_hbm, skb), "sd": (sd_hbm, sdb), "c": (c_hbm, cb_), "wd": (wd_hbm, wdb),
           }
    for j in range(NT):
        cps[f"ssm{j}"] = (ssm_hbm.at[pl.ds(j * L, L), :], ssmb.at[j])
    for a in range(NC):
        n = C * NT // WF
        cps[f"k{a}"] = (k_hbm.at[pl.ds(a * n, n), :], kb.at[pl.ds(2 * PAD // WF + a * n, n), :])
        cps[f"v{a}"] = (v_hbm.at[pl.ds(a * n, n), :], vb.at[pl.ds(a * n, n), :])
    for n, (c0, c1) in WM.items():
        cps[n] = (wm_hbm.at[:, pl.ds(c0, c1 - c0)], wmb.at[:, pl.ds(c0, c1 - c0)])
    cps["q0"] = (q_hbm.at[0, pl.ds(0, TM0), :], qb0)
    for i in range(NB):
        cps[f"q{i + 1}"] = (q_hbm.at[0, pl.ds(TM0 + i * TM, TM), :], qb.at[i])
    for p in range(len(WP) - 1):
        cols = pl.ds(WP[p], WP[p + 1] - WP[p])
        cps[f"wg{p}"] = (wg_hbm.at[:, cols], wgb.at[:, cols])
        cps[f"wu{p}"] = (wu_hbm.at[:, cols], wub.at[:, cols])
    assert sorted(cps) == sorted(DMA_ORDER)

    def cp(name):
        src, dst = cps[name]
        return pltpu.make_async_copy(src, dst, sem.at[DMA_ORDER.index(name)])

    def wait(*names):
        if SCOPES:
            with jax.named_scope("w_" + names[0]):
                for n in names:
                    cp(n).wait()
        else:
            for n in names:
                cp(n).wait()

    for n in DMA_ORDER:
        cp(n).start()

    tabs, ginv = _tables(False), []
    kb[0:2 * PAD // WF, :] = jnp.zeros((2 * PAD // WF, L), kb.dtype)
    kw, vw = (kb, vb) if WF == 2 else (kb.bitcast(u32), vb.bitcast(u32))
    ub[0, 0, 0, 0, pl.ds(0, 8, stride=2), :] = jnp.zeros((8, L), f32)
    ri = lax.broadcasted_iota(jnp.int32, (L, L), 0)
    ci = lax.broadcasted_iota(jnp.int32, (L, L), 1)
    sel = jnp.where(ci == R * _perm(ri & 31) + (ri >> 5), 1.0, 0.0).astype(bf16)

    wait("sk", "sd", "c")
    skt = skb[...].astype(f32)
    sdv = sdb[...].astype(f32).reshape(1, D)
    cv = cb_[...].astype(f32)
    sig = jax.nn.sigmoid(cv)
    cs = jnp.broadcast_to((cv * sig).astype(bf16), (16, D))
    one = sig[:, 0:L]

    def gate(x, deps):
        dep = jnp.concatenate(deps, axis=0).reshape(x.shape)
        return jnp.where(jnp.broadcast_to(one, x.shape) > 2.0, dep, x)

    def put(dst, j, a, xs):
        for qi in range(R):
            dst[j, a, qi] = jnp.concatenate(xs[qi], axis=1)

    zs = {}
    mod = {}

    def grp_z(j, a):
        z = [lax.dot_general(sel, ssmb[j, :, t * L:(t + 1) * L], (((1,), (1,)), ((), ())),
                             preferred_element_type=f32) for t in range(R * a, R * a + R)]
        zs[j, a] = [jnp.concatenate([z[p][32 * r:32 * (r + 1)] for p in range(R)],
                                    axis=0).astype(bf16) for r in range(R)]
        return [z[0][16 * t:16 * t + 8] for t in range(8)]

    def grp_fwd(ws, dst, j, a, dvec=None):
        t = [jnp.dot(tabs[r], ws[r], preferred_element_type=f32) for r in range(R)]
        x = [_split(v) for v in t]
        if dvec is not None:
            x[0] = (x[0][0] + dvec[None], x[0][1])
        put(dst, j, a, _radix4(x, -1))
        return [t[0][16 * s:16 * s + 8] for s in range(16)]

    def grp_k(j, a):
        return grp_fwd(zs.pop((j, a)), kpb, j, a,
                       sdv[:, j * L:(j + 1) * L] if a == 0 else None)

    def grp_u(j, a):
        uw = [uwb[j, a, r] for r in range(R)]
        return grp_fwd(uw, ub, j, a)

    def grp_i(j, a):
        ys = []
        for r in range(R):
            y = jnp.dot(ginv[r], pb[j, a, r], preferred_element_type=f32)
            yb[j, pl.ds(a * C + r, L, stride=R), :] = y
            ys.append(y)
        return ([ys[0][16 * s:16 * s + 8] for s in range(8)]
                + [ys[2][16 * s:16 * s + 8] for s in range(8)])

    def grp_mod(name):
        c0, c1 = WM[name]
        m = jnp.dot(cs, wmb[:, c0:c1], preferred_element_type=f32)
        for c in range(c0, c1, L):
            mod[c // L] = m[0:1, c - c0:c - c0 + L]
        return [m[0:8, c:c + L] for c in range(0, c1 - c0, L)]

    def modv(i):
        return jnp.concatenate([mod[i * NT + n] for n in range(NT)], axis=1)

    def job_kv(j, a, deps):
        lo = lambda x: lax.bitcast_convert_type(x << 16, f32)
        hi = lambda x: lax.bitcast_convert_type(x & jnp.uint32(0xFFFF0000), f32)
        n = C // 8
        ld = lambda ref, o: ref[pl.ds(a * n * WPT + 4 * j + o, n, stride=WPT), :]
        k = {}
        for m in range(4):
            x = ld(kw, PAD + m)
            k[2 * m], k[2 * m + 1] = lo(x), hi(x)
        k[-3] = hi(ld(kw, PAD - WPT + 2))
        x = ld(kw, PAD - WPT + 3)
        k[-2], k[-1] = lo(x), hi(x)
        w = [skt[t:t + 1, j * L:(j + 1) * L] for t in range(KS)]
        w[0] = gate(jnp.broadcast_to(w[0], (n, L)), deps)
        kv = {}
        for m in range(4):
            x = ld(vw, m)
            for ph, v in ((2 * m, lo(x)), (2 * m + 1, hi(x))):
                ks = k[ph] * w[0]
                for t in range(1, KS):
                    ks = ks + k[ph - t] * w[t]
                kv[ph] = (ks * v).reshape(n // 8, 8, L)
        for r in range(R):
            uwb[j, a, r] = jnp.concatenate([kv[r], kv[r + R]], axis=1).reshape(L, L).astype(bf16)

    def job_mac(j, us, outs, deps):
        ld = lambda ref, a: (ref[j, a, :, :, 0:8, :], ref[j, a, :, :, 8:16, :])
        lo, hi = us[0], us[-1]
        u = {a: ld(ub, a) for a in us}
        if len(deps) == 16:
            ur = jnp.concatenate([gate(u[lo][0][0:1], deps), u[lo][0][1:]], axis=0)
        else:
            ur = gate(u[lo][0], [deps[R * i + qi] for qi in range(R) for i in range(16)])
        u[lo] = (ur, u[lo][1])
        ms = sorted({a - n for a in outs for n in us if n <= a})
        k = {m: ld(kpb, m) for m in sorted(set(ms) | {m - 1 for m in ms if m > 0})}
        kp = {m: k[m] if m == 0 else (k[m][0] - k[m - 1][1], k[m][1] + k[m - 1][0]) for m in ms}
        for a in outs:
            yr, yi = ld(yp, a) if lo > 0 else (None, None)
            for n in us:
                if n > a:
                    continue
                (kr, ki), (ur, ui) = kp[a - n], u[n]
                tr = kr * ur - ki * ui
                ti = kr * ui + ki * ur
                yr = tr if yr is None else yr + tr
                yi = ti if yi is None else yi + ti
            if a > hi:
                yp[j, a] = jnp.concatenate([yr, yi], axis=2)
                continue
            ps = _radix4([(yr[qi], yi[qi]) for qi in range(R)], +1)
            for r in range(R):
                pb[j, a, r] = jnp.concatenate(ps[r], axis=1).reshape(2 * L, L).astype(bf16)

    grp_fn = {"z": grp_z, "k": grp_k, "u": grp_u, "i": grp_i}
    job_fn = {"kv": job_kv, "mac": job_mac}

    for waits, groups, jobs in SCHEDULE:
        wait(*waits)
        plan = _plan(groups, jobs)
        anchors, done = [], 0
        for g in groups + [None]:
            while done < len(jobs) and max(plan[done]) < len(anchors):
                job_fn[jobs[done][0]](*jobs[done][1:], [anchors[n] for n in plan[done]])
                done += 1
            if g is not None:
                anchors += grp_fn[g[0]](*g[1:])
        assert done == len(jobs)
        if waits == ["ssm1"]:
            ginv += _tables(True)

    n1, dep = [], None
    for r in range(0, TM0, PR1):
        x = qb0[r:r + PR1, :].astype(f32)
        if dep is not None:
            x = jnp.concatenate([gate(x[:, 0:L], [dep]), x[:, L:]], axis=1)
        n1.append(_layernorm(x))
        dep = n1[-1][:, 0:L]
    n1 = jnp.concatenate(n1, axis=0)
    wait("wmA")
    grp_mod("wmA")
    for g in PREP_GROUPS:
        grp_fn[g[0]](*g[1:])
    sa, ca, ga = [modv(i) for i in range(3)]
    a1 = ga * (1.0 + ca)
    b1 = ga * sa

    def o_cp(i, c0, c1):
        cols = pl.ds(c0, c1 - c0)
        if i is None:
            return pltpu.make_async_copy(ob0.at[:, cols], o_hbm.at[0, pl.ds(0, TM0), cols],
                                         osem.at[NB])
        r0 = TM0 + i * TM
        if not isinstance(i, int):
            r0 = pl.multiple_of(r0, L)
        return pltpu.make_async_copy(ob.at[i, :, cols], o_hbm.at[0, pl.ds(r0, TM), cols],
                                     osem.at[i])

    def prep_norm(q_ref, x1_ref, y0, r0, n, dep=None, n1=None):
        x = q_ref[r0:r0 + n, :].astype(f32)
        if dep is not None:
            x = jnp.concatenate([gate(x[:, 0:L], [dep]), x[:, L:]], axis=1)
        y = jnp.concatenate([yb[j, pl.ds(y0 + r0, n), :] for j in range(NT)], axis=1)
        x1 = x + ((_layernorm(x) if n1 is None else n1) * a1 + b1) * y
        x1_ref[r0:r0 + n, :] = x1
        return _layernorm(x1)

    n2 = prep_norm(qb0, x1b0, 0, 0, TM0, None, n1)
    wait("wmB")
    grp_mod("wmB")
    sb = modv(3)
    a2 = 1.0 + modv(4)

    def prep_chain(i, r0, r1):
        y0 = TM0 + i * TM
        if not isinstance(i, int):
            y0 = pl.multiple_of(y0, L)
        dep = None
        for r in range(r0, r1, PR):
            h2 = prep_norm(qb.at[i], x1b.at[i], y0, r, PR, dep) * a2 + sb
            h2b[i, r:r + PR, :] = h2.astype(bf16)
            dep = h2[:, 0:L]

    def gate_up(h2, f0, f1, anchors=None):
        hs = []
        for f in range(f0, f1, TF):
            n = min(TF, f1 - f)
            parts = [h2] if n == TF else [h2[:h2.shape[0] // 2], h2[h2.shape[0] // 2:]]
            prod = []
            for x in parts:
                g = jnp.dot(x, wgb[:, f:f + n], preferred_element_type=f32)
                u = jnp.dot(x, wub[:, f:f + n], preferred_element_type=f32)
                prod.append(g * u)
                if anchors is not None:
                    anchors += [t[s:s + 8, c:c + L] for t in (g, u) for c in range(0, n, L)
                                for s in range(0, x.shape[0], 16)]
            hs.append(jnp.concatenate(prod, axis=0))
        return jnp.concatenate(hs, axis=1).astype(bf16)

    OC = (0, D - L, D)

    def down(hh, gb, i, hook=None):
        n = hh.shape[0]
        x1_ref, o_ref = (x1b0, ob0) if i is None else (x1b.at[i], ob.at[i])
        for c0, c1 in zip(OC[:-1], OC[1:]):
            os = []
            for c in range(c0, c1, L):
                if hook is None:
                    os.append(jnp.dot(hh, wdb[:, c:c + L], preferred_element_type=f32))
                else:
                    ps = [jnp.dot(hh[:, f:f + 4 * L], wdb[f:f + 4 * L, c:c + L],
                                  preferred_element_type=f32) for f in range(0, F, 4 * L)]
                    os.append(ps[0] + ps[1] + ps[2])
                    hook(c // L, [x[s:s + 8] for x in ps for s in range(0, n, 16)])
            o = jnp.concatenate(os, axis=1)
            o_ref[:, c0:c1] = (x1_ref[:, c0:c1] + gb[:, c0:c1] * o).astype(bf16)
            o_cp(i, c0, c1).start()

    def spread(jobs, anchors):
        total, n = sum(len(_costs(j)) for j in jobs), 0
        for job in jobs:
            m = len(_costs(job))
            job_fn[job[0]](*job[1:], [anchors[(n + i) * len(anchors) // total] for i in range(m)])
            n += m

    last = NC - 1
    for p in range(len(WP) - 1):
        wait(f"wg{p}", f"wu{p}", *(["q1"] if p == len(WP) - 2 else []))
        anchors = []
        if p == 0:
            h2 = (n2 * a2 + sb).astype(bf16)
        hb[:, WP[p]:WP[p + 1]] = gate_up(h2, WP[p], WP[p + 1], anchors)
        if p == len(WP) - 3:
            spread(_m(T, A3, (last,)), anchors)
    prep_chain(0, 0, 10 * PR)
    wait("wd", "wmC", f"k{last}", f"v{last}")
    grp_mod("wmC")
    gb = modv(5)

    prep_chain(0, 10 * PR, TM)
    held = []

    def hook(n, anchors):
        if n in (0, 2):
            held[:] = anchors
        if n == 1:
            spread(_kv(last), held + anchors[:len(anchors) // 2])
            for g in _u(last):
                grp_u(*g[1:])
        if n == 3:
            spread(_m(T, (last,), (last,)), held + anchors[:len(anchors) // 2])
            for g in _iv(T, [last]):
                grp_i(*g[1:])

    down(hb[...], gb, None, hook)
    wait(*[f"q{i + 1}" for i in range(1, NB)])

    def ffn(i, carry):
        h2 = h2b[i]
        prep_chain(jnp.minimum(i + 1, NB - 1), 0, TM)
        down(gate_up(h2, 0, F), gb, i)
        return carry

    lax.fori_loop(0, NB, ffn, 0)

    def final_waits():
        for i in [None] + list(range(NB)):
            for c0, c1 in zip(OC[:-1], OC[1:]):
                o_cp(i, c0, c1).wait()

    if SCOPES:
        with jax.named_scope("w_out"):
            final_waits()
    else:
        final_waits()


@jax.jit
def pallas_adaLN_cond__ssm_conv_h3__glu_gated_bilinear__prompt_kernel(
    A_q: jax.Array,
    A_k: jax.Array,
    A_v: jax.Array,
    A_shift_k: jax.Array,
    A_ssm_k: jax.Array,
    A_ssm_D: jax.Array,
    B_x: jax.Array,
    B_w_gate: jax.Array,
    B_w_up: jax.Array,
    B_w_down: jax.Array,
    c: jax.Array,
    w_mod: jax.Array,
):
    del B_x
    tiles = lambda x: x.reshape(S // 8, 8, NT, L).transpose(0, 2, 1, 3).reshape(S * NT, L)
    kdt = bf16
    if WF == 2:
        kdt = u32
        tiles = lambda x: lax.bitcast_convert_type(
            x.reshape(S // 8, 4, 2, NT, L).transpose(0, 3, 1, 4, 2), u32).reshape(S * NT // 2, L)
    any_spec = pl.BlockSpec(memory_space=pl.ANY)
    return pl.pallas_call(
        _kernel,
        in_specs=[any_spec] * 11,
        out_specs=any_spec,
        out_shape=jax.ShapeDtypeStruct((1, S, D), bf16),
        scratch_shapes=[
            pltpu.VMEM((TM0, D), bf16),
            pltpu.VMEM((NB, TM, D), bf16),
            pltpu.VMEM(((4 * PAD + S * NT) // WF, L), kdt),
            pltpu.VMEM(((2 * PAD + S * NT) // WF, L), kdt),
            pltpu.VMEM((NT, L, S), bf16),
            pltpu.VMEM((D, F), bf16),
            pltpu.VMEM((D, F), bf16),
            pltpu.VMEM((F, D), bf16),
            pltpu.VMEM((D, 6 * D), bf16),
            pltpu.VMEM((NT, NC, R, L, L), bf16),
            pltpu.VMEM((NT, NC, R, 16, 16, L), f32),
            pltpu.VMEM((NT, NC, R, 16, 16, L), f32),
            pltpu.VMEM((NT, NC, R, 16, 16, L), f32),
            pltpu.VMEM((NT, NC, R, 2 * L, L), bf16),
            pltpu.VMEM((NT, S + 32, L), f32),
            pltpu.VMEM((TM0, D), f32),
            pltpu.VMEM((NB, TM, D), f32),
            pltpu.VMEM((NB, TM, D), bf16),
            pltpu.VMEM((TM0, F), bf16),
            pltpu.VMEM((TM0, D), bf16),
            pltpu.VMEM((NB, TM, D), bf16),
            pltpu.VMEM((KS, D), bf16),
            pltpu.VMEM((D,), bf16),
            pltpu.VMEM((1, D), bf16),
            pltpu.SemaphoreType.DMA((len(DMA_ORDER),)),
            pltpu.SemaphoreType.DMA((NB + 1,)),
        ],
        compiler_params=pltpu.CompilerParams(
            vmem_limit_bytes=120 * 1024 * 1024,
            disable_bounds_checks=True, disable_semaphore_checks=True),
        name="adaln_h3_glu",
    )(A_q, tiles(A_k), tiles(A_v), A_shift_k.T, A_ssm_k, A_ssm_D, B_w_gate, B_w_up, B_w_down, c, w_mod)
```

```python
import jax
import jax.numpy as jnp
from jax import lax
import jax.experimental.pallas as pl
import jax.experimental.pallas.tpu as pltpu

S = 2048
D = 640
F = 1536
KS = 4
L = 128
NT = D // L
R = 4
C = R * L
NC = S // C
EPS = 1e-5
WPT = 4 * NT
PAD = 32
PR = 24
TM0 = 512
TM = 384
NB = (S - TM0) // TM
TF = 256
KP = (0, 1, 2, 3, 5)

WM = {"mA": (0, 10), "c0": (20, 21), "mB": (10, 16), "s1": (16, 17), "c1": (21, 22),
      "s2": (17, 18), "c2": (22, 23), "s3": (18, 20), "c3": (23, 25), "mG": (25, 30)}
WF = 1
PR1 = 64
H0 = 320
PR2 = 64
SCOPES = False

f32 = jnp.float32
bf16 = jnp.bfloat16
u32 = jnp.uint32


def _cos_turns(t):
    x = jnp.abs(t - jnp.floor(t) - 0.5) - 0.25
    x2 = x * x
    return x * (6.283164024 + x2 * (-41.33713150 + x2 * (81.34038544 + x2 * -70.98993683)))


def _tables(inverse):
    shape = (L, 2 * L) if inverse else (2 * L, L)
    rho = lax.broadcasted_iota(jnp.int32, shape, 1 if inverse else 0)
    j = lax.broadcasted_iota(jnp.int32, shape, 0 if inverse else 1)
    if not inverse:
        j = _perm(j)
    a = (4 * (8 * (rho >> 4) + (rho & 7)) + 1).astype(f32) * (1.0 / (4 * C))
    off = ((rho >> 3) & 1).astype(f32) * 0.25
    ts = [_cos_turns(a * (R * j + r).astype(f32) + off) for r in range(R)]
    return [(t * (1.0 / C) if inverse else t).astype(bf16) for t in ts]


def _perm(c):
    return 16 * (c >> 4) + 2 * (c & 7) + ((c >> 3) & 1)


def _layernorm(x):
    m = jnp.mean(x, axis=-1, keepdims=True)
    xc = x - m
    v = jnp.mean(xc * xc, axis=-1, keepdims=True)
    return xc * lax.rsqrt(v + EPS)


def _split(t):
    t = t.reshape(16, 16, L)
    return t[:, :8, :], t[:, 8:, :]


def _radix4(x, sgn):
    (ar, ai), (br, bi), (cr, ci), (dr, di) = x
    s0r, s0i, d0r, d0i = ar + cr, ai + ci, ar - cr, ai - ci
    s1r, s1i, d1r, d1i = br + dr, bi + di, br - dr, bi - di
    o0 = (s0r + s1r, s0i + s1i)
    o2 = (s0r - s1r, s0i - s1i)
    pl_ = (d0r - d1i, d0i + d1r)
    mi_ = (d0r + d1i, d0i - d1r)
    return [o0, pl_, o2, mi_] if sgn > 0 else [o0, mi_, o2, pl_]


T = range(NT)
_z = lambda j: [("z", j, a) for a in range(NC)]
_k = lambda j, al: [("k", j, a) for a in al]
_u = lambda a: [("u", j, a) for j in T]
_iv = lambda jl, al: [("i", j, a) for j in jl for a in al]
_kv = lambda a: [("kv", j, a) for j in T]
_m = lambda jl, us, outs: [("mac", j, us, outs) for j in jl]
A3 = (0, 1, 2)

SCHEDULE = [
    (["ssm0"], _z(0) + _k(0, range(NC)), []),
    (["ssm1"], _z(1) + _k(1, [0, 1]), []),
    (["k0", "v0"], _k(1, [2, 3]) + _u(0), _kv(0)),
    (["ssm2"], _z(2) + _k(2, [0, 1]), _m([0, 1], (0,), (0,))),
    (["k1", "v1"], _k(2, [2, 3]) + _u(1), _kv(1) + _m([2], (0,), (0,))),
    (["ssm3"], _iv([0], [0]) + _z(3) + _k(3, [0, 1]), _m([0, 1, 2], (0, 1), (1,))),
    (["k2", "v2"], _k(3, [2, 3]) + _u(2), _kv(2) + _m([3], (0,), (0,))),
    (["ssm4"], _iv([1, 2, 3], [0]) + _iv([0], [1]) + _z(4) + _k(4, range(NC)),
     _m([0, 1, 2], A3, (2,)) + _m([3], A3, (1, 2))),
    (["q0", "mA", "c0"], _iv([1, 2, 3], [1]) + _iv([0, 1, 2], [2]) + _iv([4], [0]),
     _m([4], A3, A3)),
]
PREP_GROUPS = _iv([3], [2]) + _iv([4], [1, 2])

DMA_ORDER = (["sk", "sd", "c", "ssm0", "ssm1", "k0", "v0", "ssm2", "k1", "v1", "ssm3", "k2", "v2",
              "ssm4", "q0", "mA", "c0", "mB", "qh", "wg0", "wu0", "s1", "c1", "wg1", "wu1", "s2", "c2",
              "wg2", "wu2", "s3", "c3", "wg3", "wu3", "q1", "wd", "mG", "k3", "v3"]
             + [f"q{i + 1}" for i in range(1, NB)])


def _costs(job):
    if job[0] == "kv":
        return [88] * (C // 64)
    us, outs = job[2], job[3]
    pairs = [(a, n) for a in outs for n in us if n <= a]
    mac = (2 * len({a - n for a, n in pairs if a > n}) + 8 * len(pairs)
           - (2 * len(outs) if us[0] == 0 else 0))
    fin = 20 * sum(a <= us[-1] for a in outs)
    if mac < 12 and outs[-1] <= us[-1]:
        return [1 + R * mac + fin] * 16
    return [1 + mac, 1 + mac, 1 + mac, 1 + mac + fin] * 16


def _plan(groups, jobs):
    free = {"i": 56, "z": 56, "k": 47, "u": 46}
    steps = {"i": 16, "z": 8, "k": 16, "u": 16}
    slots = [free[g[0]] for g in groups for _ in range(steps[g[0]])]
    rate = max(1.03 * sum(sum(_costs(j)) for j in jobs) / sum(slots), 1.0)
    plan, credit, n = [], slots[0] * rate, 0
    for job in jobs:
        limit, first = len(slots), 0
        for g in groups:
            if g[1] == job[1] and ((g[0], job[0]) == ("u", "kv") and g[2] == job[2]
                                   or (g[0], job[0]) == ("i", "mac") and g[2] in job[3]):
                limit = min(limit, first)
            first += steps[g[0]]
        idx = []
        for c in _costs(job):
            while credit <= 0 and n + 1 < limit:
                n += 1
                credit += slots[n] * rate
            credit -= c
            idx.append(n)
        plan.append(idx)
    return plan


def _kernel(q_hbm, k_hbm, v_hbm, sk_hbm, ssm_hbm, sd_hbm, wg_hbm, wu_hbm, wd_hbm,
            c_hbm, wm_hbm, o_hbm,
            qb0, qb, kb, vb, ssmb, wgb, wub, wdb, wmb, uwb, ub, kpb, yp, pb, yb, x1b0, x1b, h2b, gub, hb, ob0, ob, skb, sdb, cb_, sem, osem):
    cps = {"sk": (sk_hbm, skb), "sd": (sd_hbm, sdb), "c": (c_hbm, cb_), "wd": (wd_hbm, wdb),
           }
    for j in range(NT):
        cps[f"ssm{j}"] = (ssm_hbm.at[pl.ds(j * L, L), :], ssmb.at[j])
    for a in range(NC):
        n = C * NT // WF
        cps[f"k{a}"] = (k_hbm.at[pl.ds(a * n, n), :], kb.at[pl.ds(2 * PAD // WF + a * n, n), :])
        cps[f"v{a}"] = (v_hbm.at[pl.ds(a * n, n), :], vb.at[pl.ds(a * n, n), :])
    for n, (c0, c1) in WM.items():
        cols = pl.ds(c0 * L, (c1 - c0) * L)
        cps[n] = (wm_hbm.at[:, cols], wmb.at[:, cols])
    cps["q0"] = (q_hbm.at[0, pl.ds(0, H0), :], qb0.at[pl.ds(0, H0), :])
    cps["qh"] = (q_hbm.at[0, pl.ds(H0, TM0 - H0), :], qb0.at[pl.ds(H0, TM0 - H0), :])
    for i in range(NB):
        cps[f"q{i + 1}"] = (q_hbm.at[0, pl.ds(TM0 + i * TM, TM), :], qb.at[i])
    for p in range(len(KP) - 1):
        rows = pl.ds(KP[p] * L, (KP[p + 1] - KP[p]) * L)
        cps[f"wg{p}"] = (wg_hbm.at[rows, :], wgb.at[rows, :])
        cps[f"wu{p}"] = (wu_hbm.at[rows, :], wub.at[rows, :])
    assert sorted(cps) == sorted(DMA_ORDER)

    def cp(name):
        src, dst = cps[name]
        return pltpu.make_async_copy(src, dst, sem.at[DMA_ORDER.index(name)])

    def wait(*names):
        if SCOPES:
            with jax.named_scope("w_" + names[0]):
                for n in names:
                    cp(n).wait()
        else:
            for n in names:
                cp(n).wait()

    for n in DMA_ORDER:
        cp(n).start()

    tabs, ginv = _tables(False), []
    kb[0:2 * PAD // WF, :] = jnp.zeros((2 * PAD // WF, L), kb.dtype)
    kw, vw = (kb, vb) if WF == 2 else (kb.bitcast(u32), vb.bitcast(u32))
    ub[0, 0, 0, 0, pl.ds(0, 8, stride=2), :] = jnp.zeros((8, L), f32)
    ri = lax.broadcasted_iota(jnp.int32, (L, L), 0)
    ci = lax.broadcasted_iota(jnp.int32, (L, L), 1)
    sel = jnp.where(ci == R * _perm(ri & 31) + (ri >> 5), 1.0, 0.0).astype(bf16)

    wait("sk", "sd", "c")
    skt = skb[...].astype(f32)
    sdv = sdb[...].astype(f32).reshape(1, D)
    cv = cb_[...].astype(f32)
    sig = jax.nn.sigmoid(cv)
    cs = jnp.broadcast_to((cv * sig).astype(bf16), (16, D))
    one = sig[:, 0:L]

    def gate(x, deps):
        dep = jnp.concatenate(deps, axis=0).reshape(x.shape)
        return jnp.where(jnp.broadcast_to(one, x.shape) > 2.0, dep, x)

    def put(dst, j, a, xs):
        for qi in range(R):
            dst[j, a, qi] = jnp.concatenate(xs[qi], axis=1)

    zs = {}
    mod = {}

    def grp_z(j, a):
        z = [lax.dot_general(sel, ssmb[j, :, t * L:(t + 1) * L], (((1,), (1,)), ((), ())),
                             preferred_element_type=f32) for t in range(R * a, R * a + R)]
        zs[j, a] = [jnp.concatenate([z[p][32 * r:32 * (r + 1)] for p in range(R)],
                                    axis=0).astype(bf16) for r in range(R)]
        return [z[0][16 * t:16 * t + 8] for t in range(8)]

    def grp_fwd(ws, dst, j, a, dvec=None):
        t = [jnp.dot(tabs[r], ws[r], preferred_element_type=f32) for r in range(R)]
        x = [_split(v) for v in t]
        if dvec is not None:
            x[0] = (x[0][0] + dvec[None], x[0][1])
        put(dst, j, a, _radix4(x, -1))
        return [t[0][16 * s:16 * s + 8] for s in range(16)]

    def grp_k(j, a):
        return grp_fwd(zs.pop((j, a)), kpb, j, a,
                       sdv[:, j * L:(j + 1) * L] if a == 0 else None)

    def grp_u(j, a):
        uw = [uwb[j, a, r] for r in range(R)]
        return grp_fwd(uw, ub, j, a)

    def grp_i(j, a):
        ys = []
        for r in range(R):
            y = jnp.dot(ginv[r], pb[j, a, r], preferred_element_type=f32)
            yb[j, pl.ds(a * C + r, L, stride=R), :] = y
            ys.append(y)
        return ([ys[0][16 * s:16 * s + 8] for s in range(8)]
                + [ys[2][16 * s:16 * s + 8] for s in range(8)])

    def grp_mod(*names):
        for name in names:
            c0, c1 = WM[name]
            m = jnp.dot(cs, wmb[:, c0 * L:c1 * L], preferred_element_type=f32)
            for c in range(c0, c1):
                mod[c] = m[0:1, (c - c0) * L:(c - c0 + 1) * L]

    def modv(i, t0=0, t1=NT):
        return jnp.concatenate([mod[i * NT + n] for n in range(t0, t1)], axis=1)

    def job_kv(j, a, deps):
        lo = lambda x: lax.bitcast_convert_type(x << 16, f32)
        hi = lambda x: lax.bitcast_convert_type(x & jnp.uint32(0xFFFF0000), f32)
        n = C // 8
        ld = lambda ref, o: ref[pl.ds(a * n * WPT + 4 * j + o, n, stride=WPT), :]
        k = {}
        for m in range(4):
            x = ld(kw, PAD + m)
            k[2 * m], k[2 * m + 1] = lo(x), hi(x)
        k[-3] = hi(ld(kw, PAD - WPT + 2))
        x = ld(kw, PAD - WPT + 3)
        k[-2], k[-1] = lo(x), hi(x)
        w = [skt[t:t + 1, j * L:(j + 1) * L] for t in range(KS)]
        w[0] = gate(jnp.broadcast_to(w[0], (n, L)), deps)
        kv = {}
        for m in range(4):
            x = ld(vw, m)
            for ph, v in ((2 * m, lo(x)), (2 * m + 1, hi(x))):
                ks = k[ph] * w[0]
                for t in range(1, KS):
                    ks = ks + k[ph - t] * w[t]
                kv[ph] = (ks * v).reshape(n // 8, 8, L)
        for r in range(R):
            uwb[j, a, r] = jnp.concatenate([kv[r], kv[r + R]], axis=1).reshape(L, L).astype(bf16)

    def job_mac(j, us, outs, deps):
        ld = lambda ref, a: (ref[j, a, :, :, 0:8, :], ref[j, a, :, :, 8:16, :])
        lo, hi = us[0], us[-1]
        u = {a: ld(ub, a) for a in us}
        if len(deps) == 16:
            ur = jnp.concatenate([gate(u[lo][0][0:1], deps), u[lo][0][1:]], axis=0)
        else:
            ur = gate(u[lo][0], [deps[R * i + qi] for qi in range(R) for i in range(16)])
        u[lo] = (ur, u[lo][1])
        ms = sorted({a - n for a in outs for n in us if n <= a})
        k = {m: ld(kpb, m) for m in sorted(set(ms) | {m - 1 for m in ms if m > 0})}
        kp = {m: k[m] if m == 0 else (k[m][0] - k[m - 1][1], k[m][1] + k[m - 1][0]) for m in ms}
        for a in outs:
            yr, yi = ld(yp, a) if lo > 0 else (None, None)
            for n in us:
                if n > a:
                    continue
                (kr, ki), (ur, ui) = kp[a - n], u[n]
                tr = kr * ur - ki * ui
                ti = kr * ui + ki * ur
                yr = tr if yr is None else yr + tr
                yi = ti if yi is None else yi + ti
            if a > hi:
                yp[j, a] = jnp.concatenate([yr, yi], axis=2)
                continue
            ps = _radix4([(yr[qi], yi[qi]) for qi in range(R)], +1)
            for r in range(R):
                pb[j, a, r] = jnp.concatenate(ps[r], axis=1).reshape(2 * L, L).astype(bf16)

    grp_fn = {"z": grp_z, "k": grp_k, "u": grp_u, "i": grp_i}
    job_fn = {"kv": job_kv, "mac": job_mac}

    for waits, groups, jobs in SCHEDULE:
        wait(*waits)
        plan = _plan(groups, jobs)
        anchors, done = [], 0
        for g in groups + [None]:
            while done < len(jobs) and max(plan[done]) < len(anchors):
                job_fn[jobs[done][0]](*jobs[done][1:], [anchors[n] for n in plan[done]])
                done += 1
            if g is not None:
                anchors += grp_fn[g[0]](*g[1:])
        assert done == len(jobs)
        if waits == ["ssm1"]:
            ginv += _tables(True)

    n1, dep = [], None
    for r in range(0, H0, PR1):
        x = qb0[r:r + PR1, :].astype(f32)
        if dep is not None:
            x = jnp.concatenate([gate(x[:, 0:L], [dep]), x[:, L:]], axis=1)
        n1.append(_layernorm(x))
        dep = n1[-1][:, 0:L]
    n1 = jnp.concatenate(n1, axis=0)
    grp_mod("mA", "c0")
    wait("mB")
    grp_mod("mB")
    for g in PREP_GROUPS:
        grp_fn[g[0]](*g[1:])
    sa, ca, ga = [modv(i) for i in range(3)]
    a1 = ga * (1.0 + ca)
    b1 = ga * sa

    def o_cp(i, c0, c1):
        cols = pl.ds(c0, c1 - c0)
        if i is None:
            return pltpu.make_async_copy(ob0.at[:, cols], o_hbm.at[0, pl.ds(0, TM0), cols],
                                         osem.at[NB])
        r0 = TM0 + i * TM
        if not isinstance(i, int):
            r0 = pl.multiple_of(r0, L)
        return pltpu.make_async_copy(ob.at[i, :, cols], o_hbm.at[0, pl.ds(r0, TM), cols],
                                     osem.at[i])

    def prep_norm(q_ref, x1_ref, y0, r0, n, dep=None, n1=None):
        x = q_ref[r0:r0 + n, :].astype(f32)
        if dep is not None:
            x = jnp.concatenate([gate(x[:, 0:L], [dep]), x[:, L:]], axis=1)
        y = jnp.concatenate([yb[j, pl.ds(y0 + r0, n), :] for j in range(NT)], axis=1)
        x1 = x + ((_layernorm(x) if n1 is None else n1) * a1 + b1) * y
        x1_ref[r0:r0 + n, :] = x1
        return _layernorm(x1)

    n2 = [prep_norm(qb0, x1b0, 0, 0, H0, None, n1)]

    aff = []

    def prep_chain(i, r0, r1):
        y0 = TM0 + i * TM
        if not isinstance(i, int):
            y0 = pl.multiple_of(y0, L)
        dep = None
        for r in range(r0, r1, PR):
            h2 = prep_norm(qb.at[i], x1b.at[i], y0, r, PR, dep) * aff[0] + aff[1]
            h2b[i, r:r + PR, :] = h2.astype(bf16)
            dep = h2[:, 0:L]

    def gate_up(h2):
        hs = []
        for f in range(0, F, TF):
            g = jnp.dot(h2, wgb[:, f:f + TF], preferred_element_type=f32)
            u = jnp.dot(h2, wub[:, f:f + TF], preferred_element_type=f32)
            hs.append(g * u)
        return jnp.concatenate(hs, axis=1).astype(bf16)

    OC = (0, D - L, D)

    def down(hh, gb, i):
        for c0, c1 in zip(OC[:-1], OC[1:]):
            o = jnp.dot(hh, wdb[:, c0:c1], preferred_element_type=f32)
            ob[i, :, c0:c1] = (x1b[i, :, c0:c1] + gb[:, c0:c1] * o).astype(bf16)
            o_cp(i, c0, c1).start()

    def spread(jobs, anchors):
        total, n = sum(len(_costs(j)) for j in jobs), 0
        for job in jobs:
            m = len(_costs(job))
            job_fn[job[0]](*job[1:], [anchors[(n + i) * len(anchors) // total] for i in range(m)])
            n += m

    last = NC - 1
    acc = {}

    hcache = {}

    def unit(p, n, f, half=None):
        t0, t1 = KP[p], KP[p + 1]
        if (p, half) not in hcache:
            x = jnp.concatenate(n2, axis=0) if half is None else n2[half]
            hcache[p, half] = (x[:, t0 * L:t1 * L] * (1.0 + modv(4, t0, t1))
                               + modv(3, t0, t1)).astype(bf16)
        rows = {None: slice(0, TM0), 0: slice(0, H0), 1: slice(H0, TM0)}[half]
        d = jnp.dot(hcache[p, half], (wgb if n == "g" else wub)[t0 * L:t1 * L, f:f + 4 * L],
                    preferred_element_type=f32)
        ref = gub.at["gu".index(n), rows, f:f + 4 * L]
        if p == len(KP) - 2:
            acc[n, f] = ref[...] + d
        else:
            ref[...] = d if p == 0 else ref[...] + d
        return [d[s:s + 8, 0:L] for s in range(0, d.shape[0], 16)]

    def units(us):
        return [x for u in us for x in unit(*u)]

    FS = range(0, F, 4 * L)
    full = lambda p: [(p, n, f) for f in FS for n in "gu"]
    wait("wg0", "wu0", "qh")
    units([(0, n, f, 0) for n in "gu" for f in FS])
    nb, dep = [], None
    for r in range(H0, TM0, PR2):
        nb.append(prep_norm(qb0, x1b0, 0, r, PR2, dep))
        dep = nb[-1][:, 0:L]
    n2.append(jnp.concatenate(nb, axis=0))
    units([(0, "g", f, 1) for f in FS])
    wait("wg1", "wu1", "s1", "c1")
    grp_mod("s1", "c1")
    spread(_m([0, 1], A3, (last,)), units([(0, "u", f, 1) for f in FS] + full(1)[:-1]))
    wait("wg2", "wu2", "s2", "c2")
    grp_mod("s2", "c2")
    spread(_m([2, 3], A3, (last,)), units(full(1)[-1:] + full(2)[:-1]))
    wait("wg3", "wu3", "s3", "c3", "q1")
    grp_mod("s3", "c3")
    units(full(2)[-1:] + full(3))
    aff += [1.0 + modv(4), modv(3)]
    prep_chain(0, 0, 11 * PR)
    for f in FS:
        hb[:, f:f + 4 * L] = (acc.pop(("g", f)) * acc.pop(("u", f))).astype(bf16)

    def down0(n):
        c = slice(n * L, (n + 1) * L)
        ps = [jnp.dot(hb[:, f:f + 4 * L], wdb[f:f + 4 * L, c], preferred_element_type=f32)
              for f in range(0, F, 4 * L)]
        ob0[:, c] = (x1b0[:, c] + gb[:, c] * (ps[0] + ps[1] + ps[2])).astype(bf16)
        return [x[s:s + 8] for x in ps for s in range(0, TM0, 16)]

    wait("wd", "mG")
    grp_mod("mG")
    gb = modv(5)
    spread(_m([4], A3, (last,)), down0(0))
    wait(f"k{last}", f"v{last}")
    prep_chain(0, 11 * PR, TM)
    a0, a1_ = down0(1), down0(2)
    spread(_kv(last), a0 + a1_[:len(a1_) // 2])
    for g in _u(last):
        grp_u(*g[1:])
    a0 = down0(3)
    o_cp(None, OC[0], OC[1]).start()
    a1_ = down0(4)
    o_cp(None, OC[1], OC[2]).start()
    spread(_m(T, (last,), (last,)), a0 + a1_[:len(a1_) // 2])
    for g in _iv(T, [last]):
        grp_i(*g[1:])
    wait(*[f"q{i + 1}" for i in range(1, NB)])

    def ffn(i, carry):
        h2 = h2b[i]
        prep_chain(jnp.minimum(i + 1, NB - 1), 0, TM)
        down(gate_up(h2), gb, i)
        return carry

    lax.fori_loop(0, NB, ffn, 0)

    def final_waits():
        for i in [None] + list(range(NB)):
            for c0, c1 in zip(OC[:-1], OC[1:]):
                o_cp(i, c0, c1).wait()

    if SCOPES:
        with jax.named_scope("w_out"):
            final_waits()
    else:
        final_waits()


@jax.jit
def pallas_adaLN_cond__ssm_conv_h3__glu_gated_bilinear__prompt_kernel(
    A_q: jax.Array,
    A_k: jax.Array,
    A_v: jax.Array,
    A_shift_k: jax.Array,
    A_ssm_k: jax.Array,
    A_ssm_D: jax.Array,
    B_x: jax.Array,
    B_w_gate: jax.Array,
    B_w_up: jax.Array,
    B_w_down: jax.Array,
    c: jax.Array,
    w_mod: jax.Array,
):
    del B_x
    tiles = lambda x: x.reshape(S // 8, 8, NT, L).transpose(0, 2, 1, 3).reshape(S * NT, L)
    kdt = bf16
    if WF == 2:
        kdt = u32
        tiles = lambda x: lax.bitcast_convert_type(
            x.reshape(S // 8, 4, 2, NT, L).transpose(0, 3, 1, 4, 2), u32).reshape(S * NT // 2, L)
    any_spec = pl.BlockSpec(memory_space=pl.ANY)
    return pl.pallas_call(
        _kernel,
        in_specs=[any_spec] * 11,
        out_specs=any_spec,
        out_shape=jax.ShapeDtypeStruct((1, S, D), bf16),
        scratch_shapes=[
            pltpu.VMEM((TM0, D), bf16),
            pltpu.VMEM((NB, TM, D), bf16),
            pltpu.VMEM(((4 * PAD + S * NT) // WF, L), kdt),
            pltpu.VMEM(((2 * PAD + S * NT) // WF, L), kdt),
            pltpu.VMEM((NT, L, S), bf16),
            pltpu.VMEM((D, F), bf16),
            pltpu.VMEM((D, F), bf16),
            pltpu.VMEM((F, D), bf16),
            pltpu.VMEM((D, 6 * D), bf16),
            pltpu.VMEM((NT, NC, R, L, L), bf16),
            pltpu.VMEM((NT, NC, R, 16, 16, L), f32),
            pltpu.VMEM((NT, NC, R, 16, 16, L), f32),
            pltpu.VMEM((NT, NC, R, 16, 16, L), f32),
            pltpu.VMEM((NT, NC, R, 2 * L, L), bf16),
            pltpu.VMEM((NT, S + 32, L), f32),
            pltpu.VMEM((TM0, D), f32),
            pltpu.VMEM((NB, TM, D), f32),
            pltpu.VMEM((NB, TM, D), bf16),
            pltpu.VMEM((2, TM0, F), f32),
            pltpu.VMEM((TM0, F), bf16),
            pltpu.VMEM((TM0, D), bf16),
            pltpu.VMEM((NB, TM, D), bf16),
            pltpu.VMEM((KS, D), bf16),
            pltpu.VMEM((D,), bf16),
            pltpu.VMEM((1, D), bf16),
            pltpu.SemaphoreType.DMA((len(DMA_ORDER),)),
            pltpu.SemaphoreType.DMA((NB + 1,)),
        ],
        compiler_params=pltpu.CompilerParams(
            vmem_limit_bytes=120 * 1024 * 1024,
            disable_bounds_checks=True, disable_semaphore_checks=True),
        name="adaln_h3_glu",
    )(A_q, tiles(A_k), tiles(A_v), A_shift_k.T, A_ssm_k, A_ssm_D, B_w_gate, B_w_up, B_w_down, c, w_mod)
```

```python
import jax
import jax.numpy as jnp
from jax import lax
import jax.experimental.pallas as pl
import jax.experimental.pallas.tpu as pltpu

S = 2048
D = 640
F = 1536
KS = 4
L = 128
NT = D // L
R = 4
C = R * L
NC = S // C
EPS = 1e-5
WPT = 4 * NT
PAD = 32
PR = 24
TM0 = 512
TM = 384
NB = (S - TM0) // TM
TF = 256
KP = (0, 1, 2, 3, 5)

WM = {"mA": (0, 10), "c0": (20, 21), "mB": (10, 16), "s1": (16, 17), "c1": (21, 22),
      "s2": (17, 18), "c2": (22, 23), "s3": (18, 20), "c3": (23, 25), "mG": (25, 30)}
WF = 1
H0 = 320
PR2 = 64
VM = 5
PR1 = 160
SCOPES = False

f32 = jnp.float32
bf16 = jnp.bfloat16
u32 = jnp.uint32


def _cos_turns(t):
    x = jnp.abs(t - jnp.floor(t) - 0.5) - 0.25
    x2 = x * x
    return x * (6.283164024 + x2 * (-41.33713150 + x2 * (81.34038544 + x2 * -70.98993683)))


def _tables(inverse, hold=None):
    shape = (L, 2 * L) if inverse else (2 * L, L)
    rho = lax.broadcasted_iota(jnp.int32, shape, 1 if inverse else 0)
    j = lax.broadcasted_iota(jnp.int32, shape, 0 if inverse else 1)
    if not inverse:
        j = _perm(j)
    a = (4 * (8 * (rho >> 4) + (rho & 7)) + 1).astype(f32) * (1.0 / (4 * C))
    off = ((rho >> 3) & 1).astype(f32) * 0.25
    ns = [(R * j + r).astype(f32) for r in range(R)]
    if hold is not None:
        ns = [hold(r, n) for r, n in enumerate(ns)]
    ts = [_cos_turns(a * n + off) for n in ns]
    return [(t * (1.0 / C) if inverse else t).astype(bf16) for t in ts]


def _perm(c):
    return 16 * (c >> 4) + 2 * (c & 7) + ((c >> 3) & 1)


def _layernorm(x):
    m = jnp.mean(x, axis=-1, keepdims=True)
    xc = x - m
    v = jnp.mean(xc * xc, axis=-1, keepdims=True)
    return xc * lax.rsqrt(v + EPS)


def _split(t):
    t = t.reshape(16, 16, L)
    return t[:, :8, :], t[:, 8:, :]


def _radix4(x, sgn):
    (ar, ai), (br, bi), (cr, ci), (dr, di) = x
    s0r, s0i, d0r, d0i = ar + cr, ai + ci, ar - cr, ai - ci
    s1r, s1i, d1r, d1i = br + dr, bi + di, br - dr, bi - di
    o0 = (s0r + s1r, s0i + s1i)
    o2 = (s0r - s1r, s0i - s1i)
    pl_ = (d0r - d1i, d0i + d1r)
    mi_ = (d0r + d1i, d0i - d1r)
    return [o0, pl_, o2, mi_] if sgn > 0 else [o0, mi_, o2, pl_]


T = range(NT)
_z = lambda j: [("z", j, a) for a in range(NC)]
_k = lambda j, al: [("k", j, a) for a in al]
_u = lambda a: [("u", j, a) for j in T]
_iv = lambda jl, al: [("i", j, a) for j in jl for a in al]
_kv = lambda a: [("kv", j, a) for j in T]
_m = lambda jl, us, outs: [("mac", j, us, outs) for j in jl]
A3 = (0, 1, 2)

SCHEDULE = [
    (["ssm0"], _z(0) + _k(0, range(NC)), [("setup", None)]),
    (["ssm1"], _z(1) + _k(1, range(NC)), []),
    (["ssm2"], _z(2) + _k(2, [0, 1]), []),
    (["k0", "v0"], _k(2, [2, 3]) + _u(0), _kv(0)),
    (["ssm3"], _z(3) + _k(3, [0, 1]), _m([0, 1, 2], (0,), (0,))),
    (["k1", "v1"], _k(3, [2, 3]) + _u(1), _kv(1) + _m([3], (0,), (0,))),
    (["ssm4"], _z(4) + _k(4, range(NC)), _m([0, 1], (0, 1), (1, 2))),
    (["k2", "v2"], _iv([0, 1, 2, 3], [0]) + _u(2) + _iv([0, 1], [1]) + _iv([4], [0, 1])
     + _iv([0, 1, 4], [2]),
     _kv(2) + _m([4], (0, 1), A3) + _m([0, 1, 4], (2,), (2,)) + _m([2, 3], A3, (1, 2))),
    (["q0", "mA", "c0"], [("mod", "mA", "c0")] + _iv([2], [1, 2]), []),
]
PREP_GROUPS = _iv([3], [1, 2])

DMA_ORDER = (["sk", "sd", "c", "ssm0", "ssm1", "ssm2", "k0", "v0", "ssm3", "k1", "v1", "ssm4",
              "k2", "v2", "q0", "mA", "c0", "mB", "qh", "wg0", "wu0", "s1", "c1", "wg1", "wu1", "s2", "c2",
              "wg2", "wu2", "s3", "c3", "wg3", "wu3", "q1", "wd", "mG", "k3", "v3"]
             + [f"q{i + 1}" for i in range(1, NB)])


def _costs(job):
    if job[0] == "kv":
        return [88] * (C // 64)
    if job[0] == "setup":
        return [100] * (8 * R)
    if job[0] == "vmod":
        return [3 * D // VM // 8] * (VM * (WM[job[1]][1] - WM[job[1]][0]))
    us, outs = job[2], job[3]
    pairs = [(a, n) for a in outs for n in us if n <= a]
    mac = (2 * len({a - n for a, n in pairs if a > n}) + 8 * len(pairs)
           - (2 * len(outs) if us[0] == 0 else 0))
    fin = 20 * sum(a <= us[-1] for a in outs)
    if mac < 12 and outs[-1] <= us[-1]:
        return [1 + R * mac + fin] * 16
    return [1 + mac, 1 + mac, 1 + mac, 1 + mac + fin] * 16


def _plan(groups, jobs):
    free = {"i": 56, "z": 56, "k": 47, "u": 46}
    steps = {"i": 16, "z": 8, "k": 16, "u": 16, "mod": 0}
    slots = [free[g[0]] for g in groups for _ in range(steps[g[0]])]
    rate = max(1.03 * sum(sum(_costs(j)) for j in jobs) / sum(slots), 1.0)
    plan, credit, n = [], slots[0] * rate, 0
    for job in jobs:
        limit, first = len(slots), 0
        for g in groups:
            if g[1] == job[1] and ((g[0], job[0]) == ("u", "kv") and g[2] == job[2]
                                   or (g[0], job[0]) == ("i", "mac") and g[2] in job[3]
                                   and g[2] <= job[2][-1]):
                limit = min(limit, first)
            first += steps[g[0]]
            if g[1] == job[1] and (g[0], job[0]) == ("u", "mac") and g[2] in job[2]:
                while n < first:
                    n += 1
                    credit = min(credit + slots[n] * rate, slots[n] * rate)
        idx = []
        for c in _costs(job):
            while credit <= 0 and n + 1 < limit:
                n += 1
                credit += slots[n] * rate
            credit -= c
            idx.append(n)
        plan.append(idx)
    return plan


def _kernel(q_hbm, k_hbm, v_hbm, sk_hbm, ssm_hbm, sd_hbm, wg_hbm, wu_hbm, wd_hbm,
            c_hbm, wm_hbm, o_hbm,
            qb0, qb, kb, vb, ssmb, wgb, wub, wdb, wmb, uwb, ub, kpb, yp, pb, yb, x1b0, x1b, h2b, gub, hb, ob0, ob, mv, skb, sdb, cb_, sem, osem):
    cps = {"sk": (sk_hbm, skb), "sd": (sd_hbm, sdb), "c": (c_hbm, cb_), "wd": (wd_hbm, wdb),
           }
    for j in range(NT):
        cps[f"ssm{j}"] = (ssm_hbm.at[pl.ds(j * L, L), :], ssmb.at[j])
    for a in range(NC):
        n = C * NT // WF
        cps[f"k{a}"] = (k_hbm.at[pl.ds(a * n, n), :], kb.at[pl.ds(2 * PAD // WF + a * n, n), :])
        cps[f"v{a}"] = (v_hbm.at[pl.ds(a * n, n), :], vb.at[pl.ds(a * n, n), :])
    for n, (c0, c1) in WM.items():
        cols = pl.ds(c0 * L, (c1 - c0) * L)
        cps[n] = (wm_hbm.at[:, cols], wmb.at[:, cols])
    cps["q0"] = (q_hbm.at[0, pl.ds(0, H0), :], qb0.at[pl.ds(0, H0), :])
    cps["qh"] = (q_hbm.at[0, pl.ds(H0, TM0 - H0), :], qb0.at[pl.ds(H0, TM0 - H0), :])
    for i in range(NB):
        cps[f"q{i + 1}"] = (q_hbm.at[0, pl.ds(TM0 + i * TM, TM), :], qb.at[i])
    for p in range(len(KP) - 1):
        rows = pl.ds(KP[p] * L, (KP[p + 1] - KP[p]) * L)
        cps[f"wg{p}"] = (wg_hbm.at[rows, :], wgb.at[rows, :])
        cps[f"wu{p}"] = (wu_hbm.at[rows, :], wub.at[rows, :])
    assert sorted(cps) == sorted(DMA_ORDER)

    def cp(name):
        src, dst = cps[name]
        return pltpu.make_async_copy(src, dst, sem.at[DMA_ORDER.index(name)])

    def wait(*names):
        if SCOPES:
            with jax.named_scope("w_" + names[0]):
                for n in names:
                    cp(n).wait()
        else:
            for n in names:
                cp(n).wait()

    for n in DMA_ORDER:
        cp(n).start()

    tabs, ginv, ccol = _tables(False), [], []
    kb[0:2 * PAD // WF, :] = jnp.zeros((2 * PAD // WF, L), kb.dtype)
    kw, vw = (kb, vb) if WF == 2 else (kb.bitcast(u32), vb.bitcast(u32))
    ub[0, 0, 0, 0, pl.ds(0, 8, stride=2), :] = jnp.zeros((8, L), f32)
    mv[0, pl.ds(0, 8, stride=2), :] = jnp.zeros((8, L), f32)
    ri = lax.broadcasted_iota(jnp.int32, (L, L), 0)
    ci = lax.broadcasted_iota(jnp.int32, (L, L), 1)
    sel = jnp.where(ci == R * _perm(ri & 31) + (ri >> 5), 1.0, 0.0).astype(bf16)

    wait("sk", "sd", "c")
    skt = skb[...].astype(f32)
    sdv = sdb[...].astype(f32).reshape(1, D)
    cv = cb_[...].astype(f32)
    sig = jax.nn.sigmoid(cv)
    cs = jnp.broadcast_to((cv * sig).astype(bf16), (16, D))
    one = sig[:, 0:L]

    def gate(x, deps):
        dep = jnp.concatenate(deps, axis=0).reshape(x.shape)
        return jnp.where(jnp.broadcast_to(one, x.shape) > 2.0, dep, x)

    def put(dst, j, a, xs):
        for qi in range(R):
            dst[j, a, qi] = jnp.concatenate(xs[qi], axis=1)

    zs = {}
    mod = {}

    def grp_z(j, a):
        z = [lax.dot_general(sel, ssmb[j, :, t * L:(t + 1) * L], (((1,), (1,)), ((), ())),
                             preferred_element_type=f32) for t in range(R * a, R * a + R)]
        zs[j, a] = [jnp.concatenate([z[p][32 * r:32 * (r + 1)] for p in range(R)],
                                    axis=0).astype(bf16) for r in range(R)]
        return [z[0][16 * t:16 * t + 8] for t in range(8)]

    def grp_fwd(ws, dst, j, a, dvec=None):
        t = [jnp.dot(tabs[r], ws[r], preferred_element_type=f32) for r in range(R)]
        x = [_split(v) for v in t]
        if dvec is not None:
            x[0] = (x[0][0] + dvec[None], x[0][1])
        put(dst, j, a, _radix4(x, -1))
        return [t[0][16 * s:16 * s + 8] for s in range(16)]

    def grp_k(j, a):
        return grp_fwd(zs.pop((j, a)), kpb, j, a,
                       sdv[:, j * L:(j + 1) * L] if a == 0 else None)

    def grp_u(j, a):
        uw = [uwb[j, a, r] for r in range(R)]
        return grp_fwd(uw, ub, j, a)

    def grp_i(j, a):
        ys = []
        for r in range(R):
            y = jnp.dot(ginv[r], pb[j, a, r], preferred_element_type=f32)
            yb[j, pl.ds(a * C + r, L, stride=R), :] = y
            ys.append(y)
        return ([ys[0][16 * s:16 * s + 8] for s in range(8)]
                + [ys[2][16 * s:16 * s + 8] for s in range(8)])

    def grp_mod(*names):
        for name in names:
            c0, c1 = WM[name]
            m = jnp.dot(cs, wmb[:, c0 * L:c1 * L], preferred_element_type=f32)
            for c in range(c0, c1):
                mod[c] = m[0:1, (c - c0) * L:(c - c0 + 1) * L]
        return []

    def modv(i, t0=0, t1=NT):
        return jnp.concatenate([mod[i * NT + n] for n in range(t0, t1)], axis=1)

    def job_kv(j, a, deps):
        lo = lambda x: lax.bitcast_convert_type(x << 16, f32)
        hi = lambda x: lax.bitcast_convert_type(x & jnp.uint32(0xFFFF0000), f32)
        n = C // 8
        ld = lambda ref, o: ref[pl.ds(a * n * WPT + 4 * j + o, n, stride=WPT), :]
        k = {}
        for m in range(4):
            x = ld(kw, PAD + m)
            k[2 * m], k[2 * m + 1] = lo(x), hi(x)
        k[-3] = hi(ld(kw, PAD - WPT + 2))
        x = ld(kw, PAD - WPT + 3)
        k[-2], k[-1] = lo(x), hi(x)
        w = [skt[t:t + 1, j * L:(j + 1) * L] for t in range(KS)]
        w[0] = gate(jnp.broadcast_to(w[0], (n, L)), deps)
        kv = {}
        for m in range(4):
            x = ld(vw, m)
            for ph, v in ((2 * m, lo(x)), (2 * m + 1, hi(x))):
                ks = k[ph] * w[0]
                for t in range(1, KS):
                    ks = ks + k[ph - t] * w[t]
                kv[ph] = (ks * v).reshape(n // 8, 8, L)
        for r in range(R):
            uwb[j, a, r] = jnp.concatenate([kv[r], kv[r + R]], axis=1).reshape(L, L).astype(bf16)

    def job_mac(j, us, outs, deps):
        ld = lambda ref, a: (ref[j, a, :, :, 0:8, :], ref[j, a, :, :, 8:16, :])
        lo, hi = us[0], us[-1]
        u = {a: ld(ub, a) for a in us}
        if len(deps) == 16:
            ur = jnp.concatenate([gate(u[lo][0][0:1], deps), u[lo][0][1:]], axis=0)
        else:
            ur = gate(u[lo][0], [deps[R * i + qi] for qi in range(R) for i in range(16)])
        u[lo] = (ur, u[lo][1])
        ms = sorted({a - n for a in outs for n in us if n <= a})
        k = {m: ld(kpb, m) for m in sorted(set(ms) | {m - 1 for m in ms if m > 0})}
        kp = {m: k[m] if m == 0 else (k[m][0] - k[m - 1][1], k[m][1] + k[m - 1][0]) for m in ms}
        for a in outs:
            yr, yi = ld(yp, a) if lo > 0 else (None, None)
            for n in us:
                if n > a:
                    continue
                (kr, ki), (ur, ui) = kp[a - n], u[n]
                tr = kr * ur - ki * ui
                ti = kr * ui + ki * ur
                yr = tr if yr is None else yr + tr
                yi = ti if yi is None else yi + ti
            if a > hi:
                yp[j, a] = jnp.concatenate([yr, yi], axis=2)
                continue
            ps = _radix4([(yr[qi], yi[qi]) for qi in range(R)], +1)
            for r in range(R):
                pb[j, a, r] = jnp.concatenate(ps[r], axis=1).reshape(2 * L, L).astype(bf16)

    def job_setup(_, deps):
        def hold(r, n):
            g = gate(n[:, 0:L], [deps[8 * r + s // 2] for s in range(16)])
            return jnp.concatenate([g, g], axis=1)

        ginv.extend(_tables(True, hold))
        csf = cs[0:1].astype(f32)
        ccol.append(jnp.concatenate([jnp.broadcast_to(csf[:, t * L:(t + 1) * L], (L, L)).T
                                     for t in range(NT)], axis=0))

    def job_vmod(name, deps):
        c0, c1 = WM[name]
        n = D // VM
        for c in range(c0, c1):
            for i in range(VM):
                cc = ccol[0][i * n:(i + 1) * n]
                cc = jnp.concatenate([gate(cc[0:8], [deps[(c - c0) * VM + i]]), cc[8:]], axis=0)
                p = wmb[i * n:(i + 1) * n, c * L:(c + 1) * L].astype(f32) * cc
                mv[c, 8 * i:8 * i + 8, :] = jnp.sum(p.reshape(n // 8, 8, L), axis=0)
            mod[c] = jnp.sum(mv[c], axis=0, keepdims=True)

    grp_fn = {"z": grp_z, "k": grp_k, "u": grp_u, "i": grp_i, "mod": grp_mod}
    job_fn = {"kv": job_kv, "mac": job_mac, "vmod": job_vmod, "setup": job_setup}

    for waits, groups, jobs in SCHEDULE:
        wait(*waits)
        plan = _plan(groups, jobs)
        anchors, done = [], 0
        for g in groups + [None]:
            while done < len(jobs) and max(plan[done]) < len(anchors):
                job_fn[jobs[done][0]](*jobs[done][1:], [anchors[n] for n in plan[done]])
                done += 1
            if g is not None:
                anchors += grp_fn[g[0]](*g[1:])
        assert done == len(jobs)

    n1, dep = [], None
    for r in range(0, H0, PR1):
        x = qb0[r:r + PR1, :].astype(f32)
        if dep is not None:
            x = jnp.concatenate([gate(x[:, 0:L], [dep]), x[:, L:]], axis=1)
        n1.append(_layernorm(x))
        dep = n1[-1][:, 0:L]
    n1 = jnp.concatenate(n1, axis=0)
    wait("mB")
    grp_mod("mB")
    for g in PREP_GROUPS:
        grp_fn[g[0]](*g[1:])
    sa, ca, ga = [modv(i) for i in range(3)]
    a1 = ga * (1.0 + ca)
    b1 = ga * sa

    def o_cp(i, c0, c1):
        cols = pl.ds(c0, c1 - c0)
        if i is None:
            return pltpu.make_async_copy(ob0.at[:, cols], o_hbm.at[0, pl.ds(0, TM0), cols],
                                         osem.at[NB])
        r0 = TM0 + i * TM
        if not isinstance(i, int):
            r0 = pl.multiple_of(r0, L)
        return pltpu.make_async_copy(ob.at[i, :, cols], o_hbm.at[0, pl.ds(r0, TM), cols],
                                     osem.at[i])

    def prep_norm(q_ref, x1_ref, y0, r0, n, dep=None, n1=None):
        x = q_ref[r0:r0 + n, :].astype(f32)
        if dep is not None:
            x = jnp.concatenate([gate(x[:, 0:L], [dep]), x[:, L:]], axis=1)
        y = jnp.concatenate([yb[j, pl.ds(y0 + r0, n), :] for j in range(NT)], axis=1)
        x1 = x + ((_layernorm(x) if n1 is None else n1) * a1 + b1) * y
        x1_ref[r0:r0 + n, :] = x1
        return _layernorm(x1)

    n2 = [prep_norm(qb0, x1b0, 0, 0, H0, None, n1)]

    aff = []

    def prep_chain(i, r0, r1):
        y0 = TM0 + i * TM
        if not isinstance(i, int):
            y0 = pl.multiple_of(y0, L)
        dep = None
        for r in range(r0, r1, PR):
            h2 = prep_norm(qb.at[i], x1b.at[i], y0, r, PR, dep) * aff[0] + aff[1]
            h2b[i, r:r + PR, :] = h2.astype(bf16)
            dep = h2[:, 0:L]

    def gate_up(h2):
        hs = []
        for f in range(0, F, TF):
            g = jnp.dot(h2, wgb[:, f:f + TF], preferred_element_type=f32)
            u = jnp.dot(h2, wub[:, f:f + TF], preferred_element_type=f32)
            hs.append(g * u)
        return jnp.concatenate(hs, axis=1).astype(bf16)

    OC = (0, D - L, D)

    def down(hh, gb, i):
        for c0, c1 in zip(OC[:-1], OC[1:]):
            o = jnp.dot(hh, wdb[:, c0:c1], preferred_element_type=f32)
            ob[i, :, c0:c1] = (x1b[i, :, c0:c1] + gb[:, c0:c1] * o).astype(bf16)
            o_cp(i, c0, c1).start()

    def spread(jobs, anchors):
        total, n = sum(len(_costs(j)) for j in jobs), 0
        for job in jobs:
            m = len(_costs(job))
            job_fn[job[0]](*job[1:], [anchors[(n + i) * len(anchors) // total] for i in range(m)])
            n += m

    last = NC - 1
    acc = {}

    hcache = {}

    def unit(p, n, f, half=None):
        t0, t1 = KP[p], KP[p + 1]
        if (p, half) not in hcache:
            x = jnp.concatenate(n2, axis=0) if half is None else n2[half]
            hcache[p, half] = (x[:, t0 * L:t1 * L] * (1.0 + modv(4, t0, t1))
                               + modv(3, t0, t1)).astype(bf16)
        rows = {None: slice(0, TM0), 0: slice(0, H0), 1: slice(H0, TM0)}[half]
        d = jnp.dot(hcache[p, half], (wgb if n == "g" else wub)[t0 * L:t1 * L, f:f + 4 * L],
                    preferred_element_type=f32)
        ref = gub.at["gu".index(n), rows, f:f + 4 * L]
        if p == len(KP) - 2:
            acc[n, f] = ref[...] + d
        else:
            ref[...] = d if p == 0 else ref[...] + d
        return [d[s:s + 8, 0:L] for s in range(0, d.shape[0], 16)]

    def units(us):
        return [x for u in us for x in unit(*u)]

    FS = range(0, F, 4 * L)
    full = lambda p: [(p, n, f) for f in FS for n in "gu"]
    wait("wg0", "wu0", "qh")
    units([(0, n, f, 0) for n in "gu" for f in FS])
    nb, dep = [], None
    for r in range(H0, TM0, PR2):
        nb.append(prep_norm(qb0, x1b0, 0, r, PR2, dep))
        dep = nb[-1][:, 0:L]
    n2.append(jnp.concatenate(nb, axis=0))
    units([(0, "g", f, 1) for f in FS])
    wait("wg1", "wu1", "s1", "c1")
    spread([("vmod", "s1"), ("vmod", "c1")], units([(0, "u", f, 1) for f in FS])[:20])
    spread(_m([0, 1], A3, (last,)), units(full(1)[:-1]))
    wait("wg2", "wu2", "s2", "c2")
    spread([("vmod", "s2"), ("vmod", "c2")], units(full(1)[-1:])[:20])
    spread(_m([2, 3], A3, (last,)), units(full(2)[:-1]))
    wait("wg3", "wu3", "s3", "c3", "q1")
    spread([("vmod", "s3"), ("vmod", "c3")], units(full(2)[-1:])[:20])
    units(full(3))
    aff += [1.0 + modv(4), modv(3)]
    prep_chain(0, 0, 11 * PR)
    for f in FS:
        hb[:, f:f + 4 * L] = (acc.pop(("g", f)) * acc.pop(("u", f))).astype(bf16)

    def down0(n):
        c = slice(n * L, (n + 1) * L)
        ps = [jnp.dot(hb[:, f:f + 4 * L], wdb[f:f + 4 * L, c], preferred_element_type=f32)
              for f in range(0, F, 4 * L)]
        anchors = [x[s:s + 8] for x in ps for s in range(0, TM0, 16)]
        if n == 0:
            spread([("vmod", "mG")], anchors[:40])
        ob0[:, c] = (x1b0[:, c] + mod[5 * NT + n] * (ps[0] + ps[1] + ps[2])).astype(bf16)
        return anchors

    wait("wd", "mG")
    spread(_m([4], A3, (last,)), down0(0)[40:])
    gb = modv(5)
    wait(f"k{last}", f"v{last}")
    prep_chain(0, 11 * PR, TM)
    a0, a1_ = down0(1), down0(2)
    spread(_kv(last), a0 + a1_[:len(a1_) // 2])
    for g in _u(last):
        grp_u(*g[1:])
    a0 = down0(3)
    o_cp(None, OC[0], OC[1]).start()
    a1_ = down0(4)
    o_cp(None, OC[1], OC[2]).start()
    spread(_m(T, (last,), (last,)), a0 + a1_[:len(a1_) // 2])
    for g in _iv(T, [last]):
        grp_i(*g[1:])
    wait(*[f"q{i + 1}" for i in range(1, NB)])

    def ffn(i, carry):
        h2 = h2b[i]
        prep_chain(jnp.minimum(i + 1, NB - 1), 0, TM)
        down(gate_up(h2), gb, i)
        return carry

    lax.fori_loop(0, NB, ffn, 0)

    def final_waits():
        for i in [None] + list(range(NB)):
            for c0, c1 in zip(OC[:-1], OC[1:]):
                o_cp(i, c0, c1).wait()

    if SCOPES:
        with jax.named_scope("w_out"):
            final_waits()
    else:
        final_waits()


@jax.jit
def pallas_adaLN_cond__ssm_conv_h3__glu_gated_bilinear__prompt_kernel(
    A_q: jax.Array,
    A_k: jax.Array,
    A_v: jax.Array,
    A_shift_k: jax.Array,
    A_ssm_k: jax.Array,
    A_ssm_D: jax.Array,
    B_x: jax.Array,
    B_w_gate: jax.Array,
    B_w_up: jax.Array,
    B_w_down: jax.Array,
    c: jax.Array,
    w_mod: jax.Array,
):
    del B_x
    tiles = lambda x: x.reshape(S // 8, 8, NT, L).transpose(0, 2, 1, 3).reshape(S * NT, L)
    kdt = bf16
    if WF == 2:
        kdt = u32
        tiles = lambda x: lax.bitcast_convert_type(
            x.reshape(S // 8, 4, 2, NT, L).transpose(0, 3, 1, 4, 2), u32).reshape(S * NT // 2, L)
    any_spec = pl.BlockSpec(memory_space=pl.ANY)
    return pl.pallas_call(
        _kernel,
        in_specs=[any_spec] * 11,
        out_specs=any_spec,
        out_shape=jax.ShapeDtypeStruct((1, S, D), bf16),
        scratch_shapes=[
            pltpu.VMEM((TM0, D), bf16),
            pltpu.VMEM((NB, TM, D), bf16),
            pltpu.VMEM(((4 * PAD + S * NT) // WF, L), kdt),
            pltpu.VMEM(((2 * PAD + S * NT) // WF, L), kdt),
            pltpu.VMEM((NT, L, S), bf16),
            pltpu.VMEM((D, F), bf16),
            pltpu.VMEM((D, F), bf16),
            pltpu.VMEM((F, D), bf16),
            pltpu.VMEM((D, 6 * D), bf16),
            pltpu.VMEM((NT, NC, R, L, L), bf16),
            pltpu.VMEM((NT, NC, R, 16, 16, L), f32),
            pltpu.VMEM((NT, NC, R, 16, 16, L), f32),
            pltpu.VMEM((NT, NC, R, 16, 16, L), f32),
            pltpu.VMEM((NT, NC, R, 2 * L, L), bf16),
            pltpu.VMEM((NT, S + 32, L), f32),
            pltpu.VMEM((TM0, D), f32),
            pltpu.VMEM((NB, TM, D), f32),
            pltpu.VMEM((NB, TM, D), bf16),
            pltpu.VMEM((2, TM0, F), f32),
            pltpu.VMEM((TM0, F), bf16),
            pltpu.VMEM((TM0, D), bf16),
            pltpu.VMEM((NB, TM, D), bf16),
            pltpu.VMEM((32, 8 * VM, L), f32),
            pltpu.VMEM((KS, D), bf16),
            pltpu.VMEM((D,), bf16),
            pltpu.VMEM((1, D), bf16),
            pltpu.SemaphoreType.DMA((len(DMA_ORDER),)),
            pltpu.SemaphoreType.DMA((NB + 1,)),
        ],
        compiler_params=pltpu.CompilerParams(
            vmem_limit_bytes=120 * 1024 * 1024,
            disable_bounds_checks=True, disable_semaphore_checks=True),
        name="adaln_h3_glu",
    )(A_q, tiles(A_k), tiles(A_v), A_shift_k.T, A_ssm_k, A_ssm_D, B_w_gate, B_w_up, B_w_down, c, w_mod)
```

```python
import jax
import jax.numpy as jnp
from jax import lax
import jax.experimental.pallas as pl
import jax.experimental.pallas.tpu as pltpu

S = 2048
D = 640
F = 1536
KS = 4
L = 128
NT = D // L
R = 4
C = R * L
NC = S // C
EPS = 1e-5
WPT = 4 * NT
PAD = 32
PR = 24
TM0 = 512
TM = 384
NB = (S - TM0) // TM
TF = 256
KP = (0, 1, 2, 3, 5)

WM = {"mA": (0, 10), "c0": (20, 21), "mB": (10, 16), "s1": (16, 17), "c1": (21, 22),
      "s2": (17, 18), "c2": (22, 23), "s3": (18, 20), "c3": (23, 25), "mG": (25, 30)}
WF = 1
H0 = 320
PR2 = 64
VM = 5
PR1 = 160
SCOPES = False

f32 = jnp.float32
bf16 = jnp.bfloat16
u32 = jnp.uint32


def _cos_turns(t):
    x = jnp.abs(t - jnp.floor(t) - 0.5) - 0.25
    x2 = x * x
    return x * (6.283164024 + x2 * (-41.33713150 + x2 * (81.34038544 + x2 * -70.98993683)))


def _tables(inverse, hold=None):
    shape = (L, 2 * L) if inverse else (2 * L, L)
    rho = lax.broadcasted_iota(jnp.int32, shape, 1 if inverse else 0)
    j = lax.broadcasted_iota(jnp.int32, shape, 0 if inverse else 1)
    if not inverse:
        j = _perm(j)
    a = (4 * (8 * (rho >> 4) + (rho & 7)) + 1).astype(f32) * (1.0 / (4 * C))
    off = ((rho >> 3) & 1).astype(f32) * 0.25
    ns = [(R * j + r).astype(f32) for r in range(R)]
    if hold is not None:
        ns = [hold(r, n) for r, n in enumerate(ns)]
    ts = [_cos_turns(a * n + off) for n in ns]
    return [(t * (1.0 / C) if inverse else t).astype(bf16) for t in ts]


def _perm(c):
    return 16 * (c >> 4) + 2 * (c & 7) + ((c >> 3) & 1)


def _layernorm(x):
    m = jnp.mean(x, axis=-1, keepdims=True)
    xc = x - m
    v = jnp.mean(xc * xc, axis=-1, keepdims=True)
    return xc * lax.rsqrt(v + EPS)


def _split(t):
    t = t.reshape(16, 16, L)
    return t[:, :8, :], t[:, 8:, :]


def _radix4(x, sgn):
    (ar, ai), (br, bi), (cr, ci), (dr, di) = x
    s0r, s0i, d0r, d0i = ar + cr, ai + ci, ar - cr, ai - ci
    s1r, s1i, d1r, d1i = br + dr, bi + di, br - dr, bi - di
    o0 = (s0r + s1r, s0i + s1i)
    o2 = (s0r - s1r, s0i - s1i)
    pl_ = (d0r - d1i, d0i + d1r)
    mi_ = (d0r + d1i, d0i - d1r)
    return [o0, pl_, o2, mi_] if sgn > 0 else [o0, mi_, o2, pl_]


T = range(NT)
_z = lambda j: [("z", j, a) for a in range(NC)]
_k = lambda j, al: [("k", j, a) for a in al]
_u = lambda a: [("u", j, a) for j in T]
_iv = lambda jl, al: [("i", j, a) for j in jl for a in al]
_kv = lambda a: [("kv", j, a) for j in T]
_m = lambda jl, us, outs: [("mac", j, us, outs) for j in jl]
A3 = (0, 1, 2)

SCHEDULE = [
    (["ssm0"], _z(0) + _k(0, range(NC)), [("setup", None)]),
    (["ssm1"], _z(1) + _k(1, range(NC)), []),
    (["ssm2"], _z(2) + _k(2, [0, 1]), []),
    (["k0", "v0"], _k(2, [2, 3]) + _u(0), _kv(0)),
    (["ssm3"], _z(3) + _k(3, [0, 1]), _m([0, 1, 2], (0,), (0,))),
    (["k1", "v1"], _k(3, [2, 3]) + _u(1), _kv(1) + _m([3], (0,), (0,))),
    (["ssm4"], _z(4) + _k(4, range(NC)), _m([0, 1], (0, 1), (1, 2))),
    (["k2", "v2"], _iv([0, 1, 2, 3], [0]) + _u(2) + _iv([0, 1], [1]) + _iv([4], [0, 1])
     + _iv([0, 1, 4], [2]),
     _kv(2) + _m([4], (0, 1), A3) + _m([0, 1, 4], (2,), (2,)) + _m([2, 3], A3, (1, 2))),
    (["q0", "mA", "c0"], [("mod", "mA", "c0")] + _iv([2], [1, 2]), []),
]
PREP_GROUPS = _iv([3], [1, 2])

DMA_ORDER = (["sk", "sd", "c", "ssm0", "ssm1", "ssm2", "k0", "v0", "ssm3", "k1", "v1", "ssm4",
              "k2", "v2", "q0", "mA", "c0", "mB", "qh", "wg0", "wu0", "s1", "c1", "wg1", "wu1", "s2", "c2",
              "wg2", "wu2", "s3", "c3", "wg3", "wu3", "q1", "wd", "mG", "k3", "v3"]
             + [f"q{i + 1}" for i in range(1, NB)])


def _costs(job):
    if job[0] == "kv":
        return [88] * (C // 64)
    if job[0] == "setup":
        return [100] * (8 * R)
    if job[0] == "vmod":
        return [3 * D // VM // 8] * (VM * (WM[job[1]][1] - WM[job[1]][0]))
    us, outs = job[2], job[3]
    pairs = [(a, n) for a in outs for n in us if n <= a]
    mac = (2 * len({a - n for a, n in pairs if a > n}) + 8 * len(pairs)
           - (2 * len(outs) if us[0] == 0 else 0))
    fin = 20 * sum(a <= us[-1] for a in outs)
    if mac < 12 and outs[-1] <= us[-1]:
        return [1 + R * mac + fin] * 16
    return [1 + mac, 1 + mac, 1 + mac, 1 + mac + fin] * 16


def _plan(groups, jobs):
    free = {"i": 56, "z": 56, "k": 47, "u": 46}
    steps = {"i": 16, "z": 8, "k": 16, "u": 16, "mod": 0}
    slots = [free[g[0]] for g in groups for _ in range(steps[g[0]])]
    rate = max(1.03 * sum(sum(_costs(j)) for j in jobs) / sum(slots), 1.0)
    plan, credit, n = [], slots[0] * rate, 0
    for job in jobs:
        limit, first = len(slots), 0
        for g in groups:
            if g[1] == job[1] and ((g[0], job[0]) == ("u", "kv") and g[2] == job[2]
                                   or (g[0], job[0]) == ("i", "mac") and g[2] in job[3]
                                   and g[2] <= job[2][-1]):
                limit = min(limit, first)
            first += steps[g[0]]
            if g[1] == job[1] and (g[0], job[0]) == ("u", "mac") and g[2] in job[2]:
                while n < first:
                    n += 1
                    credit = min(credit + slots[n] * rate, slots[n] * rate)
        idx = []
        for c in _costs(job):
            while credit <= 0 and n + 1 < limit:
                n += 1
                credit += slots[n] * rate
            credit -= c
            idx.append(n)
        plan.append(idx)
    return plan


def _kernel(q_hbm, k_hbm, v_hbm, sk_hbm, ssm_hbm, sd_hbm, wg_hbm, wu_hbm, wd_hbm,
            c_hbm, wm_hbm, o_hbm,
            qb0, qb, kb, vb, ssmb, wgb, wub, wdb, wmb, uwb, ub, kpb, yp, pb, yb, x1b0, x1b, h2b, gub, hb, ob0, ob, mv, skb, sdb, cb_, sem, osem):
    cps = {"sk": (sk_hbm, skb), "sd": (sd_hbm, sdb), "c": (c_hbm, cb_), "wd": (wd_hbm, wdb),
           }
    for j in range(NT):
        cps[f"ssm{j}"] = (ssm_hbm.at[pl.ds(j * L, L), :], ssmb.at[j])
    for a in range(NC):
        n = C * NT // WF
        cps[f"k{a}"] = (k_hbm.at[pl.ds(a * n, n), :], kb.at[pl.ds(2 * PAD // WF + a * n, n), :])
        cps[f"v{a}"] = (v_hbm.at[pl.ds(a * n, n), :], vb.at[pl.ds(a * n, n), :])
    for n, (c0, c1) in WM.items():
        cols = pl.ds(c0 * L, (c1 - c0) * L)
        cps[n] = (wm_hbm.at[:, cols], wmb.at[:, cols])
    cps["q0"] = (q_hbm.at[0, pl.ds(0, H0), :], qb0.at[pl.ds(0, H0), :])
    cps["qh"] = (q_hbm.at[0, pl.ds(H0, TM0 - H0), :], qb0.at[pl.ds(H0, TM0 - H0), :])
    for i in range(NB):
        cps[f"q{i + 1}"] = (q_hbm.at[0, pl.ds(TM0 + i * TM, TM), :], qb.at[i])
    for p in range(len(KP) - 1):
        rows = pl.ds(KP[p] * L, (KP[p + 1] - KP[p]) * L)
        cps[f"wg{p}"] = (wg_hbm.at[rows, :], wgb.at[rows, :])
        cps[f"wu{p}"] = (wu_hbm.at[rows, :], wub.at[rows, :])
    assert sorted(cps) == sorted(DMA_ORDER)

    def cp(name):
        src, dst = cps[name]
        return pltpu.make_async_copy(src, dst, sem.at[DMA_ORDER.index(name)])

    def wait(*names):
        if SCOPES:
            with jax.named_scope("w_" + names[0]):
                for n in names:
                    cp(n).wait()
        else:
            for n in names:
                cp(n).wait()

    for n in DMA_ORDER:
        cp(n).start()

    tabs, ginv, ccol = _tables(False), [], []
    kb[0:2 * PAD // WF, :] = jnp.zeros((2 * PAD // WF, L), kb.dtype)
    kw, vw = (kb, vb) if WF == 2 else (kb.bitcast(u32), vb.bitcast(u32))
    ub[0, 0, 0, 0, pl.ds(0, 8, stride=2), :] = jnp.zeros((8, L), f32)
    mv[0, pl.ds(0, 8, stride=2), :] = jnp.zeros((8, L), f32)
    ri = lax.broadcasted_iota(jnp.int32, (L, L), 0)
    ci = lax.broadcasted_iota(jnp.int32, (L, L), 1)
    sel = jnp.where(ci == R * _perm(ri & 31) + (ri >> 5), 1.0, 0.0).astype(bf16)

    wait("sk", "sd", "c")
    skt = skb[...].astype(f32)
    sdv = sdb[...].astype(f32).reshape(1, D)
    cv = cb_[...].astype(f32)
    sig = jax.nn.sigmoid(cv)
    cs = jnp.broadcast_to((cv * sig).astype(bf16), (16, D))
    one = sig[:, 0:L]

    def gate(x, deps):
        dep = jnp.concatenate(deps, axis=0).reshape(x.shape)
        return jnp.where(jnp.broadcast_to(one, x.shape) > 2.0, dep, x)

    def put(dst, j, a, xs):
        for qi in range(R):
            dst[j, a, qi] = jnp.concatenate(xs[qi], axis=1)

    zs = {}
    mod = {}

    def grp_z(j, a):
        z = [lax.dot_general(sel, ssmb[j, :, t * L:(t + 1) * L], (((1,), (1,)), ((), ())),
                             preferred_element_type=f32) for t in range(R * a, R * a + R)]
        zs[j, a] = [jnp.concatenate([z[p][32 * r:32 * (r + 1)] for p in range(R)],
                                    axis=0).astype(bf16) for r in range(R)]
        return [z[0][16 * t:16 * t + 8] for t in range(8)]

    def grp_fwd(ws, dst, j, a, dvec=None):
        t = [jnp.dot(tabs[r], ws[r], preferred_element_type=f32) for r in range(R)]
        x = [_split(v) for v in t]
        if dvec is not None:
            x[0] = (x[0][0] + dvec[None], x[0][1])
        put(dst, j, a, _radix4(x, -1))
        return [t[0][16 * s:16 * s + 8] for s in range(16)]

    def grp_k(j, a):
        return grp_fwd(zs.pop((j, a)), kpb, j, a,
                       sdv[:, j * L:(j + 1) * L] if a == 0 else None)

    def grp_u(j, a):
        uw = [uwb[j, a, r] for r in range(R)]
        return grp_fwd(uw, ub, j, a)

    def grp_i(j, a):
        ys = []
        for r in range(R):
            y = jnp.dot(ginv[r], pb[j, a, r], preferred_element_type=f32)
            yb[j, pl.ds(a * C + r, L, stride=R), :] = y
            ys.append(y)
        return ([ys[0][16 * s:16 * s + 8] for s in range(8)]
                + [ys[2][16 * s:16 * s + 8] for s in range(8)])

    def grp_mod(*names):
        for name in names:
            c0, c1 = WM[name]
            m = jnp.dot(cs, wmb[:, c0 * L:c1 * L], preferred_element_type=f32)
            for c in range(c0, c1):
                mod[c] = m[0:1, (c - c0) * L:(c - c0 + 1) * L]
        return []

    def modv(i, t0=0, t1=NT):
        return jnp.concatenate([mod[i * NT + n] for n in range(t0, t1)], axis=1)

    def job_kv(j, a, deps):
        lo = lambda x: lax.bitcast_convert_type(x << 16, f32)
        hi = lambda x: lax.bitcast_convert_type(x & jnp.uint32(0xFFFF0000), f32)
        n = C // 8
        ld = lambda ref, o: ref[pl.ds(a * n * WPT + 4 * j + o, n, stride=WPT), :]
        k = {}
        for m in range(4):
            x = ld(kw, PAD + m)
            k[2 * m], k[2 * m + 1] = lo(x), hi(x)
        k[-3] = hi(ld(kw, PAD - WPT + 2))
        x = ld(kw, PAD - WPT + 3)
        k[-2], k[-1] = lo(x), hi(x)
        w = [skt[t:t + 1, j * L:(j + 1) * L] for t in range(KS)]
        w[0] = gate(jnp.broadcast_to(w[0], (n, L)), deps)
        kv = {}
        for m in range(4):
            x = ld(vw, m)
            for ph, v in ((2 * m, lo(x)), (2 * m + 1, hi(x))):
                ks = k[ph] * w[0]
                for t in range(1, KS):
                    ks = ks + k[ph - t] * w[t]
                kv[ph] = (ks * v).reshape(n // 8, 8, L)
        for r in range(R):
            uwb[j, a, r] = jnp.concatenate([kv[r], kv[r + R]], axis=1).reshape(L, L).astype(bf16)

    def job_mac(j, us, outs, deps):
        ld = lambda ref, a: (ref[j, a, :, :, 0:8, :], ref[j, a, :, :, 8:16, :])
        lo, hi = us[0], us[-1]
        u = {a: ld(ub, a) for a in us}
        if len(deps) == 16:
            ur = jnp.concatenate([gate(u[lo][0][0:1], deps), u[lo][0][1:]], axis=0)
        else:
            ur = gate(u[lo][0], [deps[R * i + qi] for qi in range(R) for i in range(16)])
        u[lo] = (ur, u[lo][1])
        ms = sorted({a - n for a in outs for n in us if n <= a})
        k = {m: ld(kpb, m) for m in sorted(set(ms) | {m - 1 for m in ms if m > 0})}
        kp = {m: k[m] if m == 0 else (k[m][0] - k[m - 1][1], k[m][1] + k[m - 1][0]) for m in ms}
        for a in outs:
            yr, yi = ld(yp, a) if lo > 0 else (None, None)
            for n in us:
                if n > a:
                    continue
                (kr, ki), (ur, ui) = kp[a - n], u[n]
                tr = kr * ur - ki * ui
                ti = kr * ui + ki * ur
                yr = tr if yr is None else yr + tr
                yi = ti if yi is None else yi + ti
            if a > hi:
                yp[j, a] = jnp.concatenate([yr, yi], axis=2)
                continue
            ps = _radix4([(yr[qi], yi[qi]) for qi in range(R)], +1)
            for r in range(R):
                pb[j, a, r] = jnp.concatenate(ps[r], axis=1).reshape(2 * L, L).astype(bf16)

    def job_setup(_, deps):
        def hold(r, n):
            g = gate(n[:, 0:L], [deps[8 * r + s // 2] for s in range(16)])
            return jnp.concatenate([g, g], axis=1)

        ginv.extend(_tables(True, hold))
        csf = cs[0:1].astype(f32)
        ccol.append(jnp.concatenate([jnp.broadcast_to(csf[:, t * L:(t + 1) * L], (L, L)).T
                                     for t in range(NT)], axis=0))

    def job_vmod(name, deps):
        c0, c1 = WM[name]
        n = D // VM
        for c in range(c0, c1):
            for i in range(VM):
                cc = ccol[0][i * n:(i + 1) * n]
                cc = jnp.concatenate([gate(cc[0:8], [deps[(c - c0) * VM + i]]), cc[8:]], axis=0)
                p = wmb[i * n:(i + 1) * n, c * L:(c + 1) * L].astype(f32) * cc
                mv[c, 8 * i:8 * i + 8, :] = jnp.sum(p.reshape(n // 8, 8, L), axis=0)
            mod[c] = jnp.sum(mv[c], axis=0, keepdims=True)

    grp_fn = {"z": grp_z, "k": grp_k, "u": grp_u, "i": grp_i, "mod": grp_mod}
    job_fn = {"kv": job_kv, "mac": job_mac, "vmod": job_vmod, "setup": job_setup}

    for waits, groups, jobs in SCHEDULE:
        wait(*waits)
        plan = _plan(groups, jobs)
        anchors, done = [], 0
        for g in groups + [None]:
            while done < len(jobs) and max(plan[done]) < len(anchors):
                job_fn[jobs[done][0]](*jobs[done][1:], [anchors[n] for n in plan[done]])
                done += 1
            if g is not None:
                anchors += grp_fn[g[0]](*g[1:])
        assert done == len(jobs)

    n1, dep = [], None
    for r in range(0, H0, PR1):
        x = qb0[r:r + PR1, :].astype(f32)
        if dep is not None:
            x = jnp.concatenate([gate(x[:, 0:L], [dep]), x[:, L:]], axis=1)
        n1.append(_layernorm(x))
        dep = n1[-1][:, 0:L]
    n1 = jnp.concatenate(n1, axis=0)
    wait("mB")
    grp_mod("mB")
    for g in PREP_GROUPS:
        grp_fn[g[0]](*g[1:])
    sa, ca, ga = [modv(i) for i in range(3)]
    a1 = ga * (1.0 + ca)
    b1 = ga * sa

    def o_cp(i, c0, c1, r0=0, r1=TM):
        cols = pl.ds(c0, c1 - c0)
        if i is None:
            return pltpu.make_async_copy(ob0.at[:, cols], o_hbm.at[0, pl.ds(0, TM0), cols],
                                         osem.at[NB])
        base = TM0 + i * TM + r0
        if not isinstance(i, int):
            base = pl.multiple_of(base, L)
        return pltpu.make_async_copy(ob.at[i, pl.ds(r0, r1 - r0), cols],
                                     o_hbm.at[0, pl.ds(base, r1 - r0), cols], osem.at[i])

    def prep_norm(q_ref, x1_ref, y0, r0, n, dep=None, n1=None):
        x = q_ref[r0:r0 + n, :].astype(f32)
        if dep is not None:
            x = jnp.concatenate([gate(x[:, 0:L], [dep]), x[:, L:]], axis=1)
        y = jnp.concatenate([yb[j, pl.ds(y0 + r0, n), :] for j in range(NT)], axis=1)
        x1 = x + ((_layernorm(x) if n1 is None else n1) * a1 + b1) * y
        x1_ref[r0:r0 + n, :] = x1
        return _layernorm(x1)

    n2 = [prep_norm(qb0, x1b0, 0, 0, H0, None, n1)]

    aff = []

    def prep_chain(i, r0, r1):
        y0 = TM0 + i * TM
        if not isinstance(i, int):
            y0 = pl.multiple_of(y0, L)
        dep = None
        for r in range(r0, r1, PR):
            h2 = prep_norm(qb.at[i], x1b.at[i], y0, r, PR, dep) * aff[0] + aff[1]
            h2b[i, r:r + PR, :] = h2.astype(bf16)
            dep = h2[:, 0:L]

    def gate_up(h2):
        hs = []
        for f in range(0, F, TF):
            g = jnp.dot(h2, wgb[:, f:f + TF], preferred_element_type=f32)
            u = jnp.dot(h2, wub[:, f:f + TF], preferred_element_type=f32)
            hs.append(g * u)
        return jnp.concatenate(hs, axis=1).astype(bf16)

    OC = (0, D - L, D)

    OP = ((0, D - L, 0, TM), (D - L, D, 0, TM - L), (D - L, D, TM - L, TM))

    def down(hh, gb, i):
        for c0, c1, r0, r1 in OP:
            o = jnp.dot(hh[r0:r1], wdb[:, c0:c1], preferred_element_type=f32)
            ob[i, r0:r1, c0:c1] = (x1b[i, r0:r1, c0:c1] + gb[:, c0:c1] * o).astype(bf16)
            o_cp(i, c0, c1, r0, r1).start()

    def spread(jobs, anchors):
        total, n = sum(len(_costs(j)) for j in jobs), 0
        for job in jobs:
            m = len(_costs(job))
            job_fn[job[0]](*job[1:], [anchors[(n + i) * len(anchors) // total] for i in range(m)])
            n += m

    last = NC - 1
    acc = {}

    hcache = {}

    def unit(p, n, f, half=None):
        t0, t1 = KP[p], KP[p + 1]
        if (p, half) not in hcache:
            x = jnp.concatenate(n2, axis=0) if half is None else n2[half]
            hcache[p, half] = (x[:, t0 * L:t1 * L] * (1.0 + modv(4, t0, t1))
                               + modv(3, t0, t1)).astype(bf16)
        rows = {None: slice(0, TM0), 0: slice(0, H0), 1: slice(H0, TM0)}[half]
        d = jnp.dot(hcache[p, half], (wgb if n == "g" else wub)[t0 * L:t1 * L, f:f + 4 * L],
                    preferred_element_type=f32)
        ref = gub.at["gu".index(n), rows, f:f + 4 * L]
        if p == len(KP) - 2:
            acc[n, f] = ref[...] + d
        else:
            ref[...] = d if p == 0 else ref[...] + d
        return [d[s:s + 8, 0:L] for s in range(0, d.shape[0], 16)]

    def units(us):
        return [x for u in us for x in unit(*u)]

    FS = range(0, F, 4 * L)
    full = lambda p: [(p, n, f) for f in FS for n in "gu"]
    wait("wg0", "wu0", "qh")
    units([(0, n, f, 0) for n in "gu" for f in FS])
    nb, dep = [], None
    for r in range(H0, TM0, PR2):
        nb.append(prep_norm(qb0, x1b0, 0, r, PR2, dep))
        dep = nb[-1][:, 0:L]
    n2.append(jnp.concatenate(nb, axis=0))
    units([(0, "g", f, 1) for f in FS])
    wait("wg1", "wu1", "s1", "c1")
    spread([("vmod", "s1"), ("vmod", "c1")], units([(0, "u", f, 1) for f in FS])[:20])
    spread(_m([0, 1], A3, (last,)), units(full(1)[:-1]))
    wait("wg2", "wu2", "s2", "c2")
    spread([("vmod", "s2"), ("vmod", "c2")], units(full(1)[-1:])[:20])
    spread(_m([2, 3], A3, (last,)), units(full(2)[:-1]))
    wait("wg3", "wu3", "s3", "c3", "q1")
    spread([("vmod", "s3"), ("vmod", "c3")], units(full(2)[-1:])[:20])
    units(full(3))
    aff += [1.0 + modv(4), modv(3)]
    prep_chain(0, 0, 11 * PR)
    for f in FS:
        hb[:, f:f + 4 * L] = (acc.pop(("g", f)) * acc.pop(("u", f))).astype(bf16)

    def down0(n):
        c = slice(n * L, (n + 1) * L)
        ps = [jnp.dot(hb[:, f:f + 4 * L], wdb[f:f + 4 * L, c], preferred_element_type=f32)
              for f in range(0, F, 4 * L)]
        anchors = [x[s:s + 8] for x in ps for s in range(0, TM0, 16)]
        if n == 0:
            spread([("vmod", "mG")], anchors[:40])
        ob0[:, c] = (x1b0[:, c] + mod[5 * NT + n] * (ps[0] + ps[1] + ps[2])).astype(bf16)
        return anchors

    wait("wd", "mG")
    spread(_m([4], A3, (last,)), down0(0)[40:])
    gb = modv(5)
    wait(f"k{last}", f"v{last}")
    prep_chain(0, 11 * PR, TM)
    a0, a1_ = down0(1), down0(2)
    spread(_kv(last), a0 + a1_[:len(a1_) // 2])
    for g in _u(last):
        grp_u(*g[1:])
    a0 = down0(3)
    o_cp(None, OC[0], OC[1]).start()
    a1_ = down0(4)
    o_cp(None, OC[1], OC[2]).start()
    spread(_m(T, (last,), (last,)), a0 + a1_[:len(a1_) // 2])
    for g in _iv(T, [last]):
        grp_i(*g[1:])
    wait(*[f"q{i + 1}" for i in range(1, NB)])

    def ffn(i, carry):
        h2 = h2b[i]
        prep_chain(jnp.minimum(i + 1, NB - 1), 0, TM)
        down(gate_up(h2), gb, i)
        return carry

    lax.fori_loop(0, NB, ffn, 0)

    def final_waits():
        for c0, c1 in zip(OC[:-1], OC[1:]):
            o_cp(None, c0, c1).wait()
        for i in range(NB):
            for op in OP:
                o_cp(i, *op).wait()

    if SCOPES:
        with jax.named_scope("w_out"):
            final_waits()
    else:
        final_waits()


@jax.jit
def pallas_adaLN_cond__ssm_conv_h3__glu_gated_bilinear__prompt_kernel(
    A_q: jax.Array,
    A_k: jax.Array,
    A_v: jax.Array,
    A_shift_k: jax.Array,
    A_ssm_k: jax.Array,
    A_ssm_D: jax.Array,
    B_x: jax.Array,
    B_w_gate: jax.Array,
    B_w_up: jax.Array,
    B_w_down: jax.Array,
    c: jax.Array,
    w_mod: jax.Array,
):
    del B_x
    tiles = lambda x: x.reshape(S // 8, 8, NT, L).transpose(0, 2, 1, 3).reshape(S * NT, L)
    kdt = bf16
    if WF == 2:
        kdt = u32
        tiles = lambda x: lax.bitcast_convert_type(
            x.reshape(S // 8, 4, 2, NT, L).transpose(0, 3, 1, 4, 2), u32).reshape(S * NT // 2, L)
    any_spec = pl.BlockSpec(memory_space=pl.ANY)
    return pl.pallas_call(
        _kernel,
        in_specs=[any_spec] * 11,
        out_specs=any_spec,
        out_shape=jax.ShapeDtypeStruct((1, S, D), bf16),
        scratch_shapes=[
            pltpu.VMEM((TM0, D), bf16),
            pltpu.VMEM((NB, TM, D), bf16),
            pltpu.VMEM(((4 * PAD + S * NT) // WF, L), kdt),
            pltpu.VMEM(((2 * PAD + S * NT) // WF, L), kdt),
            pltpu.VMEM((NT, L, S), bf16),
            pltpu.VMEM((D, F), bf16),
            pltpu.VMEM((D, F), bf16),
            pltpu.VMEM((F, D), bf16),
            pltpu.VMEM((D, 6 * D), bf16),
            pltpu.VMEM((NT, NC, R, L, L), bf16),
            pltpu.VMEM((NT, NC, R, 16, 16, L), f32),
            pltpu.VMEM((NT, NC, R, 16, 16, L), f32),
            pltpu.VMEM((NT, NC, R, 16, 16, L), f32),
            pltpu.VMEM((NT, NC, R, 2 * L, L), bf16),
            pltpu.VMEM((NT, S + 32, L), f32),
            pltpu.VMEM((TM0, D), f32),
            pltpu.VMEM((NB, TM, D), f32),
            pltpu.VMEM((NB, TM, D), bf16),
            pltpu.VMEM((2, TM0, F), f32),
            pltpu.VMEM((TM0, F), bf16),
            pltpu.VMEM((TM0, D), bf16),
            pltpu.VMEM((NB, TM, D), bf16),
            pltpu.VMEM((32, 8 * VM, L), f32),
            pltpu.VMEM((KS, D), bf16),
            pltpu.VMEM((D,), bf16),
            pltpu.VMEM((1, D), bf16),
            pltpu.SemaphoreType.DMA((len(DMA_ORDER),)),
            pltpu.SemaphoreType.DMA((NB + 1,)),
        ],
        compiler_params=pltpu.CompilerParams(
            vmem_limit_bytes=120 * 1024 * 1024,
            disable_bounds_checks=True, disable_semaphore_checks=True),
        name="adaln_h3_glu",
    )(A_q, tiles(A_k), tiles(A_v), A_shift_k.T, A_ssm_k, A_ssm_D, B_w_gate, B_w_up, B_w_down, c, w_mod)
```

```python
import jax
import jax.numpy as jnp
from jax import lax
import jax.experimental.pallas as pl
import jax.experimental.pallas.tpu as pltpu

S = 2048
D = 640
F = 1536
KS = 4
L = 128
NT = D // L
R = 4
C = R * L
NC = S // C
EPS = 1e-5
WPT = 4 * NT
PAD = 32
PR = 24
TM0 = 512
TM = 384
NB = (S - TM0) // TM
TF = 256
KP = (0, 1, 2, 3, 5)

WM = {"mA": (0, 10), "c0": (20, 21), "mB": (10, 16), "s1": (16, 17), "c1": (21, 22),
      "s2": (17, 18), "c2": (22, 23), "s3": (18, 20), "c3": (23, 25), "mG": (25, 30)}
WF = 1
H0 = 320
PR2 = 64
VM = 5
PR1 = 160
Q1 = 8 * PR
Q2 = 12 * PR
SCOPES = False

f32 = jnp.float32
bf16 = jnp.bfloat16
u32 = jnp.uint32


def _cos_turns(t):
    x = jnp.abs(t - jnp.floor(t) - 0.5) - 0.25
    x2 = x * x
    return x * (6.283164024 + x2 * (-41.33713150 + x2 * (81.34038544 + x2 * -70.98993683)))


def _tables(inverse, hold=None):
    shape = (L, 2 * L) if inverse else (2 * L, L)
    rho = lax.broadcasted_iota(jnp.int32, shape, 1 if inverse else 0)
    j = lax.broadcasted_iota(jnp.int32, shape, 0 if inverse else 1)
    if not inverse:
        j = _perm(j)
    a = (4 * (8 * (rho >> 4) + (rho & 7)) + 1).astype(f32) * (1.0 / (4 * C))
    off = ((rho >> 3) & 1).astype(f32) * 0.25
    ns = [(R * j + r).astype(f32) for r in range(R)]
    if hold is not None:
        ns = [hold(r, n) for r, n in enumerate(ns)]
    ts = [_cos_turns(a * n + off) for n in ns]
    return [(t * (1.0 / C) if inverse else t).astype(bf16) for t in ts]


def _perm(c):
    return 16 * (c >> 4) + 2 * (c & 7) + ((c >> 3) & 1)


def _layernorm(x):
    m = jnp.mean(x, axis=-1, keepdims=True)
    xc = x - m
    v = jnp.mean(xc * xc, axis=-1, keepdims=True)
    return xc * lax.rsqrt(v + EPS)


def _split(t):
    t = t.reshape(16, 16, L)
    return t[:, :8, :], t[:, 8:, :]


def _radix4(x, sgn):
    (ar, ai), (br, bi), (cr, ci), (dr, di) = x
    s0r, s0i, d0r, d0i = ar + cr, ai + ci, ar - cr, ai - ci
    s1r, s1i, d1r, d1i = br + dr, bi + di, br - dr, bi - di
    o0 = (s0r + s1r, s0i + s1i)
    o2 = (s0r - s1r, s0i - s1i)
    pl_ = (d0r - d1i, d0i + d1r)
    mi_ = (d0r + d1i, d0i - d1r)
    return [o0, pl_, o2, mi_] if sgn > 0 else [o0, mi_, o2, pl_]


T = range(NT)
_z = lambda j: [("z", j, a) for a in range(NC)]
_k = lambda j, al: [("k", j, a) for a in al]
_u = lambda a: [("u", j, a) for j in T]
_iv = lambda jl, al: [("i", j, a) for j in jl for a in al]
_kv = lambda a: [("kv", j, a) for j in T]
_m = lambda jl, us, outs: [("mac", j, us, outs) for j in jl]
A3 = (0, 1, 2)

SCHEDULE = [
    (["ssm0"], _z(0) + _k(0, range(NC)), [("setup", None)]),
    (["ssm1"], _z(1) + _k(1, range(NC)), []),
    (["ssm2"], _z(2) + _k(2, [0, 1]), []),
    (["k0", "v0"], _k(2, [2, 3]) + _u(0), _kv(0)),
    (["ssm3"], _z(3) + _k(3, [0, 1]), _m([0, 1, 2], (0,), (0,))),
    (["k1", "v1"], _k(3, [2, 3]) + _u(1), _kv(1) + _m([3], (0,), (0,))),
    (["ssm4"], _z(4) + _k(4, range(NC)), _m([0, 1], (0, 1), (1, 2))),
    (["k2", "v2"], _iv([0, 1, 2, 3], [0]) + _u(2) + _iv([0, 1], [1]) + _iv([4], [0, 1])
     + _iv([0, 1, 4], [2]),
     _kv(2) + _m([4], (0, 1), A3) + _m([0, 1, 4], (2,), (2,)) + _m([2, 3], A3, (1, 2))),
    (["q0", "mA", "c0"], [("mod", "mA", "c0")] + _iv([2], [1, 2]), []),
]
PREP_GROUPS = _iv([3], [1, 2])

DMA_ORDER = (["sk", "sd", "c", "ssm0", "ssm1", "ssm2", "k0", "v0", "ssm3", "k1", "v1", "ssm4",
              "k2", "v2", "q0", "mA", "c0", "mB", "qh", "wg0", "wu0", "s1", "c1", "wg1", "wu1", "s2", "c2",
              "wg2", "wu2", "s3", "c3", "wg3", "wu3", "q1", "wd", "mG", "q1b", "k3", "v3"]
             + [f"q{i + 1}" for i in range(1, NB)])


def _costs(job):
    if job[0] == "kv":
        return [88] * (C // 64)
    if job[0] == "setup":
        return [100] * (8 * R)
    if job[0] == "vmod":
        return [3 * D // VM // 8] * (VM * (WM[job[1]][1] - WM[job[1]][0]))
    us, outs = job[2], job[3]
    pairs = [(a, n) for a in outs for n in us if n <= a]
    mac = (2 * len({a - n for a, n in pairs if a > n}) + 8 * len(pairs)
           - (2 * len(outs) if us[0] == 0 else 0))
    fin = 20 * sum(a <= us[-1] for a in outs)
    if mac < 12 and outs[-1] <= us[-1]:
        return [1 + R * mac + fin] * 16
    return [1 + mac, 1 + mac, 1 + mac, 1 + mac + fin] * 16


def _plan(groups, jobs):
    free = {"i": 56, "z": 56, "k": 47, "u": 46}
    steps = {"i": 16, "z": 8, "k": 16, "u": 16, "mod": 0}
    slots = [free[g[0]] for g in groups for _ in range(steps[g[0]])]
    rate = max(1.03 * sum(sum(_costs(j)) for j in jobs) / sum(slots), 1.0)
    plan, credit, n = [], slots[0] * rate, 0
    for job in jobs:
        limit, first = len(slots), 0
        for g in groups:
            if g[1] == job[1] and ((g[0], job[0]) == ("u", "kv") and g[2] == job[2]
                                   or (g[0], job[0]) == ("i", "mac") and g[2] in job[3]
                                   and g[2] <= job[2][-1]):
                limit = min(limit, first)
            first += steps[g[0]]
            if g[1] == job[1] and (g[0], job[0]) == ("u", "mac") and g[2] in job[2]:
                while n < first:
                    n += 1
                    credit = min(credit + slots[n] * rate, slots[n] * rate)
        idx = []
        for c in _costs(job):
            while credit <= 0 and n + 1 < limit:
                n += 1
                credit += slots[n] * rate
            credit -= c
            idx.append(n)
        plan.append(idx)
    return plan


def _kernel(q_hbm, k_hbm, v_hbm, sk_hbm, ssm_hbm, sd_hbm, wg_hbm, wu_hbm, wd_hbm,
            c_hbm, wm_hbm, o_hbm,
            qb0, qb, kb, vb, ssmb, wgb, wub, wdb, wmb, uwb, ub, kpb, yp, pb, yb, x1b0, x1b, h2b, gub, hb, ob0, ob, mv, skb, sdb, cb_, sem, osem):
    cps = {"sk": (sk_hbm, skb), "sd": (sd_hbm, sdb), "c": (c_hbm, cb_), "wd": (wd_hbm, wdb),
           }
    for j in range(NT):
        cps[f"ssm{j}"] = (ssm_hbm.at[pl.ds(j * L, L), :], ssmb.at[j])
    for a in range(NC):
        n = C * NT // WF
        cps[f"k{a}"] = (k_hbm.at[pl.ds(a * n, n), :], kb.at[pl.ds(2 * PAD // WF + a * n, n), :])
        cps[f"v{a}"] = (v_hbm.at[pl.ds(a * n, n), :], vb.at[pl.ds(a * n, n), :])
    for n, (c0, c1) in WM.items():
        cols = pl.ds(c0 * L, (c1 - c0) * L)
        cps[n] = (wm_hbm.at[:, cols], wmb.at[:, cols])
    cps["q0"] = (q_hbm.at[0, pl.ds(0, H0), :], qb0.at[pl.ds(0, H0), :])
    cps["qh"] = (q_hbm.at[0, pl.ds(H0, TM0 - H0), :], qb0.at[pl.ds(H0, TM0 - H0), :])
    cps["q1"] = (q_hbm.at[0, pl.ds(TM0, Q1), :], qb.at[0, pl.ds(0, Q1), :])
    cps["q1b"] = (q_hbm.at[0, pl.ds(TM0 + Q1, TM - Q1), :], qb.at[0, pl.ds(Q1, TM - Q1), :])
    for i in range(1, NB):
        cps[f"q{i + 1}"] = (q_hbm.at[0, pl.ds(TM0 + i * TM, TM), :], qb.at[i])
    for p in range(len(KP) - 1):
        rows = pl.ds(KP[p] * L, (KP[p + 1] - KP[p]) * L)
        cps[f"wg{p}"] = (wg_hbm.at[rows, :], wgb.at[rows, :])
        cps[f"wu{p}"] = (wu_hbm.at[rows, :], wub.at[rows, :])
    assert sorted(cps) == sorted(DMA_ORDER)

    def cp(name):
        src, dst = cps[name]
        return pltpu.make_async_copy(src, dst, sem.at[DMA_ORDER.index(name)])

    def wait(*names):
        if SCOPES:
            with jax.named_scope("w_" + names[0]):
                for n in names:
                    cp(n).wait()
        else:
            for n in names:
                cp(n).wait()

    for n in DMA_ORDER:
        cp(n).start()

    tabs, ginv, ccol = _tables(False), [], []
    kb[0:2 * PAD // WF, :] = jnp.zeros((2 * PAD // WF, L), kb.dtype)
    kw, vw = (kb, vb) if WF == 2 else (kb.bitcast(u32), vb.bitcast(u32))
    ub[0, 0, 0, 0, pl.ds(0, 8, stride=2), :] = jnp.zeros((8, L), f32)
    mv[0, pl.ds(0, 8, stride=2), :] = jnp.zeros((8, L), f32)
    ri = lax.broadcasted_iota(jnp.int32, (L, L), 0)
    ci = lax.broadcasted_iota(jnp.int32, (L, L), 1)
    sel = jnp.where(ci == R * _perm(ri & 31) + (ri >> 5), 1.0, 0.0).astype(bf16)

    wait("sk", "sd", "c")
    skt = skb[...].astype(f32)
    sdv = sdb[...].astype(f32).reshape(1, D)
    cv = cb_[...].astype(f32)
    sig = jax.nn.sigmoid(cv)
    cs = jnp.broadcast_to((cv * sig).astype(bf16), (16, D))
    one = sig[:, 0:L]

    def gate(x, deps):
        dep = jnp.concatenate(deps, axis=0).reshape(x.shape)
        return jnp.where(jnp.broadcast_to(one, x.shape) > 2.0, dep, x)

    def put(dst, j, a, xs):
        for qi in range(R):
            dst[j, a, qi] = jnp.concatenate(xs[qi], axis=1)

    zs = {}
    mod = {}

    def grp_z(j, a):
        z = [lax.dot_general(sel, ssmb[j, :, t * L:(t + 1) * L], (((1,), (1,)), ((), ())),
                             preferred_element_type=f32) for t in range(R * a, R * a + R)]
        zs[j, a] = [jnp.concatenate([z[p][32 * r:32 * (r + 1)] for p in range(R)],
                                    axis=0).astype(bf16) for r in range(R)]
        return [z[0][16 * t:16 * t + 8] for t in range(8)]

    def grp_fwd(ws, dst, j, a, dvec=None):
        t = [jnp.dot(tabs[r], ws[r], preferred_element_type=f32) for r in range(R)]
        x = [_split(v) for v in t]
        if dvec is not None:
            x[0] = (x[0][0] + dvec[None], x[0][1])
        put(dst, j, a, _radix4(x, -1))
        return [t[0][16 * s:16 * s + 8] for s in range(16)]

    def grp_k(j, a):
        return grp_fwd(zs.pop((j, a)), kpb, j, a,
                       sdv[:, j * L:(j + 1) * L] if a == 0 else None)

    def grp_u(j, a):
        uw = [uwb[j, a, r] for r in range(R)]
        return grp_fwd(uw, ub, j, a)

    def grp_i(j, a):
        ys = []
        for r in range(R):
            y = jnp.dot(ginv[r], pb[j, a, r], preferred_element_type=f32)
            yb[j, pl.ds(a * C + r, L, stride=R), :] = y
            ys.append(y)
        return ([ys[0][16 * s:16 * s + 8] for s in range(8)]
                + [ys[2][16 * s:16 * s + 8] for s in range(8)])

    def grp_mod(*names):
        for name in names:
            c0, c1 = WM[name]
            m = jnp.dot(cs, wmb[:, c0 * L:c1 * L], preferred_element_type=f32)
            for c in range(c0, c1):
                mod[c] = m[0:1, (c - c0) * L:(c - c0 + 1) * L]
        return []

    def modv(i, t0=0, t1=NT):
        return jnp.concatenate([mod[i * NT + n] for n in range(t0, t1)], axis=1)

    def job_kv(j, a, deps):
        lo = lambda x: lax.bitcast_convert_type(x << 16, f32)
        hi = lambda x: lax.bitcast_convert_type(x & jnp.uint32(0xFFFF0000), f32)
        n = C // 8
        ld = lambda ref, o: ref[pl.ds(a * n * WPT + 4 * j + o, n, stride=WPT), :]
        k = {}
        for m in range(4):
            x = ld(kw, PAD + m)
            k[2 * m], k[2 * m + 1] = lo(x), hi(x)
        k[-3] = hi(ld(kw, PAD - WPT + 2))
        x = ld(kw, PAD - WPT + 3)
        k[-2], k[-1] = lo(x), hi(x)
        w = [skt[t:t + 1, j * L:(j + 1) * L] for t in range(KS)]
        w[0] = gate(jnp.broadcast_to(w[0], (n, L)), deps)
        kv = {}
        for m in range(4):
            x = ld(vw, m)
            for ph, v in ((2 * m, lo(x)), (2 * m + 1, hi(x))):
                ks = k[ph] * w[0]
                for t in range(1, KS):
                    ks = ks + k[ph - t] * w[t]
                kv[ph] = (ks * v).reshape(n // 8, 8, L)
        for r in range(R):
            uwb[j, a, r] = jnp.concatenate([kv[r], kv[r + R]], axis=1).reshape(L, L).astype(bf16)

    def job_mac(j, us, outs, deps):
        ld = lambda ref, a: (ref[j, a, :, :, 0:8, :], ref[j, a, :, :, 8:16, :])
        lo, hi = us[0], us[-1]
        u = {a: ld(ub, a) for a in us}
        if len(deps) == 16:
            ur = jnp.concatenate([gate(u[lo][0][0:1], deps), u[lo][0][1:]], axis=0)
        else:
            ur = gate(u[lo][0], [deps[R * i + qi] for qi in range(R) for i in range(16)])
        u[lo] = (ur, u[lo][1])
        ms = sorted({a - n for a in outs for n in us if n <= a})
        k = {m: ld(kpb, m) for m in sorted(set(ms) | {m - 1 for m in ms if m > 0})}
        kp = {m: k[m] if m == 0 else (k[m][0] - k[m - 1][1], k[m][1] + k[m - 1][0]) for m in ms}
        for a in outs:
            yr, yi = ld(yp, a) if lo > 0 else (None, None)
            for n in us:
                if n > a:
                    continue
                (kr, ki), (ur, ui) = kp[a - n], u[n]
                tr = kr * ur - ki * ui
                ti = kr * ui + ki * ur
                yr = tr if yr is None else yr + tr
                yi = ti if yi is None else yi + ti
            if a > hi:
                yp[j, a] = jnp.concatenate([yr, yi], axis=2)
                continue
            ps = _radix4([(yr[qi], yi[qi]) for qi in range(R)], +1)
            for r in range(R):
                pb[j, a, r] = jnp.concatenate(ps[r], axis=1).reshape(2 * L, L).astype(bf16)

    def job_setup(_, deps):
        def hold(r, n):
            g = gate(n[:, 0:L], [deps[8 * r + s // 2] for s in range(16)])
            return jnp.concatenate([g, g], axis=1)

        ginv.extend(_tables(True, hold))
        csf = cs[0:1].astype(f32)
        ccol.append(jnp.concatenate([jnp.broadcast_to(csf[:, t * L:(t + 1) * L], (L, L)).T
                                     for t in range(NT)], axis=0))

    def job_vmod(name, deps):
        c0, c1 = WM[name]
        n = D // VM
        for c in range(c0, c1):
            for i in range(VM):
                cc = ccol[0][i * n:(i + 1) * n]
                cc = jnp.concatenate([gate(cc[0:8], [deps[(c - c0) * VM + i]]), cc[8:]], axis=0)
                p = wmb[i * n:(i + 1) * n, c * L:(c + 1) * L].astype(f32) * cc
                mv[c, 8 * i:8 * i + 8, :] = jnp.sum(p.reshape(n // 8, 8, L), axis=0)
            mod[c] = jnp.sum(mv[c], axis=0, keepdims=True)

    grp_fn = {"z": grp_z, "k": grp_k, "u": grp_u, "i": grp_i, "mod": grp_mod}
    job_fn = {"kv": job_kv, "mac": job_mac, "vmod": job_vmod, "setup": job_setup}

    for waits, groups, jobs in SCHEDULE:
        wait(*waits)
        plan = _plan(groups, jobs)
        anchors, done = [], 0
        for g in groups + [None]:
            while done < len(jobs) and max(plan[done]) < len(anchors):
                job_fn[jobs[done][0]](*jobs[done][1:], [anchors[n] for n in plan[done]])
                done += 1
            if g is not None:
                anchors += grp_fn[g[0]](*g[1:])
        assert done == len(jobs)

    n1, dep = [], None
    for r in range(0, H0, PR1):
        x = qb0[r:r + PR1, :].astype(f32)
        if dep is not None:
            x = jnp.concatenate([gate(x[:, 0:L], [dep]), x[:, L:]], axis=1)
        n1.append(_layernorm(x))
        dep = n1[-1][:, 0:L]
    n1 = jnp.concatenate(n1, axis=0)
    wait("mB")
    grp_mod("mB")
    for g in PREP_GROUPS:
        grp_fn[g[0]](*g[1:])
    sa, ca, ga = [modv(i) for i in range(3)]
    a1 = ga * (1.0 + ca)
    b1 = ga * sa

    def o_cp(i, c0, c1, r0=0, r1=TM):
        cols = pl.ds(c0, c1 - c0)
        if i is None:
            return pltpu.make_async_copy(ob0.at[:, cols], o_hbm.at[0, pl.ds(0, TM0), cols],
                                         osem.at[NB])
        base = TM0 + i * TM + r0
        if not isinstance(i, int):
            base = pl.multiple_of(base, L)
        return pltpu.make_async_copy(ob.at[i, pl.ds(r0, r1 - r0), cols],
                                     o_hbm.at[0, pl.ds(base, r1 - r0), cols], osem.at[i])

    def prep_norm(q_ref, x1_ref, y0, r0, n, dep=None, n1=None):
        x = q_ref[r0:r0 + n, :].astype(f32)
        if dep is not None:
            x = jnp.concatenate([gate(x[:, 0:L], [dep]), x[:, L:]], axis=1)
        y = jnp.concatenate([yb[j, pl.ds(y0 + r0, n), :] for j in range(NT)], axis=1)
        x1 = x + ((_layernorm(x) if n1 is None else n1) * a1 + b1) * y
        x1_ref[r0:r0 + n, :] = x1
        return _layernorm(x1)

    n2 = [prep_norm(qb0, x1b0, 0, 0, H0, None, n1)]

    aff = []

    def prep_chain(i, r0, r1):
        y0 = TM0 + i * TM
        if not isinstance(i, int):
            y0 = pl.multiple_of(y0, L)
        dep = None
        for r in range(r0, r1, PR):
            h2 = prep_norm(qb.at[i], x1b.at[i], y0, r, PR, dep) * aff[0] + aff[1]
            h2b[i, r:r + PR, :] = h2.astype(bf16)
            dep = h2[:, 0:L]

    def gate_up(h2):
        hs = []
        for f in range(0, F, TF):
            g = jnp.dot(h2, wgb[:, f:f + TF], preferred_element_type=f32)
            u = jnp.dot(h2, wub[:, f:f + TF], preferred_element_type=f32)
            hs.append(g * u)
        return jnp.concatenate(hs, axis=1).astype(bf16)

    OC = (0, D - L, D)

    OP = ((0, D - L, 0, TM), (D - L, D, 0, TM - L), (D - L, D, TM - L, TM))

    def down(hh, gb, i):
        for c0, c1, r0, r1 in OP:
            o = jnp.dot(hh[r0:r1], wdb[:, c0:c1], preferred_element_type=f32)
            ob[i, r0:r1, c0:c1] = (x1b[i, r0:r1, c0:c1] + gb[:, c0:c1] * o).astype(bf16)
            o_cp(i, c0, c1, r0, r1).start()

    def spread(jobs, anchors):
        total, n = sum(len(_costs(j)) for j in jobs), 0
        for job in jobs:
            m = len(_costs(job))
            job_fn[job[0]](*job[1:], [anchors[(n + i) * len(anchors) // total] for i in range(m)])
            n += m

    last = NC - 1
    acc = {}

    hcache = {}

    def unit(p, n, f, half=None):
        t0, t1 = KP[p], KP[p + 1]
        if (p, half) not in hcache:
            x = jnp.concatenate(n2, axis=0) if half is None else n2[half]
            hcache[p, half] = (x[:, t0 * L:t1 * L] * (1.0 + modv(4, t0, t1))
                               + modv(3, t0, t1)).astype(bf16)
        rows = {None: slice(0, TM0), 0: slice(0, H0), 1: slice(H0, TM0)}[half]
        d = jnp.dot(hcache[p, half], (wgb if n == "g" else wub)[t0 * L:t1 * L, f:f + 4 * L],
                    preferred_element_type=f32)
        ref = gub.at["gu".index(n), rows, f:f + 4 * L]
        if p == len(KP) - 2:
            acc[n, f] = ref[...] + d
        else:
            ref[...] = d if p == 0 else ref[...] + d
        return [d[s:s + 8, 0:L] for s in range(0, d.shape[0], 16)]

    def units(us):
        return [x for u in us for x in unit(*u)]

    FS = range(0, F, 4 * L)
    full = lambda p: [(p, n, f) for f in FS for n in "gu"]
    wait("wg0", "wu0", "qh")
    units([(0, n, f, 0) for n in "gu" for f in FS])
    nb, dep = [], None
    for r in range(H0, TM0, PR2):
        nb.append(prep_norm(qb0, x1b0, 0, r, PR2, dep))
        dep = nb[-1][:, 0:L]
    n2.append(jnp.concatenate(nb, axis=0))
    units([(0, "g", f, 1) for f in FS])
    wait("wg1", "wu1", "s1", "c1")
    spread([("vmod", "s1"), ("vmod", "c1")], units([(0, "u", f, 1) for f in FS])[:20])
    spread(_m([0, 1], A3, (last,)), units(full(1)[:-1]))
    wait("wg2", "wu2", "s2", "c2")
    spread([("vmod", "s2"), ("vmod", "c2")], units(full(1)[-1:])[:20])
    spread(_m([2, 3], A3, (last,)), units(full(2)[:-1]))
    wait("wg3", "wu3", "s3", "c3", "q1")
    spread([("vmod", "s3"), ("vmod", "c3")], units(full(2)[-1:])[:20])
    units(full(3))
    aff += [1.0 + modv(4), modv(3)]
    prep_chain(0, 0, Q1)
    for f in FS:
        hb[:, f:f + 4 * L] = (acc.pop(("g", f)) * acc.pop(("u", f))).astype(bf16)

    parts = {}

    def down0(n, fs):
        c = slice(n * L, (n + 1) * L)
        anchors = []
        for f in fs:
            k = slice(f * 4 * L, (f + 1) * 4 * L)
            d = jnp.dot(hb[:, k], wdb[k, c], preferred_element_type=f32)
            parts[n] = d if f == 0 else parts[n] + d
            anchors += [d[s:s + 8] for s in range(0, TM0, 16)]
            if (n, f) == (0, 1):
                spread([("vmod", "mG")], anchors[:50])
        if fs[-1] == 2:
            ob0[:, c] = (x1b0[:, c] + mod[5 * NT + n] * parts.pop(n)).astype(bf16)
        else:
            gub[0, :, 0:L] = parts.pop(n)
        return anchors

    wait("wd", "mG", "q1b")
    prep_chain(0, Q1, Q2)
    spread(_m([4], A3, (last,)), down0(0, A3)[50:] + down0(1, (0, 1)))
    gb = modv(5)
    wait(f"k{last}", f"v{last}")
    prep_chain(0, Q2, TM)
    parts[1] = gub[0, :, 0:L]
    spread(_kv(last), down0(1, (2,)) + down0(2, A3)[:72])
    for g in _u(last):
        grp_u(*g[1:])
    a0 = down0(3, A3)
    o_cp(None, OC[0], OC[1]).start()
    a1_ = down0(4, A3)
    o_cp(None, OC[1], OC[2]).start()
    spread(_m(T, (last,), (last,)), a0 + a1_[:len(a1_) // 2])
    for g in _iv(T, [last]):
        grp_i(*g[1:])
    wait(*[f"q{i + 1}" for i in range(1, NB)])

    def ffn(i, carry):
        h2 = h2b[i]
        prep_chain(jnp.minimum(i + 1, NB - 1), 0, TM)
        down(gate_up(h2), gb, i)
        return carry

    lax.fori_loop(0, NB, ffn, 0)

    def final_waits():
        for c0, c1 in zip(OC[:-1], OC[1:]):
            o_cp(None, c0, c1).wait()
        for i in range(NB):
            for op in OP:
                o_cp(i, *op).wait()

    if SCOPES:
        with jax.named_scope("w_out"):
            final_waits()
    else:
        final_waits()


@jax.jit
def pallas_adaLN_cond__ssm_conv_h3__glu_gated_bilinear__prompt_kernel(
    A_q: jax.Array,
    A_k: jax.Array,
    A_v: jax.Array,
    A_shift_k: jax.Array,
    A_ssm_k: jax.Array,
    A_ssm_D: jax.Array,
    B_x: jax.Array,
    B_w_gate: jax.Array,
    B_w_up: jax.Array,
    B_w_down: jax.Array,
    c: jax.Array,
    w_mod: jax.Array,
):
    del B_x
    tiles = lambda x: x.reshape(S // 8, 8, NT, L).transpose(0, 2, 1, 3).reshape(S * NT, L)
    kdt = bf16
    if WF == 2:
        kdt = u32
        tiles = lambda x: lax.bitcast_convert_type(
            x.reshape(S // 8, 4, 2, NT, L).transpose(0, 3, 1, 4, 2), u32).reshape(S * NT // 2, L)
    any_spec = pl.BlockSpec(memory_space=pl.ANY)
    return pl.pallas_call(
        _kernel,
        in_specs=[any_spec] * 11,
        out_specs=any_spec,
        out_shape=jax.ShapeDtypeStruct((1, S, D), bf16),
        scratch_shapes=[
            pltpu.VMEM((TM0, D), bf16),
            pltpu.VMEM((NB, TM, D), bf16),
            pltpu.VMEM(((4 * PAD + S * NT) // WF, L), kdt),
            pltpu.VMEM(((2 * PAD + S * NT) // WF, L), kdt),
            pltpu.VMEM((NT, L, S), bf16),
            pltpu.VMEM((D, F), bf16),
            pltpu.VMEM((D, F), bf16),
            pltpu.VMEM((F, D), bf16),
            pltpu.VMEM((D, 6 * D), bf16),
            pltpu.VMEM((NT, NC, R, L, L), bf16),
            pltpu.VMEM((NT, NC, R, 16, 16, L), f32),
            pltpu.VMEM((NT, NC, R, 16, 16, L), f32),
            pltpu.VMEM((NT, NC, R, 16, 16, L), f32),
            pltpu.VMEM((NT, NC, R, 2 * L, L), bf16),
            pltpu.VMEM((NT, S + 32, L), f32),
            pltpu.VMEM((TM0, D), f32),
            pltpu.VMEM((NB, TM, D), f32),
            pltpu.VMEM((NB, TM, D), bf16),
            pltpu.VMEM((2, TM0, F), f32),
            pltpu.VMEM((TM0, F), bf16),
            pltpu.VMEM((TM0, D), bf16),
            pltpu.VMEM((NB, TM, D), bf16),
            pltpu.VMEM((32, 8 * VM, L), f32),
            pltpu.VMEM((KS, D), bf16),
            pltpu.VMEM((D,), bf16),
            pltpu.VMEM((1, D), bf16),
            pltpu.SemaphoreType.DMA((len(DMA_ORDER),)),
            pltpu.SemaphoreType.DMA((NB + 1,)),
        ],
        compiler_params=pltpu.CompilerParams(
            vmem_limit_bytes=120 * 1024 * 1024,
            disable_bounds_checks=True, disable_semaphore_checks=True),
        name="adaln_h3_glu",
    )(A_q, tiles(A_k), tiles(A_v), A_shift_k.T, A_ssm_k, A_ssm_D, B_w_gate, B_w_up, B_w_down, c, w_mod)
```

```python
import jax
import jax.numpy as jnp
from jax import lax
import jax.experimental.pallas as pl
import jax.experimental.pallas.tpu as pltpu

S = 2048
D = 640
F = 1536
KS = 4
L = 128
NT = D // L
R = 4
C = R * L
NC = S // C
EPS = 1e-5
WPT = 4 * NT
PAD = 32
PR = 24
TM0 = 512
TM = 384
NB = (S - TM0) // TM
TF = 256
KP = (0, 1, 2, 3, 5)

MA = 12
WM = {"mA": (0, MA), "c0": (20, 21), "mB": (MA, 16), "s1": (16, 17), "c1": (21, 22),
      "s2": (17, 18), "c2": (22, 23), "s3": (18, 20), "c3": (23, 25), "mG": (25, 30)}
WF = 1
H0 = 352
PR2 = 160
VM = 5
PR1 = 176
Q1 = 8 * PR
Q2 = 12 * PR
NJUNK = 11
SCOPES = False

f32 = jnp.float32
bf16 = jnp.bfloat16
u32 = jnp.uint32


def _cos_turns(t):
    x = jnp.abs(t - jnp.floor(t) - 0.5) - 0.25
    x2 = x * x
    return x * (6.283164024 + x2 * (-41.33713150 + x2 * (81.34038544 + x2 * -70.98993683)))


def _tables(inverse, hold=None):
    shape = (L, 2 * L) if inverse else (2 * L, L)
    rho = lax.broadcasted_iota(jnp.int32, shape, 1 if inverse else 0)
    j = lax.broadcasted_iota(jnp.int32, shape, 0 if inverse else 1)
    if not inverse:
        j = _perm(j)
    a = (4 * (8 * (rho >> 4) + (rho & 7)) + 1).astype(f32) * (1.0 / (4 * C))
    off = ((rho >> 3) & 1).astype(f32) * 0.25
    ns = [(R * j + r).astype(f32) for r in range(R)]
    if hold is not None:
        ns = [hold(r, n) for r, n in enumerate(ns)]
    ts = [_cos_turns(a * n + off) for n in ns]
    return [(t * (1.0 / C) if inverse else t).astype(bf16) for t in ts]


def _perm(c):
    return 16 * (c >> 4) + 2 * (c & 7) + ((c >> 3) & 1)


def _layernorm(x):
    m = jnp.mean(x, axis=-1, keepdims=True)
    xc = x - m
    v = jnp.mean(xc * xc, axis=-1, keepdims=True)
    return xc * lax.rsqrt(v + EPS)


def _split(t):
    t = t.reshape(16, 16, L)
    return t[:, :8, :], t[:, 8:, :]


def _radix4(x, sgn):
    (ar, ai), (br, bi), (cr, ci), (dr, di) = x
    s0r, s0i, d0r, d0i = ar + cr, ai + ci, ar - cr, ai - ci
    s1r, s1i, d1r, d1i = br + dr, bi + di, br - dr, bi - di
    o0 = (s0r + s1r, s0i + s1i)
    o2 = (s0r - s1r, s0i - s1i)
    pl_ = (d0r - d1i, d0i + d1r)
    mi_ = (d0r + d1i, d0i - d1r)
    return [o0, pl_, o2, mi_] if sgn > 0 else [o0, mi_, o2, pl_]


T = range(NT)
_z = lambda j: [("z", j, a) for a in range(NC)]
_k = lambda j, al: [("k", j, a) for a in al]
_u = lambda a: [("u", j, a) for j in T]
_iv = lambda jl, al: [("i", j, a) for j in jl for a in al]
_kv = lambda a: [("kv", j, a) for j in T]
_m = lambda jl, us, outs: [("mac", j, us, outs) for j in jl]
A3 = (0, 1, 2)

SCHEDULE = [
    (["ssm0"], _z(0) + _k(0, range(NC)), [("setup", None)]),
    (["ssm1"], _z(1) + _k(1, range(NC)), []),
    (["ssm2"], _z(2) + _k(2, [0, 1]), []),
    (["k0", "v0"], _k(2, [2, 3]) + _u(0), _kv(0)),
    (["ssm3"], _z(3) + _k(3, [0, 1]), _m([0, 1, 2], (0,), (0,))),
    (["k1", "v1"], _k(3, [2, 3]) + _u(1), _kv(1) + _m([3], (0,), (0,))),
    (["ssm4"], _z(4) + _k(4, range(NC)), _m([0, 1], (0, 1), (1, 2))),
    (["k2", "v2"], _iv([0, 1, 2, 3], [0]) + _u(2) + _iv([0, 1], [1]) + _iv([4], [0, 1])
     + _iv([0, 1, 4], [2]),
     _kv(2) + _m([4], (0, 1), A3) + _m([0, 1, 4], (2,), (2,)) + _m([2, 3], A3, (1, 2))),
    (["q0", "mA", "c0"], [("mod", "mA", "c0")] + _iv([2], [1, 2]), []),
]
PREP_GROUPS = _iv([3], [1, 2])

DMA_ORDER = (["sk", "sd", "c", "ssm0", "ssm1", "ssm2", "k0", "v0", "ssm3", "k1", "v1", "ssm4",
              "k2", "v2", "q0", "c0", "mA", "mB", "wg0", "qh", "wu0", "s1", "c1", "wg1", "wu1", "s2", "c2",
              "wg2", "wu2", "s3", "c3", "wg3", "wu3", "q1", "wd", "mG", "q1b", "k3", "v3"]
             + [f"q{i + 1}" for i in range(1, NB)])


def _costs(job):
    if job[0] == "kv":
        return [88] * (C // 64)
    if job[0] == "setup":
        return [100] * (8 * R)
    if job[0] == "vmod":
        return [3 * D // VM // 8] * (VM * (WM[job[1]][1] - WM[job[1]][0]))
    us, outs = job[2], job[3]
    pairs = [(a, n) for a in outs for n in us if n <= a]
    mac = (2 * len({a - n for a, n in pairs if a > n}) + 8 * len(pairs)
           - (2 * len(outs) if us[0] == 0 else 0))
    fin = 20 * sum(a <= us[-1] for a in outs)
    if mac < 12 and outs[-1] <= us[-1]:
        return [1 + R * mac + fin] * 16
    return [1 + mac, 1 + mac, 1 + mac, 1 + mac + fin] * 16


def _plan(groups, jobs):
    free = {"i": 56, "z": 56, "k": 47, "u": 46}
    steps = {"i": 16, "z": 8, "k": 16, "u": 16, "mod": 0}
    slots = [free[g[0]] for g in groups for _ in range(steps[g[0]])]
    rate = max(1.03 * sum(sum(_costs(j)) for j in jobs) / sum(slots), 1.0)
    plan, credit, n = [], slots[0] * rate, 0
    for job in jobs:
        limit, first = len(slots), 0
        for g in groups:
            if g[1] == job[1] and ((g[0], job[0]) == ("u", "kv") and g[2] == job[2]
                                   or (g[0], job[0]) == ("i", "mac") and g[2] in job[3]
                                   and g[2] <= job[2][-1]):
                limit = min(limit, first)
            first += steps[g[0]]
            if g[1] == job[1] and (g[0], job[0]) == ("u", "mac") and g[2] in job[2]:
                while n < first:
                    n += 1
                    credit = min(credit + slots[n] * rate, slots[n] * rate)
        idx = []
        for c in _costs(job):
            while credit <= 0 and n + 1 < limit:
                n += 1
                credit += slots[n] * rate
            credit -= c
            idx.append(n)
        plan.append(idx)
    return plan


def _kernel(q_hbm, k_hbm, v_hbm, sk_hbm, ssm_hbm, sd_hbm, wg_hbm, wu_hbm, wd_hbm,
            c_hbm, wm_hbm, o_hbm,
            qb0, qb, kb, vb, ssmb, wgb, wub, wdb, wmb, uwb, ub, kpb, yp, pb, yb, x1b0, x1b, h2b, gub, hb, ob0, ob, mv, skb, sdb, cb_, sem, osem):
    cps = {"sk": (sk_hbm, skb), "sd": (sd_hbm, sdb), "c": (c_hbm, cb_), "wd": (wd_hbm, wdb),
           }
    for j in range(NT):
        cps[f"ssm{j}"] = (ssm_hbm.at[pl.ds(j * L, L), :], ssmb.at[j])
    for a in range(NC):
        n = C * NT // WF
        cps[f"k{a}"] = (k_hbm.at[pl.ds(a * n, n), :], kb.at[pl.ds(2 * PAD // WF + a * n, n), :])
        cps[f"v{a}"] = (v_hbm.at[pl.ds(a * n, n), :], vb.at[pl.ds(a * n, n), :])
    for n, (c0, c1) in WM.items():
        cols = pl.ds(c0 * L, (c1 - c0) * L)
        cps[n] = (wm_hbm.at[:, cols], wmb.at[:, cols])
    cps["q0"] = (q_hbm.at[0, pl.ds(0, H0), :], qb0.at[pl.ds(0, H0), :])
    cps["qh"] = (q_hbm.at[0, pl.ds(H0, TM0 - H0), :], qb0.at[pl.ds(H0, TM0 - H0), :])
    cps["q1"] = (q_hbm.at[0, pl.ds(TM0, Q1), :], qb.at[0, pl.ds(0, Q1), :])
    cps["q1b"] = (q_hbm.at[0, pl.ds(TM0 + Q1, TM - Q1), :], qb.at[0, pl.ds(Q1, TM - Q1), :])
    for i in range(1, NB):
        cps[f"q{i + 1}"] = (q_hbm.at[0, pl.ds(TM0 + i * TM, TM), :], qb.at[i])
    for p in range(len(KP) - 1):
        rows = pl.ds(KP[p] * L, (KP[p + 1] - KP[p]) * L)
        cps[f"wg{p}"] = (wg_hbm.at[rows, :], wgb.at[rows, :])
        cps[f"wu{p}"] = (wu_hbm.at[rows, :], wub.at[rows, :])
    assert sorted(cps) == sorted(DMA_ORDER)

    def cp(name):
        src, dst = cps[name]
        return pltpu.make_async_copy(src, dst, sem.at[DMA_ORDER.index(name)])

    def wait(*names):
        if SCOPES:
            with jax.named_scope("w_" + names[0]):
                for n in names:
                    cp(n).wait()
        else:
            for n in names:
                cp(n).wait()

    for n in DMA_ORDER:
        cp(n).start()

    tabs, ginv, ccol = _tables(False), [], []
    kb[0:2 * PAD // WF, :] = jnp.zeros((2 * PAD // WF, L), kb.dtype)
    kw, vw = (kb, vb) if WF == 2 else (kb.bitcast(u32), vb.bitcast(u32))
    ub[0, 0, 0, 0, pl.ds(0, 8, stride=2), :] = jnp.zeros((8, L), f32)
    mv[0, pl.ds(0, 8, stride=2), :] = jnp.zeros((8, L), f32)
    ri = lax.broadcasted_iota(jnp.int32, (L, L), 0)
    ci = lax.broadcasted_iota(jnp.int32, (L, L), 1)
    sel = jnp.where(ci == R * _perm(ri & 31) + (ri >> 5), 1.0, 0.0).astype(bf16)

    wait("sk", "sd", "c")
    skt = skb[...].astype(f32)
    sdv = sdb[...].astype(f32).reshape(1, D)
    cv = cb_[...].astype(f32)
    sig = jax.nn.sigmoid(cv)
    cs = jnp.broadcast_to((cv * sig).astype(bf16), (16, D))
    one = sig[:, 0:L]

    def gate(x, deps):
        dep = jnp.concatenate(deps, axis=0).reshape(x.shape)
        return jnp.where(jnp.broadcast_to(one, x.shape) > 2.0, dep, x)

    def put(dst, j, a, xs):
        for qi in range(R):
            dst[j, a, qi] = jnp.concatenate(xs[qi], axis=1)

    zs = {}
    mod = {}

    def grp_z(j, a):
        z = [lax.dot_general(sel, ssmb[j, :, t * L:(t + 1) * L], (((1,), (1,)), ((), ())),
                             preferred_element_type=f32) for t in range(R * a, R * a + R)]
        zs[j, a] = [jnp.concatenate([z[p][32 * r:32 * (r + 1)] for p in range(R)],
                                    axis=0).astype(bf16) for r in range(R)]
        return [z[0][16 * t:16 * t + 8] for t in range(8)]

    def grp_fwd(ws, dst, j, a, dvec=None):
        t = [jnp.dot(tabs[r], ws[r], preferred_element_type=f32) for r in range(R)]
        x = [_split(v) for v in t]
        if dvec is not None:
            x[0] = (x[0][0] + dvec[None], x[0][1])
        put(dst, j, a, _radix4(x, -1))
        return [t[0][16 * s:16 * s + 8] for s in range(16)]

    def grp_k(j, a):
        return grp_fwd(zs.pop((j, a)), kpb, j, a,
                       sdv[:, j * L:(j + 1) * L] if a == 0 else None)

    def grp_u(j, a):
        uw = [uwb[j, a, r] for r in range(R)]
        return grp_fwd(uw, ub, j, a)

    def grp_i(j, a):
        ys = []
        for r in range(R):
            y = jnp.dot(ginv[r], pb[j, a, r], preferred_element_type=f32)
            yb[j, pl.ds(a * C + r, L, stride=R), :] = y
            ys.append(y)
        return ([ys[0][16 * s:16 * s + 8] for s in range(8)]
                + [ys[2][16 * s:16 * s + 8] for s in range(8)])

    def grp_mod(*names):
        for name in names:
            c0, c1 = WM[name]
            m = jnp.dot(cs, wmb[:, c0 * L:c1 * L], preferred_element_type=f32)
            for c in range(c0, c1):
                mod[c] = m[0:1, (c - c0) * L:(c - c0 + 1) * L]
        return []

    def modv(i, t0=0, t1=NT):
        return jnp.concatenate([mod[i * NT + n] for n in range(t0, t1)], axis=1)

    def job_kv(j, a, deps):
        lo = lambda x: lax.bitcast_convert_type(x << 16, f32)
        hi = lambda x: lax.bitcast_convert_type(x & jnp.uint32(0xFFFF0000), f32)
        n = C // 8
        ld = lambda ref, o: ref[pl.ds(a * n * WPT + 4 * j + o, n, stride=WPT), :]
        k = {}
        for m in range(4):
            x = ld(kw, PAD + m)
            k[2 * m], k[2 * m + 1] = lo(x), hi(x)
        k[-3] = hi(ld(kw, PAD - WPT + 2))
        x = ld(kw, PAD - WPT + 3)
        k[-2], k[-1] = lo(x), hi(x)
        w = [skt[t:t + 1, j * L:(j + 1) * L] for t in range(KS)]
        w[0] = gate(jnp.broadcast_to(w[0], (n, L)), deps)
        kv = {}
        for m in range(4):
            x = ld(vw, m)
            for ph, v in ((2 * m, lo(x)), (2 * m + 1, hi(x))):
                ks = k[ph] * w[0]
                for t in range(1, KS):
                    ks = ks + k[ph - t] * w[t]
                kv[ph] = (ks * v).reshape(n // 8, 8, L)
        for r in range(R):
            uwb[j, a, r] = jnp.concatenate([kv[r], kv[r + R]], axis=1).reshape(L, L).astype(bf16)

    def job_mac(j, us, outs, deps):
        ld = lambda ref, a: (ref[j, a, :, :, 0:8, :], ref[j, a, :, :, 8:16, :])
        lo, hi = us[0], us[-1]
        u = {a: ld(ub, a) for a in us}
        if len(deps) == 16:
            ur = jnp.concatenate([gate(u[lo][0][0:1], deps), u[lo][0][1:]], axis=0)
        else:
            ur = gate(u[lo][0], [deps[R * i + qi] for qi in range(R) for i in range(16)])
        u[lo] = (ur, u[lo][1])
        ms = sorted({a - n for a in outs for n in us if n <= a})
        k = {m: ld(kpb, m) for m in sorted(set(ms) | {m - 1 for m in ms if m > 0})}
        kp = {m: k[m] if m == 0 else (k[m][0] - k[m - 1][1], k[m][1] + k[m - 1][0]) for m in ms}
        for a in outs:
            yr, yi = ld(yp, a) if lo > 0 else (None, None)
            for n in us:
                if n > a:
                    continue
                (kr, ki), (ur, ui) = kp[a - n], u[n]
                tr = kr * ur - ki * ui
                ti = kr * ui + ki * ur
                yr = tr if yr is None else yr + tr
                yi = ti if yi is None else yi + ti
            if a > hi:
                yp[j, a] = jnp.concatenate([yr, yi], axis=2)
                continue
            ps = _radix4([(yr[qi], yi[qi]) for qi in range(R)], +1)
            for r in range(R):
                pb[j, a, r] = jnp.concatenate(ps[r], axis=1).reshape(2 * L, L).astype(bf16)

    def job_setup(_, deps):
        def hold(r, n):
            g = gate(n[:, 0:L], [deps[8 * r + s // 2] for s in range(16)])
            return jnp.concatenate([g, g], axis=1)

        ginv.extend(_tables(True, hold))
        csf = cs[0:1].astype(f32)
        ccol.append(jnp.concatenate([jnp.broadcast_to(csf[:, t * L:(t + 1) * L], (L, L)).T
                                     for t in range(NT)], axis=0))

    def job_vmod(name, deps):
        c0, c1 = WM[name]
        n = D // VM
        for c in range(c0, c1):
            for i in range(VM):
                cc = ccol[0][i * n:(i + 1) * n]
                cc = jnp.concatenate([gate(cc[0:8], [deps[(c - c0) * VM + i]]), cc[8:]], axis=0)
                p = wmb[i * n:(i + 1) * n, c * L:(c + 1) * L].astype(f32) * cc
                mv[c, 8 * i:8 * i + 8, :] = jnp.sum(p.reshape(n // 8, 8, L), axis=0)
            mod[c] = jnp.sum(mv[c], axis=0, keepdims=True)

    grp_fn = {"z": grp_z, "k": grp_k, "u": grp_u, "i": grp_i, "mod": grp_mod}
    job_fn = {"kv": job_kv, "mac": job_mac, "vmod": job_vmod, "setup": job_setup}

    for waits, groups, jobs in SCHEDULE:
        wait(*waits)
        plan = _plan(groups, jobs)
        anchors, done = [], 0
        for g in groups + [None]:
            while done < len(jobs) and max(plan[done]) < len(anchors):
                job_fn[jobs[done][0]](*jobs[done][1:], [anchors[n] for n in plan[done]])
                done += 1
            if g is not None:
                anchors += grp_fn[g[0]](*g[1:])
        assert done == len(jobs)

    n1, dep = [], None
    for r in range(0, H0, PR1):
        x = qb0[r:r + PR1, :].astype(f32)
        if dep is not None:
            x = jnp.concatenate([gate(x[:, 0:L], [dep]), x[:, L:]], axis=1)
        n1.append(_layernorm(x))
        dep = n1[-1][:, 0:L]
    n1 = jnp.concatenate(n1, axis=0)
    wait("mB")
    grp_mod("mB")
    for g in PREP_GROUPS:
        grp_fn[g[0]](*g[1:])
    sa, ca, ga = [modv(i) for i in range(3)]
    a1 = ga * (1.0 + ca)
    b1 = ga * sa

    def o_cp(i, c0, c1, r0=0, r1=TM):
        cols = pl.ds(c0, c1 - c0)
        if i is None:
            return pltpu.make_async_copy(ob0.at[:, cols], o_hbm.at[0, pl.ds(0, TM0), cols],
                                         osem.at[NB])
        base = TM0 + i * TM + r0
        if not isinstance(i, int):
            base = pl.multiple_of(base, L)
        return pltpu.make_async_copy(ob.at[i, pl.ds(r0, r1 - r0), cols],
                                     o_hbm.at[0, pl.ds(base, r1 - r0), cols], osem.at[i])

    def prep_norm(q_ref, x1_ref, y0, r0, n, dep=None, n1=None):
        x = q_ref[r0:r0 + n, :].astype(f32)
        if dep is not None:
            x = jnp.concatenate([gate(x[:, 0:L], [dep]), x[:, L:]], axis=1)
        y = jnp.concatenate([yb[j, pl.ds(y0 + r0, n), :] for j in range(NT)], axis=1)
        x1 = x + ((_layernorm(x) if n1 is None else n1) * a1 + b1) * y
        x1_ref[r0:r0 + n, :] = x1
        return _layernorm(x1)

    n2 = [prep_norm(qb0, x1b0, 0, 0, H0, None, n1)]

    aff = []

    def prep_chain(i, r0, r1):
        y0 = TM0 + i * TM
        if not isinstance(i, int):
            y0 = pl.multiple_of(y0, L)
        dep = None
        for r in range(r0, r1, PR):
            h2 = prep_norm(qb.at[i], x1b.at[i], y0, r, PR, dep) * aff[0] + aff[1]
            h2b[i, r:r + PR, :] = h2.astype(bf16)
            dep = h2[:, 0:L]

    def gate_up(h2):
        hs = []
        for f in range(0, F, TF):
            g = jnp.dot(h2, wgb[:, f:f + TF], preferred_element_type=f32)
            u = jnp.dot(h2, wub[:, f:f + TF], preferred_element_type=f32)
            hs.append(g * u)
        return jnp.concatenate(hs, axis=1).astype(bf16)

    OC = (0, D - L, D)

    OP = ((0, D - L, 0, TM), (D - L, D, 0, TM - L), (D - L, D, TM - L, TM))

    def down(hh, gb, i):
        for c0, c1, r0, r1 in OP:
            o = jnp.dot(hh[r0:r1], wdb[:, c0:c1], preferred_element_type=f32)
            ob[i, r0:r1, c0:c1] = (x1b[i, r0:r1, c0:c1] + gb[:, c0:c1] * o).astype(bf16)
            o_cp(i, c0, c1, r0, r1).start()

    def spread(jobs, anchors):
        total, n = sum(len(_costs(j)) for j in jobs), 0
        for job in jobs:
            m = len(_costs(job))
            job_fn[job[0]](*job[1:], [anchors[(n + i) * len(anchors) // total] for i in range(m)])
            n += m

    last = NC - 1
    acc = {}

    hcache = {}

    def unit(p, n, f, half=None):
        t0, t1 = KP[p], KP[p + 1]
        if (p, half) not in hcache:
            x = jnp.concatenate(n2, axis=0) if half is None else n2[half]
            hcache[p, half] = (x[:, t0 * L:t1 * L] * (1.0 + modv(4, t0, t1))
                               + modv(3, t0, t1)).astype(bf16)
        rows = {None: slice(0, TM0), 0: slice(0, H0), 1: slice(H0, TM0)}[half]
        d = jnp.dot(hcache[p, half], (wgb if n == "g" else wub)[t0 * L:t1 * L, f:f + 4 * L],
                    preferred_element_type=f32)
        ref = gub.at["gu".index(n), rows, f:f + 4 * L]
        if p == len(KP) - 2:
            acc[n, f] = ref[...] + d
        else:
            ref[...] = d if p == 0 else ref[...] + d
        return [d[s:s + 8, 0:L] for s in range(0, d.shape[0], 16)]

    def units(us):
        return [x for u in us for x in unit(*u)]

    FS = range(0, F, 4 * L)
    full = lambda p: [(p, n, f) for f in FS for n in "gu"]

    @pl.when(jnp.max(one) > 2.0)
    def _():
        for g in _iv(T, A3)[:NJUNK]:
            grp_i(*g[1:])

    wait("wg0", "qh")
    units([(0, "g", f, 0) for f in FS])
    nb, dep = [], None
    for r in range(H0, TM0, PR2):
        nb.append(prep_norm(qb0, x1b0, 0, r, PR2, dep))
        dep = nb[-1][:, 0:L]
    n2.append(jnp.concatenate(nb, axis=0))
    units([(0, "g", f, 1) for f in FS])
    wait("wu0", "s1", "c1")
    spread([("vmod", "s1"), ("vmod", "c1")], units([(0, "u", f) for f in FS])[:80])
    wait("wg1", "wu1", "s2", "c2")
    spread([("vmod", "s2"), ("vmod", "c2")] + _m([0, 1], A3, (last,)), units(full(1)))
    wait("wg2", "wu2", "s3", "c3")
    spread([("vmod", "s3"), ("vmod", "c3")] + _m([2, 3], A3, (last,)), units(full(2)))
    wait("wg3", "wu3", "q1")
    units(full(3))
    aff += [1.0 + modv(4), modv(3)]
    prep_chain(0, 0, Q1)
    for f in FS:
        hb[:, f:f + 4 * L] = (acc.pop(("g", f)) * acc.pop(("u", f))).astype(bf16)

    parts = {}

    def down0(n, fs):
        c = slice(n * L, (n + 1) * L)
        anchors = []
        for f in fs:
            k = slice(f * 4 * L, (f + 1) * 4 * L)
            d = jnp.dot(hb[:, k], wdb[k, c], preferred_element_type=f32)
            parts[n] = d if f == 0 else parts[n] + d
            anchors += [d[s:s + 8] for s in range(0, TM0, 16)]
            if (n, f) == (0, 1):
                spread([("vmod", "mG")], anchors[:50])
        if fs[-1] == 2:
            ob0[:, c] = (x1b0[:, c] + mod[5 * NT + n] * parts.pop(n)).astype(bf16)
        else:
            gub[0, :, 0:L] = parts.pop(n)
        return anchors

    wait("wd", "mG", "q1b")
    prep_chain(0, Q1, Q2)
    spread(_m([4], A3, (last,)), down0(0, A3)[50:] + down0(1, (0, 1)))
    gb = modv(5)
    wait(f"k{last}", f"v{last}")
    prep_chain(0, Q2, TM)
    parts[1] = gub[0, :, 0:L]
    spread(_kv(last), down0(1, (2,)) + down0(2, A3)[:72])
    for g in _u(last):
        grp_u(*g[1:])
    a0 = down0(3, A3)
    o_cp(None, OC[0], OC[1]).start()
    a1_ = down0(4, A3)
    o_cp(None, OC[1], OC[2]).start()
    spread(_m(T, (last,), (last,)), a0 + a1_[:len(a1_) // 2])
    for g in _iv(T, [last]):
        grp_i(*g[1:])
    wait(*[f"q{i + 1}" for i in range(1, NB)])

    def ffn(i, carry):
        h2 = h2b[i]
        prep_chain(jnp.minimum(i + 1, NB - 1), 0, TM)
        down(gate_up(h2), gb, i)
        return carry

    lax.fori_loop(0, NB, ffn, 0)

    def final_waits():
        for c0, c1 in zip(OC[:-1], OC[1:]):
            o_cp(None, c0, c1).wait()
        for i in range(NB):
            for op in OP:
                o_cp(i, *op).wait()

    if SCOPES:
        with jax.named_scope("w_out"):
            final_waits()
    else:
        final_waits()


@jax.jit
def pallas_adaLN_cond__ssm_conv_h3__glu_gated_bilinear__prompt_kernel(
    A_q: jax.Array,
    A_k: jax.Array,
    A_v: jax.Array,
    A_shift_k: jax.Array,
    A_ssm_k: jax.Array,
    A_ssm_D: jax.Array,
    B_x: jax.Array,
    B_w_gate: jax.Array,
    B_w_up: jax.Array,
    B_w_down: jax.Array,
    c: jax.Array,
    w_mod: jax.Array,
):
    del B_x
    tiles = lambda x: x.reshape(S // 8, 8, NT, L).transpose(0, 2, 1, 3).reshape(S * NT, L)
    kdt = bf16
    if WF == 2:
        kdt = u32
        tiles = lambda x: lax.bitcast_convert_type(
            x.reshape(S // 8, 4, 2, NT, L).transpose(0, 3, 1, 4, 2), u32).reshape(S * NT // 2, L)
    any_spec = pl.BlockSpec(memory_space=pl.ANY)
    return pl.pallas_call(
        _kernel,
        in_specs=[any_spec] * 11,
        out_specs=any_spec,
        out_shape=jax.ShapeDtypeStruct((1, S, D), bf16),
        scratch_shapes=[
            pltpu.VMEM((TM0, D), bf16),
            pltpu.VMEM((NB, TM, D), bf16),
            pltpu.VMEM(((4 * PAD + S * NT) // WF, L), kdt),
            pltpu.VMEM(((2 * PAD + S * NT) // WF, L), kdt),
            pltpu.VMEM((NT, L, S), bf16),
            pltpu.VMEM((D, F), bf16),
            pltpu.VMEM((D, F), bf16),
            pltpu.VMEM((F, D), bf16),
            pltpu.VMEM((D, 6 * D), bf16),
            pltpu.VMEM((NT, NC, R, L, L), bf16),
            pltpu.VMEM((NT, NC, R, 16, 16, L), f32),
            pltpu.VMEM((NT, NC, R, 16, 16, L), f32),
            pltpu.VMEM((NT, NC, R, 16, 16, L), f32),
            pltpu.VMEM((NT, NC, R, 2 * L, L), bf16),
            pltpu.VMEM((NT, S + 32, L), f32),
            pltpu.VMEM((TM0, D), f32),
            pltpu.VMEM((NB, TM, D), f32),
            pltpu.VMEM((NB, TM, D), bf16),
            pltpu.VMEM((2, TM0, F), f32),
            pltpu.VMEM((TM0, F), bf16),
            pltpu.VMEM((TM0, D), bf16),
            pltpu.VMEM((NB, TM, D), bf16),
            pltpu.VMEM((32, 8 * VM, L), f32),
            pltpu.VMEM((KS, D), bf16),
            pltpu.VMEM((D,), bf16),
            pltpu.VMEM((1, D), bf16),
            pltpu.SemaphoreType.DMA((len(DMA_ORDER),)),
            pltpu.SemaphoreType.DMA((NB + 1,)),
        ],
        compiler_params=pltpu.CompilerParams(
            vmem_limit_bytes=120 * 1024 * 1024,
            disable_bounds_checks=True, disable_semaphore_checks=True),
        name="adaln_h3_glu",
    )(A_q, tiles(A_k), tiles(A_v), A_shift_k.T, A_ssm_k, A_ssm_D, B_w_gate, B_w_up, B_w_down, c, w_mod)
```

```python
import jax
import jax.numpy as jnp
from jax import lax
import jax.experimental.pallas as pl
import jax.experimental.pallas.tpu as pltpu

S = 2048
D = 640
F = 1536
KS = 4
L = 128
NT = D // L
R = 4
C = R * L
NC = S // C
EPS = 1e-5
WPT = 4 * NT
PAD = 32
PR = 24
TM0 = 512
TM = 384
NB = (S - TM0) // TM
TF = 256
KP = (0, 1, 2, 3, 5)

MA = 12
WM = {"mA": (0, MA), "c0": (20, 21), "mB": (MA, 16), "s1": (16, 17), "c1": (21, 22),
      "s2": (17, 18), "c2": (22, 23), "s3": (18, 20), "c3": (23, 25), "mG": (25, 30)}
WF = 1
H0 = 352
PR2 = 160
VM = 5
PR1 = 176
Q1 = 8 * PR
Q2 = 12 * PR
NJUNK = 12
RATE = 1.05
MIN_RATE = 0.8
SCOPES = False

f32 = jnp.float32
bf16 = jnp.bfloat16
u32 = jnp.uint32


def _cos_turns(t):
    x = jnp.abs(t - jnp.floor(t) - 0.5) - 0.25
    x2 = x * x
    return x * (6.283164024 + x2 * (-41.33713150 + x2 * (81.34038544 + x2 * -70.98993683)))


def _tables(inverse, hold=None):
    shape = (L, 2 * L) if inverse else (2 * L, L)
    rho = lax.broadcasted_iota(jnp.int32, shape, 1 if inverse else 0)
    j = lax.broadcasted_iota(jnp.int32, shape, 0 if inverse else 1)
    if not inverse:
        j = _perm(j)
    a = (4 * (8 * (rho >> 4) + (rho & 7)) + 1).astype(f32) * (1.0 / (4 * C))
    off = ((rho >> 3) & 1).astype(f32) * 0.25
    ns = [(R * j + r).astype(f32) for r in range(R)]
    if hold is not None:
        ns = [hold(r, n) for r, n in enumerate(ns)]
    ts = [_cos_turns(a * n + off) for n in ns]
    return [(t * (1.0 / C) if inverse else t).astype(bf16) for t in ts]


def _perm(c):
    return 16 * (c >> 4) + 2 * (c & 7) + ((c >> 3) & 1)


def _layernorm(x):
    m = jnp.mean(x, axis=-1, keepdims=True)
    xc = x - m
    v = jnp.mean(xc * xc, axis=-1, keepdims=True)
    return xc * lax.rsqrt(v + EPS)


def _split(t):
    t = t.reshape(16, 16, L)
    return t[:, :8, :], t[:, 8:, :]


def _radix4(x, sgn):
    (ar, ai), (br, bi), (cr, ci), (dr, di) = x
    s0r, s0i, d0r, d0i = ar + cr, ai + ci, ar - cr, ai - ci
    s1r, s1i, d1r, d1i = br + dr, bi + di, br - dr, bi - di
    o0 = (s0r + s1r, s0i + s1i)
    o2 = (s0r - s1r, s0i - s1i)
    pl_ = (d0r - d1i, d0i + d1r)
    mi_ = (d0r + d1i, d0i - d1r)
    return [o0, pl_, o2, mi_] if sgn > 0 else [o0, mi_, o2, pl_]


T = range(NT)
_z = lambda j: [("z", j, a) for a in range(NC)]
_k = lambda j, al: [("k", j, a) for a in al]
_u = lambda a: [("u", j, a) for j in T]
_iv = lambda jl, al: [("i", j, a) for j in jl for a in al]
_kv = lambda a: [("kv", j, a) for j in T]
_m = lambda jl, us, outs: [("mac", j, us, outs) for j in jl]
A3 = (0, 1, 2)

SCHEDULE = [
    (["ssm0"], _z(0) + _k(0, range(NC)), [("setup", None)]),
    (["ssm1"], _z(1) + _k(1, range(NC)), []),
    (["ssm2"], _z(2) + _k(2, [0, 1]), []),
    (["k0", "v0"], _k(2, [2, 3]) + _u(0), _kv(0) + _m([0], (0,), (0,))),
    (["ssm3"], _iv([0], [0]) + _z(3) + _k(3, [0, 1]), _m([1, 2], (0,), A3)),
    (["k1", "v1"], _k(3, [2, 3]) + _u(1), _kv(1) + _m([3], (0,), (0,))),
    (["ssm4"], _iv([1], [0]) + _z(4) + _k(4, range(NC)),
     _m([0], (0, 1), (1, 2)) + _m([1, 2], (1,), (1, 2))),
    (["k2", "v2"], _iv([2, 3], [0]) + _iv([0], [1]) + _u(2) + _iv([1, 2], [1]) + _iv([4], [0, 1])
     + _iv([0, 1, 2, 4], [2]),
     _kv(2) + _m([4], (0, 1), A3) + _m([0, 1, 2, 4], (2,), (2,)) + _m([3], A3, (1, 2))),
    (["q0", "mA", "c0"], [("mod", "mA", "c0")] + _iv([3], [1]), []),
]
PREP_GROUPS = _iv([3], [2])

DMA_ORDER = (["sk", "sd", "c", "ssm0", "ssm1", "ssm2", "k0", "v0", "ssm3", "k1", "v1", "ssm4",
              "k2", "v2", "q0", "c0", "mA", "mB", "wg0", "qh", "wu0", "s1", "c1", "wg1", "wu1", "s2", "c2",
              "wg2", "wu2", "s3", "c3", "wg3", "wu3", "q1", "wd", "mG", "q1b", "k3", "v3"]
             + [f"q{i + 1}" for i in range(1, NB)])


def _costs(job):
    if job[0] == "kv":
        return [88] * (C // 64)
    if job[0] == "setup":
        return [100] * (8 * R)
    if job[0] == "vmod":
        return [3 * D // VM // 8] * (VM * (WM[job[1]][1] - WM[job[1]][0]))
    us, outs = job[2], job[3]
    pairs = [(a, n) for a in outs for n in us if n <= a]
    mac = (2 * len({a - n for a, n in pairs if a > n}) + 8 * len(pairs)
           - (2 * len(outs) if us[0] == 0 else 0))
    fin = 20 * sum(a <= us[-1] for a in outs)
    if mac < 12 and outs[-1] <= us[-1]:
        return [1 + R * mac + fin] * 16
    return [1 + mac, 1 + mac, 1 + mac, 1 + mac + fin] * 16


def _plan(groups, jobs):
    free = {"i": 56, "z": 56, "k": 47, "u": 46}
    steps = {"i": 16, "z": 8, "k": 16, "u": 16, "mod": 0}
    slots = [free[g[0]] for g in groups for _ in range(steps[g[0]])]
    plan, credit, n = [], slots[0], 0
    for k, job in enumerate(jobs):
        rate = RATE * sum(sum(_costs(j)) for j in jobs[k:]) / sum(slots[n:])
        rate = max(rate, 1.0 if job[0] == "kv" else MIN_RATE)
        limit, first = len(slots), 0
        for g in groups:
            if g[1] == job[1] and ((g[0], job[0]) == ("u", "kv") and g[2] == job[2]
                                   or (g[0], job[0]) == ("i", "mac") and g[2] in job[3]
                                   and g[2] <= job[2][-1]):
                limit = min(limit, first)
            first += steps[g[0]]
            if g[1] == job[1] and (g[0], job[0]) == ("u", "mac") and g[2] in job[2]:
                while n < first:
                    n += 1
                    credit = min(credit + slots[n] * rate, slots[n] * rate)
        idx = []
        for c in _costs(job):
            while credit <= 0 and n + 1 < limit:
                n += 1
                credit += slots[n] * rate
            credit -= c
            idx.append(n)
        plan.append(idx)
    return plan


def _kernel(q_hbm, k_hbm, v_hbm, sk_hbm, ssm_hbm, sd_hbm, wg_hbm, wu_hbm, wd_hbm,
            c_hbm, wm_hbm, o_hbm,
            qb0, qb, kb, vb, ssmb, wgb, wub, wdb, wmb, uwb, ub, kpb, yp, pb, yb, x1b0, x1b, h2b, gub, hb, ob0, ob, mv, skb, sdb, cb_, sem, osem):
    cps = {"sk": (sk_hbm, skb), "sd": (sd_hbm, sdb), "c": (c_hbm, cb_), "wd": (wd_hbm, wdb),
           }
    for j in range(NT):
        cps[f"ssm{j}"] = (ssm_hbm.at[pl.ds(j * L, L), :], ssmb.at[j])
    for a in range(NC):
        n = C * NT // WF
        cps[f"k{a}"] = (k_hbm.at[pl.ds(a * n, n), :], kb.at[pl.ds(2 * PAD // WF + a * n, n), :])
        cps[f"v{a}"] = (v_hbm.at[pl.ds(a * n, n), :], vb.at[pl.ds(a * n, n), :])
    for n, (c0, c1) in WM.items():
        cols = pl.ds(c0 * L, (c1 - c0) * L)
        cps[n] = (wm_hbm.at[:, cols], wmb.at[:, cols])
    cps["q0"] = (q_hbm.at[0, pl.ds(0, H0), :], qb0.at[pl.ds(0, H0), :])
    cps["qh"] = (q_hbm.at[0, pl.ds(H0, TM0 - H0), :], qb0.at[pl.ds(H0, TM0 - H0), :])
    cps["q1"] = (q_hbm.at[0, pl.ds(TM0, Q1), :], qb.at[0, pl.ds(0, Q1), :])
    cps["q1b"] = (q_hbm.at[0, pl.ds(TM0 + Q1, TM - Q1), :], qb.at[0, pl.ds(Q1, TM - Q1), :])
    for i in range(1, NB):
        cps[f"q{i + 1}"] = (q_hbm.at[0, pl.ds(TM0 + i * TM, TM), :], qb.at[i])
    for p in range(len(KP) - 1):
        rows = pl.ds(KP[p] * L, (KP[p + 1] - KP[p]) * L)
        cps[f"wg{p}"] = (wg_hbm.at[rows, :], wgb.at[rows, :])
        cps[f"wu{p}"] = (wu_hbm.at[rows, :], wub.at[rows, :])
    assert sorted(cps) == sorted(DMA_ORDER)

    def cp(name):
        src, dst = cps[name]
        return pltpu.make_async_copy(src, dst, sem.at[DMA_ORDER.index(name)])

    def wait(*names):
        if SCOPES:
            with jax.named_scope("w_" + names[0]):
                for n in names:
                    cp(n).wait()
        else:
            for n in names:
                cp(n).wait()

    for n in DMA_ORDER:
        cp(n).start()

    tabs, ginv, ccol = _tables(False), [], []
    kb[0:2 * PAD // WF, :] = jnp.zeros((2 * PAD // WF, L), kb.dtype)
    kw, vw = (kb, vb) if WF == 2 else (kb.bitcast(u32), vb.bitcast(u32))
    ub[0, 0, 0, 0, pl.ds(0, 8, stride=2), :] = jnp.zeros((8, L), f32)
    mv[0, pl.ds(0, 8, stride=2), :] = jnp.zeros((8, L), f32)
    ri = lax.broadcasted_iota(jnp.int32, (L, L), 0)
    ci = lax.broadcasted_iota(jnp.int32, (L, L), 1)
    sel = jnp.where(ci == R * _perm(ri & 31) + (ri >> 5), 1.0, 0.0).astype(bf16)

    wait("sk", "sd", "c")
    skt = skb[...].astype(f32)
    sdv = sdb[...].astype(f32).reshape(1, D)
    cv = cb_[...].astype(f32)
    sig = jax.nn.sigmoid(cv)
    cs = jnp.broadcast_to((cv * sig).astype(bf16), (16, D))
    one = sig[:, 0:L]

    def gate(x, deps):
        dep = jnp.concatenate(deps, axis=0).reshape(x.shape)
        return jnp.where(jnp.broadcast_to(one, x.shape) > 2.0, dep, x)

    def put(dst, j, a, xs):
        for qi in range(R):
            dst[j, a, qi] = jnp.concatenate(xs[qi], axis=1)

    zs = {}
    mod = {}

    def grp_z(j, a):
        z = [lax.dot_general(sel, ssmb[j, :, t * L:(t + 1) * L], (((1,), (1,)), ((), ())),
                             preferred_element_type=f32) for t in range(R * a, R * a + R)]
        zs[j, a] = [jnp.concatenate([z[p][32 * r:32 * (r + 1)] for p in range(R)],
                                    axis=0).astype(bf16) for r in range(R)]
        return [z[0][16 * t:16 * t + 8] for t in range(8)]

    def grp_fwd(ws, dst, j, a, dvec=None):
        t = [jnp.dot(tabs[r], ws[r], preferred_element_type=f32) for r in range(R)]
        x = [_split(v) for v in t]
        if dvec is not None:
            x[0] = (x[0][0] + dvec[None], x[0][1])
        put(dst, j, a, _radix4(x, -1))
        return [t[0][16 * s:16 * s + 8] for s in range(16)]

    def grp_k(j, a):
        return grp_fwd(zs.pop((j, a)), kpb, j, a,
                       sdv[:, j * L:(j + 1) * L] if a == 0 else None)

    def grp_u(j, a):
        uw = [uwb[j, a, r] for r in range(R)]
        return grp_fwd(uw, ub, j, a)

    def grp_i(j, a):
        ys = []
        for r in range(R):
            y = jnp.dot(ginv[r], pb[j, a, r], preferred_element_type=f32)
            yb[j, pl.ds(a * C + r, L, stride=R), :] = y
            ys.append(y)
        return ([ys[0][16 * s:16 * s + 8] for s in range(8)]
                + [ys[2][16 * s:16 * s + 8] for s in range(8)])

    def grp_mod(*names):
        for name in names:
            c0, c1 = WM[name]
            m = jnp.dot(cs, wmb[:, c0 * L:c1 * L], preferred_element_type=f32)
            for c in range(c0, c1):
                mod[c] = m[0:1, (c - c0) * L:(c - c0 + 1) * L]
        return []

    def modv(i, t0=0, t1=NT):
        return jnp.concatenate([mod[i * NT + n] for n in range(t0, t1)], axis=1)

    def job_kv(j, a, deps):
        lo = lambda x: lax.bitcast_convert_type(x << 16, f32)
        hi = lambda x: lax.bitcast_convert_type(x & jnp.uint32(0xFFFF0000), f32)
        n = C // 8
        ld = lambda ref, o: ref[pl.ds(a * n * WPT + 4 * j + o, n, stride=WPT), :]
        k = {}
        for m in range(4):
            x = ld(kw, PAD + m)
            k[2 * m], k[2 * m + 1] = lo(x), hi(x)
        k[-3] = hi(ld(kw, PAD - WPT + 2))
        x = ld(kw, PAD - WPT + 3)
        k[-2], k[-1] = lo(x), hi(x)
        w = [skt[t:t + 1, j * L:(j + 1) * L] for t in range(KS)]
        w[0] = gate(jnp.broadcast_to(w[0], (n, L)), deps)
        kv = {}
        for m in range(4):
            x = ld(vw, m)
            for ph, v in ((2 * m, lo(x)), (2 * m + 1, hi(x))):
                ks = k[ph] * w[0]
                for t in range(1, KS):
                    ks = ks + k[ph - t] * w[t]
                kv[ph] = (ks * v).reshape(n // 8, 8, L)
        for r in range(R):
            uwb[j, a, r] = jnp.concatenate([kv[r], kv[r + R]], axis=1).reshape(L, L).astype(bf16)

    def job_mac(j, us, outs, deps):
        ld = lambda ref, a: (ref[j, a, :, :, 0:8, :], ref[j, a, :, :, 8:16, :])
        lo, hi = us[0], us[-1]
        u = {a: ld(ub, a) for a in us}
        if len(deps) == 16:
            ur = jnp.concatenate([gate(u[lo][0][0:1], deps), u[lo][0][1:]], axis=0)
        else:
            ur = gate(u[lo][0], [deps[R * i + qi] for qi in range(R) for i in range(16)])
        u[lo] = (ur, u[lo][1])
        ms = sorted({a - n for a in outs for n in us if n <= a})
        k = {m: ld(kpb, m) for m in sorted(set(ms) | {m - 1 for m in ms if m > 0})}
        kp = {m: k[m] if m == 0 else (k[m][0] - k[m - 1][1], k[m][1] + k[m - 1][0]) for m in ms}
        for a in outs:
            yr, yi = ld(yp, a) if lo > 0 else (None, None)
            for n in us:
                if n > a:
                    continue
                (kr, ki), (ur, ui) = kp[a - n], u[n]
                tr = kr * ur - ki * ui
                ti = kr * ui + ki * ur
                yr = tr if yr is None else yr + tr
                yi = ti if yi is None else yi + ti
            if a > hi:
                yp[j, a] = jnp.concatenate([yr, yi], axis=2)
                continue
            ps = _radix4([(yr[qi], yi[qi]) for qi in range(R)], +1)
            for r in range(R):
                pb[j, a, r] = jnp.concatenate(ps[r], axis=1).reshape(2 * L, L).astype(bf16)

    def job_setup(_, deps):
        def hold(r, n):
            g = gate(n[:, 0:L], [deps[8 * r + s // 2] for s in range(16)])
            return jnp.concatenate([g, g], axis=1)

        ginv.extend(_tables(True, hold))
        csf = cs[0:1].astype(f32)
        ccol.append(jnp.concatenate([jnp.broadcast_to(csf[:, t * L:(t + 1) * L], (L, L)).T
                                     for t in range(NT)], axis=0))

    def job_vmod(name, deps):
        c0, c1 = WM[name]
        n = D // VM
        for c in range(c0, c1):
            for i in range(VM):
                cc = ccol[0][i * n:(i + 1) * n]
                cc = jnp.concatenate([gate(cc[0:8], [deps[(c - c0) * VM + i]]), cc[8:]], axis=0)
                p = wmb[i * n:(i + 1) * n, c * L:(c + 1) * L].astype(f32) * cc
                mv[c, 8 * i:8 * i + 8, :] = jnp.sum(p.reshape(n // 8, 8, L), axis=0)
            mod[c] = jnp.sum(mv[c], axis=0, keepdims=True)

    grp_fn = {"z": grp_z, "k": grp_k, "u": grp_u, "i": grp_i, "mod": grp_mod}
    job_fn = {"kv": job_kv, "mac": job_mac, "vmod": job_vmod, "setup": job_setup}

    for waits, groups, jobs in SCHEDULE:
        wait(*waits)
        plan = _plan(groups, jobs)
        anchors, done = [], 0
        for g in groups + [None]:
            while done < len(jobs) and max(plan[done]) < len(anchors):
                job_fn[jobs[done][0]](*jobs[done][1:], [anchors[n] for n in plan[done]])
                done += 1
            if g is not None:
                anchors += grp_fn[g[0]](*g[1:])
        assert done == len(jobs)

    n1, dep = [], None
    for r in range(0, H0, PR1):
        x = qb0[r:r + PR1, :].astype(f32)
        if dep is not None:
            x = jnp.concatenate([gate(x[:, 0:L], [dep]), x[:, L:]], axis=1)
        n1.append(_layernorm(x))
        dep = n1[-1][:, 0:L]
    n1 = jnp.concatenate(n1, axis=0)
    wait("mB")
    grp_mod("mB")
    for g in PREP_GROUPS:
        grp_fn[g[0]](*g[1:])
    sa, ca, ga = [modv(i) for i in range(3)]
    a1 = ga * (1.0 + ca)
    b1 = ga * sa

    def o_cp(i, c0, c1, r0=0, r1=TM):
        cols = pl.ds(c0, c1 - c0)
        if i is None:
            return pltpu.make_async_copy(ob0.at[:, cols], o_hbm.at[0, pl.ds(0, TM0), cols],
                                         osem.at[NB])
        base = TM0 + i * TM + r0
        if not isinstance(i, int):
            base = pl.multiple_of(base, L)
        return pltpu.make_async_copy(ob.at[i, pl.ds(r0, r1 - r0), cols],
                                     o_hbm.at[0, pl.ds(base, r1 - r0), cols], osem.at[i])

    def prep_norm(q_ref, x1_ref, y0, r0, n, dep=None, n1=None):
        x = q_ref[r0:r0 + n, :].astype(f32)
        if dep is not None:
            x = jnp.concatenate([gate(x[:, 0:L], [dep]), x[:, L:]], axis=1)
        y = jnp.concatenate([yb[j, pl.ds(y0 + r0, n), :] for j in range(NT)], axis=1)
        x1 = x + ((_layernorm(x) if n1 is None else n1) * a1 + b1) * y
        x1_ref[r0:r0 + n, :] = x1
        return _layernorm(x1)

    n2 = [prep_norm(qb0, x1b0, 0, 0, H0, None, n1)]

    aff = []

    def prep_chain(i, r0, r1):
        y0 = TM0 + i * TM
        if not isinstance(i, int):
            y0 = pl.multiple_of(y0, L)
        dep = None
        for r in range(r0, r1, PR):
            h2 = prep_norm(qb.at[i], x1b.at[i], y0, r, PR, dep) * aff[0] + aff[1]
            h2b[i, r:r + PR, :] = h2.astype(bf16)
            dep = h2[:, 0:L]

    def gate_up(h2):
        hs = []
        for f in range(0, F, TF):
            g = jnp.dot(h2, wgb[:, f:f + TF], preferred_element_type=f32)
            u = jnp.dot(h2, wub[:, f:f + TF], preferred_element_type=f32)
            hs.append(g * u)
        return jnp.concatenate(hs, axis=1).astype(bf16)

    OC = (0, D - L, D)

    OP = ((0, D - L, 0, TM), (D - L, D, 0, TM - L), (D - L, D, TM - L, TM))

    def down(hh, gb, i):
        for c0, c1, r0, r1 in OP:
            o = jnp.dot(hh[r0:r1], wdb[:, c0:c1], preferred_element_type=f32)
            ob[i, r0:r1, c0:c1] = (x1b[i, r0:r1, c0:c1] + gb[:, c0:c1] * o).astype(bf16)
            o_cp(i, c0, c1, r0, r1).start()

    def spread(jobs, anchors):
        total, n = sum(len(_costs(j)) for j in jobs), 0
        for job in jobs:
            m = len(_costs(job))
            job_fn[job[0]](*job[1:], [anchors[(n + i) * len(anchors) // total] for i in range(m)])
            n += m

    last = NC - 1
    acc = {}

    hcache = {}

    def unit(p, n, f, half=None):
        t0, t1 = KP[p], KP[p + 1]
        if (p, half) not in hcache:
            x = jnp.concatenate(n2, axis=0) if half is None else n2[half]
            hcache[p, half] = (x[:, t0 * L:t1 * L] * (1.0 + modv(4, t0, t1))
                               + modv(3, t0, t1)).astype(bf16)
        rows = {None: slice(0, TM0), 0: slice(0, H0), 1: slice(H0, TM0)}[half]
        d = jnp.dot(hcache[p, half], (wgb if n == "g" else wub)[t0 * L:t1 * L, f:f + 4 * L],
                    preferred_element_type=f32)
        ref = gub.at["gu".index(n), rows, f:f + 4 * L]
        if p == len(KP) - 2:
            acc[n, f] = ref[...] + d
        else:
            ref[...] = d if p == 0 else ref[...] + d
        return [d[s:s + 8, 0:L] for s in range(0, d.shape[0], 16)]

    def units(us):
        return [x for u in us for x in unit(*u)]

    FS = range(0, F, 4 * L)
    full = lambda p: [(p, n, f) for f in FS for n in "gu"]

    @pl.when(jnp.max(one) > 2.0)
    def _():
        for g in _iv(T, A3)[:NJUNK]:
            grp_i(*g[1:])

    wait("wg0", "qh")
    units([(0, "g", f, 0) for f in FS])
    nb, dep = [], None
    for r in range(H0, TM0, PR2):
        nb.append(prep_norm(qb0, x1b0, 0, r, PR2, dep))
        dep = nb[-1][:, 0:L]
    n2.append(jnp.concatenate(nb, axis=0))
    units([(0, "g", f, 1) for f in FS])
    wait("wu0", "s1", "c1")
    spread([("vmod", "s1"), ("vmod", "c1")], units([(0, "u", f) for f in FS])[:80])
    wait("wg1", "wu1", "s2", "c2")
    spread([("vmod", "s2"), ("vmod", "c2")] + _m([0, 1], A3, (last,)), units(full(1)))
    wait("wg2", "wu2", "s3", "c3")
    spread([("vmod", "s3"), ("vmod", "c3")] + _m([2, 3], A3, (last,)), units(full(2)))
    wait("wg3", "wu3", "q1")
    units(full(3))
    aff += [1.0 + modv(4), modv(3)]
    prep_chain(0, 0, Q1)
    for f in FS:
        hb[:, f:f + 4 * L] = (acc.pop(("g", f)) * acc.pop(("u", f))).astype(bf16)

    parts = {}

    def down0(n, fs):
        c = slice(n * L, (n + 1) * L)
        anchors = []
        for f in fs:
            k = slice(f * 4 * L, (f + 1) * 4 * L)
            d = jnp.dot(hb[:, k], wdb[k, c], preferred_element_type=f32)
            parts[n] = d if f == 0 else parts[n] + d
            anchors += [d[s:s + 8] for s in range(0, TM0, 16)]
            if (n, f) == (0, 1):
                spread([("vmod", "mG")], anchors[:50])
        if fs[-1] == 2:
            ob0[:, c] = (x1b0[:, c] + mod[5 * NT + n] * parts.pop(n)).astype(bf16)
        else:
            gub[0, :, 0:L] = parts.pop(n)
        return anchors

    wait("wd", "mG", "q1b")
    prep_chain(0, Q1, Q2)
    spread(_m([4], A3, (last,)), down0(0, A3)[50:] + down0(1, (0, 1)))
    gb = modv(5)
    wait(f"k{last}", f"v{last}")
    prep_chain(0, Q2, TM)
    parts[1] = gub[0, :, 0:L]
    spread(_kv(last), down0(1, (2,)) + down0(2, A3)[:72])
    for g in _u(last):
        grp_u(*g[1:])
    a0 = down0(3, A3)
    o_cp(None, OC[0], OC[1]).start()
    a1_ = down0(4, A3)
    o_cp(None, OC[1], OC[2]).start()
    spread(_m(T, (last,), (last,)), a0 + a1_[:len(a1_) // 2])
    for g in _iv(T, [last]):
        grp_i(*g[1:])
    wait(*[f"q{i + 1}" for i in range(1, NB)])

    def ffn(i, carry):
        h2 = h2b[i]
        prep_chain(jnp.minimum(i + 1, NB - 1), 0, TM)
        down(gate_up(h2), gb, i)
        return carry

    lax.fori_loop(0, NB, ffn, 0)

    def final_waits():
        for c0, c1 in zip(OC[:-1], OC[1:]):
            o_cp(None, c0, c1).wait()
        for i in range(NB):
            for op in OP:
                o_cp(i, *op).wait()

    if SCOPES:
        with jax.named_scope("w_out"):
            final_waits()
    else:
        final_waits()


@jax.jit
def pallas_adaLN_cond__ssm_conv_h3__glu_gated_bilinear__prompt_kernel(
    A_q: jax.Array,
    A_k: jax.Array,
    A_v: jax.Array,
    A_shift_k: jax.Array,
    A_ssm_k: jax.Array,
    A_ssm_D: jax.Array,
    B_x: jax.Array,
    B_w_gate: jax.Array,
    B_w_up: jax.Array,
    B_w_down: jax.Array,
    c: jax.Array,
    w_mod: jax.Array,
):
    del B_x
    tiles = lambda x: x.reshape(S // 8, 8, NT, L).transpose(0, 2, 1, 3).reshape(S * NT, L)
    kdt = bf16
    if WF == 2:
        kdt = u32
        tiles = lambda x: lax.bitcast_convert_type(
            x.reshape(S // 8, 4, 2, NT, L).transpose(0, 3, 1, 4, 2), u32).reshape(S * NT // 2, L)
    any_spec = pl.BlockSpec(memory_space=pl.ANY)
    return pl.pallas_call(
        _kernel,
        in_specs=[any_spec] * 11,
        out_specs=any_spec,
        out_shape=jax.ShapeDtypeStruct((1, S, D), bf16),
        scratch_shapes=[
            pltpu.VMEM((TM0, D), bf16),
            pltpu.VMEM((NB, TM, D), bf16),
            pltpu.VMEM(((4 * PAD + S * NT) // WF, L), kdt),
            pltpu.VMEM(((2 * PAD + S * NT) // WF, L), kdt),
            pltpu.VMEM((NT, L, S), bf16),
            pltpu.VMEM((D, F), bf16),
            pltpu.VMEM((D, F), bf16),
            pltpu.VMEM((F, D), bf16),
            pltpu.VMEM((D, 6 * D), bf16),
            pltpu.VMEM((NT, NC, R, L, L), bf16),
            pltpu.VMEM((NT, NC, R, 16, 16, L), f32),
            pltpu.VMEM((NT, NC, R, 16, 16, L), f32),
            pltpu.VMEM((NT, NC, R, 16, 16, L), f32),
            pltpu.VMEM((NT, NC, R, 2 * L, L), bf16),
            pltpu.VMEM((NT, S + 32, L), f32),
            pltpu.VMEM((TM0, D), f32),
            pltpu.VMEM((NB, TM, D), f32),
            pltpu.VMEM((NB, TM, D), bf16),
            pltpu.VMEM((2, TM0, F), f32),
            pltpu.VMEM((TM0, F), bf16),
            pltpu.VMEM((TM0, D), bf16),
            pltpu.VMEM((NB, TM, D), bf16),
            pltpu.VMEM((32, 8 * VM, L), f32),
            pltpu.VMEM((KS, D), bf16),
            pltpu.VMEM((D,), bf16),
            pltpu.VMEM((1, D), bf16),
            pltpu.SemaphoreType.DMA((len(DMA_ORDER),)),
            pltpu.SemaphoreType.DMA((NB + 1,)),
        ],
        compiler_params=pltpu.CompilerParams(
            vmem_limit_bytes=120 * 1024 * 1024,
            disable_bounds_checks=True, disable_semaphore_checks=True),
        name="adaln_h3_glu",
    )(A_q, tiles(A_k), tiles(A_v), A_shift_k.T, A_ssm_k, A_ssm_D, B_w_gate, B_w_up, B_w_down, c, w_mod)
```

```python
import jax
import jax.numpy as jnp
from jax import lax
import jax.experimental.pallas as pl
import jax.experimental.pallas.tpu as pltpu

S = 2048
D = 640
F = 1536
KS = 4
L = 128
NT = D // L
R = 4
C = R * L
NC = S // C
EPS = 1e-5

WPT = 4 * NT
PAD = 32

TM0 = 512
H0 = 352
TM = 384
NB = (S - TM0) // TM
TF = 256
PR = 24
Q1, Q2 = 8 * PR, 12 * PR
KP = (0, 1, 2, 3, 5)
WM = {"mA": (0, 12), "c0": (20, 21), "mB": (12, 16), "s1": (16, 17), "c1": (21, 22),
      "s2": (17, 18), "c2": (22, 23), "s3": (18, 20), "c3": (23, 25), "mG": (25, 30)}
VM = 5

f32 = jnp.float32
bf16 = jnp.bfloat16
u32 = jnp.uint32


def _cos_turns(t):
    x = jnp.abs(t - jnp.floor(t) - 0.5) - 0.25
    x2 = x * x
    return x * (6.283164024 + x2 * (-41.33713150 + x2 * (81.34038544 + x2 * -70.98993683)))


def _tables(inverse, hold=None):
    shape = (L, 2 * L) if inverse else (2 * L, L)
    rho = lax.broadcasted_iota(jnp.int32, shape, 1 if inverse else 0)
    j = lax.broadcasted_iota(jnp.int32, shape, 0 if inverse else 1)
    if not inverse:
        j = _perm(j)
    a = (4 * (8 * (rho >> 4) + (rho & 7)) + 1).astype(f32) * (1.0 / (4 * C))
    off = ((rho >> 3) & 1).astype(f32) * 0.25
    ns = [(R * j + r).astype(f32) for r in range(R)]
    if hold is not None:
        ns = [hold(r, n) for r, n in enumerate(ns)]
    ts = [_cos_turns(a * n + off) for n in ns]
    return [(t * (1.0 / C) if inverse else t).astype(bf16) for t in ts]


def _perm(c):
    return 16 * (c >> 4) + 2 * (c & 7) + ((c >> 3) & 1)


def _layernorm(x):
    m = jnp.mean(x, axis=-1, keepdims=True)
    xc = x - m
    v = jnp.mean(xc * xc, axis=-1, keepdims=True)
    return xc * lax.rsqrt(v + EPS)


def _split(t):
    t = t.reshape(16, 16, L)
    return t[:, :8, :], t[:, 8:, :]


def _radix4(x, sgn):
    (ar, ai), (br, bi), (cr, ci), (dr, di) = x
    s0r, s0i, d0r, d0i = ar + cr, ai + ci, ar - cr, ai - ci
    s1r, s1i, d1r, d1i = br + dr, bi + di, br - dr, bi - di
    o0 = (s0r + s1r, s0i + s1i)
    o2 = (s0r - s1r, s0i - s1i)
    pl_ = (d0r - d1i, d0i + d1r)
    mi_ = (d0r + d1i, d0i - d1r)
    return [o0, pl_, o2, mi_] if sgn > 0 else [o0, mi_, o2, pl_]


T = range(NT)
_z = lambda j: [("z", j, a) for a in range(NC)]
_k = lambda j, al: [("k", j, a) for a in al]
_u = lambda a: [("u", j, a) for j in T]
_iv = lambda jl, al: [("i", j, a) for j in jl for a in al]
_kv = lambda a: [("kv", j, a) for j in T]
_m = lambda jl, us, outs: [("mac", j, us, outs) for j in jl]
A3 = (0, 1, 2)

SCHEDULE = [
    (["ssm0"], _z(0) + _k(0, range(NC)), [("setup", None)]),
    (["ssm1"], _z(1) + _k(1, range(NC)), []),
    (["ssm2"], _z(2) + _k(2, [0, 1]), []),
    (["k0", "v0"], _k(2, [2, 3]) + _u(0), _kv(0) + _m([0], (0,), (0,))),
    (["ssm3"], _iv([0], [0]) + _z(3) + _k(3, [0, 1]), _m([1, 2], (0,), A3)),
    (["k1", "v1"], _k(3, [2, 3]) + _u(1), _kv(1) + _m([3], (0,), (0,))),
    (["ssm4"], _iv([1], [0]) + _z(4) + _k(4, range(NC)),
     _m([0], (0, 1), (1, 2)) + _m([1, 2], (1,), (1, 2))),
    (["k2", "v2"], _iv([2, 3], [0]) + _iv([0], [1]) + _u(2) + _iv([1, 2], [1]) + _iv([4], [0, 1])
     + _iv([0, 1, 2, 4], [2]),
     _kv(2) + _m([4], (0, 1), A3) + _m([0, 1, 2, 4], (2,), (2,)) + _m([3], A3, (1, 2))),
    (["q0", "mA", "c0"], [("mod", "mA", "c0")] + _iv([3], [1]), []),
]
PREP_GROUPS = _iv([3], [2])

DMA_ORDER = (["sk", "sd", "c", "ssm0", "ssm1", "ssm2", "k0", "v0", "ssm3", "k1", "v1", "ssm4",
              "k2", "v2", "q0", "c0", "mA", "mB", "wg0", "qh", "wu0", "s1", "c1", "wg1", "wu1",
              "s2", "c2", "wg2", "wu2", "s3", "c3", "wg3", "wu3", "q1", "wd", "mG", "q1b",
              "k3", "v3", "q1c"]
             + [f"q{i + 1}" for i in range(1, NB)])


def _costs(job):
    if job[0] == "kv":
        return [88] * (C // 64)
    if job[0] == "setup":
        return [100] * (8 * R)
    if job[0] == "vmod":
        return [3 * D // VM // 8] * (VM * (WM[job[1]][1] - WM[job[1]][0]))
    us, outs = job[2], job[3]
    pairs = [(a, n) for a in outs for n in us if n <= a]
    mac = (2 * len({a - n for a, n in pairs if a > n}) + 8 * len(pairs)
           - (2 * len(outs) if us[0] == 0 else 0))
    fin = 20 * sum(a <= us[-1] for a in outs)
    if mac < 12 and outs[-1] <= us[-1]:
        return [1 + R * mac + fin] * 16
    return [1 + mac, 1 + mac, 1 + mac, 1 + mac + fin] * 16


def _plan(groups, jobs):
    free = {"i": 56, "z": 56, "k": 47, "u": 46}
    steps = {"i": 16, "z": 8, "k": 16, "u": 16, "mod": 0}
    slots = [free[g[0]] for g in groups for _ in range(steps[g[0]])]
    plan, credit, n = [], slots[0], 0
    for k, job in enumerate(jobs):
        rate = 1.05 * sum(sum(_costs(j)) for j in jobs[k:]) / sum(slots[n:])
        rate = max(rate, 1.0 if job[0] == "kv" else 0.8)
        limit, first = len(slots), 0
        for g in groups:
            if g[1] == job[1] and ((g[0], job[0]) == ("u", "kv") and g[2] == job[2]
                                   or (g[0], job[0]) == ("i", "mac") and g[2] in job[3]
                                   and g[2] <= job[2][-1]):
                limit = min(limit, first)
            first += steps[g[0]]
            if g[1] == job[1] and (g[0], job[0]) == ("u", "mac") and g[2] in job[2]:
                while n < first:
                    n += 1
                    credit = min(credit + slots[n] * rate, slots[n] * rate)
        idx = []
        for c in _costs(job):
            while credit <= 0 and n + 1 < limit:
                n += 1
                credit += slots[n] * rate
            credit -= c
            idx.append(n)
        plan.append(idx)
    return plan


def _kernel(q_hbm, k_hbm, v_hbm, sk_hbm, ssm_hbm, sd_hbm, wg_hbm, wu_hbm, wd_hbm,
            c_hbm, wm_hbm, o_hbm,
            qb0, qb, kbs, vbs, ssmb, wgb, wub, wdb, wmb, uwb, ub, kpb, yp, pb, yb,
            x1b0, x1b, h2b, gub, hb, ob0, ob, mv, skb, sdb, cb_, sem, osem):
    cps = {"sk": (sk_hbm, skb), "sd": (sd_hbm, sdb), "c": (c_hbm, cb_), "wd": (wd_hbm, wdb)}
    for j in range(NT):
        cps[f"ssm{j}"] = (ssm_hbm.at[pl.ds(j * L, L), :], ssmb.at[j])
    for a in range(NC):
        n, h = C * NT, 2 * PAD
        if a == 0:
            cps["k0"] = (k_hbm.at[pl.ds(0, n), :], kbs[0].at[pl.ds(h, n), :])
        else:
            e = 48
            cps[f"k{a}"] = (k_hbm.at[pl.ds(a * n - e, n + e), :],
                            kbs[a].at[pl.ds(h - e, n + e), :])
        cps[f"v{a}"] = (v_hbm.at[pl.ds(a * n, n), :], vbs[a].at[pl.ds(0, n), :])
    for n, (c0, c1) in WM.items():
        cols = pl.ds(c0 * L, (c1 - c0) * L)
        cps[n] = (wm_hbm.at[:, cols], wmb.at[:, cols])
    cps["q0"] = (q_hbm.at[0, pl.ds(0, H0), :], qb0.at[pl.ds(0, H0), :])
    cps["qh"] = (q_hbm.at[0, pl.ds(H0, TM0 - H0), :], qb0.at[pl.ds(H0, TM0 - H0), :])
    cps["q1"] = (q_hbm.at[0, pl.ds(TM0, Q1), :], qb.at[0, pl.ds(0, Q1), :])
    cps["q1b"] = (q_hbm.at[0, pl.ds(TM0 + Q1, Q2 - Q1), :], qb.at[0, pl.ds(Q1, Q2 - Q1), :])
    cps["q1c"] = (q_hbm.at[0, pl.ds(TM0 + Q2, TM - Q2), :], qb.at[0, pl.ds(Q2, TM - Q2), :])
    for i in range(1, NB):
        cps[f"q{i + 1}"] = (q_hbm.at[0, pl.ds(TM0 + i * TM, TM), :], qb.at[i])
    for p in range(len(KP) - 1):
        rows = pl.ds(KP[p] * L, (KP[p + 1] - KP[p]) * L)
        cps[f"wg{p}"] = (wg_hbm.at[rows, :], wgb.at[rows, :])
        cps[f"wu{p}"] = (wu_hbm.at[rows, :], wub.at[rows, :])
    assert sorted(cps) == sorted(DMA_ORDER)

    def cp(name):
        src, dst = cps[name]
        return pltpu.make_async_copy(src, dst, sem.at[DMA_ORDER.index(name)])

    def wait(*names):
        for n in names:
            cp(n).wait()

    kbs[0][0:2 * PAD, :] = jnp.zeros((2 * PAD, L), bf16)
    for n in DMA_ORDER:
        cp(n).start()

    tabs, ginv, ccol = _tables(False), [], []
    for ref in (ub, kpb, yp):
        ref[0, 0, 0, 0, pl.ds(0, 8, stride=2), :] = jnp.zeros((8, L), f32)
    mv[0, pl.ds(0, 8, stride=2), :] = jnp.zeros((8, L), f32)
    ri = lax.broadcasted_iota(jnp.int32, (L, L), 0)
    ci = lax.broadcasted_iota(jnp.int32, (L, L), 1)
    sel = jnp.where(ci == R * _perm(ri & 31) + (ri >> 5), 1.0, 0.0).astype(bf16)

    wait("sk", "sd", "c")
    skt = skb[...].astype(f32)
    sdv = sdb[...].astype(f32).reshape(1, D)
    cv = cb_[...].astype(f32)
    sig = jax.nn.sigmoid(cv)
    cs = jnp.broadcast_to((cv * sig).astype(bf16), (16, D))
    one = sig[:, 0:L]

    def gate(x, deps):
        dep = jnp.concatenate(deps, axis=0).reshape(x.shape)
        return jnp.where(jnp.broadcast_to(one, x.shape) > 2.0, dep, x)

    def put(dst, j, a, xs):
        for qi in range(R):
            dst[j, a, qi] = jnp.concatenate(xs[qi], axis=1)

    zs = {}
    mod = {}

    def grp_z(j, a):
        z = [lax.dot_general(sel, ssmb[j, :, t * L:(t + 1) * L], (((1,), (1,)), ((), ())),
                             preferred_element_type=f32) for t in range(R * a, R * a + R)]
        zs[j, a] = [jnp.concatenate([z[p][32 * r:32 * (r + 1)] for p in range(R)],
                                    axis=0).astype(bf16) for r in range(R)]
        return [z[0][16 * t:16 * t + 8] for t in range(8)]

    def grp_fwd(ws, dst, j, a, dvec=None):
        t = [jnp.dot(tabs[r], ws[r], preferred_element_type=f32) for r in range(R)]
        x = [_split(v) for v in t]
        if dvec is not None:
            x[0] = (x[0][0] + dvec[None], x[0][1])
        put(dst, j, a, _radix4(x, -1))
        return [t[0][16 * s:16 * s + 8] for s in range(16)]

    def grp_k(j, a):
        return grp_fwd(zs.pop((j, a)), kpb, j, a,
                       sdv[:, j * L:(j + 1) * L] if a == 0 else None)

    def grp_u(j, a):
        uw = [uwb[j, a, r] for r in range(R)]
        return grp_fwd(uw, ub, j, a)

    def grp_i(j, a):
        ys = []
        for r in range(R):
            y = jnp.dot(ginv[r], pb[j, a, r], preferred_element_type=f32)
            yb[j, pl.ds(a * C + r, L, stride=R), :] = y
            ys.append(y)
        return ([ys[0][16 * s:16 * s + 8] for s in range(8)]
                + [ys[2][16 * s:16 * s + 8] for s in range(8)])

    def grp_mod(*names):
        for name in names:
            c0, c1 = WM[name]
            m = jnp.dot(cs, wmb[:, c0 * L:c1 * L], preferred_element_type=f32)
            for c in range(c0, c1):
                mod[c] = m[0:1, (c - c0) * L:(c - c0 + 1) * L]
        return []

    def modv(i, t0=0, t1=NT):
        return jnp.concatenate([mod[i * NT + n] for n in range(t0, t1)], axis=1)

    def job_kv(j, a, deps):
        lo = lambda x: lax.bitcast_convert_type(x << 16, f32)
        hi = lambda x: lax.bitcast_convert_type(x & jnp.uint32(0xFFFF0000), f32)
        n = C // 8
        kw, vw = kbs[a].bitcast(u32), vbs[a].bitcast(u32)
        ld = lambda ref, o: ref[pl.ds(4 * j + o, n, stride=WPT), :]
        k = {}
        for m in range(4):
            x = ld(kw, PAD + m)
            k[2 * m], k[2 * m + 1] = lo(x), hi(x)
        k[-3] = hi(ld(kw, PAD - WPT + 2))
        x = ld(kw, PAD - WPT + 3)
        k[-2], k[-1] = lo(x), hi(x)
        w = [skt[t:t + 1, j * L:(j + 1) * L] for t in range(KS)]
        w[0] = gate(jnp.broadcast_to(w[0], (n, L)), deps)
        kv = {}
        for m in range(4):
            x = ld(vw, m)
            for ph, v in ((2 * m, lo(x)), (2 * m + 1, hi(x))):
                ks = k[ph] * w[0]
                for t in range(1, KS):
                    ks = ks + k[ph - t] * w[t]
                kv[ph] = (ks * v).reshape(n // 8, 8, L)
        for r in range(R):
            uwb[j, a, r] = jnp.concatenate([kv[r], kv[r + R]], axis=1).reshape(L, L).astype(bf16)

    def job_mac(j, us, outs, deps):
        ld = lambda ref, a: (ref[j, a, :, :, 0:8, :], ref[j, a, :, :, 8:16, :])
        lo, hi = us[0], us[-1]
        u = {a: ld(ub, a) for a in us}
        if len(deps) == 16:
            ur = jnp.concatenate([gate(u[lo][0][0:1], deps), u[lo][0][1:]], axis=0)
        else:
            ur = gate(u[lo][0], [deps[R * i + qi] for qi in range(R) for i in range(16)])
        u[lo] = (ur, u[lo][1])
        ms = sorted({a - n for a in outs for n in us if n <= a})
        k = {m: ld(kpb, m) for m in sorted(set(ms) | {m - 1 for m in ms if m > 0})}
        kp = {m: k[m] if m == 0 else (k[m][0] - k[m - 1][1], k[m][1] + k[m - 1][0]) for m in ms}
        for a in outs:
            yr, yi = ld(yp, a) if lo > 0 else (None, None)
            for n in us:
                if n > a:
                    continue
                (kr, ki), (ur, ui) = kp[a - n], u[n]
                tr = kr * ur - ki * ui
                ti = kr * ui + ki * ur
                yr = tr if yr is None else yr + tr
                yi = ti if yi is None else yi + ti
            if a > hi:
                yp[j, a] = jnp.concatenate([yr, yi], axis=2)
                continue
            ps = _radix4([(yr[qi], yi[qi]) for qi in range(R)], +1)
            for r in range(R):
                pb[j, a, r] = jnp.concatenate(ps[r], axis=1).reshape(2 * L, L).astype(bf16)

    def job_setup(_, deps):
        def hold(r, n):
            g = gate(n[:, 0:L], [deps[8 * r + s // 2] for s in range(16)])
            return jnp.concatenate([g, g], axis=1)

        ginv.extend(_tables(True, hold))
        csf = cs[0:1].astype(f32)
        ccol.append(jnp.concatenate([jnp.broadcast_to(csf[:, t * L:(t + 1) * L], (L, L)).T
                                     for t in range(NT)], axis=0))

    def job_vmod(name, deps):
        c0, c1 = WM[name]
        n = D // VM
        for c in range(c0, c1):
            for i in range(VM):
                cc = ccol[0][i * n:(i + 1) * n]
                cc = jnp.concatenate([gate(cc[0:8], [deps[(c - c0) * VM + i]]), cc[8:]], axis=0)
                p = wmb[i * n:(i + 1) * n, c * L:(c + 1) * L].astype(f32) * cc
                mv[c, 8 * i:8 * i + 8, :] = jnp.sum(p.reshape(n // 8, 8, L), axis=0)
            mod[c] = jnp.sum(mv[c], axis=0, keepdims=True)

    grp_fn = {"z": grp_z, "k": grp_k, "u": grp_u, "i": grp_i, "mod": grp_mod}
    job_fn = {"kv": job_kv, "mac": job_mac, "vmod": job_vmod, "setup": job_setup}

    for waits, groups, jobs in SCHEDULE:
        wait(*waits)
        plan = _plan(groups, jobs)
        anchors, done = [], 0
        for g in groups + [None]:
            while done < len(jobs) and max(plan[done]) < len(anchors):
                job_fn[jobs[done][0]](*jobs[done][1:], [anchors[n] for n in plan[done]])
                done += 1
            if g is not None:
                anchors += grp_fn[g[0]](*g[1:])
        assert done == len(jobs)

    n1, dep = [], None
    for r in range(0, H0, H0 // 2):
        x = qb0[r:r + H0 // 2, :].astype(f32)
        if dep is not None:
            x = jnp.concatenate([gate(x[:, 0:L], [dep]), x[:, L:]], axis=1)
        n1.append(_layernorm(x))
        dep = n1[-1][:, 0:L]
    n1 = jnp.concatenate(n1, axis=0)
    wait("mB")
    grp_mod("mB")
    for g in PREP_GROUPS:
        grp_fn[g[0]](*g[1:])
    sa, ca, ga = [modv(i) for i in range(3)]
    a1 = ga * (1.0 + ca)
    b1 = ga * sa

    def o_cp(i, c0, c1, r0=0, r1=TM):
        cols = pl.ds(c0, c1 - c0)
        if i is None:
            return pltpu.make_async_copy(ob0.at[:, cols], o_hbm.at[0, pl.ds(0, TM0), cols],
                                         osem.at[NB])
        base = TM0 + i * TM + r0
        if not isinstance(i, int):
            base = pl.multiple_of(base, L)
        return pltpu.make_async_copy(ob.at[i, pl.ds(r0, r1 - r0), cols],
                                     o_hbm.at[0, pl.ds(base, r1 - r0), cols], osem.at[i])

    def prep_norm(q_ref, x1_ref, y0, r0, n, dep=None, n1=None):
        x = q_ref[r0:r0 + n, :].astype(f32)
        if dep is not None:
            x = jnp.concatenate([gate(x[:, 0:L], [dep]), x[:, L:]], axis=1)
        y = jnp.concatenate([yb[j, pl.ds(y0 + r0, n), :] for j in range(NT)], axis=1)
        x1 = x + ((_layernorm(x) if n1 is None else n1) * a1 + b1) * y
        x1_ref[r0:r0 + n, :] = x1
        return _layernorm(x1)

    n2 = [prep_norm(qb0, x1b0, 0, 0, H0, None, n1)]

    aff = []

    def prep_chain(i, r0, r1):
        y0 = TM0 + i * TM
        if not isinstance(i, int):
            y0 = pl.multiple_of(y0, L)
        dep = None
        for r in range(r0, r1, PR):
            h2 = prep_norm(qb.at[i], x1b.at[i], y0, r, PR, dep) * aff[0] + aff[1]
            h2b[i, r:r + PR, :] = h2.astype(bf16)
            dep = h2[:, 0:L]

    def gate_up(h2):
        hs = []
        for f in range(0, F, TF):
            g = jnp.dot(h2, wgb[:, f:f + TF], preferred_element_type=f32)
            u = jnp.dot(h2, wub[:, f:f + TF], preferred_element_type=f32)
            hs.append(g * u)
        return jnp.concatenate(hs, axis=1).astype(bf16)

    OC = (0, D - L, D)

    OP = ((0, D - L, 0, TM), (D - L, D, 0, TM - L), (D - L, D, TM - L, TM))

    def down(hh, gb, i):
        for c0, c1, r0, r1 in OP:
            o = jnp.dot(hh[r0:r1], wdb[:, c0:c1], preferred_element_type=f32)
            ob[i, r0:r1, c0:c1] = (x1b[i, r0:r1, c0:c1] + gb[:, c0:c1] * o).astype(bf16)
            o_cp(i, c0, c1, r0, r1).start()

    def spread(jobs, anchors):
        total, n = sum(len(_costs(j)) for j in jobs), 0
        for job in jobs:
            m = len(_costs(job))
            job_fn[job[0]](*job[1:], [anchors[(n + i) * len(anchors) // total] for i in range(m)])
            n += m

    last = NC - 1
    acc = {}

    hcache = {}

    def unit(p, n, f, half=None):
        t0, t1 = KP[p], KP[p + 1]
        if (p, half) not in hcache:
            x = jnp.concatenate(n2, axis=0) if half is None else n2[half]
            hcache[p, half] = (x[:, t0 * L:t1 * L] * (1.0 + modv(4, t0, t1))
                               + modv(3, t0, t1)).astype(bf16)
        rows = {None: slice(0, TM0), 0: slice(0, H0), 1: slice(H0, TM0)}[half]
        d = jnp.dot(hcache[p, half], (wgb if n == "g" else wub)[t0 * L:t1 * L, f:f + 4 * L],
                    preferred_element_type=f32)
        ref = gub.at["gu".index(n), rows, f:f + 4 * L]
        if p == len(KP) - 2:
            acc[n, f] = ref[...] + d
        else:
            ref[...] = d if p == 0 else ref[...] + d
        return [d[s:s + 8, 0:L] for s in range(0, d.shape[0], 16)]

    def units(us):
        return [x for u in us for x in unit(*u)]

    FS = range(0, F, 4 * L)
    full = lambda p: [(p, n, f) for f in FS for n in "gu"]

    wait("wg0", "qh")
    units([(0, "g", f, 0) for f in FS])
    n2.append(prep_norm(qb0, x1b0, 0, H0, TM0 - H0))
    units([(0, "g", f, 1) for f in FS])
    wait("wu0", "s1", "c1")
    spread([("vmod", "s1"), ("vmod", "c1")], units([(0, "u", f) for f in FS])[:80])
    wait("wg1", "wu1", "s2", "c2")
    spread([("vmod", "s2"), ("vmod", "c2")] + _m([0, 1], A3, (last,)), units(full(1)))
    wait("wg2", "wu2", "s3", "c3")
    spread([("vmod", "s3"), ("vmod", "c3")] + _m([2, 3], A3, (last,)), units(full(2)))
    wait("wg3", "wu3", "q1")
    units(full(3))
    aff += [1.0 + modv(4), modv(3)]
    prep_chain(0, 0, Q1)
    for f in FS:
        hb[:, f:f + 4 * L] = (acc.pop(("g", f)) * acc.pop(("u", f))).astype(bf16)

    parts = {}

    def down0(n, fs):
        c = slice(n * L, (n + 1) * L)
        anchors = []
        for f in fs:
            k = slice(f * 4 * L, (f + 1) * 4 * L)
            d = jnp.dot(hb[:, k], wdb[k, c], preferred_element_type=f32)
            parts[n] = d if f == 0 else parts[n] + d
            anchors += [d[s:s + 8] for s in range(0, TM0, 16)]
            if (n, f) == (0, 1):
                spread([("vmod", "mG")], anchors[:50])
        if fs[-1] == 2:
            ob0[:, c] = (x1b0[:, c] + mod[5 * NT + n] * parts.pop(n)).astype(bf16)
        else:
            gub[0, :, 0:L] = parts.pop(n)
        return anchors

    wait("wd", "mG", "q1b")
    prep_chain(0, Q1, Q2)
    spread(_m([4], A3, (last,)), down0(0, A3)[50:] + down0(1, (0, 1)))
    gb = modv(5)
    wait(f"k{last}", f"v{last}", "q1c")
    prep_chain(0, Q2, TM)
    parts[1] = gub[0, :, 0:L]
    spread(_kv(last), down0(1, (2,)) + down0(2, A3)[:72])
    for g in _u(last):
        grp_u(*g[1:])
    a0 = down0(3, A3)
    o_cp(None, OC[0], OC[1]).start()
    a1_ = down0(4, A3)
    o_cp(None, OC[1], OC[2]).start()
    spread(_m(T, (last,), (last,)), a0 + a1_[:len(a1_) // 2])
    for g in _iv(T, [last]):
        grp_i(*g[1:])
    wait(*[f"q{i + 1}" for i in range(1, NB)])

    def ffn(i, carry):
        h2 = h2b[i]
        prep_chain(jnp.minimum(i + 1, NB - 1), 0, TM)
        down(gate_up(h2), gb, i)
        return carry

    lax.fori_loop(0, NB, ffn, 0)

    for c0, c1 in zip(OC[:-1], OC[1:]):
        o_cp(None, c0, c1).wait()
    for i in range(NB):
        for op in OP:
            o_cp(i, *op).wait()


@jax.jit
def pallas_adaLN_cond__ssm_conv_h3__glu_gated_bilinear__prompt_kernel(
    A_q: jax.Array,
    A_k: jax.Array,
    A_v: jax.Array,
    A_shift_k: jax.Array,
    A_ssm_k: jax.Array,
    A_ssm_D: jax.Array,
    B_x: jax.Array,
    B_w_gate: jax.Array,
    B_w_up: jax.Array,
    B_w_down: jax.Array,
    c: jax.Array,
    w_mod: jax.Array,
):
    del B_x
    tiles = lambda x: x.reshape(S // 8, 8, NT, L).transpose(0, 2, 1, 3).reshape(S * NT, L)
    any_spec = pl.BlockSpec(memory_space=pl.ANY)
    return pl.pallas_call(
        _kernel,
        in_specs=[any_spec] * 11,
        out_specs=any_spec,
        out_shape=jax.ShapeDtypeStruct((1, S, D), bf16),
        scratch_shapes=[
            pltpu.VMEM((TM0, D), bf16),
            pltpu.VMEM((NB, TM, D), bf16),
            [pltpu.VMEM((4 * PAD + C * NT, L), bf16)] * NC,
            [pltpu.VMEM((2 * PAD + C * NT, L), bf16)] * NC,
            pltpu.VMEM((NT, L, S), bf16),
            pltpu.VMEM((D, F), bf16),
            pltpu.VMEM((D, F), bf16),
            pltpu.VMEM((F, D), bf16),
            pltpu.VMEM((D, 6 * D), bf16),
            pltpu.VMEM((NT, NC, R, L, L), bf16),
            pltpu.VMEM((NT, NC, R, 16, 16, L), f32),
            pltpu.VMEM((NT, NC, R, 16, 16, L), f32),
            pltpu.VMEM((NT, NC, R, 16, 16, L), f32),
            pltpu.VMEM((NT, NC, R, 2 * L, L), bf16),
            pltpu.VMEM((NT, S + 32, L), f32),
            pltpu.VMEM((TM0, D), f32),
            pltpu.VMEM((NB, TM, D), f32),
            pltpu.VMEM((NB, TM, D), bf16),
            pltpu.VMEM((2, TM0, F), f32),
            pltpu.VMEM((TM0, F), bf16),
            pltpu.VMEM((TM0, D), bf16),
            pltpu.VMEM((NB, TM, D), bf16),
            pltpu.VMEM((32, 8 * VM, L), f32),
            pltpu.VMEM((KS, D), bf16),
            pltpu.VMEM((D,), bf16),
            pltpu.VMEM((1, D), bf16),
            pltpu.SemaphoreType.DMA((len(DMA_ORDER),)),
            pltpu.SemaphoreType.DMA((NB + 1,)),
        ],
        compiler_params=pltpu.CompilerParams(
            vmem_limit_bytes=120 * 1024 * 1024,
            disable_bounds_checks=True, disable_semaphore_checks=True),
        name="adaln_h3_glu",
    )(A_q, tiles(A_k), tiles(A_v), A_shift_k.T, A_ssm_k, A_ssm_D,
      B_w_gate, B_w_up, B_w_down, c, w_mod)
```

```python
import jax
import jax.numpy as jnp
from jax import lax
import jax.experimental.pallas as pl
import jax.experimental.pallas.tpu as pltpu

S = 2048
D = 640
F = 1536
KS = 4
L = 128
NT = D // L
R = 4
C = R * L
NC = S // C
EPS = 1e-5
RSQ2 = 0.7071067811865476

WPT = 4 * NT
PAD = 32

TM0 = 512
H0 = 352
TM = 384
NB = (S - TM0) // TM
TF = 256
PR = 24
Q1, Q2 = 8 * PR, 12 * PR
KP = (0, 1, 2, 3, 5)
WM = {"mA": (0, 12), "c0": (20, 21), "mB": (12, 16), "s1": (16, 17), "c1": (21, 22),
      "s2": (17, 18), "c2": (22, 23), "s3": (18, 20), "c3": (23, 25), "mG": (25, 30)}
VM = 5
RATE = 1.05
LEAD = 32

f32 = jnp.float32
bf16 = jnp.bfloat16
u32 = jnp.uint32


def _cos_turns(t):
    x = jnp.abs(t - jnp.floor(t) - 0.5) - 0.25
    x2 = x * x
    return x * (6.283164024 + x2 * (-41.33713150 + x2 * (81.34038544 + x2 * -70.98993683)))


def _tables(inverse, hold=None):
    shape = (L // 2, L) if inverse else (2 * L, L)
    rho = lax.broadcasted_iota(jnp.int32, shape, 1 if inverse else 0)
    j = lax.broadcasted_iota(jnp.int32, shape, 0 if inverse else 1)
    if inverse:
        g, rad = 8 * (rho >> 4) + (rho & 7), 2 * R
    else:
        g, rad, j = 8 * (rho >> 5) + (rho & 7) + 64 * ((rho >> 4) & 1), R, _perm(j)
    a = (4 * g + 1).astype(f32) * (1.0 / (4 * C))
    off = ((rho >> 3) & 1).astype(f32) * 0.25
    ns = [(rad * j + r).astype(f32) for r in range(rad)]
    if hold is not None:
        ns = [hold(r, n) for r, n in enumerate(ns)]
    ts = [_cos_turns(a * n + off) for n in ns]
    return [(t * (1.0 / C) if inverse else t).astype(bf16) for t in ts]


def _perm(c):
    return 16 * (c >> 4) + 2 * (c & 7) + ((c >> 3) & 1)


def _layernorm(x):
    m = jnp.mean(x, axis=-1, keepdims=True)
    xc = x - m
    v = jnp.mean(xc * xc, axis=-1, keepdims=True)
    return xc * lax.rsqrt(v + EPS)


def _split(t):
    t = t.reshape(16, 16, L)
    return t[:, :8, :], t[:, 8:, :]


def _radix4(x, sgn):
    (ar, ai), (br, bi), (cr, ci), (dr, di) = x
    s0r, s0i, d0r, d0i = ar + cr, ai + ci, ar - cr, ai - ci
    s1r, s1i, d1r, d1i = br + dr, bi + di, br - dr, bi - di
    o0 = (s0r + s1r, s0i + s1i)
    o2 = (s0r - s1r, s0i - s1i)
    pl_ = (d0r - d1i, d0i + d1r)
    mi_ = (d0r + d1i, d0i - d1r)
    return [o0, pl_, o2, mi_] if sgn > 0 else [o0, mi_, o2, pl_]


T = range(NT)
_z = lambda j: [("z", j, a) for a in range(NC)]
_k = lambda j, al: [("k", j, a) for a in al]
_u = lambda a: [("u", j, a) for j in T]
_iv = lambda jl, al: [("i", j, a) for j in jl for a in al]
_kv = lambda a: [("kv", j, a) for j in T]
_m = lambda jl, us, outs: [("mac", j, us, outs) for j in jl]
A3 = (0, 1, 2)

SCHEDULE = [
    (["ssm0"], _z(0) + _k(0, range(NC)), [("setup", None)]),
    (["ssm1"], _z(1) + _k(1, range(NC)), []),
    (["ssm2"], _z(2) + _k(2, [0, 1]), []),
    (["k0", "v0"], _k(2, [2, 3]) + _u(0), _kv(0) + _m([0], (0,), (0,))),
    (["ssm3"], _iv([0], [0]) + _z(3) + _k(3, [0, 1]), _m([1, 2], (0,), A3)),
    (["k1", "v1"], _k(3, [2, 3]) + _u(1), _kv(1) + _m([3], (0,), (0,))),
    (["ssm4"], _iv([1], [0]) + _z(4) + _k(4, range(NC)),
     _m([0], (0, 1), (1, 2)) + _m([1, 2], (1,), (1, 2))),
    (["k2", "v2"], _iv([2, 3], [0]) + _iv([0], [1]) + _u(2) + _iv([1, 2], [1]) + _iv([4], [0, 1])
     + _iv([0, 1, 2, 4], [2]),
     _kv(2) + _m([4], (0, 1), A3) + _m([0, 1, 2, 4], (2,), (2,)) + _m([3], A3, (1, 2))),
    (["q0", "mA", "c0"], [("mod", "mA", "c0")] + _iv([3], [1]), []),
]
PREP_GROUPS = _iv([3], [2])

PART = [_m([0, 1], A3, (3,)), _m([2, 3], A3, (3,))]
_d = [("d", n, f) for n in T for f in range(3)]
TAIL = [
    (["wd", "mG", "q1b"], (Q1, Q2), _d[:5], [("vmod", "mG")] + _m([4], A3, (3,))),
    (["k3", "v3", "q1c"], (Q2, TM), _d[5:9] + _u(3) + _d[9:] + _iv(T, [3]),
     _kv(3) + _m(T, (3,), (3,))),
]

DMA_ORDER = (["sk", "sd", "c", "ssm0", "ssm1", "ssm2", "k0", "v0", "ssm3", "k1", "v1", "ssm4",
              "k2", "v2", "q0", "c0", "mA", "mB", "wg0", "qh", "wu0", "s1", "c1", "wg1", "wu1",
              "s2", "c2", "wg2", "wu2", "s3", "c3", "wg3", "wu3", "q1", "wd", "mG", "q1b",
              "k3", "v3", "q1c"]
             + [f"q{i + 1}" for i in range(1, NB)])


def _costs(job):
    if job[0] == "kv":
        return [48, 42] * (C // 64)
    if job[0] == "setup":
        return [100] * (4 * R)
    if job[0] == "vmod":
        return [3 * D // VM // 8] * (VM * (WM[job[1]][1] - WM[job[1]][0]))
    us, outs = job[2], job[3]
    pairs = [(a, n) for a in outs for n in us if n <= a]
    mac = (2 * len({a - n for a, n in pairs if a > n}) + 8 * len(pairs)
           - (2 * len(outs) if us[0] == 0 else 0))
    fin = sum(a <= us[-1] for a in outs)
    if mac < 12 and outs[-1] <= us[-1] < NC - 1:
        return [1 + R * mac + 16 * fin, 1 + R * mac + 48 * fin] * 8
    return ([1 + mac] * 3 + [1 + mac + 16 * fin] + [1 + mac] * 3 + [1 + mac + 48 * fin]) * 8


def _plan(groups, jobs, lead=0, floor=(1.0, 0.8)):
    free = {"i": 56, "z": 56, "k": 47, "u": 46, "d": 48}
    steps = {"i": 8, "z": 8, "k": 16, "u": 16, "mod": 0, "d": TM0 // 16}
    slots = [free[g[0]] for g in groups for _ in range(steps[g[0]])]
    lo, hi = [], []
    for job in jobs:
        begin, limit, first = 0, len(slots), 0
        for g in groups:
            kind = (g[0], job[0])
            if (kind == ("u", "kv") and g[1:] == job[1:]
                    or kind == ("i", "mac") and g[1] == job[1] and g[2] in job[3]
                    and g[2] <= job[2][-1] or kind == ("d", "vmod") and g[2] == 2):
                limit = min(limit, first - lead)
            first += steps[g[0]]
            if kind == ("u", "mac") and g[1] == job[1] and g[2] in job[2]:
                begin = first
        lo.append(begin)
        hi.append(limit)
    plan, credit, n = [], slots[0], 0
    for k, job in enumerate(jobs):
        if n < lo[k]:
            n, credit = lo[k], min(credit, 0) + slots[lo[k]]
        work = [sum(_costs(j)) for j in jobs]
        if lead:
            rate = max(RATE * sum(work[k:m + 1]) / max(sum(slots[n:hi[m]]), 1)
                       for m in range(k, len(jobs)))
        else:
            rate = RATE * sum(work[k:]) / sum(slots[n:])
        rate = max(rate, floor[0] if job[0] == "kv" else floor[1])
        idx = []
        for c in _costs(job):
            while credit <= 0 and n + 1 < hi[k]:
                n += 1
                credit += slots[n] * rate
            credit -= c
            idx.append(n)
        plan.append(idx)
    return plan


def _kernel(q_hbm, k_hbm, v_hbm, sk_hbm, ssm_hbm, sd_hbm, wg_hbm, wu_hbm, wd_hbm,
            c_hbm, wm_hbm, o_hbm,
            qb0, qb, kbs, vbs, ssmb, wgb, wub, wdb, wmb, uwb, ub, kpb, yp, pb, yb,
            x1b0, x1b, h2b, gub, hb, ob0, ob, mv, skb, sdb, cb_, sem, osem):
    cps = {"sk": (sk_hbm, skb), "sd": (sd_hbm, sdb), "c": (c_hbm, cb_), "wd": (wd_hbm, wdb)}
    for j in range(NT):
        cps[f"ssm{j}"] = (ssm_hbm.at[pl.ds(j * L, L), :], ssmb.at[j])
    for a in range(NC):
        n, h = C * NT, 2 * PAD
        if a == 0:
            cps["k0"] = (k_hbm.at[pl.ds(0, n), :], kbs[0].at[pl.ds(h, n), :])
        else:
            e = 48
            cps[f"k{a}"] = (k_hbm.at[pl.ds(a * n - e, n + e), :],
                            kbs[a].at[pl.ds(h - e, n + e), :])
        cps[f"v{a}"] = (v_hbm.at[pl.ds(a * n, n), :], vbs[a].at[pl.ds(0, n), :])
    for n, (c0, c1) in WM.items():
        cols = pl.ds(c0 * L, (c1 - c0) * L)
        cps[n] = (wm_hbm.at[:, cols], wmb.at[:, cols])
    cps["q0"] = (q_hbm.at[0, pl.ds(0, H0), :], qb0.at[pl.ds(0, H0), :])
    cps["qh"] = (q_hbm.at[0, pl.ds(H0, TM0 - H0), :], qb0.at[pl.ds(H0, TM0 - H0), :])
    cps["q1"] = (q_hbm.at[0, pl.ds(TM0, Q1), :], qb.at[0, pl.ds(0, Q1), :])
    cps["q1b"] = (q_hbm.at[0, pl.ds(TM0 + Q1, Q2 - Q1), :], qb.at[0, pl.ds(Q1, Q2 - Q1), :])
    cps["q1c"] = (q_hbm.at[0, pl.ds(TM0 + Q2, TM - Q2), :], qb.at[0, pl.ds(Q2, TM - Q2), :])
    for i in range(1, NB):
        cps[f"q{i + 1}"] = (q_hbm.at[0, pl.ds(TM0 + i * TM, TM), :], qb.at[i])
    for p in range(len(KP) - 1):
        rows = pl.ds(KP[p] * L, (KP[p + 1] - KP[p]) * L)
        cps[f"wg{p}"] = (wg_hbm.at[rows, :], wgb.at[rows, :])
        cps[f"wu{p}"] = (wu_hbm.at[rows, :], wub.at[rows, :])
    assert sorted(cps) == sorted(DMA_ORDER)

    def cp(name):
        src, dst = cps[name]
        return pltpu.make_async_copy(src, dst, sem.at[DMA_ORDER.index(name)])

    def wait(*names):
        for n in names:
            cp(n).wait()

    kbs[0][0:2 * PAD, :] = jnp.zeros((2 * PAD, L), bf16)
    for n in DMA_ORDER:
        cp(n).start()

    tabs, ginv, ccol = _tables(False), [], []
    for ref in (ub, kpb, yp):
        ref[0, 0, 0, 0, pl.ds(0, 8, stride=2), :] = jnp.zeros((8, L), f32)
    mv[0, pl.ds(0, 8, stride=2), :] = jnp.zeros((8, L), f32)
    ri = lax.broadcasted_iota(jnp.int32, (L, L), 0)
    ci = lax.broadcasted_iota(jnp.int32, (L, L), 1)
    sel = jnp.where(ci == R * _perm(ri & 31) + (ri >> 5), 1.0, 0.0).astype(bf16)

    wait("sk", "sd", "c")
    skt = skb[...].astype(f32)
    sdv = sdb[...].astype(f32).reshape(1, D)
    cv = cb_[...].astype(f32)
    sig = jax.nn.sigmoid(cv)
    cs = jnp.broadcast_to((cv * sig).astype(bf16), (16, D))
    one = sig[:, 0:L]

    def gate(x, deps):
        dep = jnp.concatenate(deps, axis=0).reshape(x.shape)
        return jnp.where(jnp.broadcast_to(one, x.shape) > 2.0, dep, x)

    def put(dst, j, a, xs):
        for qi in range(R):
            dst[j, a, qi] = jnp.concatenate(xs[qi], axis=1)

    zs = {}
    mod = {}

    def grp_z(j, a):
        z = [lax.dot_general(sel, ssmb[j, :, t * L:(t + 1) * L], (((1,), (1,)), ((), ())),
                             preferred_element_type=f32) for t in range(R * a, R * a + R)]
        zs[j, a] = [jnp.concatenate([z[p][32 * r:32 * (r + 1)] for p in range(R)],
                                    axis=0).astype(bf16) for r in range(R)]
        return [z[0][16 * t:16 * t + 8] for t in range(8)]

    def grp_fwd(ws, dst, j, a, dvec=None):
        t = [jnp.dot(tabs[r], ws[r], preferred_element_type=f32) for r in range(R)]
        x = [_split(v) for v in t]
        if dvec is not None:
            x[0] = (x[0][0] + dvec[None], x[0][1])
        put(dst, j, a, _radix4(x, -1))
        return [t[0][16 * s:16 * s + 8] for s in range(16)]

    def grp_k(j, a):
        return grp_fwd(zs.pop((j, a)), kpb, j, a,
                       sdv[:, j * L:(j + 1) * L] if a == 0 else None)

    def grp_u(j, a):
        uw = [uwb[j, a, r] for r in range(R)]
        return grp_fwd(uw, ub, j, a)

    def grp_i(j, a):
        ys = []
        for r in range(2 * R):
            y = jnp.dot(ginv[r], pb[j, a, r], preferred_element_type=f32)
            yb[j, pl.ds(a * C + r, L // 2, stride=2 * R), :] = y
            ys.append(y)
        return [ys[r][16 * s:16 * s + 8] for r in (0, R) for s in range(4)]

    def grp_mod(*names):
        for name in names:
            c0, c1 = WM[name]
            m = jnp.dot(cs, wmb[:, c0 * L:c1 * L], preferred_element_type=f32)
            for c in range(c0, c1):
                mod[c] = m[0:1, (c - c0) * L:(c - c0 + 1) * L]
        return []

    def modv(i, t0=0, t1=NT):
        return jnp.concatenate([mod[i * NT + n] for n in range(t0, t1)], axis=1)

    def job_kv(j, a, deps):
        lo = lambda x: lax.bitcast_convert_type(x << 16, f32)
        hi = lambda x: lax.bitcast_convert_type(x & jnp.uint32(0xFFFF0000), f32)
        n = C // 8
        kw, vw = kbs[a].bitcast(u32), vbs[a].bitcast(u32)
        ld = lambda ref, o: ref[pl.ds(4 * j + o, n, stride=WPT), :]
        k = {}
        for m in range(4):
            x = ld(kw, PAD + m)
            k[2 * m], k[2 * m + 1] = lo(x), hi(x)
        k[-3] = hi(ld(kw, PAD - WPT + 2))
        x = ld(kw, PAD - WPT + 3)
        k[-2], k[-1] = lo(x), hi(x)
        w = [skt[t:t + 1, j * L:(j + 1) * L] for t in range(KS)]
        w0 = [gate(jnp.broadcast_to(w[0], (n, L)), deps[e::2]) for e in (0, 1)]
        kv = {}
        for m in range(4):
            x = ld(vw, m)
            for ph, v in ((2 * m, lo(x)), (2 * m + 1, hi(x))):
                ks = k[ph] * w0[m % 2]
                for t in range(1, KS):
                    ks = ks + k[ph - t] * w[t]
                kv[ph] = (ks * v).reshape(n // 8, 8, L)
        for r in range(R):
            uwb[j, a, r] = jnp.concatenate([kv[r], kv[r + R]], axis=1).reshape(L, L).astype(bf16)

    def job_mac(j, us, outs, deps):
        ld = lambda ref, a: (ref[j, a, :, :, 0:8, :], ref[j, a, :, :, 8:16, :])
        lo, hi = us[0], us[-1]
        u = {a: ld(ub, a) for a in us}
        if len(deps) == 16:
            ur = jnp.concatenate([gate(u[lo][0][0:1], deps), u[lo][0][1:]], axis=0)
        else:
            ur = gate(u[lo][0], [deps[R * i + qi] for qi in range(R) for i in range(16)])
        u[lo] = (ur, u[lo][1])
        ms = sorted({a - n for a in outs for n in us if n <= a})
        k = {m: ld(kpb, m) for m in sorted(set(ms) | {m - 1 for m in ms if m > 0})}
        kp = {m: k[m] if m == 0 else (k[m][0] - k[m - 1][1], k[m][1] + k[m - 1][0]) for m in ms}
        for a in outs:
            yr, yi = ld(yp, a) if lo > 0 else (None, None)
            for n in us:
                if n > a:
                    continue
                (kr, ki), (ur, ui) = kp[a - n], u[n]
                tr = kr * ur - ki * ui
                ti = kr * ui + ki * ur
                yr = tr if yr is None else yr + tr
                yi = ti if yi is None else yi + ti
            if a > hi:
                yp[j, a] = jnp.concatenate([yr, yi], axis=2)
                continue
            ps = _radix4([(yr[qi], yi[qi]) for qi in range(R)], +1)
            for r in range(R):
                pr, pi = [p.reshape(8, 2, 8, L) for p in ps[r]]
                lr, li, hr, hi_ = pr[:, 0], pi[:, 0], pr[:, 1], pi[:, 1]
                if r % 2:
                    hr, hi_ = (hr - hi_) * RSQ2, (hr + hi_) * RSQ2
                if r < 2:
                    outs2 = (lr + hr, li + hi_), (lr - hr, li - hi_)
                else:
                    outs2 = (lr - hi_, li + hr), (lr + hi_, li - hr)
                for e in range(2):
                    pb[j, a, r + R * e] = jnp.concatenate(
                        outs2[e], axis=1).reshape(L, L).astype(bf16)

    def job_setup(_, deps):
        def hold(r, n):
            return gate(n, [deps[2 * r + s // 4] for s in range(8)])

        ginv.extend(_tables(True, hold))
        csf = cs[0:1].astype(f32)
        ccol.append(jnp.concatenate([jnp.broadcast_to(csf[:, t * L:(t + 1) * L], (L, L)).T
                                     for t in range(NT)], axis=0))

    def job_vmod(name, deps):
        c0, c1 = WM[name]
        n = D // VM
        for c in range(c0, c1):
            for i in range(VM):
                cc = ccol[0][i * n:(i + 1) * n]
                cc = jnp.concatenate([gate(cc[0:8], [deps[(c - c0) * VM + i]]), cc[8:]], axis=0)
                p = wmb[i * n:(i + 1) * n, c * L:(c + 1) * L].astype(f32) * cc
                mv[c, 8 * i:8 * i + 8, :] = jnp.sum(p.reshape(n // 8, 8, L), axis=0)
            mod[c] = jnp.sum(mv[c], axis=0, keepdims=True)

    grp_fn = {"z": grp_z, "k": grp_k, "u": grp_u, "i": grp_i, "mod": grp_mod}
    job_fn = {"kv": job_kv, "mac": job_mac, "vmod": job_vmod, "setup": job_setup}

    def run(groups, jobs, **kw):
        plan = _plan(groups, jobs, **kw)
        anchors, done = [], 0
        for g in groups + [None]:
            while done < len(jobs) and max(plan[done]) < len(anchors):
                job_fn[jobs[done][0]](*jobs[done][1:], [anchors[n] for n in plan[done]])
                done += 1
            if g is not None:
                anchors += grp_fn[g[0]](*g[1:])
        assert done == len(jobs)

    for waits, groups, jobs in SCHEDULE:
        wait(*waits)
        run(groups, jobs)

    n1, dep = [], None
    for r in range(0, H0, H0 // 2):
        x = qb0[r:r + H0 // 2, :].astype(f32)
        if dep is not None:
            x = jnp.concatenate([gate(x[:, 0:L], [dep]), x[:, L:]], axis=1)
        n1.append(_layernorm(x))
        dep = n1[-1][:, 0:L]
    n1 = jnp.concatenate(n1, axis=0)
    wait("mB")
    grp_mod("mB")
    for g in PREP_GROUPS:
        grp_fn[g[0]](*g[1:])
    sa, ca, ga = [modv(i) for i in range(3)]
    a1 = ga * (1.0 + ca)
    b1 = ga * sa

    def o_cp(i, c0, c1, r0=0, r1=TM):
        cols = pl.ds(c0, c1 - c0)
        if i is None:
            return pltpu.make_async_copy(ob0.at[:, cols], o_hbm.at[0, pl.ds(0, TM0), cols],
                                         osem.at[NB])
        base = TM0 + i * TM + r0
        if not isinstance(i, int):
            base = pl.multiple_of(base, L)
        return pltpu.make_async_copy(ob.at[i, pl.ds(r0, r1 - r0), cols],
                                     o_hbm.at[0, pl.ds(base, r1 - r0), cols], osem.at[i])

    def prep_norm(q_ref, x1_ref, y0, r0, n, dep=None, n1=None):
        x = q_ref[r0:r0 + n, :].astype(f32)
        if dep is not None:
            x = jnp.concatenate([gate(x[:, 0:L], [dep]), x[:, L:]], axis=1)
        y = jnp.concatenate([yb[j, pl.ds(y0 + r0, n), :] for j in range(NT)], axis=1)
        x1 = x + ((_layernorm(x) if n1 is None else n1) * a1 + b1) * y
        x1_ref[r0:r0 + n, :] = x1
        return _layernorm(x1)

    n2 = [prep_norm(qb0, x1b0, 0, 0, H0, None, n1)]

    aff = []

    def prep_chain(i, r0, r1):
        y0 = TM0 + i * TM
        if not isinstance(i, int):
            y0 = pl.multiple_of(y0, L)
        dep = None
        for r in range(r0, r1, PR):
            h2 = prep_norm(qb.at[i], x1b.at[i], y0, r, PR, dep) * aff[0] + aff[1]
            h2b[i, r:r + PR, :] = h2.astype(bf16)
            dep = h2[:, 0:L]

    def gate_up(h2):
        hs = []
        for f in range(0, F, TF):
            g = jnp.dot(h2, wgb[:, f:f + TF], preferred_element_type=f32)
            u = jnp.dot(h2, wub[:, f:f + TF], preferred_element_type=f32)
            hs.append(g * u)
        return jnp.concatenate(hs, axis=1).astype(bf16)

    OC = (0, D - L, D)

    OP = ((0, D - L, 0, TM), (D - L, D, 0, TM - L), (D - L, D, TM - L, TM))

    def down(hh, gb, i):
        for c0, c1, r0, r1 in OP:
            o = jnp.dot(hh[r0:r1], wdb[:, c0:c1], preferred_element_type=f32)
            ob[i, r0:r1, c0:c1] = (x1b[i, r0:r1, c0:c1] + gb[:, c0:c1] * o).astype(bf16)
            o_cp(i, c0, c1, r0, r1).start()

    def spread(jobs, anchors):
        total, n = sum(len(_costs(j)) for j in jobs), 0
        for job in jobs:
            m = len(_costs(job))
            job_fn[job[0]](*job[1:], [anchors[(n + i) * len(anchors) // total] for i in range(m)])
            n += m

    acc, hcache = {}, {}

    def unit(p, n, f, half=None):
        t0, t1 = KP[p], KP[p + 1]
        if (p, half) not in hcache:
            x = jnp.concatenate(n2, axis=0) if half is None else n2[half]
            hcache[p, half] = (x[:, t0 * L:t1 * L] * (1.0 + modv(4, t0, t1))
                               + modv(3, t0, t1)).astype(bf16)
        rows = {None: slice(0, TM0), 0: slice(0, H0), 1: slice(H0, TM0)}[half]
        d = jnp.dot(hcache[p, half], (wgb if n == "g" else wub)[t0 * L:t1 * L, f:f + 4 * L],
                    preferred_element_type=f32)
        ref = gub.at["gu".index(n), rows, f:f + 4 * L]
        if p == len(KP) - 2:
            acc[n, f] = ref[...] + d
        else:
            ref[...] = d if p == 0 else ref[...] + d
        return [d[s:s + 8, 0:L] for s in range(0, d.shape[0], 16)]

    def units(us):
        return [x for u in us for x in unit(*u)]

    FS = range(0, F, 4 * L)
    full = lambda p: [(p, n, f) for f in FS for n in "gu"]

    wait("wg0", "qh")
    units([(0, "g", f, 0) for f in FS])
    n2.append(prep_norm(qb0, x1b0, 0, H0, TM0 - H0))
    units([(0, "g", f, 1) for f in FS])
    wait("wu0", "s1", "c1")
    spread([("vmod", "s1"), ("vmod", "c1")], units([(0, "u", f) for f in FS])[:80])
    wait("wg1", "wu1", "s2", "c2")
    spread([("vmod", "s2"), ("vmod", "c2")] + PART[0], units(full(1)))
    wait("wg2", "wu2", "s3", "c3")
    spread([("vmod", "s3"), ("vmod", "c3")] + PART[1], units(full(2)))
    wait("wg3", "wu3", "q1")
    units(full(3))
    aff += [1.0 + modv(4), modv(3)]
    prep_chain(0, 0, Q1)
    for f in FS:
        hb[:, f:f + 4 * L] = (acc.pop(("g", f)) * acc.pop(("u", f))).astype(bf16)

    parts = {}

    def grp_d(n, f):
        c = slice(n * L, (n + 1) * L)
        k = slice(f * 4 * L, (f + 1) * 4 * L)
        d = jnp.dot(hb[:, k], wdb[k, c], preferred_element_type=f32)
        parts[n] = d if f == 0 else parts[n] + d
        if f == 2:
            ob0[:, c] = (x1b0[:, c] + mod[5 * NT + n] * parts.pop(n)).astype(bf16)
            if (n + 1) * L in OC:
                o_cp(None, OC[OC.index((n + 1) * L) - 1], (n + 1) * L).start()
        return [d[s:s + 8] for s in range(0, TM0, 16)]

    grp_fn["d"] = grp_d
    for waits, rows, groups, jobs in TAIL:
        wait(*waits)
        for n in list(parts):
            parts[n] = gub[0, :, 0:L]
        prep_chain(0, *rows)
        run(groups, jobs, lead=LEAD, floor=(0.0, 0.0))
        for n in parts:
            gub[0, :, 0:L] = parts[n]
    gb = modv(5)
    wait(*[f"q{i + 1}" for i in range(1, NB)])

    def ffn(i, carry):
        h2 = h2b[i]
        prep_chain(jnp.minimum(i + 1, NB - 1), 0, TM)
        down(gate_up(h2), gb, i)
        return carry

    lax.fori_loop(0, NB, ffn, 0)

    for c0, c1 in zip(OC[:-1], OC[1:]):
        o_cp(None, c0, c1).wait()
    for i in range(NB):
        for op in OP:
            o_cp(i, *op).wait()


@jax.jit
def pallas_adaLN_cond__ssm_conv_h3__glu_gated_bilinear__prompt_kernel(
    A_q: jax.Array,
    A_k: jax.Array,
    A_v: jax.Array,
    A_shift_k: jax.Array,
    A_ssm_k: jax.Array,
    A_ssm_D: jax.Array,
    B_x: jax.Array,
    B_w_gate: jax.Array,
    B_w_up: jax.Array,
    B_w_down: jax.Array,
    c: jax.Array,
    w_mod: jax.Array,
):
    del B_x
    tiles = lambda x: x.reshape(S // 8, 8, NT, L).transpose(0, 2, 1, 3).reshape(S * NT, L)
    any_spec = pl.BlockSpec(memory_space=pl.ANY)
    return pl.pallas_call(
        _kernel,
        in_specs=[any_spec] * 11,
        out_specs=any_spec,
        out_shape=jax.ShapeDtypeStruct((1, S, D), bf16),
        scratch_shapes=[
            pltpu.VMEM((TM0, D), bf16),
            pltpu.VMEM((NB, TM, D), bf16),
            [pltpu.VMEM((4 * PAD + C * NT, L), bf16)] * NC,
            [pltpu.VMEM((2 * PAD + C * NT, L), bf16)] * NC,
            pltpu.VMEM((NT, L, S), bf16),
            pltpu.VMEM((D, F), bf16),
            pltpu.VMEM((D, F), bf16),
            pltpu.VMEM((F, D), bf16),
            pltpu.VMEM((D, 6 * D), bf16),
            pltpu.VMEM((NT, NC, R, L, L), bf16),
            pltpu.VMEM((NT, NC, R, 16, 16, L), f32),
            pltpu.VMEM((NT, NC, R, 16, 16, L), f32),
            pltpu.VMEM((NT, NC, R, 16, 16, L), f32),
            pltpu.VMEM((NT, NC, 2 * R, L, L), bf16),
            pltpu.VMEM((NT, S + 32, L), f32),
            pltpu.VMEM((TM0, D), f32),
            pltpu.VMEM((NB, TM, D), f32),
            pltpu.VMEM((NB, TM, D), bf16),
            pltpu.VMEM((2, TM0, F), f32),
            pltpu.VMEM((TM0, F), bf16),
            pltpu.VMEM((TM0, D), bf16),
            pltpu.VMEM((NB, TM, D), bf16),
            pltpu.VMEM((32, 8 * VM, L), f32),
            pltpu.VMEM((KS, D), bf16),
            pltpu.VMEM((D,), bf16),
            pltpu.VMEM((1, D), bf16),
            pltpu.SemaphoreType.DMA((len(DMA_ORDER),)),
            pltpu.SemaphoreType.DMA((NB + 1,)),
        ],
        compiler_params=pltpu.CompilerParams(
            vmem_limit_bytes=120 * 1024 * 1024,
            disable_bounds_checks=True, disable_semaphore_checks=True),
        name="adaln_h3_glu",
    )(A_q, tiles(A_k), tiles(A_v), A_shift_k.T, A_ssm_k, A_ssm_D,
      B_w_gate, B_w_up, B_w_down, c, w_mod)
```

```python
import jax
import jax.numpy as jnp
from jax import lax
import jax.experimental.pallas as pl
import jax.experimental.pallas.tpu as pltpu

S = 2048
D = 640
F = 1536
KS = 4
L = 128
NT = D // L
R = 4
C = R * L
NC = S // C
EPS = 1e-5
RSQ2 = 0.7071067811865476

WPT = 4 * NT
PAD = 32

TM0 = 512
H0 = 352
TM = 384
NB = (S - TM0) // TM
HM = TM // 2
PL = 16
TF = 256
PR = 24
KP = (0, 1, 2, 3, 4, 5)
WM = {"mA": (0, 12), "c0": (20, 21), "mB": (12, 16), "s1": (16, 17), "c1": (21, 22),
      "s2": (17, 19), "c2": (22, 24), "s4": (19, 20), "c4": (24, 25), "mG": (25, 30)}
VM = 5
RATE = 1.05
LEAD = 32

f32 = jnp.float32
bf16 = jnp.bfloat16
u32 = jnp.uint32


def _cos_turns(t):
    x = jnp.abs(t - jnp.floor(t) - 0.5) - 0.25
    x2 = x * x
    return x * (6.283164024 + x2 * (-41.33713150 + x2 * (81.34038544 + x2 * -70.98993683)))


def _tables(inverse, hold=None):
    shape = (L // 2, L) if inverse else (2 * L, L)
    rho = lax.broadcasted_iota(jnp.int32, shape, 1 if inverse else 0)
    j = lax.broadcasted_iota(jnp.int32, shape, 0 if inverse else 1)
    if inverse:
        g, rad = 8 * (rho >> 4) + (rho & 7), 2 * R
    else:
        g, rad, j = 8 * (rho >> 5) + (rho & 7) + 64 * ((rho >> 4) & 1), R, _perm(j)
    a = (4 * g + 1).astype(f32) * (1.0 / (4 * C))
    off = ((rho >> 3) & 1).astype(f32) * 0.25
    ns = [(rad * j + r).astype(f32) for r in range(rad)]
    if hold is not None:
        ns = [hold(r, n) for r, n in enumerate(ns)]
    ts = [_cos_turns(a * n + off) for n in ns]
    return [(t * (1.0 / C) if inverse else t).astype(bf16) for t in ts]


def _perm(c):
    return 16 * (c >> 4) + 2 * (c & 7) + ((c >> 3) & 1)


def _layernorm(x):
    m = jnp.mean(x, axis=-1, keepdims=True)
    xc = x - m
    v = jnp.mean(xc * xc, axis=-1, keepdims=True)
    return xc * lax.rsqrt(v + EPS)


def _split(t):
    t = t.reshape(16, 16, L)
    return t[:, :8, :], t[:, 8:, :]


def _radix4(x, sgn):
    (ar, ai), (br, bi), (cr, ci), (dr, di) = x
    s0r, s0i, d0r, d0i = ar + cr, ai + ci, ar - cr, ai - ci
    s1r, s1i, d1r, d1i = br + dr, bi + di, br - dr, bi - di
    o0 = (s0r + s1r, s0i + s1i)
    o2 = (s0r - s1r, s0i - s1i)
    pl_ = (d0r - d1i, d0i + d1r)
    mi_ = (d0r + d1i, d0i - d1r)
    return [o0, pl_, o2, mi_] if sgn > 0 else [o0, mi_, o2, pl_]


T = range(NT)
_z = lambda j: [("z", j, a) for a in range(NC)]
_k = lambda j, al: [("k", j, a) for a in al]
_u = lambda a: [("u", j, a) for j in T]
_iv = lambda jl, al: [("i", j, a) for j in jl for a in al]
_kv = lambda a: [("kv", j, a) for j in T]
_m = lambda jl, us, outs: [("mac", j, us, outs) for j in jl]
A3 = (0, 1, 2)

A2 = (0, 1)
SCHEDULE = [
    (["ssm0"], _z(0) + _k(0, range(NC)), [("setup", None)]),
    (["ssm1"], _z(1) + _k(1, range(NC)), []),
    (["ssm2"], _z(2) + _k(2, [0, 1]), []),
    (["k0", "v0"], _k(2, [2, 3]) + _u(0), _kv(0) + _m([0], (0,), (0,))),
    (["ssm3"], _iv([0], [0]) + _z(3) + _k(3, [0, 1]), _m([1, 2], (0,), (0,))),
    (["k1", "v1"], _k(3, [2, 3]) + _u(1), _kv(1) + _m([3], (0,), (0,))),
    (["ssm4"], _iv([1, 2, 3], [0]) + _z(4) + _k(4, range(NC)), _m([0, 1, 2, 3], A2, (1,))),
    (["q0"], _iv([0, 1, 2, 3], [1]) + _iv([4], A2), _m([4], A2, A2)),
    (["mA", "c0"], [("mod", "mA", "c0")], []),
]
PREP_GROUPS = []

_g = lambda p: [("g", p, n, f) for f in range(3) for n in "gu"]
_d = [("d", n, f) for n in T for f in range(3)]
_v = lambda *names: [("vmod", n) for n in names]
_e = [("d", n, f) for n in T for f in (0, 1)]
FIRST = [
    (["wg0", "qh"], None, [("g", 0, "g", f, h) for h in (0, 1) for f in range(3)], []),
    (["wu0", "s1", "c1"], None, [("g", 0, "u", f) for f in range(3)],
     _v("s1", "c1") + _m([0], A2, (2, 3))),
    (["wg1", "wu1"], None, _g(1)[:-1], _m([1, 2], A2, (2, 3))),
    (["wg2", "wu2", "s2", "c2"], None, _g(1)[-1:] + _g(2),
     _v("s2", "c2") + _m([3, 4], A2, (2, 3))),
    (["wg3", "wu3", "wg4", "wu4", "s4", "c4", "q1"], (0, HM), _g(3) + _g(4), _v("s4", "c4")),
    (["wd", "k2", "v2"], None, _e[:2] + _u(2) + _e[2:6],
     _kv(2) + _m([0, 1, 2, 3], (2,), (2, 3))),
    (["mG", "k3", "v3"], None,
     _e[6:] + _u(3) + _iv(T, [2]) + [("d", n, 2) for n in T] + _iv(T, [3]),
     _kv(3) + _m([4], (2,), (2, 3)) + _v("mG") + _m(T, (3,), (3,))),
]

DMA_ORDER = (["sk", "sd", "c", "ssm0", "ssm1", "ssm2", "k0", "v0", "ssm3", "k1", "v1", "ssm4",
              "q0", "c0", "mA", "mB", "wg0", "qh", "wu0", "s1", "c1", "wg1", "wu1", "s2", "c2",
              "wg2", "wu2", "s4", "c4", "wg3", "wu3", "wg4", "wu4", "q1", "wd", "k2", "v2", "mG", "k3", "v3",
              "q1c"] + [f"q{i + 1}" for i in range(1, NB)])


def _costs(job):
    if job[0] == "kv":
        return [48, 42] * (C // 64)
    if job[0] == "setup":
        return [100] * (4 * R)
    if job[0] == "vmod":
        return [3 * D // VM // 8] * (VM * (WM[job[1]][1] - WM[job[1]][0]))
    us, outs = job[2], job[3]
    pairs = [(a, n) for a in outs for n in us if n <= a]
    mac = (2 * len({a - n for a, n in pairs if a > n}) + 8 * len(pairs)
           - (2 * len(outs) if us[0] == 0 else 0))
    fin = sum(a <= us[-1] for a in outs)
    if mac < 12 and outs[-1] <= us[-1] < NC - 1:
        return [1 + R * mac + 16 * fin, 1 + R * mac + 48 * fin] * 8
    return ([1 + mac] * 3 + [1 + mac + 16 * fin] + [1 + mac] * 3 + [1 + mac + 48 * fin]) * 8


def _plan(groups, jobs, lead=0, floor=(1.0, 0.8)):
    free = {"i": 56, "z": 56, "k": 47, "u": 46, "d": 48, "g": 50}
    nstep = {"i": 8, "z": 8, "k": 16, "u": 16, "mod": 0, "d": TM0 // 16}
    steps = lambda g: (KP[g[1] + 1] - KP[g[1]]) * TM0 // 16 if g[0] == "g" else nstep[g[0]]
    slots = [free[g[0]] for g in groups for _ in range(steps(g))]
    lo, hi = [], []
    for job in jobs:
        begin, limit, first = 0, len(slots), 0
        for g in groups:
            kind = (g[0], job[0])
            if (kind == ("u", "kv") and g[1:] == job[1:]
                    or kind == ("i", "mac") and g[1] == job[1] and g[2] in job[3]
                    and g[2] <= job[2][-1] or kind == ("d", "vmod") and g[2] == 2):
                limit = min(limit, first - lead)
            if kind == ("g", "vmod") and job[1][1] == str(g[1]):
                limit = min(limit, first - 11)
            first += steps(g)
            if kind == ("u", "mac") and g[1] == job[1] and g[2] in job[2]:
                begin = first
        lo.append(begin)
        hi.append(limit)
    plan, credit, n = [], (slots or [0])[0], 0
    for k, job in enumerate(jobs):
        if n < lo[k]:
            n, credit = lo[k], min(credit, 0) + slots[lo[k]]
        work = [sum(_costs(j)) for j in jobs]
        if lead:
            rate = max(RATE * sum(work[k:m + 1]) / max(sum(slots[n:hi[m]]), 1)
                       for m in range(k, len(jobs)))
        else:
            rate = RATE * sum(work[k:]) / sum(slots[n:])
        rate = max(rate, floor[0] if job[0] == "kv" else floor[1])
        idx = []
        for c in _costs(job):
            while credit <= 0 and n + 1 < hi[k]:
                n += 1
                credit += slots[n] * rate
            credit -= c
            idx.append(n)
        plan.append(idx)
    return plan


def _kernel(q_hbm, k_hbm, v_hbm, sk_hbm, ssm_hbm, sd_hbm, wg_hbm, wu_hbm, wd_hbm,
            c_hbm, wm_hbm, o_hbm,
            qb0, qb, kbs, vbs, ssmb, wgb, wub, wdb, wmb, uwb, ub, kpb, yp, pb, yb,
            x1b0, x1b, h2b, gub, dpart, hb, ob0, ob, mv, skb, sdb, cb_, sem, osem):
    cps = {"sk": (sk_hbm, skb), "sd": (sd_hbm, sdb), "c": (c_hbm, cb_), "wd": (wd_hbm, wdb)}
    for j in range(NT):
        cps[f"ssm{j}"] = (ssm_hbm.at[pl.ds(j * L, L), :], ssmb.at[j])
    for a in range(NC):
        n, h = C * NT, 2 * PAD
        if a == 0:
            cps["k0"] = (k_hbm.at[pl.ds(0, n), :], kbs[0].at[pl.ds(h, n), :])
        else:
            e = 48
            cps[f"k{a}"] = (k_hbm.at[pl.ds(a * n - e, n + e), :],
                            kbs[a].at[pl.ds(h - e, n + e), :])
        cps[f"v{a}"] = (v_hbm.at[pl.ds(a * n, n), :], vbs[a].at[pl.ds(0, n), :])
    for n, (c0, c1) in WM.items():
        cols = pl.ds(c0 * L, (c1 - c0) * L)
        cps[n] = (wm_hbm.at[:, cols], wmb.at[:, cols])
    cps["q0"] = (q_hbm.at[0, pl.ds(0, H0), :], qb0.at[pl.ds(0, H0), :])
    cps["qh"] = (q_hbm.at[0, pl.ds(H0, TM0 - H0), :], qb0.at[pl.ds(H0, TM0 - H0), :])
    cps["q1"] = (q_hbm.at[0, pl.ds(TM0, HM), :], qb.at[0, pl.ds(0, HM), :])
    cps["q1c"] = (q_hbm.at[0, pl.ds(TM0 + HM, HM), :], qb.at[0, pl.ds(HM, HM), :])
    for i in range(1, NB):
        cps[f"q{i + 1}"] = (q_hbm.at[0, pl.ds(TM0 + i * TM, TM), :], qb.at[i])
    for p in range(len(KP) - 1):
        rows = pl.ds(KP[p] * L, (KP[p + 1] - KP[p]) * L)
        cps[f"wg{p}"] = (wg_hbm.at[rows, :], wgb.at[rows, :])
        cps[f"wu{p}"] = (wu_hbm.at[rows, :], wub.at[rows, :])
    assert sorted(cps) == sorted(DMA_ORDER)

    def cp(name):
        src, dst = cps[name]
        return pltpu.make_async_copy(src, dst, sem.at[DMA_ORDER.index(name)])

    def wait(*names):
        for n in names:
            cp(n).wait()

    kbs[0][0:2 * PAD, :] = jnp.zeros((2 * PAD, L), bf16)
    for n in DMA_ORDER:
        cp(n).start()

    tabs, ginv, ccol = _tables(False), [], []
    for ref in (ub, kpb, yp):
        ref[0, 0, 0, 0, pl.ds(0, 8, stride=2), :] = jnp.zeros((8, L), f32)
    mv[0, pl.ds(0, 8, stride=2), :] = jnp.zeros((8, L), f32)
    ri = lax.broadcasted_iota(jnp.int32, (L, L), 0)
    ci = lax.broadcasted_iota(jnp.int32, (L, L), 1)
    sel = jnp.where(ci == R * _perm(ri & 31) + (ri >> 5), 1.0, 0.0).astype(bf16)

    wait("sk", "sd", "c")
    skt = skb[...].astype(f32)
    sdv = sdb[...].astype(f32).reshape(1, D)
    cv = cb_[...].astype(f32)
    sig = jax.nn.sigmoid(cv)
    cs = jnp.broadcast_to((cv * sig).astype(bf16), (16, D))
    one = sig[:, 0:L]

    def gate(x, deps):
        dep = jnp.concatenate(deps, axis=0).reshape(x.shape)
        return jnp.where(jnp.broadcast_to(one, x.shape) > 2.0, dep, x)

    def put(dst, j, a, xs):
        for qi in range(R):
            dst[j, a, qi] = jnp.concatenate(xs[qi], axis=1)

    zs = {}
    mod = {}

    def grp_z(j, a):
        z = [lax.dot_general(sel, ssmb[j, :, t * L:(t + 1) * L], (((1,), (1,)), ((), ())),
                             preferred_element_type=f32) for t in range(R * a, R * a + R)]
        zs[j, a] = [jnp.concatenate([z[p][32 * r:32 * (r + 1)] for p in range(R)],
                                    axis=0).astype(bf16) for r in range(R)]
        return [z[0][16 * t:16 * t + 8] for t in range(8)]

    def grp_fwd(ws, dst, j, a, dvec=None):
        t = [jnp.dot(tabs[r], ws[r], preferred_element_type=f32) for r in range(R)]
        x = [_split(v) for v in t]
        if dvec is not None:
            x[0] = (x[0][0] + dvec[None], x[0][1])
        put(dst, j, a, _radix4(x, -1))
        return [t[0][16 * s:16 * s + 8] for s in range(16)]

    def grp_k(j, a):
        return grp_fwd(zs.pop((j, a)), kpb, j, a,
                       sdv[:, j * L:(j + 1) * L] if a == 0 else None)

    def grp_u(j, a):
        uw = [uwb[j, a, r] for r in range(R)]
        return grp_fwd(uw, ub, j, a)

    def grp_i(j, a):
        ys = []
        for r in range(2 * R):
            y = jnp.dot(ginv[r], pb[j, a, r], preferred_element_type=f32)
            yb[j, pl.ds(a * C + r, L // 2, stride=2 * R), :] = y
            ys.append(y)
        return [ys[r][16 * s:16 * s + 8] for r in (0, R) for s in range(4)]

    def grp_mod(*names):
        for name in names:
            c0, c1 = WM[name]
            m = jnp.dot(cs, wmb[:, c0 * L:c1 * L], preferred_element_type=f32)
            for c in range(c0, c1):
                mod[c] = m[0:1, (c - c0) * L:(c - c0 + 1) * L]
        return []

    def modv(i, t0=0, t1=NT):
        return jnp.concatenate([mod[i * NT + n] for n in range(t0, t1)], axis=1)

    def job_kv(j, a, deps):
        lo = lambda x: lax.bitcast_convert_type(x << 16, f32)
        hi = lambda x: lax.bitcast_convert_type(x & jnp.uint32(0xFFFF0000), f32)
        n = C // 8
        kw, vw = kbs[a].bitcast(u32), vbs[a].bitcast(u32)
        ld = lambda ref, o: ref[pl.ds(4 * j + o, n, stride=WPT), :]
        k = {}
        for m in range(4):
            x = ld(kw, PAD + m)
            k[2 * m], k[2 * m + 1] = lo(x), hi(x)
        k[-3] = hi(ld(kw, PAD - WPT + 2))
        x = ld(kw, PAD - WPT + 3)
        k[-2], k[-1] = lo(x), hi(x)
        w = [skt[t:t + 1, j * L:(j + 1) * L] for t in range(KS)]
        w0 = [gate(jnp.broadcast_to(w[0], (n, L)), deps[e::2]) for e in (0, 1)]
        kv = {}
        for m in range(4):
            x = ld(vw, m)
            for ph, v in ((2 * m, lo(x)), (2 * m + 1, hi(x))):
                ks = k[ph] * w0[m % 2]
                for t in range(1, KS):
                    ks = ks + k[ph - t] * w[t]
                kv[ph] = (ks * v).reshape(n // 8, 8, L)
        for r in range(R):
            uwb[j, a, r] = jnp.concatenate([kv[r], kv[r + R]], axis=1).reshape(L, L).astype(bf16)

    def job_mac(j, us, outs, deps):
        ld = lambda ref, a: (ref[j, a, :, :, 0:8, :], ref[j, a, :, :, 8:16, :])
        lo, hi = us[0], us[-1]
        u = {a: ld(ub, a) for a in us}
        if len(deps) == 16:
            ur = jnp.concatenate([gate(u[lo][0][0:1], deps), u[lo][0][1:]], axis=0)
        else:
            ur = gate(u[lo][0], [deps[R * i + qi] for qi in range(R) for i in range(16)])
        u[lo] = (ur, u[lo][1])
        ms = sorted({a - n for a in outs for n in us if n <= a})
        k = {m: ld(kpb, m) for m in sorted(set(ms) | {m - 1 for m in ms if m > 0})}
        kp = {m: k[m] if m == 0 else (k[m][0] - k[m - 1][1], k[m][1] + k[m - 1][0]) for m in ms}
        for a in outs:
            yr, yi = ld(yp, a) if lo > 0 else (None, None)
            for n in us:
                if n > a:
                    continue
                (kr, ki), (ur, ui) = kp[a - n], u[n]
                tr = kr * ur - ki * ui
                ti = kr * ui + ki * ur
                yr = tr if yr is None else yr + tr
                yi = ti if yi is None else yi + ti
            if a > hi:
                yp[j, a] = jnp.concatenate([yr, yi], axis=2)
                continue
            ps = _radix4([(yr[qi], yi[qi]) for qi in range(R)], +1)
            for r in range(R):
                pr, pi = [p.reshape(8, 2, 8, L) for p in ps[r]]
                lr, li, hr, hi_ = pr[:, 0], pi[:, 0], pr[:, 1], pi[:, 1]
                if r % 2:
                    hr, hi_ = (hr - hi_) * RSQ2, (hr + hi_) * RSQ2
                if r < 2:
                    outs2 = (lr + hr, li + hi_), (lr - hr, li - hi_)
                else:
                    outs2 = (lr - hi_, li + hr), (lr + hi_, li - hr)
                for e in range(2):
                    pb[j, a, r + R * e] = jnp.concatenate(
                        outs2[e], axis=1).reshape(L, L).astype(bf16)

    def job_setup(_, deps):
        def hold(r, n):
            return gate(n, [deps[2 * r + s // 4] for s in range(8)])

        ginv.extend(_tables(True, hold))
        csf = cs[0:1].astype(f32)
        ccol.append(jnp.concatenate([jnp.broadcast_to(csf[:, t * L:(t + 1) * L], (L, L)).T
                                     for t in range(NT)], axis=0))

    def job_vmod(name, deps):
        c0, c1 = WM[name]
        n = D // VM
        for c in range(c0, c1):
            for i in range(VM):
                cc = ccol[0][i * n:(i + 1) * n]
                cc = jnp.concatenate([gate(cc[0:8], [deps[(c - c0) * VM + i]]), cc[8:]], axis=0)
                p = wmb[i * n:(i + 1) * n, c * L:(c + 1) * L].astype(f32) * cc
                mv[c, 8 * i:8 * i + 8, :] = jnp.sum(p.reshape(n // 8, 8, L), axis=0)
            mod[c] = jnp.sum(mv[c], axis=0, keepdims=True)

    grp_fn = {"z": grp_z, "k": grp_k, "u": grp_u, "i": grp_i, "mod": grp_mod}
    job_fn = {"kv": job_kv, "mac": job_mac, "vmod": job_vmod, "setup": job_setup}

    def run(groups, jobs, **kw):
        plan = _plan(groups, jobs, **kw)
        anchors, done = [], 0
        for g in groups + [None]:
            while done < len(jobs) and max(plan[done]) < len(anchors):
                job_fn[jobs[done][0]](*jobs[done][1:], [anchors[n] for n in plan[done]])
                done += 1
            if g is not None:
                anchors += grp_fn[g[0]](*g[1:])
        assert done == len(jobs)

    for waits, groups, jobs in SCHEDULE:
        wait(*waits)
        run(groups, jobs)

    n1, dep = [], None
    for r in range(0, H0, H0 // 2):
        x = qb0[r:r + H0 // 2, :].astype(f32)
        if dep is not None:
            x = jnp.concatenate([gate(x[:, 0:L], [dep]), x[:, L:]], axis=1)
        n1.append(_layernorm(x))
        dep = n1[-1][:, 0:L]
    n1 = jnp.concatenate(n1, axis=0)
    wait("mB")
    grp_mod("mB")
    for g in PREP_GROUPS:
        grp_fn[g[0]](*g[1:])
    sa, ca, ga = [modv(i) for i in range(3)]
    a1 = ga * (1.0 + ca)
    b1 = ga * sa

    def o_cp(i, c0, c1, r0=0, r1=TM):
        cols = pl.ds(c0, c1 - c0)
        if i is None:
            return pltpu.make_async_copy(ob0.at[:, cols], o_hbm.at[0, pl.ds(0, TM0), cols],
                                         osem.at[NB])
        base = TM0 + i * TM + r0
        if not isinstance(i, int):
            base = pl.multiple_of(base, 64)
        return pltpu.make_async_copy(ob.at[i, pl.ds(r0, r1 - r0), cols],
                                     o_hbm.at[0, pl.ds(base, r1 - r0), cols], osem.at[i])

    def prep_norm(q_ref, x1_ref, y0, r0, n, dep=None, n1=None):
        x = q_ref[r0:r0 + n, :].astype(f32)
        if dep is not None:
            x = jnp.concatenate([gate(x[:, 0:L], [dep]), x[:, L:]], axis=1)
        y = jnp.concatenate([yb[j, pl.ds(y0 + r0, n), :] for j in range(NT)], axis=1)
        x1 = x + ((_layernorm(x) if n1 is None else n1) * a1 + b1) * y
        x1_ref[r0:r0 + n, :] = x1
        return _layernorm(x1)

    n2 = [prep_norm(qb0, x1b0, 0, 0, H0, None, n1)]
    aff = []

    def prep_chain(i, r0, r1, pr):
        y0 = TM0 + i * TM
        if not isinstance(i, int):
            y0 = pl.multiple_of(y0, L)
        dep = None
        for r in range(r0, r1, pr):
            h2 = prep_norm(qb.at[i], x1b, y0, r, pr, dep) * aff[0] + aff[1]
            h2b[r:r + pr, :] = h2.astype(bf16)
            dep = h2[:, 0:L]

    OC = (0, D - L, D)
    OP = (((0, D, 0, HM),),
          ((0, D - L, HM, TM), (D - L, D, HM, TM - 64), (D - L, D, TM - 64, TM)))

    def ffn_half(i, half, gb):
        h2 = h2b[half * HM:(half + 1) * HM, :]
        hs = []
        for f in range(0, F, TF):
            g = jnp.dot(h2, wgb[:, f:f + TF], preferred_element_type=f32)
            u = jnp.dot(h2, wub[:, f:f + TF], preferred_element_type=f32)
            hs.append(g * u)
        hh = jnp.concatenate(hs, axis=1).astype(bf16)
        for c0, c1, r0, r1 in OP[half]:
            o = jnp.dot(hh[r0 - half * HM:r1 - half * HM], wdb[:, c0:c1],
                        preferred_element_type=f32)
            ob[i, r0:r1, c0:c1] = (x1b[r0:r1, c0:c1] + gb[:, c0:c1] * o).astype(bf16)
            o_cp(i, c0, c1, r0, r1).start()

    acc, hcache, parts = {}, {}, {}

    def grp_g(p, n, f, half=None):
        t0, t1 = KP[p], KP[p + 1]
        if (p, half) not in hcache:
            if len(n2) == 1 and half != 0:
                n2.append(prep_norm(qb0, x1b0, 0, H0, TM0 - H0))
            x = jnp.concatenate(n2, axis=0) if half is None else n2[half]
            hcache[p, half] = (x[:, t0 * L:t1 * L] * (1.0 + modv(4, t0, t1))
                               + modv(3, t0, t1)).astype(bf16)
        rows = {None: slice(0, TM0), 0: slice(0, H0), 1: slice(H0, TM0)}[half]
        cols = slice(f * 4 * L, (f + 1) * 4 * L)
        d = jnp.dot(hcache[p, half], (wgb if n == "g" else wub)[t0 * L:t1 * L, cols],
                    preferred_element_type=f32)
        ref = gub.at["gu".index(n), rows, cols]
        if p < len(KP) - 2:
            ref[...] = d if p == 0 else ref[...] + d
        elif n == "g":
            acc[f] = ref[...] + d
        else:
            hb[:, cols] = (acc.pop(f) * (ref[...] + d)).astype(bf16)
        return [d[s:s + 8, c * L:(c + 1) * L] for c in range(0, 4, 4 // (t1 - t0))
                for s in range(0, d.shape[0], 16)]

    def grp_d(n, f):
        c = slice(n * L, (n + 1) * L)
        k = slice(f * 4 * L, (f + 1) * 4 * L)
        d = jnp.dot(hb[:, k], wdb[k, c], preferred_element_type=f32)
        parts[n] = d if f == 0 else parts[n] + d
        if f == 2:
            ob0[:, c] = (x1b0[:, c] + mod[5 * NT + n] * parts.pop(n)).astype(bf16)
            if (n + 1) * L in OC:
                o_cp(None, OC[OC.index((n + 1) * L) - 1], (n + 1) * L).start()
        return [d[s:s + 8] for s in range(0, TM0, 16)]

    grp_fn.update(g=grp_g, d=grp_d)
    for waits, rows, groups, jobs in FIRST:
        wait(*waits)
        for n in parts:
            parts[n] = dpart[:, n * L:(n + 1) * L]
        run(groups, jobs, lead=LEAD, floor=(0.0, 0.5 if rows else 0.0))
        if rows:
            aff += [1.0 + modv(4), modv(3)]
            prep_chain(0, *rows, PR)
        for n in parts:
            dpart[:, n * L:(n + 1) * L] = parts[n]
    gb = modv(5)
    wait("q1c", *[f"q{i + 1}" for i in range(1, NB)])

    def ffn(i, carry):
        prep_chain(i, HM, TM, PL)
        ffn_half(i, 0, gb)
        prep_chain(jnp.minimum(i + 1, NB - 1), 0, HM, PL)
        ffn_half(i, 1, gb)
        return carry

    lax.fori_loop(0, NB, ffn, 0)

    for c0, c1 in zip(OC[:-1], OC[1:]):
        o_cp(None, c0, c1).wait()
    for i in range(NB):
        for op in OP[0] + OP[1]:
            o_cp(i, *op).wait()


@jax.jit
def pallas_adaLN_cond__ssm_conv_h3__glu_gated_bilinear__prompt_kernel(
    A_q: jax.Array,
    A_k: jax.Array,
    A_v: jax.Array,
    A_shift_k: jax.Array,
    A_ssm_k: jax.Array,
    A_ssm_D: jax.Array,
    B_x: jax.Array,
    B_w_gate: jax.Array,
    B_w_up: jax.Array,
    B_w_down: jax.Array,
    c: jax.Array,
    w_mod: jax.Array,
):
    del B_x
    tiles = lambda x: x.reshape(S // 8, 8, NT, L).transpose(0, 2, 1, 3).reshape(S * NT, L)
    any_spec = pl.BlockSpec(memory_space=pl.ANY)
    return pl.pallas_call(
        _kernel,
        in_specs=[any_spec] * 11,
        out_specs=any_spec,
        out_shape=jax.ShapeDtypeStruct((1, S, D), bf16),
        scratch_shapes=[
            pltpu.VMEM((TM0, D), bf16),
            pltpu.VMEM((NB, TM, D), bf16),
            [pltpu.VMEM((4 * PAD + C * NT, L), bf16)] * NC,
            [pltpu.VMEM((2 * PAD + C * NT, L), bf16)] * NC,
            pltpu.VMEM((NT, L, S), bf16),
            pltpu.VMEM((D, F), bf16),
            pltpu.VMEM((D, F), bf16),
            pltpu.VMEM((F, D), bf16),
            pltpu.VMEM((D, 6 * D), bf16),
            pltpu.VMEM((NT, NC, R, L, L), bf16),
            pltpu.VMEM((NT, NC, R, 16, 16, L), f32),
            pltpu.VMEM((NT, NC, R, 16, 16, L), f32),
            pltpu.VMEM((NT, NC, R, 16, 16, L), f32),
            pltpu.VMEM((NT, NC, 2 * R, L, L), bf16),
            pltpu.VMEM((NT, S + 32, L), f32),
            pltpu.VMEM((TM0, D), f32),
            pltpu.VMEM((TM, D), f32),
            pltpu.VMEM((TM, D), bf16),
            pltpu.VMEM((2, TM0, F), f32),
            pltpu.VMEM((TM0, D), f32),
            pltpu.VMEM((TM0, F), bf16),
            pltpu.VMEM((TM0, D), bf16),
            pltpu.VMEM((NB, TM, D), bf16),
            pltpu.VMEM((32, 8 * VM, L), f32),
            pltpu.VMEM((KS, D), bf16),
            pltpu.VMEM((D,), bf16),
            pltpu.VMEM((1, D), bf16),
            pltpu.SemaphoreType.DMA((len(DMA_ORDER),)),
            pltpu.SemaphoreType.DMA((NB + 1,)),
        ],
        compiler_params=pltpu.CompilerParams(
            vmem_limit_bytes=120 * 1024 * 1024,
            disable_bounds_checks=True, disable_semaphore_checks=True),
        name="adaln_h3_glu",
    )(A_q, tiles(A_k), tiles(A_v), A_shift_k.T, A_ssm_k, A_ssm_D,
      B_w_gate, B_w_up, B_w_down, c, w_mod)
```

```python
import jax
import jax.numpy as jnp
from jax import lax
import jax.experimental.pallas as pl
import jax.experimental.pallas.tpu as pltpu

S = 2048
D = 640
F = 1536
KS = 4
L = 128
NT = D // L
R = 4
C = R * L
NC = S // C
EPS = 1e-5
RSQ2 = 0.7071067811865476

WPT = 4 * NT
PAD = 32

TM0 = 512
H0 = 352
TM = 384
NB = (S - TM0) // TM
HM = TM // 2
PL = 16
TF = 256
PR = 24
KP = (0, 1, 2, 3, 4, 5)
WM = {"mA": (0, 12), "c0": (20, 21), "mB": (12, 16), "s1": (16, 17), "c1": (21, 22),
      "s2": (17, 19), "c2": (22, 24), "s4": (19, 20), "c4": (24, 25), "mG": (25, 30)}
VM = 5
RATE = 1.05
LEAD = 24
FREE = {"i": 56, "z": 56, "k": 47, "u": 46}
FREE_FFN = {"i": 4, "u": 26, "d": 48, "D": 42, "g": 50}

f32 = jnp.float32
bf16 = jnp.bfloat16
u32 = jnp.uint32


def _cos_turns(t):
    x = jnp.abs(t - jnp.floor(t) - 0.5) - 0.25
    x2 = x * x
    return x * (6.283164024 + x2 * (-41.33713150 + x2 * (81.34038544 + x2 * -70.98993683)))


def _tables(inverse, hold=None):
    shape = (L // 2, L) if inverse else (2 * L, L)
    rho = lax.broadcasted_iota(jnp.int32, shape, 1 if inverse else 0)
    j = lax.broadcasted_iota(jnp.int32, shape, 0 if inverse else 1)
    if inverse:
        g, rad = 8 * (rho >> 4) + (rho & 7), 2 * R
    else:
        g, rad, j = 8 * (rho >> 5) + (rho & 7) + 64 * ((rho >> 4) & 1), R, _perm(j)
    a = (4 * g + 1).astype(f32) * (1.0 / (4 * C))
    off = ((rho >> 3) & 1).astype(f32) * 0.25
    ns = [(rad * j + r).astype(f32) for r in range(rad)]
    if hold is not None:
        ns = [hold(r, n) for r, n in enumerate(ns)]
    ts = [_cos_turns(a * n + off) for n in ns]
    return [(t * (1.0 / C) if inverse else t).astype(bf16) for t in ts]


def _perm(c):
    return 16 * (c >> 4) + 2 * (c & 7) + ((c >> 3) & 1)


def _layernorm(x):
    m = jnp.mean(x, axis=-1, keepdims=True)
    xc = x - m
    v = jnp.mean(xc * xc, axis=-1, keepdims=True)
    return xc * lax.rsqrt(v + EPS)


def _split(t):
    t = t.reshape(16, 16, L)
    return t[:, :8, :], t[:, 8:, :]


def _radix4(x, sgn):
    (ar, ai), (br, bi), (cr, ci), (dr, di) = x
    s0r, s0i, d0r, d0i = ar + cr, ai + ci, ar - cr, ai - ci
    s1r, s1i, d1r, d1i = br + dr, bi + di, br - dr, bi - di
    o0 = (s0r + s1r, s0i + s1i)
    o2 = (s0r - s1r, s0i - s1i)
    pl_ = (d0r - d1i, d0i + d1r)
    mi_ = (d0r + d1i, d0i - d1r)
    return [o0, pl_, o2, mi_] if sgn > 0 else [o0, mi_, o2, pl_]


T = range(NT)
_z = lambda j: [("z", j, a) for a in range(NC)]
_k = lambda j, al: [("k", j, a) for a in al]
_u = lambda a: [("u", j, a) for j in T]
_iv = lambda jl, al: [("i", j, a) for j in jl for a in al]
_kv = lambda a: [("kv", j, a) for j in T]
_m = lambda jl, us, outs: [("mac", j, us, outs) for j in jl]
A3 = (0, 1, 2)

A2 = (0, 1)
SCHEDULE = [
    (["ssm0"], _z(0) + _k(0, range(NC)), [("setup", None)]),
    (["ssm1"], _z(1) + _k(1, range(NC)), []),
    (["ssm2"], _z(2) + _k(2, [0, 1]), []),
    (["k0", "v0"], _k(2, [2, 3]) + _u(0), _kv(0) + _m([0], (0,), (0,))),
    (["ssm3"], _iv([0], [0]) + _z(3) + _k(3, [0, 1]), _m([1, 2], (0,), (0,))),
    (["k1", "v1"], _k(3, [2, 3]) + _u(1), _kv(1) + _m([3], (0,), (0,))),
    (["ssm4"], _iv([1, 2, 3], [0]) + _z(4) + _k(4, range(NC)), _m([0, 1, 2, 3], A2, (1,))),
    (["q0"], _iv([0, 1, 2, 3], [1]) + _iv([4], A2), _m([4], A2, A2)),
    (["mA", "c0"], [("mod", "mA", "c0")], []),
]
PREP_GROUPS = []

_g = lambda p: [("g", p, n, f) for f in range(3) for n in "gu"]
_d = [("d", n, f) for n in T for f in range(3)]
_v = lambda *names: [("vmod", n) for n in names]
_e = [("d", n, f) for n in T for f in (0, 1)]
FIRST = [
    (["wg0", "qh"], None, [("g", 0, "g", f, h) for h in (0, 1) for f in range(3)], []),
    (["wu0", "s1", "c1"], None, [("g", 0, "u", f) for f in range(3)],
     _v("s1", "c1") + _m([0], A2, (2, 3))),
    (["wg1", "wu1"], None, _g(1)[:-1], _m([1, 2], A2, (2, 3))),
    (["wg2", "wu2", "s2", "c2"], None, _g(1)[-1:] + _g(2),
     _v("s2", "c2") + _m([3, 4], A2, (2, 3))),
    (["wg3", "wu3", "wg4", "wu4", "s4", "c4", "q1"], (0, HM), _g(3) + _g(4), _v("s4", "c4")),
    (["wd", "k2", "v2"], None, _e[:2] + _u(2) + _e[2:6],
     _kv(2) + _m([0, 1, 2, 3], (2,), (2, 3))),
    (["mG", "k3", "v3"], None,
     _e[6:] + _u(3) + [(x, n, 2) for n in T for x in "di"] + _iv(T, [3]),
     _m([4], (2,), (2, 3)) + _kv(3) + _v("mG") + _m(T, (3,), (3,))),
]

DMA_ORDER = (["sk", "sd", "c", "ssm0", "ssm1", "ssm2", "k0", "v0", "ssm3", "k1", "v1", "ssm4",
              "q0", "c0", "mA", "mB", "wg0", "qh", "wu0", "s1", "c1", "wg1", "wu1", "s2", "c2",
              "wg2", "wu2", "s4", "c4", "wg3", "wu3", "wg4", "wu4", "q1", "wd", "k2", "v2", "mG", "k3", "v3",
              "q1c"] + [f"q{i + 1}" for i in range(1, NB)])


def _costs(job):
    if job[0] == "kv":
        return [48, 42] * (C // 64)
    if job[0] == "setup":
        return [100] * (4 * R)
    if job[0] == "vmod":
        return [3 * D // VM // 8] * (VM * (WM[job[1]][1] - WM[job[1]][0]))
    us, outs = job[2], job[3]
    pairs = [(a, n) for a in outs for n in us if n <= a]
    mac = (2 * len({a - n for a, n in pairs if a > n}) + 8 * len(pairs)
           - (2 * len(outs) if us[0] == 0 else 0))
    fin = sum(a <= us[-1] for a in outs)
    if mac < 12 and outs[-1] <= us[-1] < NC - 1:
        return [1 + R * mac + 16 * fin, 1 + R * mac + 48 * fin] * 8
    return ([1 + mac] * 3 + [1 + mac + 16 * fin] + [1 + mac] * 3 + [1 + mac + 48 * fin]) * 8


def _plan(groups, jobs, lead=0, floor=(1.0, 0.8)):
    free = FREE_FFN if lead else FREE
    nstep = {"i": 8, "z": 8, "k": 16, "u": 16, "mod": 0, "d": TM0 // 16}
    steps = lambda g: (KP[g[1] + 1] - KP[g[1]]) * TM0 // 16 if g[0] == "g" else nstep[g[0]]
    slots = [free["D" if g[0] == "d" and g[2] == 2 else g[0]]
             for g in groups for _ in range(steps(g))]
    lo, hi = [], []
    for job in jobs:
        begin, limit, first = 0, len(slots), 0
        for g in groups:
            kind = (g[0], job[0])
            if (kind == ("u", "kv") and g[1:] == job[1:]
                    or kind == ("i", "mac") and g[1] == job[1] and g[2] in job[3]
                    and g[2] <= job[2][-1] or kind == ("d", "vmod") and g[2] == 2):
                limit = min(limit, first - lead)
            if kind == ("g", "vmod") and job[1][1] == str(g[1]):
                limit = min(limit, first - 11)
            first += steps(g)
            if kind == ("u", "mac") and g[1] == job[1] and g[2] in job[2]:
                begin = first
        lo.append(begin)
        hi.append(limit)
    plan, credit, n = [], (slots or [0])[0], 0
    for k, job in enumerate(jobs):
        if n < lo[k]:
            n, credit = lo[k], min(credit, 0) + slots[lo[k]]
        work = [sum(_costs(j)) for j in jobs]
        if lead:
            rate = max(RATE * sum(work[k:m + 1]) / max(sum(slots[n:hi[m]]), 1)
                       for m in range(k, len(jobs)))
        else:
            rate = RATE * sum(work[k:]) / sum(slots[n:])
        rate = max(rate, floor[0] if job[0] == "kv" else floor[1])
        idx = []
        for c in _costs(job):
            while credit <= 0 and n + 1 < hi[k]:
                n += 1
                credit += slots[n] * rate
            credit -= c
            idx.append(n)
        plan.append(idx)
    return plan


def _kernel(q_hbm, k_hbm, v_hbm, sk_hbm, ssm_hbm, sd_hbm, wg_hbm, wu_hbm, wd_hbm,
            c_hbm, wm_hbm, o_hbm,
            qb0, qb, kbs, vbs, ssmb, wgb, wub, wdb, wmb, uwb, ub, kpb, yp, pb, yb,
            x1b0, x1b, h2b, gub, dpart, hb, ob0, ob, mv, skb, sdb, cb_, sem, osem):
    cps = {"sk": (sk_hbm, skb), "sd": (sd_hbm, sdb), "c": (c_hbm, cb_), "wd": (wd_hbm, wdb)}
    for j in range(NT):
        cps[f"ssm{j}"] = (ssm_hbm.at[pl.ds(j * L, L), :], ssmb.at[j])
    for a in range(NC):
        n, h = C * NT, 2 * PAD
        if a == 0:
            cps["k0"] = (k_hbm.at[pl.ds(0, n), :], kbs[0].at[pl.ds(h, n), :])
        else:
            e = 48
            cps[f"k{a}"] = (k_hbm.at[pl.ds(a * n - e, n + e), :],
                            kbs[a].at[pl.ds(h - e, n + e), :])
        cps[f"v{a}"] = (v_hbm.at[pl.ds(a * n, n), :], vbs[a].at[pl.ds(0, n), :])
    for n, (c0, c1) in WM.items():
        cols = pl.ds(c0 * L, (c1 - c0) * L)
        cps[n] = (wm_hbm.at[:, cols], wmb.at[:, cols])
    cps["q0"] = (q_hbm.at[0, pl.ds(0, H0), :], qb0.at[pl.ds(0, H0), :])
    cps["qh"] = (q_hbm.at[0, pl.ds(H0, TM0 - H0), :], qb0.at[pl.ds(H0, TM0 - H0), :])
    cps["q1"] = (q_hbm.at[0, pl.ds(TM0, HM), :], qb.at[0, pl.ds(0, HM), :])
    cps["q1c"] = (q_hbm.at[0, pl.ds(TM0 + HM, HM), :], qb.at[0, pl.ds(HM, HM), :])
    for i in range(1, NB):
        cps[f"q{i + 1}"] = (q_hbm.at[0, pl.ds(TM0 + i * TM, TM), :], qb.at[i])
    for p in range(len(KP) - 1):
        rows = pl.ds(KP[p] * L, (KP[p + 1] - KP[p]) * L)
        cps[f"wg{p}"] = (wg_hbm.at[rows, :], wgb.at[rows, :])
        cps[f"wu{p}"] = (wu_hbm.at[rows, :], wub.at[rows, :])
    assert sorted(cps) == sorted(DMA_ORDER)

    def cp(name):
        src, dst = cps[name]
        return pltpu.make_async_copy(src, dst, sem.at[DMA_ORDER.index(name)])

    def wait(*names):
        for n in names:
            cp(n).wait()

    kbs[0][0:2 * PAD, :] = jnp.zeros((2 * PAD, L), bf16)
    for n in DMA_ORDER:
        cp(n).start()

    tabs, ginv, ccol = _tables(False), [], []
    for ref in (ub, kpb, yp):
        ref[0, 0, 0, 0, pl.ds(0, 8, stride=2), :] = jnp.zeros((8, L), f32)
    mv[0, pl.ds(0, 8, stride=2), :] = jnp.zeros((8, L), f32)
    ri = lax.broadcasted_iota(jnp.int32, (L, L), 0)
    ci = lax.broadcasted_iota(jnp.int32, (L, L), 1)
    sel = jnp.where(ci == R * _perm(ri & 31) + (ri >> 5), 1.0, 0.0).astype(bf16)

    wait("sk", "sd", "c")
    skt = skb[...].astype(f32)
    sdv = sdb[...].astype(f32).reshape(1, D)
    cv = cb_[...].astype(f32)
    sig = jax.nn.sigmoid(cv)
    cs = jnp.broadcast_to((cv * sig).astype(bf16), (16, D))
    one = sig[:, 0:L]

    def gate(x, deps):
        dep = jnp.concatenate(deps, axis=0).reshape(x.shape)
        return jnp.where(jnp.broadcast_to(one, x.shape) > 2.0, dep, x)

    def put(dst, j, a, xs):
        for qi in range(R):
            dst[j, a, qi] = jnp.concatenate(xs[qi], axis=1)

    zs = {}
    mod = {}

    def grp_z(j, a):
        z = [lax.dot_general(sel, ssmb[j, :, t * L:(t + 1) * L], (((1,), (1,)), ((), ())),
                             preferred_element_type=f32) for t in range(R * a, R * a + R)]
        zs[j, a] = [jnp.concatenate([z[p][32 * r:32 * (r + 1)] for p in range(R)],
                                    axis=0).astype(bf16) for r in range(R)]
        return [z[0][16 * t:16 * t + 8] for t in range(8)]

    def grp_fwd(ws, dst, j, a, dvec=None):
        t = [jnp.dot(tabs[r], ws[r], preferred_element_type=f32) for r in range(R)]
        x = [_split(v) for v in t]
        if dvec is not None:
            x[0] = (x[0][0] + dvec[None], x[0][1])
        put(dst, j, a, _radix4(x, -1))
        return [t[0][16 * s:16 * s + 8] for s in range(16)]

    def grp_k(j, a):
        return grp_fwd(zs.pop((j, a)), kpb, j, a,
                       sdv[:, j * L:(j + 1) * L] if a == 0 else None)

    def grp_u(j, a):
        uw = [uwb[j, a, r] for r in range(R)]
        return grp_fwd(uw, ub, j, a)

    def grp_i(j, a):
        ys = []
        for r in range(2 * R):
            y = jnp.dot(ginv[r], pb[j, a, r], preferred_element_type=f32)
            yb[j, pl.ds(a * C + r, L // 2, stride=2 * R), :] = y
            ys.append(y)
        return [ys[r][16 * s:16 * s + 8] for r in (0, R) for s in range(4)]

    def grp_mod(*names):
        for name in names:
            c0, c1 = WM[name]
            m = jnp.dot(cs, wmb[:, c0 * L:c1 * L], preferred_element_type=f32)
            for c in range(c0, c1):
                mod[c] = m[0:1, (c - c0) * L:(c - c0 + 1) * L]
        return []

    def modv(i, t0=0, t1=NT):
        return jnp.concatenate([mod[i * NT + n] for n in range(t0, t1)], axis=1)

    def job_kv(j, a, deps):
        lo = lambda x: lax.bitcast_convert_type(x << 16, f32)
        hi = lambda x: lax.bitcast_convert_type(x & jnp.uint32(0xFFFF0000), f32)
        n = C // 8
        kw, vw = kbs[a].bitcast(u32), vbs[a].bitcast(u32)
        ld = lambda ref, o: ref[pl.ds(4 * j + o, n, stride=WPT), :]
        k = {}
        for m in range(4):
            x = ld(kw, PAD + m)
            k[2 * m], k[2 * m + 1] = lo(x), hi(x)
        k[-3] = hi(ld(kw, PAD - WPT + 2))
        x = ld(kw, PAD - WPT + 3)
        k[-2], k[-1] = lo(x), hi(x)
        w = [skt[t:t + 1, j * L:(j + 1) * L] for t in range(KS)]
        w0 = [gate(jnp.broadcast_to(w[0], (n, L)), deps[e::2]) for e in (0, 1)]
        kv = {}
        for m in range(4):
            x = ld(vw, m)
            for ph, v in ((2 * m, lo(x)), (2 * m + 1, hi(x))):
                ks = k[ph] * w0[m % 2]
                for t in range(1, KS):
                    ks = ks + k[ph - t] * w[t]
                kv[ph] = (ks * v).reshape(n // 8, 8, L)
        for r in range(R):
            uwb[j, a, r] = jnp.concatenate([kv[r], kv[r + R]], axis=1).reshape(L, L).astype(bf16)

    def job_mac(j, us, outs, deps):
        ld = lambda ref, a: (ref[j, a, :, :, 0:8, :], ref[j, a, :, :, 8:16, :])
        lo, hi = us[0], us[-1]
        u = {a: ld(ub, a) for a in us}
        if len(deps) == 16:
            ur = jnp.concatenate([gate(u[lo][0][0:1], deps), u[lo][0][1:]], axis=0)
        else:
            ur = gate(u[lo][0], [deps[R * i + qi] for qi in range(R) for i in range(16)])
        u[lo] = (ur, u[lo][1])
        ms = sorted({a - n for a in outs for n in us if n <= a})
        k = {m: ld(kpb, m) for m in sorted(set(ms) | {m - 1 for m in ms if m > 0})}
        kp = {m: k[m] if m == 0 else (k[m][0] - k[m - 1][1], k[m][1] + k[m - 1][0]) for m in ms}
        for a in outs:
            yr, yi = ld(yp, a) if lo > 0 else (None, None)
            for n in us:
                if n > a:
                    continue
                (kr, ki), (ur, ui) = kp[a - n], u[n]
                tr = kr * ur - ki * ui
                ti = kr * ui + ki * ur
                yr = tr if yr is None else yr + tr
                yi = ti if yi is None else yi + ti
            if a > hi:
                yp[j, a] = jnp.concatenate([yr, yi], axis=2)
                continue
            ps = _radix4([(yr[qi], yi[qi]) for qi in range(R)], +1)
            for r in range(R):
                pr, pi = [p.reshape(8, 2, 8, L) for p in ps[r]]
                lr, li, hr, hi_ = pr[:, 0], pi[:, 0], pr[:, 1], pi[:, 1]
                if r % 2:
                    hr, hi_ = (hr - hi_) * RSQ2, (hr + hi_) * RSQ2
                if r < 2:
                    outs2 = (lr + hr, li + hi_), (lr - hr, li - hi_)
                else:
                    outs2 = (lr - hi_, li + hr), (lr + hi_, li - hr)
                for e in range(2):
                    pb[j, a, r + R * e] = jnp.concatenate(
                        outs2[e], axis=1).reshape(L, L).astype(bf16)

    def job_setup(_, deps):
        def hold(r, n):
            return gate(n, [deps[2 * r + s // 4] for s in range(8)])

        ginv.extend(_tables(True, hold))
        csf = cs[0:1].astype(f32)
        ccol.append(jnp.concatenate([jnp.broadcast_to(csf[:, t * L:(t + 1) * L], (L, L)).T
                                     for t in range(NT)], axis=0))

    def job_vmod(name, deps):
        c0, c1 = WM[name]
        n = D // VM
        for c in range(c0, c1):
            for i in range(VM):
                cc = ccol[0][i * n:(i + 1) * n]
                cc = jnp.concatenate([gate(cc[0:8], [deps[(c - c0) * VM + i]]), cc[8:]], axis=0)
                p = wmb[i * n:(i + 1) * n, c * L:(c + 1) * L].astype(f32) * cc
                mv[c, 8 * i:8 * i + 8, :] = jnp.sum(p.reshape(n // 8, 8, L), axis=0)
            mod[c] = jnp.sum(mv[c], axis=0, keepdims=True)

    grp_fn = {"z": grp_z, "k": grp_k, "u": grp_u, "i": grp_i, "mod": grp_mod}
    job_fn = {"kv": job_kv, "mac": job_mac, "vmod": job_vmod, "setup": job_setup}

    def run(groups, jobs, **kw):
        plan = _plan(groups, jobs, **kw)
        anchors, done = [], 0
        for g in groups + [None]:
            while done < len(jobs) and max(plan[done]) < len(anchors):
                job_fn[jobs[done][0]](*jobs[done][1:], [anchors[n] for n in plan[done]])
                done += 1
            if g is not None:
                anchors += grp_fn[g[0]](*g[1:])
        assert done == len(jobs)

    for waits, groups, jobs in SCHEDULE:
        wait(*waits)
        run(groups, jobs)

    n1, dep = [], None
    for r in range(0, H0, H0 // 2):
        x = qb0[r:r + H0 // 2, :].astype(f32)
        if dep is not None:
            x = jnp.concatenate([gate(x[:, 0:L], [dep]), x[:, L:]], axis=1)
        n1.append(_layernorm(x))
        dep = n1[-1][:, 0:L]
    n1 = jnp.concatenate(n1, axis=0)
    wait("mB")
    grp_mod("mB")
    for g in PREP_GROUPS:
        grp_fn[g[0]](*g[1:])
    sa, ca, ga = [modv(i) for i in range(3)]
    a1 = ga * (1.0 + ca)
    b1 = ga * sa

    def o_cp(i, c0, c1, r0=0, r1=TM):
        cols = pl.ds(c0, c1 - c0)
        if i is None:
            return pltpu.make_async_copy(ob0.at[:, cols], o_hbm.at[0, pl.ds(0, TM0), cols],
                                         osem.at[NB])
        base = TM0 + i * TM + r0
        if not isinstance(i, int):
            base = pl.multiple_of(base, 64)
        return pltpu.make_async_copy(ob.at[i, pl.ds(r0, r1 - r0), cols],
                                     o_hbm.at[0, pl.ds(base, r1 - r0), cols], osem.at[i])

    def prep_norm(q_ref, x1_ref, y0, r0, n, dep=None, n1=None):
        x = q_ref[r0:r0 + n, :].astype(f32)
        if dep is not None:
            x = jnp.concatenate([gate(x[:, 0:L], [dep]), x[:, L:]], axis=1)
        y = jnp.concatenate([yb[j, pl.ds(y0 + r0, n), :] for j in range(NT)], axis=1)
        x1 = x + ((_layernorm(x) if n1 is None else n1) * a1 + b1) * y
        x1_ref[r0:r0 + n, :] = x1
        return _layernorm(x1)

    n2 = [prep_norm(qb0, x1b0, 0, 0, H0, None, n1)]
    aff = []

    def prep_chain(i, r0, r1, pr):
        y0 = TM0 + i * TM
        if not isinstance(i, int):
            y0 = pl.multiple_of(y0, L)
        dep = None
        for r in range(r0, r1, pr):
            h2 = prep_norm(qb.at[i], x1b, y0, r, pr, dep) * aff[0] + aff[1]
            h2b[r:r + pr, :] = h2.astype(bf16)
            dep = h2[:, 0:L]

    OC = (0, D - L, D)
    OP = (((0, D, 0, HM),),
          ((0, D - L, HM, TM), (D - L, D, HM, TM - 64), (D - L, D, TM - 64, TM)))

    def ffn_half(i, half, gb):
        h2 = h2b[half * HM:(half + 1) * HM, :]
        hs = []
        for f in range(0, F, TF):
            g = jnp.dot(h2, wgb[:, f:f + TF], preferred_element_type=f32)
            u = jnp.dot(h2, wub[:, f:f + TF], preferred_element_type=f32)
            hs.append(g * u)
        hh = jnp.concatenate(hs, axis=1).astype(bf16)
        for c0, c1, r0, r1 in OP[half]:
            o = jnp.dot(hh[r0 - half * HM:r1 - half * HM], wdb[:, c0:c1],
                        preferred_element_type=f32)
            ob[i, r0:r1, c0:c1] = (x1b[r0:r1, c0:c1] + gb[:, c0:c1] * o).astype(bf16)
            o_cp(i, c0, c1, r0, r1).start()

    acc, hcache, parts = {}, {}, {}

    def grp_g(p, n, f, half=None):
        t0, t1 = KP[p], KP[p + 1]
        if (p, half) not in hcache:
            if len(n2) == 1 and half != 0:
                n2.append(prep_norm(qb0, x1b0, 0, H0, TM0 - H0))
            x = jnp.concatenate(n2, axis=0) if half is None else n2[half]
            hcache[p, half] = (x[:, t0 * L:t1 * L] * (1.0 + modv(4, t0, t1))
                               + modv(3, t0, t1)).astype(bf16)
        rows = {None: slice(0, TM0), 0: slice(0, H0), 1: slice(H0, TM0)}[half]
        cols = slice(f * 4 * L, (f + 1) * 4 * L)
        d = jnp.dot(hcache[p, half], (wgb if n == "g" else wub)[t0 * L:t1 * L, cols],
                    preferred_element_type=f32)
        ref = gub.at["gu".index(n), rows, cols]
        if p < len(KP) - 2:
            ref[...] = d if p == 0 else ref[...] + d
        elif n == "g":
            acc[f] = ref[...] + d
        else:
            hb[:, cols] = (acc.pop(f) * (ref[...] + d)).astype(bf16)
        return [d[s:s + 8, c * L:(c + 1) * L] for c in range(0, 4, 4 // (t1 - t0))
                for s in range(0, d.shape[0], 16)]

    def grp_d(n, f):
        c = slice(n * L, (n + 1) * L)
        k = slice(f * 4 * L, (f + 1) * 4 * L)
        d = jnp.dot(hb[:, k], wdb[k, c], preferred_element_type=f32)
        parts[n] = d if f == 0 else parts[n] + d
        if f == 2:
            ob0[:, c] = (x1b0[:, c] + mod[5 * NT + n] * parts.pop(n)).astype(bf16)
            if (n + 1) * L in OC:
                o_cp(None, OC[OC.index((n + 1) * L) - 1], (n + 1) * L).start()
        return [d[s:s + 8] for s in range(0, TM0, 16)]

    grp_fn.update(g=grp_g, d=grp_d)
    for waits, rows, groups, jobs in FIRST:
        wait(*waits)
        for n in parts:
            parts[n] = dpart[:, n * L:(n + 1) * L]
        run(groups, jobs, lead=LEAD, floor=(0.0, 0.5 if rows else 0.0))
        if rows:
            aff += [1.0 + modv(4), modv(3)]
            prep_chain(0, *rows, PR)
        for n in parts:
            dpart[:, n * L:(n + 1) * L] = parts[n]
    gb = modv(5)
    wait("q1c", *[f"q{i + 1}" for i in range(1, NB)])

    def ffn(i, carry):
        prep_chain(i, HM, TM, PL)
        ffn_half(i, 0, gb)
        prep_chain(jnp.minimum(i + 1, NB - 1), 0, HM, PL)
        ffn_half(i, 1, gb)
        return carry

    lax.fori_loop(0, NB, ffn, 0)

    for c0, c1 in zip(OC[:-1], OC[1:]):
        o_cp(None, c0, c1).wait()
    for i in range(NB):
        for op in OP[0] + OP[1]:
            o_cp(i, *op).wait()


@jax.jit
def pallas_adaLN_cond__ssm_conv_h3__glu_gated_bilinear__prompt_kernel(
    A_q: jax.Array,
    A_k: jax.Array,
    A_v: jax.Array,
    A_shift_k: jax.Array,
    A_ssm_k: jax.Array,
    A_ssm_D: jax.Array,
    B_x: jax.Array,
    B_w_gate: jax.Array,
    B_w_up: jax.Array,
    B_w_down: jax.Array,
    c: jax.Array,
    w_mod: jax.Array,
):
    del B_x
    tiles = lambda x: x.reshape(S // 8, 8, NT, L).transpose(0, 2, 1, 3).reshape(S * NT, L)
    any_spec = pl.BlockSpec(memory_space=pl.ANY)
    return pl.pallas_call(
        _kernel,
        in_specs=[any_spec] * 11,
        out_specs=any_spec,
        out_shape=jax.ShapeDtypeStruct((1, S, D), bf16),
        scratch_shapes=[
            pltpu.VMEM((TM0, D), bf16),
            pltpu.VMEM((NB, TM, D), bf16),
            [pltpu.VMEM((4 * PAD + C * NT, L), bf16)] * NC,
            [pltpu.VMEM((2 * PAD + C * NT, L), bf16)] * NC,
            pltpu.VMEM((NT, L, S), bf16),
            pltpu.VMEM((D, F), bf16),
            pltpu.VMEM((D, F), bf16),
            pltpu.VMEM((F, D), bf16),
            pltpu.VMEM((D, 6 * D), bf16),
            pltpu.VMEM((NT, NC, R, L, L), bf16),
            pltpu.VMEM((NT, NC, R, 16, 16, L), f32),
            pltpu.VMEM((NT, NC, R, 16, 16, L), f32),
            pltpu.VMEM((NT, NC, R, 16, 16, L), f32),
            pltpu.VMEM((NT, NC, 2 * R, L, L), bf16),
            pltpu.VMEM((NT, S + 32, L), f32),
            pltpu.VMEM((TM0, D), f32),
            pltpu.VMEM((TM, D), f32),
            pltpu.VMEM((TM, D), bf16),
            pltpu.VMEM((2, TM0, F), f32),
            pltpu.VMEM((TM0, D), f32),
            pltpu.VMEM((TM0, F), bf16),
            pltpu.VMEM((TM0, D), bf16),
            pltpu.VMEM((NB, TM, D), bf16),
            pltpu.VMEM((32, 8 * VM, L), f32),
            pltpu.VMEM((KS, D), bf16),
            pltpu.VMEM((D,), bf16),
            pltpu.VMEM((1, D), bf16),
            pltpu.SemaphoreType.DMA((len(DMA_ORDER),)),
            pltpu.SemaphoreType.DMA((NB + 1,)),
        ],
        compiler_params=pltpu.CompilerParams(
            vmem_limit_bytes=120 * 1024 * 1024,
            disable_bounds_checks=True, disable_semaphore_checks=True),
        name="adaln_h3_glu",
    )(A_q, tiles(A_k), tiles(A_v), A_shift_k.T, A_ssm_k, A_ssm_D,
      B_w_gate, B_w_up, B_w_down, c, w_mod)
```

```python
import jax
import jax.numpy as jnp
from jax import lax
import jax.experimental.pallas as pl
import jax.experimental.pallas.tpu as pltpu

S = 2048
D = 640
F = 1536
KS = 4
L = 128
NT = D // L
R = 4
C = R * L
NC = S // C
EPS = 1e-5
RSQ2 = 0.7071067811865476

WPT = 4 * NT
PAD = 32

TM0 = 512
H0 = 352
TM = 512
NB = (S - TM0) // TM
HM = 240
PL = 16
TF = 256
PR = 24
KP = (0, 1, 2, 3, 4, 5)
WM = {"mA": (0, 12), "c0": (20, 21), "mB": (12, 16), "s1": (16, 17), "c1": (21, 22),
      "s2": (17, 19), "c2": (22, 24), "s4": (19, 20), "c4": (24, 25), "mG": (25, 30)}
VM = 5
RATE = 1.05
LEAD = 24
FREE = {"i": 56, "z": 56, "k": 47, "u": 46}
FREE_FFN = {"i": 4, "u": 26, "d": 48, "D": 42, "g": 50}

f32 = jnp.float32
bf16 = jnp.bfloat16
u32 = jnp.uint32


def _cos_turns(t):
    x = jnp.abs(t - jnp.floor(t) - 0.5) - 0.25
    x2 = x * x
    return x * (6.283164024 + x2 * (-41.33713150 + x2 * (81.34038544 + x2 * -70.98993683)))


def _tables(inverse, hold=None):
    shape = (L // 2, L) if inverse else (2 * L, L)
    rho = lax.broadcasted_iota(jnp.int32, shape, 1 if inverse else 0)
    j = lax.broadcasted_iota(jnp.int32, shape, 0 if inverse else 1)
    if inverse:
        g, rad = 8 * (rho >> 4) + (rho & 7), 2 * R
    else:
        g, rad, j = 8 * (rho >> 5) + (rho & 7) + 64 * ((rho >> 4) & 1), R, _perm(j)
    a = (4 * g + 1).astype(f32) * (1.0 / (4 * C))
    off = ((rho >> 3) & 1).astype(f32) * 0.25
    ns = [(rad * j + r).astype(f32) for r in range(rad)]
    if hold is not None:
        ns = [hold(r, n) for r, n in enumerate(ns)]
    ts = [_cos_turns(a * n + off) for n in ns]
    return [(t * (1.0 / C) if inverse else t).astype(bf16) for t in ts]


def _perm(c):
    return 16 * (c >> 4) + 2 * (c & 7) + ((c >> 3) & 1)


def _layernorm(x):
    m = jnp.mean(x, axis=-1, keepdims=True)
    xc = x - m
    v = jnp.mean(xc * xc, axis=-1, keepdims=True)
    return xc * lax.rsqrt(v + EPS)


def _split(t):
    t = t.reshape(16, 16, L)
    return t[:, :8, :], t[:, 8:, :]


def _radix4(x, sgn):
    (ar, ai), (br, bi), (cr, ci), (dr, di) = x
    s0r, s0i, d0r, d0i = ar + cr, ai + ci, ar - cr, ai - ci
    s1r, s1i, d1r, d1i = br + dr, bi + di, br - dr, bi - di
    o0 = (s0r + s1r, s0i + s1i)
    o2 = (s0r - s1r, s0i - s1i)
    pl_ = (d0r - d1i, d0i + d1r)
    mi_ = (d0r + d1i, d0i - d1r)
    return [o0, pl_, o2, mi_] if sgn > 0 else [o0, mi_, o2, pl_]


T = range(NT)
_z = lambda j: [("z", j, a) for a in range(NC)]
_k = lambda j, al: [("k", j, a) for a in al]
_u = lambda a: [("u", j, a) for j in T]
_iv = lambda jl, al: [("i", j, a) for j in jl for a in al]
_kv = lambda a: [("kv", j, a) for j in T]
_m = lambda jl, us, outs: [("mac", j, us, outs) for j in jl]

A2 = (0, 1)
SCHEDULE = [
    (["ssm0"], _z(0) + _k(0, range(NC)), [("setup", None)]),
    (["ssm1"], _z(1) + _k(1, range(NC)), []),
    (["ssm2"], _z(2) + _k(2, [0, 1]), []),
    (["k0", "v0"], _k(2, [2, 3]) + _u(0), _kv(0) + _m([0], (0,), (0,))),
    (["ssm3"], _iv([0], [0]) + _z(3) + _k(3, [0, 1]), _m([1, 2], (0,), (0,))),
    (["k1", "v1"], _k(3, [2, 3]) + _u(1), _kv(1) + _m([3], (0,), (0,))),
    (["ssm4"], _iv([1, 2, 3], [0]) + _z(4) + _k(4, range(NC)), _m([0, 1, 2, 3], A2, (1,))),
    (["q0"], _iv([0, 1, 2, 3], [1]) + _iv([4], A2), _m([4], A2, A2)),
    (["mA", "c0"], [("mod", "mA", "c0")], []),
]
_g = lambda p: [("g", p, n, f) for f in range(3) for n in "gu"]
_v = lambda *names: [("vmod", n) for n in names]
_e = [("d", n, f) for n in T for f in (0, 1)]
FIRST = [
    (["wg0", "qh"], None, [("g", 0, "g", f, h) for h in (0, 1) for f in range(3)], []),
    (["wu0", "s1", "c1"], None, [("g", 0, "u", f) for f in range(3)],
     _v("s1", "c1") + _m([0], A2, (2, 3))),
    (["wg1", "wu1"], None, _g(1)[:-1], _m([1, 2], A2, (2, 3))),
    (["wg2", "wu2", "s2", "c2"], None, _g(1)[-1:] + _g(2),
     _v("s2", "c2") + _m([3, 4], A2, (2, 3))),
    (["wg3", "wu3", "wg4", "wu4", "s4", "c4", "q1"], (0, HM), _g(3) + _g(4), _v("s4", "c4")),
    (["wd", "k2", "v2"], None, _e[:2] + _u(2) + _e[2:6],
     _kv(2) + _m([0, 1, 2, 3], (2,), (2, 3))),
    (["mG", "k3", "v3"], None,
     _e[6:] + _u(3) + [(x, n, 2) for n in T for x in "di"] + _iv(T, [3]),
     _m([4], (2,), (2, 3)) + _kv(3) + _v("mG") + _m(T, (3,), (3,))),
]

DMA_ORDER = (["sk", "sd", "c", "ssm0", "ssm1", "ssm2", "k0", "v0", "ssm3", "k1", "v1", "ssm4",
              "q0", "c0", "mA", "mB", "wg0", "qh", "wu0", "s1", "c1", "wg1", "wu1", "s2", "c2",
              "wg2", "wu2", "s4", "c4", "wg3", "wu3", "wg4", "wu4", "q1", "wd", "k2", "v2", "mG", "k3", "v3",
              "q1c"] + [f"q{i + 1}" for i in range(1, NB)])


def _costs(job):
    if job[0] == "kv":
        return [48, 42] * (C // 64)
    if job[0] == "setup":
        return [100] * (4 * R)
    if job[0] == "vmod":
        return [3 * D // VM // 8] * (VM * (WM[job[1]][1] - WM[job[1]][0]))
    us, outs = job[2], job[3]
    pairs = [(a, n) for a in outs for n in us if n <= a]
    mac = (2 * len({a - n for a, n in pairs if a > n}) + 8 * len(pairs)
           - (2 * len(outs) if us[0] == 0 else 0))
    fin = sum(a <= us[-1] for a in outs)
    if mac < 12 and outs[-1] <= us[-1] < NC - 1:
        return [1 + R * mac + 16 * fin, 1 + R * mac + 48 * fin] * 8
    return ([1 + mac] * 3 + [1 + mac + 16 * fin] + [1 + mac] * 3 + [1 + mac + 48 * fin]) * 8


def _plan(groups, jobs, lead=0, floor=(1.0, 0.8)):
    free = FREE_FFN if lead else FREE
    nstep = {"i": 8, "z": 8, "k": 16, "u": 16, "mod": 0, "d": TM0 // 16}
    steps = lambda g: (KP[g[1] + 1] - KP[g[1]]) * TM0 // 16 if g[0] == "g" else nstep[g[0]]
    slots = [free["D" if g[0] == "d" and g[2] == 2 else g[0]]
             for g in groups for _ in range(steps(g))]
    lo, hi = [], []
    for job in jobs:
        begin, limit, first = 0, len(slots), 0
        for g in groups:
            kind = (g[0], job[0])
            if (kind == ("u", "kv") and g[1:] == job[1:]
                    or kind == ("i", "mac") and g[1] == job[1] and g[2] in job[3]
                    and g[2] <= job[2][-1] or kind == ("d", "vmod") and g[2] == 2):
                limit = min(limit, first - lead)
            if kind == ("g", "vmod") and job[1][1] == str(g[1]):
                limit = min(limit, first - 11)
            first += steps(g)
            if kind == ("u", "mac") and g[1] == job[1] and g[2] in job[2]:
                begin = first
        lo.append(begin)
        hi.append(limit)
    plan, credit, n = [], (slots or [0])[0], 0
    for k, job in enumerate(jobs):
        if n < lo[k]:
            n, credit = lo[k], min(credit, 0) + slots[lo[k]]
        work = [sum(_costs(j)) for j in jobs]
        if lead:
            rate = max(RATE * sum(work[k:m + 1]) / max(sum(slots[n:hi[m]]), 1)
                       for m in range(k, len(jobs)))
        else:
            rate = RATE * sum(work[k:]) / sum(slots[n:])
        rate = max(rate, floor[0] if job[0] == "kv" else floor[1])
        idx = []
        for c in _costs(job):
            while credit <= 0 and n + 1 < hi[k]:
                n += 1
                credit += slots[n] * rate
            credit -= c
            idx.append(n)
        plan.append(idx)
    return plan


def _kernel(q_hbm, k_hbm, v_hbm, sk_hbm, ssm_hbm, sd_hbm, wg_hbm, wu_hbm, wd_hbm,
            c_hbm, wm_hbm, o_hbm,
            qb0, qb, kbs, vbs, ssmb, wgb, wub, wdb, wmb, uwb, ub, kpb, yp, pb, yb,
            x1b0, x1b, h2b, gub, dpart, hb, ob0, ob, mv, skb, sdb, cb_, sem, osem):
    cps = {"sk": (sk_hbm, skb), "sd": (sd_hbm, sdb), "c": (c_hbm, cb_), "wd": (wd_hbm, wdb)}
    for j in range(NT):
        cps[f"ssm{j}"] = (ssm_hbm.at[pl.ds(j * L, L), :], ssmb.at[j])
    for a in range(NC):
        n, h = C * NT, 2 * PAD
        if a == 0:
            cps["k0"] = (k_hbm.at[pl.ds(0, n), :], kbs[0].at[pl.ds(h, n), :])
        else:
            e = 48
            cps[f"k{a}"] = (k_hbm.at[pl.ds(a * n - e, n + e), :],
                            kbs[a].at[pl.ds(h - e, n + e), :])
        cps[f"v{a}"] = (v_hbm.at[pl.ds(a * n, n), :], vbs[a].at[pl.ds(0, n), :])
    for n, (c0, c1) in WM.items():
        cols = pl.ds(c0 * L, (c1 - c0) * L)
        cps[n] = (wm_hbm.at[:, cols], wmb.at[:, cols])
    cps["q0"] = (q_hbm.at[0, pl.ds(0, H0), :], qb0.at[pl.ds(0, H0), :])
    cps["qh"] = (q_hbm.at[0, pl.ds(H0, TM0 - H0), :], qb0.at[pl.ds(H0, TM0 - H0), :])
    cps["q1"] = (q_hbm.at[0, pl.ds(TM0, HM), :], qb.at[0, pl.ds(0, HM), :])
    cps["q1c"] = (q_hbm.at[0, pl.ds(TM0 + HM, TM - HM), :], qb.at[0, pl.ds(HM, TM - HM), :])
    for i in range(1, NB):
        cps[f"q{i + 1}"] = (q_hbm.at[0, pl.ds(TM0 + i * TM, TM), :], qb.at[i])
    for p in range(len(KP) - 1):
        rows = pl.ds(KP[p] * L, (KP[p + 1] - KP[p]) * L)
        cps[f"wg{p}"] = (wg_hbm.at[rows, :], wgb.at[rows, :])
        cps[f"wu{p}"] = (wu_hbm.at[rows, :], wub.at[rows, :])
    assert sorted(cps) == sorted(DMA_ORDER)

    def cp(name):
        src, dst = cps[name]
        return pltpu.make_async_copy(src, dst, sem.at[DMA_ORDER.index(name)])

    def wait(*names):
        for n in names:
            cp(n).wait()

    kbs[0][0:2 * PAD, :] = jnp.zeros((2 * PAD, L), bf16)
    for n in DMA_ORDER:
        cp(n).start()

    tabs, ginv, ccol = _tables(False), [], []
    for ref in (ub, kpb, yp):
        ref[0, 0, 0, 0, pl.ds(0, 8, stride=2), :] = jnp.zeros((8, L), f32)
    mv[0, pl.ds(0, 8, stride=2), :] = jnp.zeros((8, L), f32)
    ri = lax.broadcasted_iota(jnp.int32, (L, L), 0)
    ci = lax.broadcasted_iota(jnp.int32, (L, L), 1)
    sel = jnp.where(ci == R * _perm(ri & 31) + (ri >> 5), 1.0, 0.0).astype(bf16)

    wait("sk", "sd", "c")
    skt = skb[...].astype(f32)
    sdv = sdb[...].astype(f32).reshape(1, D)
    cv = cb_[...].astype(f32)
    sig = jax.nn.sigmoid(cv)
    cs = jnp.broadcast_to((cv * sig).astype(bf16), (16, D))
    one = sig[:, 0:L]

    def gate(x, deps):
        dep = jnp.concatenate(deps, axis=0).reshape(x.shape)
        return jnp.where(jnp.broadcast_to(one, x.shape) > 2.0, dep, x)

    def put(dst, j, a, xs):
        for qi in range(R):
            dst[j, a, qi] = jnp.concatenate(xs[qi], axis=1)

    zs = {}
    mod = {}

    def grp_z(j, a):
        z = [lax.dot_general(sel, ssmb[j, :, t * L:(t + 1) * L], (((1,), (1,)), ((), ())),
                             preferred_element_type=f32) for t in range(R * a, R * a + R)]
        zs[j, a] = [jnp.concatenate([z[p][32 * r:32 * (r + 1)] for p in range(R)],
                                    axis=0).astype(bf16) for r in range(R)]
        return [z[0][16 * t:16 * t + 8] for t in range(8)]

    def grp_fwd(ws, dst, j, a, dvec=None):
        t = [jnp.dot(tabs[r], ws[r], preferred_element_type=f32) for r in range(R)]
        x = [_split(v) for v in t]
        if dvec is not None:
            x[0] = (x[0][0] + dvec[None], x[0][1])
        put(dst, j, a, _radix4(x, -1))
        return [t[0][16 * s:16 * s + 8] for s in range(16)]

    def grp_k(j, a):
        return grp_fwd(zs.pop((j, a)), kpb, j, a,
                       sdv[:, j * L:(j + 1) * L] if a == 0 else None)

    def grp_u(j, a):
        uw = [uwb[j, a, r] for r in range(R)]
        return grp_fwd(uw, ub, j, a)

    def grp_i(j, a):
        ys = []
        for r in range(2 * R):
            y = jnp.dot(ginv[r], pb[j, a, r], preferred_element_type=f32)
            yb[j, pl.ds(a * C + r, L // 2, stride=2 * R), :] = y
            ys.append(y)
        return [ys[r][16 * s:16 * s + 8] for r in (0, R) for s in range(4)]

    def grp_mod(*names):
        for name in names:
            c0, c1 = WM[name]
            m = jnp.dot(cs, wmb[:, c0 * L:c1 * L], preferred_element_type=f32)
            for c in range(c0, c1):
                mod[c] = m[0:1, (c - c0) * L:(c - c0 + 1) * L]
        return []

    def modv(i, t0=0, t1=NT):
        return jnp.concatenate([mod[i * NT + n] for n in range(t0, t1)], axis=1)

    def job_kv(j, a, deps):
        lo = lambda x: lax.bitcast_convert_type(x << 16, f32)
        hi = lambda x: lax.bitcast_convert_type(x & jnp.uint32(0xFFFF0000), f32)
        n = C // 8
        kw, vw = kbs[a].bitcast(u32), vbs[a].bitcast(u32)
        ld = lambda ref, o: ref[pl.ds(4 * j + o, n, stride=WPT), :]
        k = {}
        for m in range(4):
            x = ld(kw, PAD + m)
            k[2 * m], k[2 * m + 1] = lo(x), hi(x)
        k[-3] = hi(ld(kw, PAD - WPT + 2))
        x = ld(kw, PAD - WPT + 3)
        k[-2], k[-1] = lo(x), hi(x)
        w = [skt[t:t + 1, j * L:(j + 1) * L] for t in range(KS)]
        w0 = [gate(jnp.broadcast_to(w[0], (n, L)), deps[e::2]) for e in (0, 1)]
        kv = {}
        for m in range(4):
            x = ld(vw, m)
            for ph, v in ((2 * m, lo(x)), (2 * m + 1, hi(x))):
                ks = k[ph] * w0[m % 2]
                for t in range(1, KS):
                    ks = ks + k[ph - t] * w[t]
                kv[ph] = (ks * v).reshape(n // 8, 8, L)
        for r in range(R):
            uwb[j, a, r] = jnp.concatenate([kv[r], kv[r + R]], axis=1).reshape(L, L).astype(bf16)

    def job_mac(j, us, outs, deps):
        ld = lambda ref, a: (ref[j, a, :, :, 0:8, :], ref[j, a, :, :, 8:16, :])
        lo, hi = us[0], us[-1]
        u = {a: ld(ub, a) for a in us}
        if len(deps) == 16:
            ur = jnp.concatenate([gate(u[lo][0][0:1], deps), u[lo][0][1:]], axis=0)
        else:
            ur = gate(u[lo][0], [deps[R * i + qi] for qi in range(R) for i in range(16)])
        u[lo] = (ur, u[lo][1])
        ms = sorted({a - n for a in outs for n in us if n <= a})
        k = {m: ld(kpb, m) for m in sorted(set(ms) | {m - 1 for m in ms if m > 0})}
        kp = {m: k[m] if m == 0 else (k[m][0] - k[m - 1][1], k[m][1] + k[m - 1][0]) for m in ms}
        for a in outs:
            yr, yi = ld(yp, a) if lo > 0 else (None, None)
            for n in us:
                if n > a:
                    continue
                (kr, ki), (ur, ui) = kp[a - n], u[n]
                tr = kr * ur - ki * ui
                ti = kr * ui + ki * ur
                yr = tr if yr is None else yr + tr
                yi = ti if yi is None else yi + ti
            if a > hi:
                yp[j, a] = jnp.concatenate([yr, yi], axis=2)
                continue
            ps = _radix4([(yr[qi], yi[qi]) for qi in range(R)], +1)
            for r in range(R):
                pr, pi = [p.reshape(8, 2, 8, L) for p in ps[r]]
                lr, li, hr, hi_ = pr[:, 0], pi[:, 0], pr[:, 1], pi[:, 1]
                if r % 2:
                    hr, hi_ = (hr - hi_) * RSQ2, (hr + hi_) * RSQ2
                if r < 2:
                    outs2 = (lr + hr, li + hi_), (lr - hr, li - hi_)
                else:
                    outs2 = (lr - hi_, li + hr), (lr + hi_, li - hr)
                for e in range(2):
                    pb[j, a, r + R * e] = jnp.concatenate(
                        outs2[e], axis=1).reshape(L, L).astype(bf16)

    def job_setup(_, deps):
        def hold(r, n):
            return gate(n, [deps[2 * r + s // 4] for s in range(8)])

        ginv.extend(_tables(True, hold))
        csf = cs[0:1].astype(f32)
        ccol.append(jnp.concatenate([jnp.broadcast_to(csf[:, t * L:(t + 1) * L], (L, L)).T
                                     for t in range(NT)], axis=0))

    def job_vmod(name, deps):
        c0, c1 = WM[name]
        n = D // VM
        for c in range(c0, c1):
            for i in range(VM):
                cc = ccol[0][i * n:(i + 1) * n]
                cc = jnp.concatenate([gate(cc[0:8], [deps[(c - c0) * VM + i]]), cc[8:]], axis=0)
                p = wmb[i * n:(i + 1) * n, c * L:(c + 1) * L].astype(f32) * cc
                mv[c, 8 * i:8 * i + 8, :] = jnp.sum(p.reshape(n // 8, 8, L), axis=0)
            mod[c] = jnp.sum(mv[c], axis=0, keepdims=True)

    grp_fn = {"z": grp_z, "k": grp_k, "u": grp_u, "i": grp_i, "mod": grp_mod}
    job_fn = {"kv": job_kv, "mac": job_mac, "vmod": job_vmod, "setup": job_setup}

    def run(groups, jobs, **kw):
        plan = _plan(groups, jobs, **kw)
        anchors, done = [], 0
        for g in groups + [None]:
            while done < len(jobs) and max(plan[done]) < len(anchors):
                job_fn[jobs[done][0]](*jobs[done][1:], [anchors[n] for n in plan[done]])
                done += 1
            if g is not None:
                anchors += grp_fn[g[0]](*g[1:])
        assert done == len(jobs)

    for waits, groups, jobs in SCHEDULE:
        wait(*waits)
        run(groups, jobs)

    n1, dep = [], None
    for r in range(0, H0, H0 // 2):
        x = qb0[r:r + H0 // 2, :].astype(f32)
        if dep is not None:
            x = jnp.concatenate([gate(x[:, 0:L], [dep]), x[:, L:]], axis=1)
        n1.append(_layernorm(x))
        dep = n1[-1][:, 0:L]
    n1 = jnp.concatenate(n1, axis=0)
    wait("mB")
    grp_mod("mB")
    sa, ca, ga = [modv(i) for i in range(3)]
    a1 = ga * (1.0 + ca)
    b1 = ga * sa

    def o_cp(i, c0, c1, r0=0, r1=TM):
        cols = pl.ds(c0, c1 - c0)
        if i is None:
            return pltpu.make_async_copy(ob0.at[:, cols], o_hbm.at[0, pl.ds(0, TM0), cols],
                                         osem.at[NB])
        base = TM0 + i * TM + r0
        if not isinstance(i, int):
            base = pl.multiple_of(base, 16)
        return pltpu.make_async_copy(ob.at[i, pl.ds(r0, r1 - r0), cols],
                                     o_hbm.at[0, pl.ds(base, r1 - r0), cols], osem.at[i])

    def prep_norm(q_ref, x1_ref, y0, r0, n, dep=None, n1=None):
        x = q_ref[r0:r0 + n, :].astype(f32)
        if dep is not None:
            x = jnp.concatenate([gate(x[:, 0:L], [dep]), x[:, L:]], axis=1)
        y = jnp.concatenate([yb[j, pl.ds(y0 + r0, n), :] for j in range(NT)], axis=1)
        x1 = x + ((_layernorm(x) if n1 is None else n1) * a1 + b1) * y
        x1_ref[r0:r0 + n, :] = x1
        return _layernorm(x1)

    n2 = [prep_norm(qb0, x1b0, 0, 0, H0, None, n1)]
    aff = []

    def prep_chain(i, r0, r1, pr):
        y0 = TM0 + i * TM
        if not isinstance(i, int):
            y0 = pl.multiple_of(y0, L)
        dep = None
        for r in range(r0, r1, pr):
            h2 = prep_norm(qb.at[i], x1b, y0, r, pr, dep) * aff[0] + aff[1]
            h2b[r:r + pr, :] = h2.astype(bf16)
            dep = h2[:, 0:L]

    OC = (0, D - L, D)
    OP = (((0, D, 0, HM),),
          ((0, D - L, HM, TM), (D - L, D, HM, TM - 64), (D - L, D, TM - 64, TM)))

    def ffn_half(i, half, gb):
        h2 = h2b[HM:, :] if half else h2b[:HM, :]
        hs = []
        for f in range(0, F, TF):
            g = jnp.dot(h2, wgb[:, f:f + TF], preferred_element_type=f32)
            u = jnp.dot(h2, wub[:, f:f + TF], preferred_element_type=f32)
            hs.append(g * u)
        hh = jnp.concatenate(hs, axis=1).astype(bf16)
        for c0, c1, r0, r1 in OP[half]:
            o = jnp.dot(hh[r0 - half * HM:r1 - half * HM], wdb[:, c0:c1],
                        preferred_element_type=f32)
            ob[i, r0:r1, c0:c1] = (x1b[r0:r1, c0:c1] + gb[:, c0:c1] * o).astype(bf16)
            o_cp(i, c0, c1, r0, r1).start()

    acc, hcache, parts = {}, {}, {}

    def grp_g(p, n, f, half=None):
        t0, t1 = KP[p], KP[p + 1]
        if (p, half) not in hcache:
            if len(n2) == 1 and half != 0:
                n2.append(prep_norm(qb0, x1b0, 0, H0, TM0 - H0))
            x = jnp.concatenate(n2, axis=0) if half is None else n2[half]
            hcache[p, half] = (x[:, t0 * L:t1 * L] * (1.0 + modv(4, t0, t1))
                               + modv(3, t0, t1)).astype(bf16)
        rows = {None: slice(0, TM0), 0: slice(0, H0), 1: slice(H0, TM0)}[half]
        cols = slice(f * 4 * L, (f + 1) * 4 * L)
        d = jnp.dot(hcache[p, half], (wgb if n == "g" else wub)[t0 * L:t1 * L, cols],
                    preferred_element_type=f32)
        ref = gub.at["gu".index(n), rows, cols]
        if p < len(KP) - 2:
            ref[...] = d if p == 0 else ref[...] + d
        elif n == "g":
            acc[f] = ref[...] + d
        else:
            hb[:, cols] = (acc.pop(f) * (ref[...] + d)).astype(bf16)
        return [d[s:s + 8, c * L:(c + 1) * L] for c in range(0, 4, 4 // (t1 - t0))
                for s in range(0, d.shape[0], 16)]

    def grp_d(n, f):
        c = slice(n * L, (n + 1) * L)
        k = slice(f * 4 * L, (f + 1) * 4 * L)
        d = jnp.dot(hb[:, k], wdb[k, c], preferred_element_type=f32)
        parts[n] = d if f == 0 else parts[n] + d
        if f == 2:
            ob0[:, c] = (x1b0[:, c] + mod[5 * NT + n] * parts.pop(n)).astype(bf16)
            if (n + 1) * L in OC:
                o_cp(None, OC[OC.index((n + 1) * L) - 1], (n + 1) * L).start()
        return [d[s:s + 8] for s in range(0, TM0, 16)]

    grp_fn.update(g=grp_g, d=grp_d)
    for waits, rows, groups, jobs in FIRST:
        wait(*waits)
        for n in parts:
            parts[n] = dpart[:, n * L:(n + 1) * L]
        run(groups, jobs, lead=LEAD, floor=(0.0, 0.5 if rows else 0.0))
        if rows:
            aff += [1.0 + modv(4), modv(3)]
            prep_chain(0, *rows, PR)
        for n in parts:
            dpart[:, n * L:(n + 1) * L] = parts[n]
    gb = modv(5)
    wait("q1c", *[f"q{i + 1}" for i in range(1, NB)])

    def ffn(i, carry):
        prep_chain(i, HM, TM, PL)
        ffn_half(i, 0, gb)
        prep_chain(jnp.minimum(i + 1, NB - 1), 0, HM, PL)
        ffn_half(i, 1, gb)
        return carry

    lax.fori_loop(0, NB, ffn, 0)

    for c0, c1 in zip(OC[:-1], OC[1:]):
        o_cp(None, c0, c1).wait()
    for i in range(NB):
        for op in OP[0] + OP[1]:
            o_cp(i, *op).wait()


@jax.jit
def pallas_adaLN_cond__ssm_conv_h3__glu_gated_bilinear__prompt_kernel(
    A_q: jax.Array,
    A_k: jax.Array,
    A_v: jax.Array,
    A_shift_k: jax.Array,
    A_ssm_k: jax.Array,
    A_ssm_D: jax.Array,
    B_x: jax.Array,
    B_w_gate: jax.Array,
    B_w_up: jax.Array,
    B_w_down: jax.Array,
    c: jax.Array,
    w_mod: jax.Array,
):
    del B_x
    tiles = lambda x: x.reshape(S // 8, 8, NT, L).transpose(0, 2, 1, 3).reshape(S * NT, L)
    any_spec = pl.BlockSpec(memory_space=pl.ANY)
    return pl.pallas_call(
        _kernel,
        in_specs=[any_spec] * 11,
        out_specs=any_spec,
        out_shape=jax.ShapeDtypeStruct((1, S, D), bf16),
        scratch_shapes=[
            pltpu.VMEM((TM0, D), bf16),
            pltpu.VMEM((NB, TM, D), bf16),
            [pltpu.VMEM((4 * PAD + C * NT, L), bf16)] * NC,
            [pltpu.VMEM((2 * PAD + C * NT, L), bf16)] * NC,
            pltpu.VMEM((NT, L, S), bf16),
            pltpu.VMEM((D, F), bf16),
            pltpu.VMEM((D, F), bf16),
            pltpu.VMEM((F, D), bf16),
            pltpu.VMEM((D, 6 * D), bf16),
            pltpu.VMEM((NT, NC, R, L, L), bf16),
            pltpu.VMEM((NT, NC, R, 16, 16, L), f32),
            pltpu.VMEM((NT, NC, R, 16, 16, L), f32),
            pltpu.VMEM((NT, NC, R, 16, 16, L), f32),
            pltpu.VMEM((NT, NC, 2 * R, L, L), bf16),
            pltpu.VMEM((NT, S + 32, L), f32),
            pltpu.VMEM((TM0, D), f32),
            pltpu.VMEM((TM, D), f32),
            pltpu.VMEM((TM, D), bf16),
            pltpu.VMEM((2, TM0, F), f32),
            pltpu.VMEM((TM0, D), f32),
            pltpu.VMEM((TM0, F), bf16),
            pltpu.VMEM((TM0, D), bf16),
            pltpu.VMEM((NB, TM, D), bf16),
            pltpu.VMEM((32, 8 * VM, L), f32),
            pltpu.VMEM((KS, D), bf16),
            pltpu.VMEM((D,), bf16),
            pltpu.VMEM((1, D), bf16),
            pltpu.SemaphoreType.DMA((len(DMA_ORDER),)),
            pltpu.SemaphoreType.DMA((NB + 1,)),
        ],
        compiler_params=pltpu.CompilerParams(
            vmem_limit_bytes=120 * 1024 * 1024,
            disable_bounds_checks=True, disable_semaphore_checks=True),
        name="adaln_h3_glu",
    )(A_q, tiles(A_k), tiles(A_v), A_shift_k.T, A_ssm_k, A_ssm_D,
      B_w_gate, B_w_up, B_w_down, c, w_mod)
```

```python
import jax
import jax.numpy as jnp
from jax import lax
import jax.experimental.pallas as pl
import jax.experimental.pallas.tpu as pltpu

S = 2048
D = 640
F = 1536
KS = 4
L = 128
NT = D // L
R = 4
C = R * L
NC = S // C
EPS = 1e-5
RSQ2 = 0.7071067811865476

WPT = 4 * NT
PAD = 32

TM0 = 512
H0 = 352
TM = 384
NB = (S - TM0) // TM
HM = 192
PL = 16
PR = 24
KP = (0, 1, 2, 3, 4, 5)
WM = {"mA": (0, 12), "c0": (20, 21), "mB": (12, 16), "s1": (16, 17), "c1": (21, 22),
      "s2": (17, 19), "c2": (22, 24), "s4": (19, 20), "c4": (24, 25), "mG": (25, 30)}
VM = 5
RATE = 1.05
LEAD = 24
FREE = {"i": 56, "z": 56, "k": 47, "u": 46}
FREE_FFN = {"i": 4, "u": 26, "d": 48, "D": 42, "g": 50}

f32 = jnp.float32
bf16 = jnp.bfloat16
u32 = jnp.uint32


def _cos_turns(t):
    x = jnp.abs(t - jnp.floor(t) - 0.5) - 0.25
    x2 = x * x
    return x * (6.283164024 + x2 * (-41.33713150 + x2 * (81.34038544 + x2 * -70.98993683)))


def _tables(inverse, hold=None):
    shape = (L // 2, L) if inverse else (2 * L, L)
    rho = lax.broadcasted_iota(jnp.int32, shape, 1 if inverse else 0)
    j = lax.broadcasted_iota(jnp.int32, shape, 0 if inverse else 1)
    if inverse:
        g, rad = 8 * (rho >> 4) + (rho & 7), 2 * R
    else:
        g, rad, j = 8 * (rho >> 5) + (rho & 7) + 64 * ((rho >> 4) & 1), R, _perm(j)
    a = (4 * g + 1).astype(f32) * (1.0 / (4 * C))
    off = ((rho >> 3) & 1).astype(f32) * 0.25
    ns = [(rad * j + r).astype(f32) for r in range(rad)]
    if hold is not None:
        ns = [hold(r, n) for r, n in enumerate(ns)]
    ts = [_cos_turns(a * n + off) for n in ns]
    return [(t * (1.0 / C) if inverse else t).astype(bf16) for t in ts]


def _perm(c):
    return 16 * (c >> 4) + 2 * (c & 7) + ((c >> 3) & 1)


def _layernorm(x):
    m = jnp.mean(x, axis=-1, keepdims=True)
    xc = x - m
    v = jnp.mean(xc * xc, axis=-1, keepdims=True)
    return xc * lax.rsqrt(v + EPS)


def _split(t):
    t = t.reshape(16, 16, L)
    return t[:, :8, :], t[:, 8:, :]


def _radix4(x, sgn):
    (ar, ai), (br, bi), (cr, ci), (dr, di) = x
    s0r, s0i, d0r, d0i = ar + cr, ai + ci, ar - cr, ai - ci
    s1r, s1i, d1r, d1i = br + dr, bi + di, br - dr, bi - di
    o0 = (s0r + s1r, s0i + s1i)
    o2 = (s0r - s1r, s0i - s1i)
    pl_ = (d0r - d1i, d0i + d1r)
    mi_ = (d0r + d1i, d0i - d1r)
    return [o0, pl_, o2, mi_] if sgn > 0 else [o0, mi_, o2, pl_]


def _strassen_lhs(a11, a12, a21, a22):
    return [x.astype(bf16)
            for x in (a11 + a22, a21 + a22, a11, a22, a11 + a12, a21 - a11, a12 - a22)]


def _strassen_out(p):
    c11, c12 = p[0] + p[3] - p[4] + p[6], p[2] + p[4]
    c21, c22 = p[1] + p[3], p[0] - p[1] + p[2] + p[5]
    return jnp.concatenate([c11, c21], axis=0), jnp.concatenate([c12, c22], axis=0)


SQ = {"g": (2 * L, F // 2), "u": (2 * L, F // 2), "d": (F // 2, 2 * L)}

T = range(NT)
_z = lambda j: [("z", j, a) for a in range(NC)]
_k = lambda j, al: [("k", j, a) for a in al]
_u = lambda a: [("u", j, a) for j in T]
_iv = lambda jl, al: [("i", j, a) for j in jl for a in al]
_kv = lambda a: [("kv", j, a) for j in T]
_m = lambda jl, us, outs: [("mac", j, us, outs) for j in jl]

A2 = (0, 1)
SCHEDULE = [
    (["ssm0"], _z(0) + _k(0, range(NC)), [("setup", None)]),
    (["ssm1"], _z(1) + _k(1, range(NC)), []),
    (["ssm2"], _z(2) + _k(2, [0, 1]), []),
    (["k0", "v0"], _k(2, [2, 3]) + _u(0), _kv(0) + _m([0], (0,), (0,))),
    (["ssm3"], _iv([0], [0]) + _z(3) + _k(3, [0, 1]), _m([1, 2], (0,), (0,))),
    (["k1", "v1"], _k(3, [2, 3]) + _u(1), _kv(1) + _m([3], (0,), (0,))),
    (["ssm4"], _iv([1, 2, 3], [0]) + _z(4) + _k(4, range(NC)), _m([0, 1, 2, 3], A2, (1,))),
    (["q0"], _iv([0, 1, 2, 3], [1]) + _iv([4], A2), _m([4], A2, A2)),
    (["mA", "c0"], [("mod", "mA", "c0")], []),
]
_g = lambda p: [("g", p, n, f) for f in range(3) for n in "gu"]
_v = lambda *names: [("vmod", n) for n in names]
_e = [("d", n, f) for n in T for f in (0, 1)]
FIRST = [
    (["wg0", "qh"], None, [("g", 0, "g", f, h) for h in (0, 1) for f in range(3)], []),
    (["wu0", "s1", "c1"], None, [("g", 0, "u", f) for f in range(3)],
     _v("s1", "c1") + _m([0], A2, (2, 3))),
    (["wg1", "wu1"], None, _g(1)[:-1], _m([1, 2], A2, (2, 3))),
    (["wg2", "wu2", "s2", "c2"], None, _g(1)[-1:] + _g(2),
     _v("s2", "c2") + _m([3, 4], A2, (2, 3))),
    (["wg3", "wu3", "wg4", "wu4", "s4", "c4", "q1"], (0, HM), _g(3) + _g(4),
     _v("s4", "c4") + [("wsum", "g"), ("wsum", "u")]),
    (["wd", "k2", "v2"], None, _e[:2] + _u(2) + _e[2:6],
     _kv(2) + _m([0, 1, 2, 3], (2,), (2, 3))),
    (["mG", "k3", "v3"], None,
     _e[6:] + _u(3) + [(x, n, 2) for n in T for x in "di"] + _iv(T, [3]),
     _m([4], (2,), (2, 3)) + _kv(3) + _v("mG") + [("wsum", "d")] + _m(T, (3,), (3,))),
]

DMA_ORDER = (["sk", "sd", "c", "ssm0", "ssm1", "ssm2", "k0", "v0", "ssm3", "k1", "v1", "ssm4",
              "q0", "c0", "mA", "mB", "wg0", "qh", "wu0", "s1", "c1", "wg1", "wu1", "s2", "c2",
              "wg2", "wu2", "s4", "c4", "wg3", "wu3", "wg4", "wu4", "q1", "wd", "k2", "v2", "mG", "k3", "v3",
              "q1c"] + [f"q{i + 1}" for i in range(1, NB)])


def _costs(job):
    if job[0] == "kv":
        return [48, 42] * (C // 64)
    if job[0] == "wsum":
        return [54] * (SQ[job[1]][0] * SQ[job[1]][1] // (16 * 2 * L))
    if job[0] == "setup":
        return [100] * (4 * R)
    if job[0] == "vmod":
        return [3 * D // VM // 8] * (VM * (WM[job[1]][1] - WM[job[1]][0]))
    us, outs = job[2], job[3]
    pairs = [(a, n) for a in outs for n in us if n <= a]
    mac = (2 * len({a - n for a, n in pairs if a > n}) + 8 * len(pairs)
           - (2 * len(outs) if us[0] == 0 else 0))
    fin = sum(a <= us[-1] for a in outs)
    if mac < 12 and outs[-1] <= us[-1] < NC - 1:
        return [1 + R * mac + 16 * fin, 1 + R * mac + 48 * fin] * 8
    return ([1 + mac] * 3 + [1 + mac + 16 * fin] + [1 + mac] * 3 + [1 + mac + 48 * fin]) * 8


def _plan(groups, jobs, lead=0, floor=(1.0, 0.8)):
    free = FREE_FFN if lead else FREE
    nstep = {"i": 8, "z": 8, "k": 16, "u": 16, "mod": 0, "d": TM0 // 16}
    steps = lambda g: (KP[g[1] + 1] - KP[g[1]]) * TM0 // 16 if g[0] == "g" else nstep[g[0]]
    slots = [free["D" if g[0] == "d" and g[2] == 2 else g[0]]
             for g in groups for _ in range(steps(g))]
    lo, hi = [], []
    for job in jobs:
        begin, limit, first = 0, len(slots), 0
        for g in groups:
            kind = (g[0], job[0])
            if (kind == ("u", "kv") and g[1:] == job[1:]
                    or kind == ("i", "mac") and g[1] == job[1] and g[2] in job[3]
                    and g[2] <= job[2][-1] or kind == ("d", "vmod") and g[2] == 2):
                limit = min(limit, first - lead)
            if kind == ("g", "vmod") and job[1][1] == str(g[1]):
                limit = min(limit, first - 11)
            first += steps(g)
            if kind == ("u", "mac") and g[1] == job[1] and g[2] in job[2]:
                begin = first
        lo.append(begin)
        hi.append(limit)
    plan, credit, n = [], (slots or [0])[0], 0
    for k, job in enumerate(jobs):
        if n < lo[k]:
            n, credit = lo[k], min(credit, 0) + slots[lo[k]]
        work = [sum(_costs(j)) for j in jobs]
        if lead:
            rate = max(RATE * sum(work[k:m + 1]) / max(sum(slots[n:hi[m]]), 1)
                       for m in range(k, len(jobs)))
        else:
            rate = RATE * sum(work[k:]) / sum(slots[n:])
        rate = max(rate, floor[0] if job[0] == "kv" else floor[1])
        idx = []
        for c in _costs(job):
            while credit <= 0 and n + 1 < hi[k]:
                n += 1
                credit += slots[n] * rate
            credit -= c
            idx.append(n)
        plan.append(idx)
    return plan


def _kernel(q_hbm, k_hbm, v_hbm, sk_hbm, ssm_hbm, sd_hbm, wg_hbm, wu_hbm, wd_hbm,
            c_hbm, wm_hbm, o_hbm,
            qb0, qb, kbs, vbs, ssmb, wgb, wub, wdb, sgb, sub, sdn, wmb, uwb, ub, kpb, yp, pb, yb,
            x1b0, x1b, h2b, gub, dpart, hb, ob0, ob, mv, skb, sdb, cb_, sem, osem):
    cps = {"sk": (sk_hbm, skb), "sd": (sd_hbm, sdb), "c": (c_hbm, cb_), "wd": (wd_hbm, wdb)}
    for j in range(NT):
        cps[f"ssm{j}"] = (ssm_hbm.at[pl.ds(j * L, L), :], ssmb.at[j])
    for a in range(NC):
        n, h = C * NT, 2 * PAD
        if a == 0:
            cps["k0"] = (k_hbm.at[pl.ds(0, n), :], kbs[0].at[pl.ds(h, n), :])
        else:
            e = 48
            cps[f"k{a}"] = (k_hbm.at[pl.ds(a * n - e, n + e), :],
                            kbs[a].at[pl.ds(h - e, n + e), :])
        cps[f"v{a}"] = (v_hbm.at[pl.ds(a * n, n), :], vbs[a].at[pl.ds(0, n), :])
    for n, (c0, c1) in WM.items():
        cols = pl.ds(c0 * L, (c1 - c0) * L)
        cps[n] = (wm_hbm.at[:, cols], wmb.at[:, cols])
    cps["q0"] = (q_hbm.at[0, pl.ds(0, H0), :], qb0.at[pl.ds(0, H0), :])
    cps["qh"] = (q_hbm.at[0, pl.ds(H0, TM0 - H0), :], qb0.at[pl.ds(H0, TM0 - H0), :])
    cps["q1"] = (q_hbm.at[0, pl.ds(TM0, HM), :], qb.at[0, pl.ds(0, HM), :])
    cps["q1c"] = (q_hbm.at[0, pl.ds(TM0 + HM, TM - HM), :], qb.at[0, pl.ds(HM, TM - HM), :])
    for i in range(1, NB):
        cps[f"q{i + 1}"] = (q_hbm.at[0, pl.ds(TM0 + i * TM, TM), :], qb.at[i])
    for p in range(len(KP) - 1):
        rows = pl.ds(KP[p] * L, (KP[p + 1] - KP[p]) * L)
        cps[f"wg{p}"] = (wg_hbm.at[rows, :], wgb.at[rows, :])
        cps[f"wu{p}"] = (wu_hbm.at[rows, :], wub.at[rows, :])
    assert sorted(cps) == sorted(DMA_ORDER)

    def cp(name):
        src, dst = cps[name]
        return pltpu.make_async_copy(src, dst, sem.at[DMA_ORDER.index(name)])

    def wait(*names):
        for n in names:
            cp(n).wait()

    kbs[0][0:2 * PAD, :] = jnp.zeros((2 * PAD, L), bf16)
    for n in DMA_ORDER:
        cp(n).start()

    tabs, ginv, ccol = _tables(False), [], []
    for ref in (ub, kpb, yp):
        ref[0, 0, 0, 0, pl.ds(0, 8, stride=2), :] = jnp.zeros((8, L), f32)
    mv[0, pl.ds(0, 8, stride=2), :] = jnp.zeros((8, L), f32)
    ri = lax.broadcasted_iota(jnp.int32, (L, L), 0)
    ci = lax.broadcasted_iota(jnp.int32, (L, L), 1)
    sel = jnp.where(ci == R * _perm(ri & 31) + (ri >> 5), 1.0, 0.0).astype(bf16)

    wait("sk", "sd", "c")
    skt = skb[...].astype(f32)
    sdv = sdb[...].astype(f32).reshape(1, D)
    cv = cb_[...].astype(f32)
    sig = jax.nn.sigmoid(cv)
    cs = jnp.broadcast_to((cv * sig).astype(bf16), (16, D))
    one = sig[:, 0:L]

    def gate(x, deps):
        dep = jnp.concatenate(deps, axis=0).reshape(x.shape)
        return jnp.where(jnp.broadcast_to(one, x.shape) > 2.0, dep, x)

    def put(dst, j, a, xs):
        for qi in range(R):
            dst[j, a, qi] = jnp.concatenate(xs[qi], axis=1)

    zs = {}
    mod = {}

    def grp_z(j, a):
        z = [lax.dot_general(sel, ssmb[j, :, t * L:(t + 1) * L], (((1,), (1,)), ((), ())),
                             preferred_element_type=f32) for t in range(R * a, R * a + R)]
        zs[j, a] = [jnp.concatenate([z[p][32 * r:32 * (r + 1)] for p in range(R)],
                                    axis=0).astype(bf16) for r in range(R)]
        return [z[0][16 * t:16 * t + 8] for t in range(8)]

    def grp_fwd(ws, dst, j, a, dvec=None):
        t = [jnp.dot(tabs[r], ws[r], preferred_element_type=f32) for r in range(R)]
        x = [_split(v) for v in t]
        if dvec is not None:
            x[0] = (x[0][0] + dvec[None], x[0][1])
        put(dst, j, a, _radix4(x, -1))
        return [t[0][16 * s:16 * s + 8] for s in range(16)]

    def grp_k(j, a):
        return grp_fwd(zs.pop((j, a)), kpb, j, a,
                       sdv[:, j * L:(j + 1) * L] if a == 0 else None)

    def grp_u(j, a):
        uw = [uwb[j, a, r] for r in range(R)]
        return grp_fwd(uw, ub, j, a)

    def grp_i(j, a):
        ys = []
        for r in range(2 * R):
            y = jnp.dot(ginv[r], pb[j, a, r], preferred_element_type=f32)
            yb[j, pl.ds(a * C + r, L // 2, stride=2 * R), :] = y
            ys.append(y)
        return [ys[r][16 * s:16 * s + 8] for r in (0, R) for s in range(4)]

    def grp_mod(*names):
        for name in names:
            c0, c1 = WM[name]
            m = jnp.dot(cs, wmb[:, c0 * L:c1 * L], preferred_element_type=f32)
            for c in range(c0, c1):
                mod[c] = m[0:1, (c - c0) * L:(c - c0 + 1) * L]
        return []

    def modv(i, t0=0, t1=NT):
        return jnp.concatenate([mod[i * NT + n] for n in range(t0, t1)], axis=1)

    def job_kv(j, a, deps):
        lo = lambda x: lax.bitcast_convert_type(x << 16, f32)
        hi = lambda x: lax.bitcast_convert_type(x & jnp.uint32(0xFFFF0000), f32)
        n = C // 8
        kw, vw = kbs[a].bitcast(u32), vbs[a].bitcast(u32)
        ld = lambda ref, o: ref[pl.ds(4 * j + o, n, stride=WPT), :]
        k = {}
        for m in range(4):
            x = ld(kw, PAD + m)
            k[2 * m], k[2 * m + 1] = lo(x), hi(x)
        k[-3] = hi(ld(kw, PAD - WPT + 2))
        x = ld(kw, PAD - WPT + 3)
        k[-2], k[-1] = lo(x), hi(x)
        w = [skt[t:t + 1, j * L:(j + 1) * L] for t in range(KS)]
        w0 = [gate(jnp.broadcast_to(w[0], (n, L)), deps[e::2]) for e in (0, 1)]
        kv = {}
        for m in range(4):
            x = ld(vw, m)
            for ph, v in ((2 * m, lo(x)), (2 * m + 1, hi(x))):
                ks = k[ph] * w0[m % 2]
                for t in range(1, KS):
                    ks = ks + k[ph - t] * w[t]
                kv[ph] = (ks * v).reshape(n // 8, 8, L)
        for r in range(R):
            uwb[j, a, r] = jnp.concatenate([kv[r], kv[r + R]], axis=1).reshape(L, L).astype(bf16)

    def job_mac(j, us, outs, deps):
        ld = lambda ref, a: (ref[j, a, :, :, 0:8, :], ref[j, a, :, :, 8:16, :])
        lo, hi = us[0], us[-1]
        u = {a: ld(ub, a) for a in us}
        if len(deps) == 16:
            ur = jnp.concatenate([gate(u[lo][0][0:1], deps), u[lo][0][1:]], axis=0)
        else:
            ur = gate(u[lo][0], [deps[R * i + qi] for qi in range(R) for i in range(16)])
        u[lo] = (ur, u[lo][1])
        ms = sorted({a - n for a in outs for n in us if n <= a})
        k = {m: ld(kpb, m) for m in sorted(set(ms) | {m - 1 for m in ms if m > 0})}
        kp = {m: k[m] if m == 0 else (k[m][0] - k[m - 1][1], k[m][1] + k[m - 1][0]) for m in ms}
        for a in outs:
            yr, yi = ld(yp, a) if lo > 0 else (None, None)
            for n in us:
                if n > a:
                    continue
                (kr, ki), (ur, ui) = kp[a - n], u[n]
                tr = kr * ur - ki * ui
                ti = kr * ui + ki * ur
                yr = tr if yr is None else yr + tr
                yi = ti if yi is None else yi + ti
            if a > hi:
                yp[j, a] = jnp.concatenate([yr, yi], axis=2)
                continue
            ps = _radix4([(yr[qi], yi[qi]) for qi in range(R)], +1)
            for r in range(R):
                pr, pi = [p.reshape(8, 2, 8, L) for p in ps[r]]
                lr, li, hr, hi_ = pr[:, 0], pi[:, 0], pr[:, 1], pi[:, 1]
                if r % 2:
                    hr, hi_ = (hr - hi_) * RSQ2, (hr + hi_) * RSQ2
                if r < 2:
                    outs2 = (lr + hr, li + hi_), (lr - hr, li - hi_)
                else:
                    outs2 = (lr - hi_, li + hr), (lr + hi_, li - hr)
                for e in range(2):
                    pb[j, a, r + R * e] = jnp.concatenate(
                        outs2[e], axis=1).reshape(L, L).astype(bf16)

    def job_setup(_, deps):
        def hold(r, n):
            return gate(n, [deps[2 * r + s // 4] for s in range(8)])

        ginv.extend(_tables(True, hold))
        csf = cs[0:1].astype(f32)
        ccol.append(jnp.concatenate([jnp.broadcast_to(csf[:, t * L:(t + 1) * L], (L, L)).T
                                     for t in range(NT)], axis=0))

    def job_vmod(name, deps):
        c0, c1 = WM[name]
        n = D // VM
        for c in range(c0, c1):
            for i in range(VM):
                cc = ccol[0][i * n:(i + 1) * n]
                cc = jnp.concatenate([gate(cc[0:8], [deps[(c - c0) * VM + i]]), cc[8:]], axis=0)
                p = wmb[i * n:(i + 1) * n, c * L:(c + 1) * L].astype(f32) * cc
                mv[c, 8 * i:8 * i + 8, :] = jnp.sum(p.reshape(n // 8, 8, L), axis=0)
            mod[c] = jnp.sum(mv[c], axis=0, keepdims=True)

    wts = {"g": (wgb, sgb), "u": (wub, sub), "d": (wdb, sdn)}

    def job_wsum(n, deps):
        (w, s), (kh, nh) = wts[n], SQ[n]

        def quad(r, c, hold):
            x = w[r * kh:(r + 1) * kh, c * nh:(c + 1) * nh].astype(f32)
            if hold:
                x = jnp.concatenate(
                    [gate(x[:, t * L:(t + 1) * L],
                          [deps[t // 2 * (kh // 16) + g // 2] for g in range(kh // 8)])
                     for t in range(nh // L)], axis=1)
            return x

        b11, b12, b21, b22 = quad(0, 0, 1), quad(0, 1, 0), quad(1, 0, 0), quad(1, 1, 1)
        for i, v in enumerate((b11 + b22, b12 - b22, b21 - b11, b11 + b12, b21 + b22)):
            s[i] = v.astype(bf16)

    def strassen(a, n, c):
        (w, s), (kh, nh) = wts[n], SQ[n]
        cs = slice(c, c + L)
        b = [s[0, :, cs], w[0:kh, cs], s[1, :, cs], s[2, :, cs],
             w[kh:2 * kh, nh + c:nh + c + L], s[3, :, cs], s[4, :, cs]]
        return _strassen_out([jnp.dot(x, y, preferred_element_type=f32) for x, y in zip(a, b)])

    grp_fn = {"z": grp_z, "k": grp_k, "u": grp_u, "i": grp_i, "mod": grp_mod}
    job_fn = {"kv": job_kv, "mac": job_mac, "vmod": job_vmod, "setup": job_setup,
              "wsum": job_wsum}

    def run(groups, jobs, **kw):
        plan = _plan(groups, jobs, **kw)
        anchors, done = [], 0
        for g in groups + [None]:
            while done < len(jobs) and max(plan[done]) < len(anchors):
                job_fn[jobs[done][0]](*jobs[done][1:], [anchors[n] for n in plan[done]])
                done += 1
            if g is not None:
                anchors += grp_fn[g[0]](*g[1:])
        assert done == len(jobs)

    for waits, groups, jobs in SCHEDULE:
        wait(*waits)
        run(groups, jobs)

    n1, dep = [], None
    for r in range(0, H0, H0 // 2):
        x = qb0[r:r + H0 // 2, :].astype(f32)
        if dep is not None:
            x = jnp.concatenate([gate(x[:, 0:L], [dep]), x[:, L:]], axis=1)
        n1.append(_layernorm(x))
        dep = n1[-1][:, 0:L]
    n1 = jnp.concatenate(n1, axis=0)
    wait("mB")
    grp_mod("mB")
    sa, ca, ga = [modv(i) for i in range(3)]
    a1 = ga * (1.0 + ca)
    b1 = ga * sa

    def o_cp(i, c0, c1, r0=0, r1=TM):
        cols = pl.ds(c0, c1 - c0)
        if i is None:
            return pltpu.make_async_copy(ob0.at[:, cols], o_hbm.at[0, pl.ds(0, TM0), cols],
                                         osem.at[NB])
        base = TM0 + i * TM + r0
        if not isinstance(i, int):
            base = pl.multiple_of(base, 16)
        return pltpu.make_async_copy(ob.at[i, pl.ds(r0, r1 - r0), cols],
                                     o_hbm.at[0, pl.ds(base, r1 - r0), cols], osem.at[i])

    def prep_norm(q_ref, x1_ref, y0, r0, n, dep=None, n1=None):
        x = q_ref[r0:r0 + n, :].astype(f32)
        if dep is not None:
            x = jnp.concatenate([gate(x[:, 0:L], [dep]), x[:, L:]], axis=1)
        y = jnp.concatenate([yb[j, pl.ds(y0 + r0, n), :] for j in range(NT)], axis=1)
        x1 = x + ((_layernorm(x) if n1 is None else n1) * a1 + b1) * y
        x1_ref[r0:r0 + n, :] = x1
        return _layernorm(x1)

    n2 = [prep_norm(qb0, x1b0, 0, 0, H0, None, n1)]
    aff = []

    def prep_chain(i, r0, r1, pr):
        y0 = TM0 + i * TM
        if not isinstance(i, int):
            y0 = pl.multiple_of(y0, L)
        dep = None
        for r in range(r0, r1, pr):
            h2 = prep_norm(qb.at[i], x1b, y0, r, pr, dep) * aff[0] + aff[1]
            h2b[r:r + pr, :] = h2
            dep = h2[:, 0:L]

    OC = (0, D - L, D)
    OP = (((0, D - L, 0, HM), (D - L, D, 0, HM)),
          ((0, D - L, HM, TM), (D - L, D, HM, TM - 64), (D - L, D, TM - 64, TM)))

    def ffn_half(i, half, gb):
        r0, r1 = (HM, TM) if half else (0, HM)
        m, k = (r1 - r0) // 2, 2 * L
        x = h2b[r0:r1, :]
        a = _strassen_lhs(x[:m, :k], x[:m, k:2 * k], x[m:, :k], x[m:, k:2 * k])
        xe = x[:, 2 * k:].astype(bf16)
        hs = ([], [])
        for c in range(0, F // 2, L):
            gu = []
            for n in "gu":
                p = strassen(a, n, c)
                gu.append([p[e] + jnp.dot(xe, wts[n][0][2 * k:, o:o + L],
                                          preferred_element_type=f32)
                           for e, o in enumerate((c, F // 2 + c))])
            for e in range(2):
                hs[e].append(gu[0][e] * gu[1][e])
        hl, hr = [jnp.concatenate(h, axis=1) for h in hs]
        a = _strassen_lhs(hl[:m], hr[:m], hl[m:], hr[m:])
        hh = jnp.concatenate([hl, hr], axis=1).astype(bf16)
        for c0, c1, s0, s1 in OP[half]:
            if c0 == 0:
                p = [strassen(a, "d", c) for c in range(0, k, L)]
                o = jnp.concatenate([q[0] for q in p] + [q[1] for q in p], axis=1)
            else:
                o = jnp.dot(hh[s0 - r0:s1 - r0], wdb[:, c0:c1], preferred_element_type=f32)
            ob[i, s0:s1, c0:c1] = (x1b[s0:s1, c0:c1] + gb[:, c0:c1] * o).astype(bf16)
            o_cp(i, c0, c1, s0, s1).start()

    acc, hcache, parts = {}, {}, {}

    def grp_g(p, n, f, half=None):
        t0, t1 = KP[p], KP[p + 1]
        if (p, half) not in hcache:
            if len(n2) == 1 and half != 0:
                n2.append(prep_norm(qb0, x1b0, 0, H0, TM0 - H0))
            x = jnp.concatenate(n2, axis=0) if half is None else n2[half]
            hcache[p, half] = (x[:, t0 * L:t1 * L] * (1.0 + modv(4, t0, t1))
                               + modv(3, t0, t1)).astype(bf16)
        rows = {None: slice(0, TM0), 0: slice(0, H0), 1: slice(H0, TM0)}[half]
        cols = slice(f * 4 * L, (f + 1) * 4 * L)
        d = jnp.dot(hcache[p, half], (wgb if n == "g" else wub)[t0 * L:t1 * L, cols],
                    preferred_element_type=f32)
        ref = gub.at["gu".index(n), rows, cols]
        if p < len(KP) - 2:
            ref[...] = d if p == 0 else ref[...] + d
        elif n == "g":
            acc[f] = ref[...] + d
        else:
            hb[:, cols] = (acc.pop(f) * (ref[...] + d)).astype(bf16)
        return [d[s:s + 8, c * L:(c + 1) * L] for c in range(0, 4, 4 // (t1 - t0))
                for s in range(0, d.shape[0], 16)]

    def grp_d(n, f):
        c = slice(n * L, (n + 1) * L)
        k = slice(f * 4 * L, (f + 1) * 4 * L)
        d = jnp.dot(hb[:, k], wdb[k, c], preferred_element_type=f32)
        parts[n] = d if f == 0 else parts[n] + d
        if f == 2:
            ob0[:, c] = (x1b0[:, c] + mod[5 * NT + n] * parts.pop(n)).astype(bf16)
            if (n + 1) * L in OC:
                o_cp(None, OC[OC.index((n + 1) * L) - 1], (n + 1) * L).start()
        return [d[s:s + 8] for s in range(0, TM0, 16)]

    grp_fn.update(g=grp_g, d=grp_d)
    for waits, rows, groups, jobs in FIRST:
        wait(*waits)
        for n in parts:
            parts[n] = dpart[:, n * L:(n + 1) * L]
        run(groups, jobs, lead=LEAD, floor=(0.0, 0.0))
        if rows:
            aff += [1.0 + modv(4), modv(3)]
            prep_chain(0, *rows, PR)
        for n in parts:
            dpart[:, n * L:(n + 1) * L] = parts[n]
    gb = modv(5)
    wait("q1c", *[f"q{i + 1}" for i in range(1, NB)])

    def ffn(i, carry):
        prep_chain(i, HM, TM, PL)
        ffn_half(i, 0, gb)
        prep_chain(jnp.minimum(i + 1, NB - 1), 0, HM, PL)
        ffn_half(i, 1, gb)
        return carry

    lax.fori_loop(0, NB, ffn, 0)

    for c0, c1 in zip(OC[:-1], OC[1:]):
        o_cp(None, c0, c1).wait()
    for i in range(NB):
        for op in OP[0] + OP[1]:
            o_cp(i, *op).wait()


@jax.jit
def pallas_adaLN_cond__ssm_conv_h3__glu_gated_bilinear__prompt_kernel(
    A_q: jax.Array,
    A_k: jax.Array,
    A_v: jax.Array,
    A_shift_k: jax.Array,
    A_ssm_k: jax.Array,
    A_ssm_D: jax.Array,
    B_x: jax.Array,
    B_w_gate: jax.Array,
    B_w_up: jax.Array,
    B_w_down: jax.Array,
    c: jax.Array,
    w_mod: jax.Array,
):
    del B_x
    tiles = lambda x: x.reshape(S // 8, 8, NT, L).transpose(0, 2, 1, 3).reshape(S * NT, L)
    any_spec = pl.BlockSpec(memory_space=pl.ANY)
    return pl.pallas_call(
        _kernel,
        in_specs=[any_spec] * 11,
        out_specs=any_spec,
        out_shape=jax.ShapeDtypeStruct((1, S, D), bf16),
        scratch_shapes=[
            pltpu.VMEM((TM0, D), bf16),
            pltpu.VMEM((NB, TM, D), bf16),
            [pltpu.VMEM((4 * PAD + C * NT, L), bf16)] * NC,
            [pltpu.VMEM((2 * PAD + C * NT, L), bf16)] * NC,
            pltpu.VMEM((NT, L, S), bf16),
            pltpu.VMEM((D, F), bf16),
            pltpu.VMEM((D, F), bf16),
            pltpu.VMEM((F, D), bf16),
            pltpu.VMEM((5,) + SQ["g"], bf16),
            pltpu.VMEM((5,) + SQ["u"], bf16),
            pltpu.VMEM((5,) + SQ["d"], bf16),
            pltpu.VMEM((D, 6 * D), bf16),
            pltpu.VMEM((NT, NC, R, L, L), bf16),
            pltpu.VMEM((NT, NC, R, 16, 16, L), f32),
            pltpu.VMEM((NT, NC, R, 16, 16, L), f32),
            pltpu.VMEM((NT, NC, R, 16, 16, L), f32),
            pltpu.VMEM((NT, NC, 2 * R, L, L), bf16),
            pltpu.VMEM((NT, S + 32, L), f32),
            pltpu.VMEM((TM0, D), f32),
            pltpu.VMEM((TM, D), f32),
            pltpu.VMEM((TM, D), f32),
            pltpu.VMEM((2, TM0, F), f32),
            pltpu.VMEM((TM0, D), f32),
            pltpu.VMEM((TM0, F), bf16),
            pltpu.VMEM((TM0, D), bf16),
            pltpu.VMEM((NB, TM, D), bf16),
            pltpu.VMEM((32, 8 * VM, L), f32),
            pltpu.VMEM((KS, D), bf16),
            pltpu.VMEM((D,), bf16),
            pltpu.VMEM((1, D), bf16),
            pltpu.SemaphoreType.DMA((len(DMA_ORDER),)),
            pltpu.SemaphoreType.DMA((NB + 1,)),
        ],
        compiler_params=pltpu.CompilerParams(
            vmem_limit_bytes=120 * 1024 * 1024,
            disable_bounds_checks=True, disable_semaphore_checks=True),
        name="adaln_h3_glu",
    )(A_q, tiles(A_k), tiles(A_v), A_shift_k.T, A_ssm_k, A_ssm_D,
      B_w_gate, B_w_up, B_w_down, c, w_mod)
```

```python
import jax
import jax.numpy as jnp
from jax import lax
import jax.experimental.pallas as pl
import jax.experimental.pallas.tpu as pltpu

S = 2048
D = 640
F = 1536
KS = 4
L = 128
NT = D // L
R = 4
C = R * L
NC = S // C
EPS = 1e-5
RSQ2 = 0.7071067811865476

WPT = 4 * NT
PAD = 32

TM0 = 512
H0 = 352
TM = 512
NB = (S - TM0) // TM
HM = 256
PL = 16
PR = 24
KP = (0, 1, 2, 3, 4, 5)
WM = {"mA": (0, 12), "c0": (20, 21), "mB": (12, 16), "s1": (16, 17), "c1": (21, 22),
      "s2": (17, 19), "c2": (22, 24), "s4": (19, 20), "c4": (24, 25), "mG": (25, 30)}
VM = 5
RATE = 1.05
LEAD = 24
FREE = {"i": 56, "z": 56, "k": 47, "u": 46}
FREE_FFN = {"i": 4, "u": 26, "d": 48, "D": 42, "g": 50}

f32 = jnp.float32
bf16 = jnp.bfloat16
u32 = jnp.uint32


def _cos_turns(t):
    x = jnp.abs(t - jnp.floor(t) - 0.5) - 0.25
    x2 = x * x
    return x * (6.283164024 + x2 * (-41.33713150 + x2 * (81.34038544 + x2 * -70.98993683)))


def _tables(inverse, hold=None):
    shape = (L // 2, L) if inverse else (2 * L, L)
    rho = lax.broadcasted_iota(jnp.int32, shape, 1 if inverse else 0)
    j = lax.broadcasted_iota(jnp.int32, shape, 0 if inverse else 1)
    if inverse:
        g, rad = 8 * (rho >> 4) + (rho & 7), 2 * R
    else:
        g, rad, j = 8 * (rho >> 5) + (rho & 7) + 64 * ((rho >> 4) & 1), R, _perm(j)
    a = (4 * g + 1).astype(f32) * (1.0 / (4 * C))
    off = ((rho >> 3) & 1).astype(f32) * 0.25
    ns = [(rad * j + r).astype(f32) for r in range(rad)]
    if hold is not None:
        ns = [hold(r, n) for r, n in enumerate(ns)]
    ts = [_cos_turns(a * n + off) for n in ns]
    return [(t * (1.0 / C) if inverse else t).astype(bf16) for t in ts]


def _perm(c):
    return 16 * (c >> 4) + 2 * (c & 7) + ((c >> 3) & 1)


def _layernorm(x):
    m = jnp.mean(x, axis=-1, keepdims=True)
    xc = x - m
    v = jnp.mean(xc * xc, axis=-1, keepdims=True)
    return xc * lax.rsqrt(v + EPS)


def _split(t):
    t = t.reshape(16, 16, L)
    return t[:, :8, :], t[:, 8:, :]


def _radix4(x, sgn):
    (ar, ai), (br, bi), (cr, ci), (dr, di) = x
    s0r, s0i, d0r, d0i = ar + cr, ai + ci, ar - cr, ai - ci
    s1r, s1i, d1r, d1i = br + dr, bi + di, br - dr, bi - di
    o0 = (s0r + s1r, s0i + s1i)
    o2 = (s0r - s1r, s0i - s1i)
    pl_ = (d0r - d1i, d0i + d1r)
    mi_ = (d0r + d1i, d0i - d1r)
    return [o0, pl_, o2, mi_] if sgn > 0 else [o0, mi_, o2, pl_]


def _strassen_lhs(a11, a12, a21, a22):
    return [x.astype(bf16)
            for x in (a11 + a22, a21 + a22, a11, a22, a11 + a12, a21 - a11, a12 - a22)]


def _strassen_out(p):
    c11, c12 = p[0] + p[3] - p[4] + p[6], p[2] + p[4]
    c21, c22 = p[1] + p[3], p[0] - p[1] + p[2] + p[5]
    return jnp.concatenate([c11, c21], axis=0), jnp.concatenate([c12, c22], axis=0)


SQ = {"g": (2 * L, F // 2), "u": (2 * L, F // 2), "d": (F // 2, 2 * L)}

SK = {"g": ((0, 2), (1, 3)), "u": ((0, 2), (1, 3)), "d": (range(6), range(6, 12))}

T = range(NT)
_z = lambda j: [("z", j, a) for a in range(NC)]
_k = lambda j, al: [("k", j, a) for a in al]
_u = lambda a: [("u", j, a) for j in T]
_iv = lambda jl, al: [("i", j, a) for j in jl for a in al]
_kv = lambda a: [("kv", j, a) for j in T]
_m = lambda jl, us, outs: [("mac", j, us, outs) for j in jl]

A2 = (0, 1)
SCHEDULE = [
    (["ssm0"], _z(0) + _k(0, range(NC)), [("setup", None)]),
    (["ssm1"], _z(1) + _k(1, range(NC)), []),
    (["ssm2"], _z(2) + _k(2, [0, 1]), []),
    (["k0", "v0"], _k(2, [2, 3]) + _u(0), _kv(0) + _m([0], (0,), (0,))),
    (["ssm3"], _iv([0], [0]) + _z(3) + _k(3, [0, 1]), _m([1, 2], (0,), (0,))),
    (["k1", "v1"], _k(3, [2, 3]) + _u(1), _kv(1) + _m([3], (0,), (0,))),
    (["ssm4"], _iv([1, 2, 3], [0]) + _z(4) + _k(4, range(NC)), _m([0, 1, 2, 3], A2, (1,))),
    (["q0"], _iv([0, 1, 2, 3], [1]) + _iv([4], A2), _m([4], A2, A2) + _m([4], A2, (2, 3))),
    (["mA", "c0"], [("mod", "mA", "c0")], []),
]
_g = lambda p: [("g", p, n, f) for f in range(3) for n in "gu"]
_v = lambda *names: [("vmod", n) for n in names]
_w = lambda names, p0, p1: [("wsum", n, p0, p1) for n in names]
_e = [("d", n, f) for n in T for f in (0, 1)]
FIRST = [
    (["wg0", "qh"], None, [("g", 0, "g", f, h) for h in (0, 1) for f in range(3)], []),
    (["wu0", "s1", "c1"], None, [("g", 0, "u", f) for f in range(3)],
     _v("s1", "c1") + _m([0], A2, (2, 3))),
    (["wg1", "wu1"], None, _g(1)[:-1], _m([1, 2], A2, (2, 3))),
    (["wg2", "wu2", "s2", "c2"], None, _g(1)[-1:] + _g(2),
     _v("s2", "c2") + _m([3], A2, (2, 3)) + _w("gu", 0, 1)),
    (["wg3", "wu3", "wg4", "wu4", "s4", "c4", "q1"], (0, HM), _g(3) + _g(4),
     _v("s4", "c4") + _w("gu", 1, 2)),
    (["wd", "k2", "v2"], None, _e[:2] + _u(2) + _e[2:6],
     _kv(2) + _m([0, 1, 2, 3], (2,), (2, 3))),
    (["mG", "k3", "v3"], None,
     _e[6:] + _u(3) + [(x, n, 2) for n in T for x in "di"] + _iv(T, [3]),
     _m([4], (2,), (2, 3)) + _kv(3) + _v("mG") + _w("d", 0, 6) + _m(T, (3,), (3,))),
]

DMA_ORDER = (["sk", "sd", "c", "ssm0", "ssm1", "ssm2", "k0", "v0", "ssm3", "k1", "v1", "ssm4",
              "q0", "c0", "mA", "mB", "wg0", "qh", "wu0", "s1", "c1", "wg1", "wu1", "s2", "c2",
              "wg2", "wu2", "s4", "c4", "wg3", "wu3", "wg4", "wu4", "q1", "wd", "k2", "v2", "mG", "k3", "v3",
              "q1c"] + [f"q{i + 1}" for i in range(1, NB)])


def _costs(job):
    if job[0] == "kv":
        return [48, 42] * (C // 64)
    if job[0] == "wsum":
        return [54] * ((job[3] - job[2]) * SQ[job[1]][1] // 32)
    if job[0] == "setup":
        return [100] * (4 * R)
    if job[0] == "vmod":
        return [3 * D // VM // 8] * (VM * (WM[job[1]][1] - WM[job[1]][0]))
    us, outs = job[2], job[3]
    pairs = [(a, n) for a in outs for n in us if n <= a]
    mac = (2 * len({a - n for a, n in pairs if a > n}) + 8 * len(pairs)
           - (2 * len(outs) if us[0] == 0 else 0))
    fin = sum(a <= us[-1] for a in outs)
    if mac < 12 and outs[-1] <= us[-1] < NC - 1:
        return [1 + R * mac + 16 * fin, 1 + R * mac + 48 * fin] * 8
    return ([1 + mac] * 3 + [1 + mac + 16 * fin] + [1 + mac] * 3 + [1 + mac + 48 * fin]) * 8


def _plan(groups, jobs, lead=0, floor=(1.0, 0.8)):
    free = FREE_FFN if lead else FREE
    nstep = {"i": 8, "z": 8, "k": 16, "u": 16, "mod": 0, "d": TM0 // 16}
    steps = lambda g: (KP[g[1] + 1] - KP[g[1]]) * TM0 // 16 if g[0] == "g" else nstep[g[0]]
    slots = [free["D" if g[0] == "d" and g[2] == 2 else g[0]]
             for g in groups for _ in range(steps(g))]
    lo, hi = [], []
    for job in jobs:
        begin, limit, first = 0, len(slots), 0
        for g in groups:
            kind = (g[0], job[0])
            if (kind == ("u", "kv") and g[1:] == job[1:]
                    or kind == ("i", "mac") and g[1] == job[1] and g[2] in job[3]
                    and g[2] <= job[2][-1] or kind == ("d", "vmod") and g[2] == 2):
                limit = min(limit, first - lead)
            if kind == ("g", "vmod") and job[1][1] == str(g[1]):
                limit = min(limit, first - 11)
            first += steps(g)
            if kind == ("u", "mac") and g[1] == job[1] and g[2] in job[2]:
                begin = first
        lo.append(begin)
        hi.append(limit)
    plan, credit, n = [], (slots or [0])[0], 0
    for k, job in enumerate(jobs):
        if n < lo[k]:
            n, credit = lo[k], min(credit, 0) + slots[lo[k]]
        work = [sum(_costs(j)) for j in jobs]
        if lead:
            rate = max(RATE * sum(work[k:m + 1]) / max(sum(slots[n:hi[m]]), 1)
                       for m in range(k, len(jobs)))
        else:
            rate = RATE * sum(work[k:]) / sum(slots[n:])
        rate = max(rate, floor[0] if job[0] == "kv" else floor[1])
        idx = []
        for c in _costs(job):
            while credit <= 0 and n + 1 < hi[k]:
                n += 1
                credit += slots[n] * rate
            credit -= c
            idx.append(n)
        plan.append(idx)
    return plan


def _kernel(q_hbm, k_hbm, v_hbm, sk_hbm, ssm_hbm, sd_hbm, wg_hbm, wu_hbm, wd_hbm,
            c_hbm, wm_hbm, o_hbm,
            qb0, qb, kbs, vbs, ssmb, wgb, wub, wdb, sgb, sub, sdn, wmb, uwb, ub, kpb, yp, pb, yb,
            x1b0, x1b, h2b, gub, dpart, hb, ob0, ob, mv, skb, sdb, cb_, sem, osem):
    cps = {"sk": (sk_hbm, skb), "sd": (sd_hbm, sdb), "c": (c_hbm, cb_), "wd": (wd_hbm, wdb)}
    for j in range(NT):
        cps[f"ssm{j}"] = (ssm_hbm.at[pl.ds(j * L, L), :], ssmb.at[j])
    for a in range(NC):
        n, h = C * NT, 2 * PAD
        if a == 0:
            cps["k0"] = (k_hbm.at[pl.ds(0, n), :], kbs[0].at[pl.ds(h, n), :])
        else:
            e = 48
            cps[f"k{a}"] = (k_hbm.at[pl.ds(a * n - e, n + e), :],
                            kbs[a].at[pl.ds(h - e, n + e), :])
        cps[f"v{a}"] = (v_hbm.at[pl.ds(a * n, n), :], vbs[a].at[pl.ds(0, n), :])
    for n, (c0, c1) in WM.items():
        cols = pl.ds(c0 * L, (c1 - c0) * L)
        cps[n] = (wm_hbm.at[:, cols], wmb.at[:, cols])
    cps["q0"] = (q_hbm.at[0, pl.ds(0, H0), :], qb0.at[pl.ds(0, H0), :])
    cps["qh"] = (q_hbm.at[0, pl.ds(H0, TM0 - H0), :], qb0.at[pl.ds(H0, TM0 - H0), :])
    cps["q1"] = (q_hbm.at[0, pl.ds(TM0, HM), :], qb.at[0, pl.ds(0, HM), :])
    cps["q1c"] = (q_hbm.at[0, pl.ds(TM0 + HM, TM - HM), :], qb.at[0, pl.ds(HM, TM - HM), :])
    for i in range(1, NB):
        cps[f"q{i + 1}"] = (q_hbm.at[0, pl.ds(TM0 + i * TM, TM), :], qb.at[i])
    for p in range(len(KP) - 1):
        rows = pl.ds(KP[p] * L, (KP[p + 1] - KP[p]) * L)
        cps[f"wg{p}"] = (wg_hbm.at[rows, :], wgb.at[rows, :])
        cps[f"wu{p}"] = (wu_hbm.at[rows, :], wub.at[rows, :])
    assert sorted(cps) == sorted(DMA_ORDER)

    def cp(name):
        src, dst = cps[name]
        return pltpu.make_async_copy(src, dst, sem.at[DMA_ORDER.index(name)])

    def wait(*names):
        for n in names:
            cp(n).wait()

    kbs[0][0:2 * PAD, :] = jnp.zeros((2 * PAD, L), bf16)
    for n in DMA_ORDER:
        cp(n).start()

    tabs, ginv, ccol = _tables(False), [], []
    for ref in (ub, kpb, yp):
        ref[0, 0, 0, 0, pl.ds(0, 8, stride=2), :] = jnp.zeros((8, L), f32)
    mv[0, pl.ds(0, 8, stride=2), :] = jnp.zeros((8, L), f32)
    ri = lax.broadcasted_iota(jnp.int32, (L, L), 0)
    ci = lax.broadcasted_iota(jnp.int32, (L, L), 1)
    sel = jnp.where(ci == R * _perm(ri & 31) + (ri >> 5), 1.0, 0.0).astype(bf16)

    wait("sk", "sd", "c")
    skt = skb[...].astype(f32)
    sdv = sdb[...].astype(f32).reshape(1, D)
    cv = cb_[...].astype(f32)
    sig = jax.nn.sigmoid(cv)
    cs = jnp.broadcast_to((cv * sig).astype(bf16), (16, D))
    one = sig[:, 0:L]

    def gate(x, deps):
        dep = jnp.concatenate(deps, axis=0).reshape(x.shape)
        return jnp.where(jnp.broadcast_to(one, x.shape) > 2.0, dep, x)

    def put(dst, j, a, xs):
        for qi in range(R):
            dst[j, a, qi] = jnp.concatenate(xs[qi], axis=1)

    zs = {}
    mod = {}

    def grp_z(j, a):
        z = [lax.dot_general(sel, ssmb[j, :, t * L:(t + 1) * L], (((1,), (1,)), ((), ())),
                             preferred_element_type=f32) for t in range(R * a, R * a + R)]
        zs[j, a] = [jnp.concatenate([z[p][32 * r:32 * (r + 1)] for p in range(R)],
                                    axis=0).astype(bf16) for r in range(R)]
        return [z[0][16 * t:16 * t + 8] for t in range(8)]

    def grp_fwd(ws, dst, j, a, dvec=None):
        t = [jnp.dot(tabs[r], ws[r], preferred_element_type=f32) for r in range(R)]
        x = [_split(v) for v in t]
        if dvec is not None:
            x[0] = (x[0][0] + dvec[None], x[0][1])
        put(dst, j, a, _radix4(x, -1))
        return [t[0][16 * s:16 * s + 8] for s in range(16)]

    def grp_k(j, a):
        return grp_fwd(zs.pop((j, a)), kpb, j, a,
                       sdv[:, j * L:(j + 1) * L] if a == 0 else None)

    def grp_u(j, a):
        uw = [uwb[j, a, r] for r in range(R)]
        return grp_fwd(uw, ub, j, a)

    def grp_i(j, a):
        ys = []
        for r in range(2 * R):
            y = jnp.dot(ginv[r], pb[j, a, r], preferred_element_type=f32)
            yb[j, pl.ds(a * C + r, L // 2, stride=2 * R), :] = y
            ys.append(y)
        return [ys[r][16 * s:16 * s + 8] for r in (0, R) for s in range(4)]

    def grp_mod(*names):
        for name in names:
            c0, c1 = WM[name]
            m = jnp.dot(cs, wmb[:, c0 * L:c1 * L], preferred_element_type=f32)
            for c in range(c0, c1):
                mod[c] = m[0:1, (c - c0) * L:(c - c0 + 1) * L]
        return []

    def modv(i, t0=0, t1=NT):
        return jnp.concatenate([mod[i * NT + n] for n in range(t0, t1)], axis=1)

    def job_kv(j, a, deps):
        lo = lambda x: lax.bitcast_convert_type(x << 16, f32)
        hi = lambda x: lax.bitcast_convert_type(x & jnp.uint32(0xFFFF0000), f32)
        n = C // 8
        kw, vw = kbs[a].bitcast(u32), vbs[a].bitcast(u32)
        ld = lambda ref, o: ref[pl.ds(4 * j + o, n, stride=WPT), :]
        k = {}
        for m in range(4):
            x = ld(kw, PAD + m)
            k[2 * m], k[2 * m + 1] = lo(x), hi(x)
        k[-3] = hi(ld(kw, PAD - WPT + 2))
        x = ld(kw, PAD - WPT + 3)
        k[-2], k[-1] = lo(x), hi(x)
        w = [skt[t:t + 1, j * L:(j + 1) * L] for t in range(KS)]
        w0 = [gate(jnp.broadcast_to(w[0], (n, L)), deps[e::2]) for e in (0, 1)]
        kv = {}
        for m in range(4):
            x = ld(vw, m)
            for ph, v in ((2 * m, lo(x)), (2 * m + 1, hi(x))):
                ks = k[ph] * w0[m % 2]
                for t in range(1, KS):
                    ks = ks + k[ph - t] * w[t]
                kv[ph] = (ks * v).reshape(n // 8, 8, L)
        for r in range(R):
            uwb[j, a, r] = jnp.concatenate([kv[r], kv[r + R]], axis=1).reshape(L, L).astype(bf16)

    def job_mac(j, us, outs, deps):
        ld = lambda ref, a: (ref[j, a, :, :, 0:8, :], ref[j, a, :, :, 8:16, :])
        lo, hi = us[0], us[-1]
        u = {a: ld(ub, a) for a in us}
        if len(deps) == 16:
            ur = jnp.concatenate([gate(u[lo][0][0:1], deps), u[lo][0][1:]], axis=0)
        else:
            ur = gate(u[lo][0], [deps[R * i + qi] for qi in range(R) for i in range(16)])
        u[lo] = (ur, u[lo][1])
        ms = sorted({a - n for a in outs for n in us if n <= a})
        k = {m: ld(kpb, m) for m in sorted(set(ms) | {m - 1 for m in ms if m > 0})}
        kp = {m: k[m] if m == 0 else (k[m][0] - k[m - 1][1], k[m][1] + k[m - 1][0]) for m in ms}
        for a in outs:
            yr, yi = ld(yp, a) if lo > 0 else (None, None)
            for n in us:
                if n > a:
                    continue
                (kr, ki), (ur, ui) = kp[a - n], u[n]
                tr = kr * ur - ki * ui
                ti = kr * ui + ki * ur
                yr = tr if yr is None else yr + tr
                yi = ti if yi is None else yi + ti
            if a > hi:
                yp[j, a] = jnp.concatenate([yr, yi], axis=2)
                continue
            ps = _radix4([(yr[qi], yi[qi]) for qi in range(R)], +1)
            for r in range(R):
                pr, pi = [p.reshape(8, 2, 8, L) for p in ps[r]]
                lr, li, hr, hi_ = pr[:, 0], pi[:, 0], pr[:, 1], pi[:, 1]
                if r % 2:
                    hr, hi_ = (hr - hi_) * RSQ2, (hr + hi_) * RSQ2
                if r < 2:
                    outs2 = (lr + hr, li + hi_), (lr - hr, li - hi_)
                else:
                    outs2 = (lr - hi_, li + hr), (lr + hi_, li - hr)
                for e in range(2):
                    pb[j, a, r + R * e] = jnp.concatenate(
                        outs2[e], axis=1).reshape(L, L).astype(bf16)

    def job_setup(_, deps):
        def hold(r, n):
            return gate(n, [deps[2 * r + s // 4] for s in range(8)])

        ginv.extend(_tables(True, hold))
        csf = cs[0:1].astype(f32)
        ccol.append(jnp.concatenate([jnp.broadcast_to(csf[:, t * L:(t + 1) * L], (L, L)).T
                                     for t in range(NT)], axis=0))

    def job_vmod(name, deps):
        c0, c1 = WM[name]
        n = D // VM
        for c in range(c0, c1):
            for i in range(VM):
                cc = ccol[0][i * n:(i + 1) * n]
                cc = jnp.concatenate([gate(cc[0:8], [deps[(c - c0) * VM + i]]), cc[8:]], axis=0)
                p = wmb[i * n:(i + 1) * n, c * L:(c + 1) * L].astype(f32) * cc
                mv[c, 8 * i:8 * i + 8, :] = jnp.sum(p.reshape(n // 8, 8, L), axis=0)
            mod[c] = jnp.sum(mv[c], axis=0, keepdims=True)

    wts = {"g": (wgb, sgb), "u": (wub, sub), "d": (wdb, sdn)}

    def job_wsum(n, p0, p1, deps):
        (w, s), nh = wts[n], SQ[n][1]
        for p in range(p0, p1):
            dp = deps[(p - p0) * nh // 32:(p - p0 + 1) * nh // 32]

            def quad(r, c, hold):
                t0 = SK[n][r][p] * L
                x = w[t0:t0 + L, c * nh:(c + 1) * nh].astype(f32)
                if hold:
                    x = jnp.concatenate(
                        [gate(x[:, t * L:(t + 1) * L], [dp[t // 2 * 8 + g // 2] for g in range(16)])
                         for t in range(nh // L)], axis=1)
                return x

            b11, b12, b21, b22 = quad(0, 0, 1), quad(0, 1, 0), quad(1, 0, 0), quad(1, 1, 1)
            for i, v in enumerate((b11 + b22, b12 - b22, b21 - b11, b11 + b12, b21 + b22)):
                s[i, p * L:(p + 1) * L, :] = v.astype(bf16)

    def strassen_lhs(x, n):
        m = x.shape[0] // 2
        k0, k1 = [jnp.concatenate([x[:, t * L:(t + 1) * L] for t in ts], axis=1) for ts in SK[n]]
        return _strassen_lhs(k0[:m], k1[:m], k0[m:], k1[m:])

    def strassen(a, n, c):
        (w, s), nh = wts[n], SQ[n][1]
        cs = slice(c, c + L)
        raw = lambda e: jnp.concatenate([w[t * L:(t + 1) * L, e * nh + c:e * nh + c + L]
                                         for t in SK[n][e]], axis=0)
        b = [s[0, :, cs], raw(0), s[1, :, cs], s[2, :, cs], raw(1), s[3, :, cs], s[4, :, cs]]
        return _strassen_out([jnp.dot(x, y, preferred_element_type=f32) for x, y in zip(a, b)])

    grp_fn = {"z": grp_z, "k": grp_k, "u": grp_u, "i": grp_i, "mod": grp_mod}
    job_fn = {"kv": job_kv, "mac": job_mac, "vmod": job_vmod, "setup": job_setup,
              "wsum": job_wsum}

    def run(groups, jobs, **kw):
        plan = _plan(groups, jobs, **kw)
        anchors, done = [], 0
        for g in groups + [None]:
            while done < len(jobs) and max(plan[done]) < len(anchors):
                job_fn[jobs[done][0]](*jobs[done][1:], [anchors[n] for n in plan[done]])
                done += 1
            if g is not None:
                anchors += grp_fn[g[0]](*g[1:])
        assert done == len(jobs)

    for waits, groups, jobs in SCHEDULE:
        wait(*waits)
        run(groups, jobs)

    n1, dep = [], None
    for r in range(0, H0, H0 // 2):
        x = qb0[r:r + H0 // 2, :].astype(f32)
        if dep is not None:
            x = jnp.concatenate([gate(x[:, 0:L], [dep]), x[:, L:]], axis=1)
        n1.append(_layernorm(x))
        dep = n1[-1][:, 0:L]
    n1 = jnp.concatenate(n1, axis=0)
    wait("mB")
    grp_mod("mB")
    sa, ca, ga = [modv(i) for i in range(3)]
    a1 = ga * (1.0 + ca)
    b1 = ga * sa

    def o_cp(i, c0, c1, r0=0, r1=TM):
        cols = pl.ds(c0, c1 - c0)
        if i is None:
            return pltpu.make_async_copy(ob0.at[:, cols], o_hbm.at[0, pl.ds(0, TM0), cols],
                                         osem.at[NB])
        base = TM0 + i * TM + r0
        if not isinstance(i, int):
            base = pl.multiple_of(base, 16)
        return pltpu.make_async_copy(ob.at[i, pl.ds(r0, r1 - r0), cols],
                                     o_hbm.at[0, pl.ds(base, r1 - r0), cols], osem.at[i])

    def prep_norm(q_ref, x1_ref, y0, r0, n, dep=None, n1=None):
        x = q_ref[r0:r0 + n, :].astype(f32)
        if dep is not None:
            x = jnp.concatenate([gate(x[:, 0:L], [dep]), x[:, L:]], axis=1)
        y = jnp.concatenate([yb[j, pl.ds(y0 + r0, n), :] for j in range(NT)], axis=1)
        x1 = x + ((_layernorm(x) if n1 is None else n1) * a1 + b1) * y
        x1_ref[r0:r0 + n, :] = x1
        return _layernorm(x1)

    n2 = [prep_norm(qb0, x1b0, 0, 0, H0, None, n1)]
    aff = []

    def prep_chain(i, r0, r1, pr):
        y0 = TM0 + i * TM
        if not isinstance(i, int):
            y0 = pl.multiple_of(y0, L)
        dep = None
        while r0 < r1:
            n = pr if (r1 - r0) % pr == 0 else pr + 8
            h2 = prep_norm(qb.at[i], x1b, y0, r0, n, dep if dep is None else dep[:n])
            h2 = h2 * aff[0] + aff[1]
            h2b[r0:r0 + n, :] = h2
            dep = h2[:, 0:L]
            r0 += n

    OC = (0, D - L, D)
    OP = (((0, D - L, 0, HM), (D - L, D, 0, HM)),
          ((0, D - L, HM, TM), (D - L, D, HM, TM - 64), (D - L, D, TM - 64, TM)))

    def ffn_half(i, half, gb):
        r0, r1 = (HM, TM) if half else (0, HM)
        k = 2 * L
        x = h2b[r0:r1, :]
        a = strassen_lhs(x, "g")
        xe = x[:, 2 * k:].astype(bf16)
        hs = ([], [])
        for c in range(0, F // 2, L):
            gu = []
            for n in "gu":
                p = strassen(a, n, c)
                gu.append([p[e] + jnp.dot(xe, wts[n][0][2 * k:, o:o + L],
                                          preferred_element_type=f32)
                           for e, o in enumerate((c, F // 2 + c))])
            for e in range(2):
                hs[e].append(gu[0][e] * gu[1][e])
        hh = jnp.concatenate(hs[0] + hs[1], axis=1)
        a = strassen_lhs(hh, "d")
        hh = hh.astype(bf16)
        for c0, c1, s0, s1 in OP[half]:
            if c0 == 0:
                p = [strassen(a, "d", c) for c in range(0, k, L)]
                o = jnp.concatenate([q[0] for q in p] + [q[1] for q in p], axis=1)
            else:
                o = jnp.dot(hh[s0 - r0:s1 - r0], wdb[:, c0:c1], preferred_element_type=f32)
            ob[i, s0:s1, c0:c1] = (x1b[s0:s1, c0:c1] + gb[:, c0:c1] * o).astype(bf16)
            o_cp(i, c0, c1, s0, s1).start()

    acc, hcache, parts = {}, {}, {}

    def grp_g(p, n, f, half=None):
        t0, t1 = KP[p], KP[p + 1]
        if (p, half) not in hcache:
            if len(n2) == 1 and half != 0:
                n2.append(prep_norm(qb0, x1b0, 0, H0, TM0 - H0))
            x = jnp.concatenate(n2, axis=0) if half is None else n2[half]
            hcache[p, half] = (x[:, t0 * L:t1 * L] * (1.0 + modv(4, t0, t1))
                               + modv(3, t0, t1)).astype(bf16)
        rows = {None: slice(0, TM0), 0: slice(0, H0), 1: slice(H0, TM0)}[half]
        cols = slice(f * 4 * L, (f + 1) * 4 * L)
        d = jnp.dot(hcache[p, half], (wgb if n == "g" else wub)[t0 * L:t1 * L, cols],
                    preferred_element_type=f32)
        ref = gub.at["gu".index(n), rows, cols]
        if p < len(KP) - 2:
            ref[...] = d if p == 0 else ref[...] + d
        elif n == "g":
            acc[f] = ref[...] + d
        else:
            hb[:, cols] = (acc.pop(f) * (ref[...] + d)).astype(bf16)
        return [d[s:s + 8, c * L:(c + 1) * L] for c in range(0, 4, 4 // (t1 - t0))
                for s in range(0, d.shape[0], 16)]

    def grp_d(n, f):
        c = slice(n * L, (n + 1) * L)
        k = slice(f * 4 * L, (f + 1) * 4 * L)
        d = jnp.dot(hb[:, k], wdb[k, c], preferred_element_type=f32)
        parts[n] = d if f == 0 else parts[n] + d
        if f == 2:
            ob0[:, c] = (x1b0[:, c] + mod[5 * NT + n] * parts.pop(n)).astype(bf16)
            if (n + 1) * L in OC:
                o_cp(None, OC[OC.index((n + 1) * L) - 1], (n + 1) * L).start()
        return [d[s:s + 8] for s in range(0, TM0, 16)]

    grp_fn.update(g=grp_g, d=grp_d)
    for waits, rows, groups, jobs in FIRST:
        wait(*waits)
        for n in parts:
            parts[n] = dpart[:, n * L:(n + 1) * L]
        run(groups, jobs, lead=LEAD, floor=(0.0, 0.0))
        if rows:
            aff += [1.0 + modv(4), modv(3)]
            prep_chain(0, *rows, PR)
        for n in parts:
            dpart[:, n * L:(n + 1) * L] = parts[n]
    gb = modv(5)
    wait("q1c", *[f"q{i + 1}" for i in range(1, NB)])

    def ffn(i, carry):
        prep_chain(i, HM, TM, PL)
        ffn_half(i, 0, gb)
        prep_chain(jnp.minimum(i + 1, NB - 1), 0, HM, PL)
        ffn_half(i, 1, gb)
        return carry

    lax.fori_loop(0, NB, ffn, 0)

    for c0, c1 in zip(OC[:-1], OC[1:]):
        o_cp(None, c0, c1).wait()
    for i in range(NB):
        for op in OP[0] + OP[1]:
            o_cp(i, *op).wait()


@jax.jit
def pallas_adaLN_cond__ssm_conv_h3__glu_gated_bilinear__prompt_kernel(
    A_q: jax.Array,
    A_k: jax.Array,
    A_v: jax.Array,
    A_shift_k: jax.Array,
    A_ssm_k: jax.Array,
    A_ssm_D: jax.Array,
    B_x: jax.Array,
    B_w_gate: jax.Array,
    B_w_up: jax.Array,
    B_w_down: jax.Array,
    c: jax.Array,
    w_mod: jax.Array,
):
    del B_x
    tiles = lambda x: x.reshape(S // 8, 8, NT, L).transpose(0, 2, 1, 3).reshape(S * NT, L)
    any_spec = pl.BlockSpec(memory_space=pl.ANY)
    return pl.pallas_call(
        _kernel,
        in_specs=[any_spec] * 11,
        out_specs=any_spec,
        out_shape=jax.ShapeDtypeStruct((1, S, D), bf16),
        scratch_shapes=[
            pltpu.VMEM((TM0, D), bf16),
            pltpu.VMEM((NB, TM, D), bf16),
            [pltpu.VMEM((4 * PAD + C * NT, L), bf16)] * NC,
            [pltpu.VMEM((2 * PAD + C * NT, L), bf16)] * NC,
            pltpu.VMEM((NT, L, S), bf16),
            pltpu.VMEM((D, F), bf16),
            pltpu.VMEM((D, F), bf16),
            pltpu.VMEM((F, D), bf16),
            pltpu.VMEM((5,) + SQ["g"], bf16),
            pltpu.VMEM((5,) + SQ["u"], bf16),
            pltpu.VMEM((5,) + SQ["d"], bf16),
            pltpu.VMEM((D, 6 * D), bf16),
            pltpu.VMEM((NT, NC, R, L, L), bf16),
            pltpu.VMEM((NT, NC, R, 16, 16, L), f32),
            pltpu.VMEM((NT, NC, R, 16, 16, L), f32),
            pltpu.VMEM((NT, NC, R, 16, 16, L), f32),
            pltpu.VMEM((NT, NC, 2 * R, L, L), bf16),
            pltpu.VMEM((NT, S + 32, L), f32),
            pltpu.VMEM((TM0, D), f32),
            pltpu.VMEM((TM, D), f32),
            pltpu.VMEM((TM, D), f32),
            pltpu.VMEM((2, TM0, F), f32),
            pltpu.VMEM((TM0, D), f32),
            pltpu.VMEM((TM0, F), bf16),
            pltpu.VMEM((TM0, D), bf16),
            pltpu.VMEM((NB, TM, D), bf16),
            pltpu.VMEM((32, 8 * VM, L), f32),
            pltpu.VMEM((KS, D), bf16),
            pltpu.VMEM((D,), bf16),
            pltpu.VMEM((1, D), bf16),
            pltpu.SemaphoreType.DMA((len(DMA_ORDER),)),
            pltpu.SemaphoreType.DMA((NB + 1,)),
        ],
        compiler_params=pltpu.CompilerParams(
            vmem_limit_bytes=120 * 1024 * 1024,
            disable_bounds_checks=True, disable_semaphore_checks=True),
        name="adaln_h3_glu",
    )(A_q, tiles(A_k), tiles(A_v), A_shift_k.T, A_ssm_k, A_ssm_D,
      B_w_gate, B_w_up, B_w_down, c, w_mod)
```

```python
import jax
import jax.numpy as jnp
from jax import lax
import jax.experimental.pallas as pl
import jax.experimental.pallas.tpu as pltpu

S = 2048
D = 640
F = 1536
KS = 4
L = 128
NT = D // L
R = 4
C = R * L
NC = S // C
EPS = 1e-5
RSQ2 = 0.7071067811865476

WPT = 4 * NT
PAD = 32

TM0 = 512
H0 = 352
TM = 512
NB = (S - TM0) // TM
HM = 256
PL = 16
PR = 24
KP = (0, 1, 2, 3, 4, 5)
WM = {"mA": (0, 12), "c0": (20, 21), "mB": (12, 16), "s1": (16, 17), "c1": (21, 22),
      "s2": (17, 19), "c2": (22, 24), "s4": (19, 20), "c4": (24, 25), "mG": (25, 30)}
VM = 5
RATE = 1.05
LEAD = 24
FREE = {"i": 56, "z": 56, "k": 47, "u": 46}
FREE_FFN = {"i": 4, "u": 26, "d": 48, "D": 42, "g": 50}

f32 = jnp.float32
bf16 = jnp.bfloat16
u32 = jnp.uint32


def _cos_turns(t):
    x = jnp.abs(t - jnp.floor(t) - 0.5) - 0.25
    x2 = x * x
    return x * (6.283164024 + x2 * (-41.33713150 + x2 * (81.34038544 + x2 * -70.98993683)))


def _tables(inverse, hold=None):
    shape = (L // 2, L) if inverse else (2 * L, L)
    rho = lax.broadcasted_iota(jnp.int32, shape, 1 if inverse else 0)
    j = lax.broadcasted_iota(jnp.int32, shape, 0 if inverse else 1)
    if inverse:
        g, rad = 8 * (rho >> 4) + (rho & 7), 2 * R
    else:
        g, rad, j = 8 * (rho >> 5) + (rho & 7) + 64 * ((rho >> 4) & 1), R, _perm(j)
    a = (4 * g + 1).astype(f32) * (1.0 / (4 * C))
    off = ((rho >> 3) & 1).astype(f32) * 0.25
    ns = [(rad * j + r).astype(f32) for r in range(rad)]
    if hold is not None:
        ns = [hold(r, n) for r, n in enumerate(ns)]
    ts = [_cos_turns(a * n + off) for n in ns]
    return [(t * (1.0 / C) if inverse else t).astype(bf16) for t in ts]


def _perm(c):
    return 16 * (c >> 4) + 2 * (c & 7) + ((c >> 3) & 1)


def _layernorm(x):
    m = jnp.mean(x, axis=-1, keepdims=True)
    xc = x - m
    v = jnp.mean(xc * xc, axis=-1, keepdims=True)
    return xc * lax.rsqrt(v + EPS)


def _split(t):
    t = t.reshape(16, 16, L)
    return t[:, :8, :], t[:, 8:, :]


def _radix4(x, sgn):
    (ar, ai), (br, bi), (cr, ci), (dr, di) = x
    s0r, s0i, d0r, d0i = ar + cr, ai + ci, ar - cr, ai - ci
    s1r, s1i, d1r, d1i = br + dr, bi + di, br - dr, bi - di
    o0 = (s0r + s1r, s0i + s1i)
    o2 = (s0r - s1r, s0i - s1i)
    pl_ = (d0r - d1i, d0i + d1r)
    mi_ = (d0r + d1i, d0i - d1r)
    return [o0, pl_, o2, mi_] if sgn > 0 else [o0, mi_, o2, pl_]


S222 = (
    ({(1, 1): 1, (0, 0): -1}, {(0, 0): 1, (1, 1): 1}, {(0, 0): -1, (1, 1): 1}),
    ({(0, 1): 1, (1, 1): 1}, {(1, 0): 1, (1, 1): 1}, {(0, 0): 1}),
    ({(0, 0): 1, (0, 1): 1}, {(1, 1): 1}, {(0, 0): -1, (0, 1): 1}),
    ({(1, 1): 1}, {(1, 0): 1, (0, 0): -1}, {(0, 0): -1, (1, 0): 1}),
    ({(1, 0): 1, (1, 1): 1}, {(0, 0): 1}, {(1, 0): 1, (1, 1): -1}),
    ({(0, 0): 1}, {(0, 1): 1, (1, 1): -1}, {(0, 1): 1, (1, 1): -1}),
    ({(0, 0): 1, (1, 0): 1}, {(0, 0): 1, (0, 1): 1}, {(1, 1): 1}),
)
S233 = (
    ({(0, 0): 1, (1, 0): 1, (1, 2): -1}, {(0, 0): 1, (2, 2): -1},
     {(0, 0): 1, (0, 2): -1, (1, 2): 1}),
    ({(1, 0): 1, (1, 2): -1}, {(0, 0): 1}, {(0, 0): -1, (0, 2): 1, (1, 0): 1, (1, 2): -1}),
    ({(0, 0): 1, (1, 0): 1, (1, 2): -1, (0, 2): -1}, {(2, 2): 1}, {(0, 0): 1, (0, 2): -1}),
    ({(0, 2): 1}, {(1, 0): 1, (2, 0): 1, (2, 2): 1}, {(0, 0): 1}),
    ({(0, 1): 1, (0, 2): -1, (1, 1): 1}, {(1, 0): 1, (2, 1): 1},
     {(0, 1): -1, (1, 0): 1, (1, 1): 1}),
    ({(0, 1): 1, (0, 2): -1}, {(1, 0): 1}, {(0, 0): 1, (0, 1): 1, (1, 0): -1, (1, 1): -1}),
    ({(0, 1): 1, (0, 2): -1, (1, 1): 1, (1, 2): -1}, {(2, 1): 1}, {(1, 0): -1, (1, 1): -1}),
    ({(1, 2): 1}, {(0, 0): 1, (2, 0): 1, (2, 1): -1}, {(1, 0): 1}),
    ({(0, 0): 1, (1, 1): 1}, {(0, 1): 1, (1, 2): -1}, {(0, 1): 1, (1, 2): -1}),
    ({(1, 0): 1, (1, 1): -1}, {(0, 1): 1}, {(1, 1): 1, (1, 2): -1}),
    ({(0, 0): 1, (0, 1): -1}, {(1, 2): 1}, {(0, 1): 1, (0, 2): -1}),
    ({(0, 0): 1}, {(0, 0): 1, (0, 2): 1, (1, 2): 1}, {(0, 2): 1, (1, 2): -1}),
    ({(0, 0): 1, (1, 0): 1}, {(0, 1): 1, (0, 2): 1, (2, 2): 1}, {(1, 2): 1}),
    ({(1, 1): 1}, {(0, 1): 1, (1, 1): 1, (1, 0): -1}, {(0, 1): -1, (1, 1): 1}),
    ({(0, 1): 1, (1, 1): 1}, {(1, 1): 1, (1, 2): 1, (2, 1): 1}, {(0, 1): 1}),
)
SCHEME = (S233, S222)
HIT = (((0, 0), (0, 1), (1, 0), (2, 1)), ((0, 0), (1, 1)))
NSUM = [sum(len(t[1]) > 1 for t in s) for s in SCHEME]
DT = ((0, 1, 2), (3, 4))
FT = ([range(0, 4), range(4, 8), range(8, 12)], [range(0, 6), range(6, 12)])


def _lin(coef, get):
    r = None
    for q, v in coef.items():
        x = get(q)
        r = (x if v > 0 else -x) if r is None else (r + x if v > 0 else r - x)
    return r


T = range(NT)
_z = lambda j: [("z", j, a) for a in range(NC)]
_k = lambda j, al: [("k", j, a) for a in al]
_u = lambda a: [("u", j, a) for j in T]
_iv = lambda jl, al: [("i", j, a) for j in jl for a in al]
_kv = lambda a: [("kv", j, a) for j in T]
_m = lambda jl, us, outs: [("mac", j, us, outs) for j in jl]

A2 = (0, 1)
SCHEDULE = [
    (["ssm0"], _z(0) + _k(0, range(NC)), [("setup", None)]),
    (["ssm1"], _z(1) + _k(1, range(NC)), []),
    (["ssm2"], _z(2) + _k(2, [0, 1]), []),
    (["k0", "v0"], _k(2, [2, 3]) + _u(0), _kv(0) + _m([0], (0,), (0,))),
    (["ssm3"], _iv([0], [0]) + _z(3) + _k(3, [0, 1]), _m([1, 2], (0,), (0,))),
    (["k1", "v1"], _k(3, [2, 3]) + _u(1), _kv(1) + _m([3], (0,), (0,))),
    (["ssm4"], _iv([1, 2, 3], [0]) + _z(4) + _k(4, range(NC)), _m([0, 1, 2, 3], A2, (1,))),
    (["q0"], _iv([0, 1, 2, 3], [1]) + _iv([4], A2), _m([4], A2, A2) + _m([4], A2, (2, 3))),
    (["mA", "c0"], [("mod", "mA", "c0")], []),
]
_g = lambda p: [("g", p, n, f) for f in range(3) for n in "gu"]
_v = lambda *names: [("vmod", n) for n in names]
_w = lambda names, si: [("wsum", n, si, t) for n in names for t in range(len(FT[si][0]))]
_e = [("d", n, f) for n in T for f in (0, 1)]
FIRST = [
    (["wg0", "qh"], None, [("g", 0, "g", f, h) for h in (0, 1) for f in range(3)], []),
    (["wu0", "s1", "c1"], None, [("g", 0, "u", f) for f in range(3)],
     _v("s1", "c1") + _m([0], A2, (2, 3))),
    (["wg1", "wu1"], None, _g(1)[:-1], _m([1, 2], A2, (2, 3))),
    (["wg2", "wu2", "s2", "c2"], None, _g(1)[-1:] + _g(2),
     _v("s2", "c2") + _m([3], A2, (2, 3)) + _w("gu", 0)),
    (["wg3", "wu3", "wg4", "wu4", "s4", "c4", "q1"], (0, HM), _g(3) + _g(4),
     _v("s4", "c4") + _w("gu", 1)),
    (["wd", "k2", "v2"], None, _e[:2] + _u(2) + _e[2:6],
     _kv(2) + _m([0, 1, 2, 3], (2,), (2, 3))),
    (["mG", "k3", "v3"], None,
     _e[6:] + _u(3) + [(x, n, 2) for n in T for x in "di"] + _iv(T, [3]),
     _m([4], (2,), (2, 3)) + _kv(3) + _v("mG") + _w("d", 0) + _w("d", 1) + _m(T, (3,), (3,))),
]

DMA_ORDER = (["sk", "sd", "c", "ssm0", "ssm1", "ssm2", "k0", "v0", "ssm3", "k1", "v1", "ssm4",
              "q0", "c0", "mA", "mB", "wg0", "qh", "wu0", "s1", "c1", "wg1", "wu1", "s2", "c2",
              "wg2", "wu2", "s4", "c4", "wg3", "wu3", "wg4", "wu4", "q1", "wd", "k2", "v2", "mG", "k3", "v3",
              "q1c"] + [f"q{i + 1}" for i in range(1, NB)])


def _costs(job):
    if job[0] == "kv":
        return [48, 42] * (C // 64)
    if job[0] == "wsum":
        return [61] * 8 if job[2] == 0 else [50] * 4
    if job[0] == "setup":
        return [100] * (4 * R)
    if job[0] == "vmod":
        return [3 * D // VM // 8] * (VM * (WM[job[1]][1] - WM[job[1]][0]))
    us, outs = job[2], job[3]
    pairs = [(a, n) for a in outs for n in us if n <= a]
    mac = (2 * len({a - n for a, n in pairs if a > n}) + 8 * len(pairs)
           - (2 * len(outs) if us[0] == 0 else 0))
    fin = sum(a <= us[-1] for a in outs)
    if mac < 12 and outs[-1] <= us[-1] < NC - 1:
        return [1 + R * mac + 16 * fin, 1 + R * mac + 48 * fin] * 8
    return ([1 + mac] * 3 + [1 + mac + 16 * fin] + [1 + mac] * 3 + [1 + mac + 48 * fin]) * 8


def _plan(groups, jobs, lead=0, floor=(1.0, 0.8)):
    free = FREE_FFN if lead else FREE
    nstep = {"i": 8, "z": 8, "k": 16, "u": 16, "mod": 0, "d": TM0 // 16}
    steps = lambda g: (KP[g[1] + 1] - KP[g[1]]) * TM0 // 16 if g[0] == "g" else nstep[g[0]]
    slots = [free["D" if g[0] == "d" and g[2] == 2 else g[0]]
             for g in groups for _ in range(steps(g))]
    lo, hi = [], []
    for job in jobs:
        begin, limit, first = 0, len(slots), 0
        for g in groups:
            kind = (g[0], job[0])
            if (kind == ("u", "kv") and g[1:] == job[1:]
                    or kind == ("i", "mac") and g[1] == job[1] and g[2] in job[3]
                    and g[2] <= job[2][-1] or kind == ("d", "vmod") and g[2] == 2):
                limit = min(limit, first - lead)
            if kind == ("g", "vmod") and job[1][1] == str(g[1]):
                limit = min(limit, first - 11)
            first += steps(g)
            if kind == ("u", "mac") and g[1] == job[1] and g[2] in job[2]:
                begin = first
        lo.append(begin)
        hi.append(limit)
    plan, credit, n = [], (slots or [0])[0], 0
    for k, job in enumerate(jobs):
        if n < lo[k]:
            n, credit = lo[k], min(credit, 0) + slots[lo[k]]
        work = [sum(_costs(j)) for j in jobs]
        if lead:
            rate = max(RATE * sum(work[k:m + 1]) / max(sum(slots[n:hi[m]]), 1)
                       for m in range(k, len(jobs)))
        else:
            rate = RATE * sum(work[k:]) / sum(slots[n:])
        rate = max(rate, floor[0] if job[0] == "kv" else floor[1])
        idx = []
        for c in _costs(job):
            while credit <= 0 and n + 1 < hi[k]:
                n += 1
                credit += slots[n] * rate
            credit -= c
            idx.append(n)
        plan.append(idx)
    return plan


def _kernel(q_hbm, k_hbm, v_hbm, sk_hbm, ssm_hbm, sd_hbm, wg_hbm, wu_hbm, wd_hbm,
            c_hbm, wm_hbm, o_hbm,
            qb0, qb, kbs, vbs, ssmb, wgb, wub, wdb, wsb, wmb, uwb, ub, kpb, yp, pb, yb,
            x1b0, x1b, h2b, hf, gub, dpart, hb, ob0, ob, mv, skb, sdb, cb_, sem, osem):
    cps = {"sk": (sk_hbm, skb), "sd": (sd_hbm, sdb), "c": (c_hbm, cb_), "wd": (wd_hbm, wdb)}
    for j in range(NT):
        cps[f"ssm{j}"] = (ssm_hbm.at[pl.ds(j * L, L), :], ssmb.at[j])
    for a in range(NC):
        n, h = C * NT, 2 * PAD
        if a == 0:
            cps["k0"] = (k_hbm.at[pl.ds(0, n), :], kbs[0].at[pl.ds(h, n), :])
        else:
            e = 48
            cps[f"k{a}"] = (k_hbm.at[pl.ds(a * n - e, n + e), :],
                            kbs[a].at[pl.ds(h - e, n + e), :])
        cps[f"v{a}"] = (v_hbm.at[pl.ds(a * n, n), :], vbs[a].at[pl.ds(0, n), :])
    for n, (c0, c1) in WM.items():
        cols = pl.ds(c0 * L, (c1 - c0) * L)
        cps[n] = (wm_hbm.at[:, cols], wmb.at[:, cols])
    cps["q0"] = (q_hbm.at[0, pl.ds(0, H0), :], qb0.at[pl.ds(0, H0), :])
    cps["qh"] = (q_hbm.at[0, pl.ds(H0, TM0 - H0), :], qb0.at[pl.ds(H0, TM0 - H0), :])
    cps["q1"] = (q_hbm.at[0, pl.ds(TM0, HM), :], qb.at[0, pl.ds(0, HM), :])
    cps["q1c"] = (q_hbm.at[0, pl.ds(TM0 + HM, TM - HM), :], qb.at[0, pl.ds(HM, TM - HM), :])
    for i in range(1, NB):
        cps[f"q{i + 1}"] = (q_hbm.at[0, pl.ds(TM0 + i * TM, TM), :], qb.at[i])
    for p in range(len(KP) - 1):
        rows = pl.ds(KP[p] * L, (KP[p + 1] - KP[p]) * L)
        cps[f"wg{p}"] = (wg_hbm.at[rows, :], wgb.at[rows, :])
        cps[f"wu{p}"] = (wu_hbm.at[rows, :], wub.at[rows, :])
    assert sorted(cps) == sorted(DMA_ORDER)

    def cp(name):
        src, dst = cps[name]
        return pltpu.make_async_copy(src, dst, sem.at[DMA_ORDER.index(name)])

    def wait(*names):
        for n in names:
            cp(n).wait()

    kbs[0][0:2 * PAD, :] = jnp.zeros((2 * PAD, L), bf16)
    for n in DMA_ORDER:
        cp(n).start()

    tabs, ginv, ccol = _tables(False), [], []
    for ref in (ub, kpb, yp):
        ref[0, 0, 0, 0, pl.ds(0, 8, stride=2), :] = jnp.zeros((8, L), f32)
    mv[0, pl.ds(0, 8, stride=2), :] = jnp.zeros((8, L), f32)
    hf[0, 0, pl.ds(0, 8, stride=2), :] = jnp.zeros((8, L), f32)
    ri = lax.broadcasted_iota(jnp.int32, (L, L), 0)
    ci = lax.broadcasted_iota(jnp.int32, (L, L), 1)
    sel = jnp.where(ci == R * _perm(ri & 31) + (ri >> 5), 1.0, 0.0).astype(bf16)

    wait("sk", "sd", "c")
    skt = skb[...].astype(f32)
    sdv = sdb[...].astype(f32).reshape(1, D)
    cv = cb_[...].astype(f32)
    sig = jax.nn.sigmoid(cv)
    cs = jnp.broadcast_to((cv * sig).astype(bf16), (16, D))
    one = sig[:, 0:L]

    def gate(x, deps):
        dep = jnp.concatenate(deps, axis=0).reshape(x.shape)
        return jnp.where(jnp.broadcast_to(one, x.shape) > 2.0, dep, x)

    def put(dst, j, a, xs):
        for qi in range(R):
            dst[j, a, qi] = jnp.concatenate(xs[qi], axis=1)

    zs = {}
    mod = {}

    def grp_z(j, a):
        z = [lax.dot_general(sel, ssmb[j, :, t * L:(t + 1) * L], (((1,), (1,)), ((), ())),
                             preferred_element_type=f32) for t in range(R * a, R * a + R)]
        zs[j, a] = [jnp.concatenate([z[p][32 * r:32 * (r + 1)] for p in range(R)],
                                    axis=0).astype(bf16) for r in range(R)]
        return [z[0][16 * t:16 * t + 8] for t in range(8)]

    def grp_fwd(ws, dst, j, a, dvec=None):
        t = [jnp.dot(tabs[r], ws[r], preferred_element_type=f32) for r in range(R)]
        x = [_split(v) for v in t]
        if dvec is not None:
            x[0] = (x[0][0] + dvec[None], x[0][1])
        put(dst, j, a, _radix4(x, -1))
        return [t[0][16 * s:16 * s + 8] for s in range(16)]

    def grp_k(j, a):
        return grp_fwd(zs.pop((j, a)), kpb, j, a,
                       sdv[:, j * L:(j + 1) * L] if a == 0 else None)

    def grp_u(j, a):
        uw = [uwb[j, a, r] for r in range(R)]
        return grp_fwd(uw, ub, j, a)

    def grp_i(j, a):
        ys = []
        for r in range(2 * R):
            y = jnp.dot(ginv[r], pb[j, a, r], preferred_element_type=f32)
            yb[j, pl.ds(a * C + r, L // 2, stride=2 * R), :] = y
            ys.append(y)
        return [ys[r][16 * s:16 * s + 8] for r in (0, R) for s in range(4)]

    def grp_mod(*names):
        for name in names:
            c0, c1 = WM[name]
            m = jnp.dot(cs, wmb[:, c0 * L:c1 * L], preferred_element_type=f32)
            for c in range(c0, c1):
                mod[c] = m[0:1, (c - c0) * L:(c - c0 + 1) * L]
        return []

    def modv(i, t0=0, t1=NT):
        return jnp.concatenate([mod[i * NT + n] for n in range(t0, t1)], axis=1)

    def job_kv(j, a, deps):
        lo = lambda x: lax.bitcast_convert_type(x << 16, f32)
        hi = lambda x: lax.bitcast_convert_type(x & jnp.uint32(0xFFFF0000), f32)
        n = C // 8
        kw, vw = kbs[a].bitcast(u32), vbs[a].bitcast(u32)
        ld = lambda ref, o: ref[pl.ds(4 * j + o, n, stride=WPT), :]
        k = {}
        for m in range(4):
            x = ld(kw, PAD + m)
            k[2 * m], k[2 * m + 1] = lo(x), hi(x)
        k[-3] = hi(ld(kw, PAD - WPT + 2))
        x = ld(kw, PAD - WPT + 3)
        k[-2], k[-1] = lo(x), hi(x)
        w = [skt[t:t + 1, j * L:(j + 1) * L] for t in range(KS)]
        w0 = [gate(jnp.broadcast_to(w[0], (n, L)), deps[e::2]) for e in (0, 1)]
        kv = {}
        for m in range(4):
            x = ld(vw, m)
            for ph, v in ((2 * m, lo(x)), (2 * m + 1, hi(x))):
                ks = k[ph] * w0[m % 2]
                for t in range(1, KS):
                    ks = ks + k[ph - t] * w[t]
                kv[ph] = (ks * v).reshape(n // 8, 8, L)
        for r in range(R):
            uwb[j, a, r] = jnp.concatenate([kv[r], kv[r + R]], axis=1).reshape(L, L).astype(bf16)

    def job_mac(j, us, outs, deps):
        ld = lambda ref, a: (ref[j, a, :, :, 0:8, :], ref[j, a, :, :, 8:16, :])
        lo, hi = us[0], us[-1]
        u = {a: ld(ub, a) for a in us}
        if len(deps) == 16:
            ur = jnp.concatenate([gate(u[lo][0][0:1], deps), u[lo][0][1:]], axis=0)
        else:
            ur = gate(u[lo][0], [deps[R * i + qi] for qi in range(R) for i in range(16)])
        u[lo] = (ur, u[lo][1])
        ms = sorted({a - n for a in outs for n in us if n <= a})
        k = {m: ld(kpb, m) for m in sorted(set(ms) | {m - 1 for m in ms if m > 0})}
        kp = {m: k[m] if m == 0 else (k[m][0] - k[m - 1][1], k[m][1] + k[m - 1][0]) for m in ms}
        for a in outs:
            yr, yi = ld(yp, a) if lo > 0 else (None, None)
            for n in us:
                if n > a:
                    continue
                (kr, ki), (ur, ui) = kp[a - n], u[n]
                tr = kr * ur - ki * ui
                ti = kr * ui + ki * ur
                yr = tr if yr is None else yr + tr
                yi = ti if yi is None else yi + ti
            if a > hi:
                yp[j, a] = jnp.concatenate([yr, yi], axis=2)
                continue
            ps = _radix4([(yr[qi], yi[qi]) for qi in range(R)], +1)
            for r in range(R):
                pr, pi = [p.reshape(8, 2, 8, L) for p in ps[r]]
                lr, li, hr, hi_ = pr[:, 0], pi[:, 0], pr[:, 1], pi[:, 1]
                if r % 2:
                    hr, hi_ = (hr - hi_) * RSQ2, (hr + hi_) * RSQ2
                if r < 2:
                    outs2 = (lr + hr, li + hi_), (lr - hr, li - hi_)
                else:
                    outs2 = (lr - hi_, li + hr), (lr + hi_, li - hr)
                for e in range(2):
                    pb[j, a, r + R * e] = jnp.concatenate(
                        outs2[e], axis=1).reshape(L, L).astype(bf16)

    def job_setup(_, deps):
        def hold(r, n):
            return gate(n, [deps[2 * r + s // 4] for s in range(8)])

        ginv.extend(_tables(True, hold))
        csf = cs[0:1].astype(f32)
        ccol.append(jnp.concatenate([jnp.broadcast_to(csf[:, t * L:(t + 1) * L], (L, L)).T
                                     for t in range(NT)], axis=0))

    def job_vmod(name, deps):
        c0, c1 = WM[name]
        n = D // VM
        for c in range(c0, c1):
            for i in range(VM):
                cc = ccol[0][i * n:(i + 1) * n]
                cc = jnp.concatenate([gate(cc[0:8], [deps[(c - c0) * VM + i]]), cc[8:]], axis=0)
                p = wmb[i * n:(i + 1) * n, c * L:(c + 1) * L].astype(f32) * cc
                mv[c, 8 * i:8 * i + 8, :] = jnp.sum(p.reshape(n // 8, 8, L), axis=0)
            mod[c] = jnp.sum(mv[c], axis=0, keepdims=True)

    wts = {"g": wgb, "u": wub, "d": wdb}

    def wtile(n, si, q, t):
        r, c = (FT[si][q[0]][t], DT[si][q[1]]) if n == "d" else (DT[si][q[0]], FT[si][q[1]][t])
        return wts[n][r * L:(r + 1) * L, c * L:(c + 1) * L]

    def job_wsum(n, si, t, deps):
        blk = {}
        for q in sorted({q for term in SCHEME[si] for q in term[1]}):
            x = wtile(n, si, q, t).astype(f32)
            if q in HIT[si]:
                x = x.reshape(8, 16, L)
                held = gate(x[:, 0:8], [deps[g * len(deps) // 8] for g in range(8)])
                x = jnp.concatenate([held, x[:, 8:]], axis=1).reshape(L, L)
            blk[q] = x
        sums = [term[1] for term in SCHEME[si] if len(term[1]) > 1]
        for i, coef in enumerate(sums):
            wsb["gud".index(n)][si][i, t * L:(t + 1) * L, :] = _lin(coef, blk.get).astype(bf16)

    def fast_lhs(x, tiles, si):
        get = lambda q: x[q[0]][:, tiles[q[1]][0] * L:(tiles[q[1]][-1] + 1) * L]
        return [_lin(term[0], get).astype(bf16) for term in SCHEME[si]]

    def fast_dot(a, n, si, ts, out, key, done=None):
        left = {q: sum(q in term[2] for term in SCHEME[si]) for term in SCHEME[si] for q in term[2]}
        i = 0
        for x, term in zip(a, SCHEME[si]):
            if len(term[1]) > 1:
                w = wsb["gud".index(n)][si][i, ts[0] * L:(ts[-1] + 1) * L, :]
                i += 1
            else:
                w = jnp.concatenate([wtile(n, si, *term[1], t) for t in ts], axis=0)
            p = jnp.dot(x, w, preferred_element_type=f32)
            for q, v in term[2].items():
                k = key(q)
                out[k] = (p if v > 0 else -p) if k not in out else (
                    out[k] + p if v > 0 else out[k] - p)
                left[q] -= 1
                if done is not None and not left[q]:
                    done(k)

    grp_fn = {"z": grp_z, "k": grp_k, "u": grp_u, "i": grp_i, "mod": grp_mod}
    job_fn = {"kv": job_kv, "mac": job_mac, "vmod": job_vmod, "setup": job_setup,
              "wsum": job_wsum}

    def run(groups, jobs, **kw):
        plan = _plan(groups, jobs, **kw)
        anchors, done = [], 0
        for g in groups + [None]:
            while done < len(jobs) and max(plan[done]) < len(anchors):
                job_fn[jobs[done][0]](*jobs[done][1:], [anchors[n] for n in plan[done]])
                done += 1
            if g is not None:
                anchors += grp_fn[g[0]](*g[1:])
        assert done == len(jobs)

    for waits, groups, jobs in SCHEDULE:
        wait(*waits)
        run(groups, jobs)

    n1, dep = [], None
    for r in range(0, H0, H0 // 2):
        x = qb0[r:r + H0 // 2, :].astype(f32)
        if dep is not None:
            x = jnp.concatenate([gate(x[:, 0:L], [dep]), x[:, L:]], axis=1)
        n1.append(_layernorm(x))
        dep = n1[-1][:, 0:L]
    n1 = jnp.concatenate(n1, axis=0)
    wait("mB")
    grp_mod("mB")
    sa, ca, ga = [modv(i) for i in range(3)]
    a1 = ga * (1.0 + ca)
    b1 = ga * sa

    def o_cp(i, c0, c1, r0=0, r1=TM):
        cols = pl.ds(c0, c1 - c0)
        if i is None:
            return pltpu.make_async_copy(ob0.at[:, cols], o_hbm.at[0, pl.ds(0, TM0), cols],
                                         osem.at[NB])
        base = TM0 + i * TM + r0
        if not isinstance(i, int):
            base = pl.multiple_of(base, 16)
        return pltpu.make_async_copy(ob.at[i, pl.ds(r0, r1 - r0), cols],
                                     o_hbm.at[0, pl.ds(base, r1 - r0), cols], osem.at[i])

    def prep_norm(q_ref, x1_ref, y0, r0, n, dep=None, n1=None):
        x = q_ref[r0:r0 + n, :].astype(f32)
        if dep is not None:
            x = jnp.concatenate([gate(x[:, 0:L], [dep]), x[:, L:]], axis=1)
        y = jnp.concatenate([yb[j, pl.ds(y0 + r0, n), :] for j in range(NT)], axis=1)
        x1 = x + ((_layernorm(x) if n1 is None else n1) * a1 + b1) * y
        x1_ref[r0:r0 + n, :] = x1
        return _layernorm(x1)

    n2 = [prep_norm(qb0, x1b0, 0, 0, H0, None, n1)]
    aff = []

    def prep_chain(i, r0, r1, pr):
        y0 = TM0 + i * TM
        if not isinstance(i, int):
            y0 = pl.multiple_of(y0, L)
        dep = None
        while r0 < r1:
            n = pr if (r1 - r0) % pr == 0 else pr + 8
            h2 = prep_norm(qb.at[i], x1b, y0, r0, n, dep if dep is None else dep[:n])
            h2 = h2 * aff[0] + aff[1]
            h2b[r0:r0 + n, :] = h2
            dep = h2[:, 0:L]
            r0 += n

    OC = (0, D - L, D)
    MH = HM // 2
    OP = [(0, D, 0, HM), (0, 3 * L, HM, TM), (3 * L, 4 * L, HM, TM),
          (4 * L, D, HM, HM + MH), (4 * L, D, HM + MH, TM)]

    def ffn_half(i, half, gb):
        r0 = half * HM
        mix = lambda x, y: (x, y - 0.5 * x)
        x = mix(h2b[r0:r0 + MH, :], h2b[r0 + MH:r0 + HM, :])
        a = [fast_lhs(x, [[t] for t in DT[si]], si) for si in range(2)]
        for par in range(2):
            gu = []
            for n in "gu":
                acc2 = {}
                for si in range(2):
                    for t in range(par, len(FT[si][0]), 2):
                        fast_dot(a[si], n, si, [t], acc2, lambda q: (q[0], FT[si][q[1]][t]))
                gu.append({(r, t): v + 0.5 * acc2[0, t] if r else v
                           for (r, t), v in acc2.items()})
            for t in range(par, F // L, 2):
                hf[0, t], hf[1, t] = mix(*[gu[0][r, t] * gu[1][r, t] for r in range(2)])
        x = [jnp.concatenate([hf[r, t] for t in range(F // L)], axis=1) for r in range(2)]
        o, ready, stored = {}, set(), set()

        def done(k):
            ready.add(k)
            for r, c in sorted(ready):
                if (0, c) in ready and (k == (r, c) or k == (0, c)):
                    v = o[r, c] + 0.5 * o[0, c] if r else o[r, c]
                    rows, cols = slice(r0 + r * MH, r0 + (r + 1) * MH), slice(c * L, (c + 1) * L)
                    ob[i, rows, cols] = (x1b[rows, cols] + gb[:, cols] * v).astype(bf16)
                    stored.add((rows.start, c * L))
            for op in OP:
                need = {(s, c) for s in range(op[2], op[3], MH) for c in range(op[0], op[1], L)}
                if need <= stored:
                    stored.difference_update(need)
                    o_cp(i, *op).start()

        for si in range(2):
            fast_dot(fast_lhs(x, FT[si], si), "d", si, range(len(FT[si][0])), o,
                     lambda q: (q[0], DT[si][q[1]]), done)

    acc, hcache, parts = {}, {}, {}

    def grp_g(p, n, f, half=None):
        t0, t1 = KP[p], KP[p + 1]
        if (p, half) not in hcache:
            if len(n2) == 1 and half != 0:
                n2.append(prep_norm(qb0, x1b0, 0, H0, TM0 - H0))
            x = jnp.concatenate(n2, axis=0) if half is None else n2[half]
            hcache[p, half] = (x[:, t0 * L:t1 * L] * (1.0 + modv(4, t0, t1))
                               + modv(3, t0, t1)).astype(bf16)
        rows = {None: slice(0, TM0), 0: slice(0, H0), 1: slice(H0, TM0)}[half]
        cols = slice(f * 4 * L, (f + 1) * 4 * L)
        d = jnp.dot(hcache[p, half], (wgb if n == "g" else wub)[t0 * L:t1 * L, cols],
                    preferred_element_type=f32)
        ref = gub.at["gu".index(n), rows, cols]
        if p < len(KP) - 2:
            ref[...] = d if p == 0 else ref[...] + d
        elif n == "g":
            acc[f] = ref[...] + d
        else:
            hb[:, cols] = (acc.pop(f) * (ref[...] + d)).astype(bf16)
        return [d[s:s + 8, c * L:(c + 1) * L] for c in range(0, 4, 4 // (t1 - t0))
                for s in range(0, d.shape[0], 16)]

    def grp_d(n, f):
        c = slice(n * L, (n + 1) * L)
        k = slice(f * 4 * L, (f + 1) * 4 * L)
        d = jnp.dot(hb[:, k], wdb[k, c], preferred_element_type=f32)
        parts[n] = d if f == 0 else parts[n] + d
        if f == 2:
            ob0[:, c] = (x1b0[:, c] + mod[5 * NT + n] * parts.pop(n)).astype(bf16)
            if (n + 1) * L in OC:
                o_cp(None, OC[OC.index((n + 1) * L) - 1], (n + 1) * L).start()
        return [d[s:s + 8] for s in range(0, TM0, 16)]

    grp_fn.update(g=grp_g, d=grp_d)
    for waits, rows, groups, jobs in FIRST:
        wait(*waits)
        for n in parts:
            parts[n] = dpart[:, n * L:(n + 1) * L]
        run(groups, jobs, lead=LEAD, floor=(0.0, 0.0))
        if rows:
            aff += [1.0 + modv(4), modv(3)]
            prep_chain(0, *rows, PR)
        for n in parts:
            dpart[:, n * L:(n + 1) * L] = parts[n]
    gb = modv(5)
    wait("q1c", *[f"q{i + 1}" for i in range(1, NB)])

    def ffn(i, carry):
        prep_chain(i, HM, TM, PL)
        ffn_half(i, 0, gb)
        prep_chain(jnp.minimum(i + 1, NB - 1), 0, HM, PL)
        ffn_half(i, 1, gb)
        return carry

    lax.fori_loop(0, NB, ffn, 0)

    for c0, c1 in zip(OC[:-1], OC[1:]):
        o_cp(None, c0, c1).wait()
    for i in range(NB):
        for op in OP:
            o_cp(i, *op).wait()


@jax.jit
def pallas_adaLN_cond__ssm_conv_h3__glu_gated_bilinear__prompt_kernel(
    A_q: jax.Array,
    A_k: jax.Array,
    A_v: jax.Array,
    A_shift_k: jax.Array,
    A_ssm_k: jax.Array,
    A_ssm_D: jax.Array,
    B_x: jax.Array,
    B_w_gate: jax.Array,
    B_w_up: jax.Array,
    B_w_down: jax.Array,
    c: jax.Array,
    w_mod: jax.Array,
):
    del B_x
    tiles = lambda x: x.reshape(S // 8, 8, NT, L).transpose(0, 2, 1, 3).reshape(S * NT, L)
    any_spec = pl.BlockSpec(memory_space=pl.ANY)
    return pl.pallas_call(
        _kernel,
        in_specs=[any_spec] * 11,
        out_specs=any_spec,
        out_shape=jax.ShapeDtypeStruct((1, S, D), bf16),
        scratch_shapes=[
            pltpu.VMEM((TM0, D), bf16),
            pltpu.VMEM((NB, TM, D), bf16),
            [pltpu.VMEM((4 * PAD + C * NT, L), bf16)] * NC,
            [pltpu.VMEM((2 * PAD + C * NT, L), bf16)] * NC,
            pltpu.VMEM((NT, L, S), bf16),
            pltpu.VMEM((D, F), bf16),
            pltpu.VMEM((D, F), bf16),
            pltpu.VMEM((F, D), bf16),
            [[pltpu.VMEM((NSUM[si], len(FT[si][0]) * L, L), bf16) for si in range(2)]] * 3,
            pltpu.VMEM((D, 6 * D), bf16),
            pltpu.VMEM((NT, NC, R, L, L), bf16),
            pltpu.VMEM((NT, NC, R, 16, 16, L), f32),
            pltpu.VMEM((NT, NC, R, 16, 16, L), f32),
            pltpu.VMEM((NT, NC, R, 16, 16, L), f32),
            pltpu.VMEM((NT, NC, 2 * R, L, L), bf16),
            pltpu.VMEM((NT, S + 32, L), f32),
            pltpu.VMEM((TM0, D), f32),
            pltpu.VMEM((TM, D), f32),
            pltpu.VMEM((TM, D), f32),
            pltpu.VMEM((2, F // L, HM // 2, L), f32),
            pltpu.VMEM((2, TM0, F), f32),
            pltpu.VMEM((TM0, D), f32),
            pltpu.VMEM((TM0, F), bf16),
            pltpu.VMEM((TM0, D), bf16),
            pltpu.VMEM((NB, TM, D), bf16),
            pltpu.VMEM((32, 8 * VM, L), f32),
            pltpu.VMEM((KS, D), bf16),
            pltpu.VMEM((D,), bf16),
            pltpu.VMEM((1, D), bf16),
            pltpu.SemaphoreType.DMA((len(DMA_ORDER),)),
            pltpu.SemaphoreType.DMA((NB + 1,)),
        ],
        compiler_params=pltpu.CompilerParams(
            vmem_limit_bytes=120 * 1024 * 1024,
            disable_bounds_checks=True, disable_semaphore_checks=True),
        name="adaln_h3_glu",
    )(A_q, tiles(A_k), tiles(A_v), A_shift_k.T, A_ssm_k, A_ssm_D,
      B_w_gate, B_w_up, B_w_down, c, w_mod)
```

```python
import jax
import jax.numpy as jnp
from jax import lax
import jax.experimental.pallas as pl
import jax.experimental.pallas.tpu as pltpu

S = 2048
D = 640
F = 1536
KS = 4
L = 128
NT = D // L
R = 4
C = R * L
NC = S // C
EPS = 1e-5
RSQ2 = 0.7071067811865476

WPT = 4 * NT
PAD = 32

TM0 = 512
H0 = 352
TM = 512
NB = (S - TM0) // TM
HM = 256
PL = 16
PR = 24
WM = {"mA": (0, 12), "c0": (20, 21), "mB": (12, 16), "s1": (16, 17), "c1": (21, 22),
      "s2": (17, 19), "c2": (22, 24), "s4": (19, 20), "c4": (24, 25), "mG": (25, 30)}
VM = 5
RATE = 1.05
LEAD = 24
FREE = {"i": 56, "z": 56, "k": 47, "u": 46}
FREE_FFN = {"i": 20, "u": 36, "f": 36, "g": 50}

f32 = jnp.float32
bf16 = jnp.bfloat16
u32 = jnp.uint32


def _cos_turns(t):
    x = jnp.abs(t - jnp.floor(t) - 0.5) - 0.25
    x2 = x * x
    return x * (6.283164024 + x2 * (-41.33713150 + x2 * (81.34038544 + x2 * -70.98993683)))


def _tables(inverse, hold=None):
    shape = (L // 2, L) if inverse else (2 * L, L)
    rho = lax.broadcasted_iota(jnp.int32, shape, 1 if inverse else 0)
    j = lax.broadcasted_iota(jnp.int32, shape, 0 if inverse else 1)
    if inverse:
        g, rad = 8 * (rho >> 4) + (rho & 7), 2 * R
    else:
        g, rad, j = 8 * (rho >> 5) + (rho & 7) + 64 * ((rho >> 4) & 1), R, _perm(j)
    a = (4 * g + 1).astype(f32) * (1.0 / (4 * C))
    off = ((rho >> 3) & 1).astype(f32) * 0.25
    ns = [(rad * j + r).astype(f32) for r in range(rad)]
    if hold is not None:
        ns = [hold(r, n) for r, n in enumerate(ns)]
    ts = [_cos_turns(a * n + off) for n in ns]
    return [(t * (1.0 / C) if inverse else t).astype(bf16) for t in ts]


def _perm(c):
    return 16 * (c >> 4) + 2 * (c & 7) + ((c >> 3) & 1)


def _layernorm(x):
    m = jnp.mean(x, axis=-1, keepdims=True)
    xc = x - m
    v = jnp.mean(xc * xc, axis=-1, keepdims=True)
    return xc * lax.rsqrt(v + EPS)


def _split(t):
    t = t.reshape(16, 16, L)
    return t[:, :8, :], t[:, 8:, :]


def _radix4(x, sgn):
    (ar, ai), (br, bi), (cr, ci), (dr, di) = x
    s0r, s0i, d0r, d0i = ar + cr, ai + ci, ar - cr, ai - ci
    s1r, s1i, d1r, d1i = br + dr, bi + di, br - dr, bi - di
    o0 = (s0r + s1r, s0i + s1i)
    o2 = (s0r - s1r, s0i - s1i)
    pl_ = (d0r - d1i, d0i + d1r)
    mi_ = (d0r + d1i, d0i - d1r)
    return [o0, pl_, o2, mi_] if sgn > 0 else [o0, mi_, o2, pl_]


S222 = (
    ({(1, 1): 1, (0, 0): -1}, {(0, 0): 1, (1, 1): 1}, {(0, 0): -1, (1, 1): 1}),
    ({(0, 1): 1, (1, 1): 1}, {(1, 0): 1, (1, 1): 1}, {(0, 0): 1}),
    ({(0, 0): 1, (0, 1): 1}, {(1, 1): 1}, {(0, 0): -1, (0, 1): 1}),
    ({(1, 1): 1}, {(1, 0): 1, (0, 0): -1}, {(0, 0): -1, (1, 0): 1}),
    ({(1, 0): 1, (1, 1): 1}, {(0, 0): 1}, {(1, 0): 1, (1, 1): -1}),
    ({(0, 0): 1}, {(0, 1): 1, (1, 1): -1}, {(0, 1): 1, (1, 1): -1}),
    ({(0, 0): 1, (1, 0): 1}, {(0, 0): 1, (0, 1): 1}, {(1, 1): 1}),
)
S233 = (
    ({(0, 0): 1, (1, 0): 1, (1, 2): -1}, {(0, 0): 1, (2, 2): -1},
     {(0, 0): 1, (0, 2): -1, (1, 2): 1}),
    ({(1, 0): 1, (1, 2): -1}, {(0, 0): 1}, {(0, 0): -1, (0, 2): 1, (1, 0): 1, (1, 2): -1}),
    ({(0, 0): 1, (1, 0): 1, (1, 2): -1, (0, 2): -1}, {(2, 2): 1}, {(0, 0): 1, (0, 2): -1}),
    ({(0, 2): 1}, {(1, 0): 1, (2, 0): 1, (2, 2): 1}, {(0, 0): 1}),
    ({(0, 1): 1, (0, 2): -1, (1, 1): 1}, {(1, 0): 1, (2, 1): 1},
     {(0, 1): -1, (1, 0): 1, (1, 1): 1}),
    ({(0, 1): 1, (0, 2): -1}, {(1, 0): 1}, {(0, 0): 1, (0, 1): 1, (1, 0): -1, (1, 1): -1}),
    ({(0, 1): 1, (0, 2): -1, (1, 1): 1, (1, 2): -1}, {(2, 1): 1}, {(1, 0): -1, (1, 1): -1}),
    ({(1, 2): 1}, {(0, 0): 1, (2, 0): 1, (2, 1): -1}, {(1, 0): 1}),
    ({(0, 0): 1, (1, 1): 1}, {(0, 1): 1, (1, 2): -1}, {(0, 1): 1, (1, 2): -1}),
    ({(1, 0): 1, (1, 1): -1}, {(0, 1): 1}, {(1, 1): 1, (1, 2): -1}),
    ({(0, 0): 1, (0, 1): -1}, {(1, 2): 1}, {(0, 1): 1, (0, 2): -1}),
    ({(0, 0): 1}, {(0, 0): 1, (0, 2): 1, (1, 2): 1}, {(0, 2): 1, (1, 2): -1}),
    ({(0, 0): 1, (1, 0): 1}, {(0, 1): 1, (0, 2): 1, (2, 2): 1}, {(1, 2): 1}),
    ({(1, 1): 1}, {(0, 1): 1, (1, 1): 1, (1, 0): -1}, {(0, 1): -1, (1, 1): 1}),
    ({(0, 1): 1, (1, 1): 1}, {(1, 1): 1, (1, 2): 1, (2, 1): 1}, {(0, 1): 1}),
)
SCHEME = (S233, S222)
HIT = (((0, 0), (0, 1), (1, 0), (2, 1)), ((0, 0), (1, 1)))
NSUM = [sum(len(t[1]) > 1 for t in s) for s in SCHEME]
DT = ((0, 1, 2), (3, 4))
FT = ([range(0, 4), range(4, 8), range(8, 12)], [range(0, 6), range(6, 12)])


def _lin(coef, get):
    r = None
    for q, v in coef.items():
        x = get(q)
        r = (x if v > 0 else -x) if r is None else (r + x if v > 0 else r - x)
    return r


T = range(NT)
_z = lambda j: [("z", j, a) for a in range(NC)]
_k = lambda j, al: [("k", j, a) for a in al]
_u = lambda a: [("u", j, a) for j in T]
_iv = lambda jl, al: [("i", j, a) for j in jl for a in al]
_kv = lambda a: [("kv", j, a) for j in T]
_m = lambda jl, us, outs: [("mac", j, us, outs) for j in jl]

A3 = (0, 1, 2)
SCHEDULE = [
    (["ssm0"], _z(0) + _k(0, range(NC)), [("setup", None)]),
    (["ssm1"], _z(1) + _k(1, range(NC)), []),
    (["ssm2"], _z(2) + _k(2, [0, 1]), []),
    (["k0", "v0"], _k(2, [2, 3]) + _u(0), _kv(0) + _m([0], (0,), (0,))),
    (["ssm3"], _iv([0], [0]) + _z(3) + _k(3, [0, 1]), _m([1, 2], (0,), A3)),
    (["k1", "v1"], _k(3, [2, 3]) + _u(1), _kv(1) + _m([3], (0,), (0,))),
    (["ssm4"], _iv([1], [0]) + _z(4) + _k(4, range(NC)),
     _m([0], (0, 1), (1, 2)) + _m([1, 2], (1,), (1, 2))),
    (["k2", "v2"], _iv([2, 3], [0]) + _iv([0], [1]) + _u(2) + _iv([1, 2], [1]) + _iv([4], [0, 1])
     + _iv([0, 1, 2, 4], [2]),
     _kv(2) + _m([4], (0, 1), A3) + _m([0, 1, 2, 4], (2,), (2,)) + _m([3], A3, (1, 2))),
    (["q0", "mA", "c0"], [("mod", "mA", "c0")] + _iv([3], [1, 2]), []),
]
_g = lambda p: [("g", p, n, f) for f in range(3) for n in "gu"]
_v = lambda *names: [("vmod", n) for n in names]
_w = lambda names, si: [("wsum", n, si, t) for n in names for t in range(len(FT[si][0]))]
_f = lambda si, *ids: [("f", si, i) for i in ids]
FIRST = [
    (["wg0", "qh"], None, [("g", 0, "g", f, h) for h in (0, 1) for f in range(3)], []),
    (["wu0", "s1", "c1"], None, [("g", 0, "u", f) for f in range(3)],
     _v("s1", "c1") + _m([0], A3, (3,))),
    (["wg1", "wu1"], None, _g(1)[:-1], _m([1, 2, 3], A3, (3,))),
    (["wg2", "wu2", "s2", "c2"], None, _g(1)[-1:] + _g(2),
     _v("s2", "c2") + _m([4], A3, (3,)) + _w("gu", 0)),
    (["wg3", "wu3", "wg4", "wu4", "s4", "c4", "q1"], (0, HM), _g(3) + _g(4),
     _v("s4", "c4") + _w("gu", 1)),
    (["wd", "k3", "v3"], None, _f(0, 1, 2, 5, 6, 9, 10) + _f(1, 2, 4) + _u(3) + _f(0, 0, 4, 8),
     _w("d", 0) + _kv(3) + _w("d", 1) + _m([0], (3,), (3,))),
    (["mG"], None, _f(0, 3, 11, 13, 7, 12, 14) + _f(1, 0, 1, 3, 5, 6) + _iv(T, [3]),
     _v("mG") + _m([1, 2, 3, 4], (3,), (3,))),
]

DMA_ORDER = (["sk", "sd", "c", "ssm0", "ssm1", "ssm2", "k0", "v0", "ssm3", "k1", "v1", "ssm4",
              "k2", "v2", "q0", "c0", "mA", "mB", "wg0", "qh", "wu0", "s1", "c1", "wg1", "wu1",
              "s2", "c2", "wg2", "wu2", "s4", "c4", "wg3", "wu3", "wg4", "wu4", "q1", "wd", "k3",
              "v3", "mG", "q1c"] + [f"q{i + 1}" for i in range(1, NB)])


def _costs(job):
    if job[0] == "kv":
        return [48, 42] * (C // 64)
    if job[0] == "wsum":
        return [61] * 8 if job[2] == 0 else [50] * 4
    if job[0] == "setup":
        return [100] * (4 * R)
    if job[0] == "vmod":
        return [3 * D // VM // 8] * (VM * (WM[job[1]][1] - WM[job[1]][0]))
    us, outs = job[2], job[3]
    pairs = [(a, n) for a in outs for n in us if n <= a]
    mac = (2 * len({a - n for a, n in pairs if a > n}) + 8 * len(pairs)
           - (2 * len(outs) if us[0] == 0 else 0))
    fin = sum(a <= us[-1] for a in outs)
    if mac < 12 and outs[-1] <= us[-1] < NC - 1:
        return [1 + R * mac + 16 * fin, 1 + R * mac + 48 * fin] * 8
    return ([1 + mac] * 3 + [1 + mac + 16 * fin] + [1 + mac] * 3 + [1 + mac + 48 * fin]) * 8


def _plan(groups, jobs, lead=0, floor=(1.0, 0.8)):
    free = FREE_FFN if lead else FREE
    nstep = {"i": 8, "z": 8, "k": 16, "u": 16, "mod": 0, "g": TM0 // 16}
    steps = lambda g: (16, 24)[g[1]] if g[0] == "f" else nstep[g[0]]
    slots = [free[g[0]] for g in groups for _ in range(steps(g))]
    lo, hi = [], []
    for job in jobs:
        begin, limit, first = 0, len(slots), 0
        for g in groups:
            kind = (g[0], job[0])
            if (kind == ("u", "kv") and g[1:] == job[1:]
                    or kind == ("i", "mac") and g[1] == job[1] and g[2] in job[3]
                    and g[2] <= job[2][-1]):
                limit = min(limit, first - lead)
            if (kind == ("f", "wsum") and g[1] == job[2] and len(SCHEME[g[1]][g[2]][1]) > 1
                    or kind == ("f", "vmod") and g[1:] == (0, 7)):
                limit = min(limit, first - lead)
            if kind == ("g", "vmod") and job[1][1] == str(g[1]):
                limit = min(limit, first - 11)
            first += steps(g)
            if kind == ("u", "mac") and g[1] == job[1] and g[2] in job[2]:
                begin = first
        lo.append(begin)
        hi.append(limit)
    plan, credit, n = [], (slots or [0])[0], 0
    for k, job in enumerate(jobs):
        if n < lo[k]:
            n, credit = lo[k], min(credit, 0) + slots[lo[k]]
        work = [sum(_costs(j)) for j in jobs]
        if lead:
            rate = max(RATE * sum(work[k:m + 1]) / max(sum(slots[n:hi[m]]), 1)
                       for m in range(k, len(jobs)))
        else:
            rate = RATE * sum(work[k:]) / sum(slots[n:])
        rate = max(rate, floor[0] if job[0] == "kv" else floor[1])
        idx = []
        for c in _costs(job):
            while credit <= 0 and n + 1 < hi[k]:
                n += 1
                credit += slots[n] * rate
            credit -= c
            idx.append(n)
        assert n < hi[k]
        plan.append(idx)
    return plan


def _kernel(q_hbm, k_hbm, v_hbm, sk_hbm, ssm_hbm, sd_hbm, wg_hbm, wu_hbm, wd_hbm,
            c_hbm, wm_hbm, o_hbm,
            qb0, qb, kbs, vbs, ssmb, wgb, wub, wdb, wsb, wmb, uwb, ub, kpb, yp, pb, yb,
            x1b0, x1b, h2b, hf, gub, dpart, hf0, ob0, ob, mv, skb, sdb, cb_, sem, osem):
    cps = {"sk": (sk_hbm, skb), "sd": (sd_hbm, sdb), "c": (c_hbm, cb_), "wd": (wd_hbm, wdb)}
    for j in range(NT):
        cps[f"ssm{j}"] = (ssm_hbm.at[pl.ds(j * L, L), :], ssmb.at[j])
    for a in range(NC):
        n, h = C * NT, 2 * PAD
        if a == 0:
            cps["k0"] = (k_hbm.at[pl.ds(0, n), :], kbs[0].at[pl.ds(h, n), :])
        else:
            e = 48
            cps[f"k{a}"] = (k_hbm.at[pl.ds(a * n - e, n + e), :],
                            kbs[a].at[pl.ds(h - e, n + e), :])
        cps[f"v{a}"] = (v_hbm.at[pl.ds(a * n, n), :], vbs[a].at[pl.ds(0, n), :])
    for n, (c0, c1) in WM.items():
        cols = pl.ds(c0 * L, (c1 - c0) * L)
        cps[n] = (wm_hbm.at[:, cols], wmb.at[:, cols])
    cps["q0"] = (q_hbm.at[0, pl.ds(0, H0), :], qb0.at[pl.ds(0, H0), :])
    cps["qh"] = (q_hbm.at[0, pl.ds(H0, TM0 - H0), :], qb0.at[pl.ds(H0, TM0 - H0), :])
    cps["q1"] = (q_hbm.at[0, pl.ds(TM0, HM), :], qb.at[0, pl.ds(0, HM), :])
    cps["q1c"] = (q_hbm.at[0, pl.ds(TM0 + HM, TM - HM), :], qb.at[0, pl.ds(HM, TM - HM), :])
    for i in range(1, NB):
        cps[f"q{i + 1}"] = (q_hbm.at[0, pl.ds(TM0 + i * TM, TM), :], qb.at[i])
    for p in range(NT):
        rows = pl.ds(p * L, L)
        cps[f"wg{p}"] = (wg_hbm.at[rows, :], wgb.at[rows, :])
        cps[f"wu{p}"] = (wu_hbm.at[rows, :], wub.at[rows, :])
    assert sorted(cps) == sorted(DMA_ORDER)

    def cp(name):
        src, dst = cps[name]
        return pltpu.make_async_copy(src, dst, sem.at[DMA_ORDER.index(name)])

    def wait(*names):
        for n in names:
            cp(n).wait()

    kbs[0][0:2 * PAD, :] = jnp.zeros((2 * PAD, L), bf16)
    for n in DMA_ORDER:
        cp(n).start()

    tabs, ginv, ccol = _tables(False), [], []
    for ref in (ub, kpb, yp):
        ref[0, 0, 0, 0, pl.ds(0, 8, stride=2), :] = jnp.zeros((8, L), f32)
    mv[0, pl.ds(0, 8, stride=2), :] = jnp.zeros((8, L), f32)
    for ref in (hf, hf0):
        ref[0, 0, pl.ds(0, 8, stride=2), :] = jnp.zeros((8, L), f32)
    ri = lax.broadcasted_iota(jnp.int32, (L, L), 0)
    ci = lax.broadcasted_iota(jnp.int32, (L, L), 1)
    sel = jnp.where(ci == R * _perm(ri & 31) + (ri >> 5), 1.0, 0.0).astype(bf16)

    wait("sk", "sd", "c")
    skt = skb[...].astype(f32)
    sdv = sdb[...].astype(f32).reshape(1, D)
    cv = cb_[...].astype(f32)
    sig = jax.nn.sigmoid(cv)
    cs = jnp.broadcast_to((cv * sig).astype(bf16), (16, D))
    one = sig[:, 0:L]

    def gate(x, deps):
        dep = jnp.concatenate(deps, axis=0).reshape(x.shape)
        return jnp.where(jnp.broadcast_to(one, x.shape) > 2.0, dep, x)

    def put(dst, j, a, xs):
        for qi in range(R):
            dst[j, a, qi] = jnp.concatenate(xs[qi], axis=1)

    zs = {}
    mod = {}

    def grp_z(j, a):
        z = [lax.dot_general(sel, ssmb[j, :, t * L:(t + 1) * L], (((1,), (1,)), ((), ())),
                             preferred_element_type=f32) for t in range(R * a, R * a + R)]
        zs[j, a] = [jnp.concatenate([z[p][32 * r:32 * (r + 1)] for p in range(R)],
                                    axis=0).astype(bf16) for r in range(R)]
        return [z[0][16 * t:16 * t + 8] for t in range(8)]

    def grp_fwd(ws, dst, j, a, dvec=None):
        t = [jnp.dot(tabs[r], ws[r], preferred_element_type=f32) for r in range(R)]
        x = [_split(v) for v in t]
        if dvec is not None:
            x[0] = (x[0][0] + dvec[None], x[0][1])
        put(dst, j, a, _radix4(x, -1))
        return [t[0][16 * s:16 * s + 8] for s in range(16)]

    def grp_k(j, a):
        return grp_fwd(zs.pop((j, a)), kpb, j, a,
                       sdv[:, j * L:(j + 1) * L] if a == 0 else None)

    def grp_u(j, a):
        uw = [uwb[j, a, r] for r in range(R)]
        return grp_fwd(uw, ub, j, a)

    def grp_i(j, a):
        ys = []
        for r in range(2 * R):
            y = jnp.dot(ginv[r], pb[j, a, r], preferred_element_type=f32)
            yb[j, pl.ds(a * C + r, L // 2, stride=2 * R), :] = y
            ys.append(y)
        return [ys[r][16 * s:16 * s + 8] for r in (0, R) for s in range(4)]

    def grp_mod(*names):
        for name in names:
            c0, c1 = WM[name]
            m = jnp.dot(cs, wmb[:, c0 * L:c1 * L], preferred_element_type=f32)
            for c in range(c0, c1):
                mod[c] = m[0:1, (c - c0) * L:(c - c0 + 1) * L]
        return []

    def modv(i):
        return jnp.concatenate([mod[i * NT + n] for n in range(NT)], axis=1)

    def job_kv(j, a, deps):
        lo = lambda x: lax.bitcast_convert_type(x << 16, f32)
        hi = lambda x: lax.bitcast_convert_type(x & jnp.uint32(0xFFFF0000), f32)
        n = C // 8
        kw, vw = kbs[a].bitcast(u32), vbs[a].bitcast(u32)
        ld = lambda ref, o: ref[pl.ds(4 * j + o, n, stride=WPT), :]
        k = {}
        for m in range(4):
            x = ld(kw, PAD + m)
            k[2 * m], k[2 * m + 1] = lo(x), hi(x)
        k[-3] = hi(ld(kw, PAD - WPT + 2))
        x = ld(kw, PAD - WPT + 3)
        k[-2], k[-1] = lo(x), hi(x)
        w = [skt[t:t + 1, j * L:(j + 1) * L] for t in range(KS)]
        w0 = [gate(jnp.broadcast_to(w[0], (n, L)), deps[e::2]) for e in (0, 1)]
        kv = {}
        for m in range(4):
            x = ld(vw, m)
            for ph, v in ((2 * m, lo(x)), (2 * m + 1, hi(x))):
                ks = k[ph] * w0[m % 2]
                for t in range(1, KS):
                    ks = ks + k[ph - t] * w[t]
                kv[ph] = (ks * v).reshape(n // 8, 8, L)
        for r in range(R):
            uwb[j, a, r] = jnp.concatenate([kv[r], kv[r + R]], axis=1).reshape(L, L).astype(bf16)

    def job_mac(j, us, outs, deps):
        ld = lambda ref, a: (ref[j, a, :, :, 0:8, :], ref[j, a, :, :, 8:16, :])
        lo, hi = us[0], us[-1]
        u = {a: ld(ub, a) for a in us}
        if len(deps) == 16:
            ur = jnp.concatenate([gate(u[lo][0][0:1], deps), u[lo][0][1:]], axis=0)
        else:
            ur = gate(u[lo][0], [deps[R * i + qi] for qi in range(R) for i in range(16)])
        u[lo] = (ur, u[lo][1])
        ms = sorted({a - n for a in outs for n in us if n <= a})
        k = {m: ld(kpb, m) for m in sorted(set(ms) | {m - 1 for m in ms if m > 0})}
        kp = {m: k[m] if m == 0 else (k[m][0] - k[m - 1][1], k[m][1] + k[m - 1][0]) for m in ms}
        for a in outs:
            yr, yi = ld(yp, a) if lo > 0 else (None, None)
            for n in us:
                if n > a:
                    continue
                (kr, ki), (ur, ui) = kp[a - n], u[n]
                tr = kr * ur - ki * ui
                ti = kr * ui + ki * ur
                yr = tr if yr is None else yr + tr
                yi = ti if yi is None else yi + ti
            if a > hi:
                yp[j, a] = jnp.concatenate([yr, yi], axis=2)
                continue
            ps = _radix4([(yr[qi], yi[qi]) for qi in range(R)], +1)
            for r in range(R):
                pr, pi = [p.reshape(8, 2, 8, L) for p in ps[r]]
                lr, li, hr, hi_ = pr[:, 0], pi[:, 0], pr[:, 1], pi[:, 1]
                if r % 2:
                    hr, hi_ = (hr - hi_) * RSQ2, (hr + hi_) * RSQ2
                if r < 2:
                    outs2 = (lr + hr, li + hi_), (lr - hr, li - hi_)
                else:
                    outs2 = (lr - hi_, li + hr), (lr + hi_, li - hr)
                for e in range(2):
                    pb[j, a, r + R * e] = jnp.concatenate(
                        outs2[e], axis=1).reshape(L, L).astype(bf16)

    def job_setup(_, deps):
        def hold(r, n):
            return gate(n, [deps[2 * r + s // 4] for s in range(8)])

        ginv.extend(_tables(True, hold))
        csf = cs[0:1].astype(f32)
        ccol.append(jnp.concatenate([jnp.broadcast_to(csf[:, t * L:(t + 1) * L], (L, L)).T
                                     for t in range(NT)], axis=0))

    def job_vmod(name, deps):
        c0, c1 = WM[name]
        n = D // VM
        for c in range(c0, c1):
            for i in range(VM):
                cc = ccol[0][i * n:(i + 1) * n]
                cc = jnp.concatenate([gate(cc[0:8], [deps[(c - c0) * VM + i]]), cc[8:]], axis=0)
                p = wmb[i * n:(i + 1) * n, c * L:(c + 1) * L].astype(f32) * cc
                mv[c, 8 * i:8 * i + 8, :] = jnp.sum(p.reshape(n // 8, 8, L), axis=0)
            mod[c] = jnp.sum(mv[c], axis=0, keepdims=True)

    wts = {"g": wgb, "u": wub, "d": wdb}

    def wtile(n, si, q, t):
        r, c = (FT[si][q[0]][t], DT[si][q[1]]) if n == "d" else (DT[si][q[0]], FT[si][q[1]][t])
        return wts[n][r * L:(r + 1) * L, c * L:(c + 1) * L]

    def job_wsum(n, si, t, deps):
        blk = {}
        for q in sorted({q for term in SCHEME[si] for q in term[1]}):
            x = wtile(n, si, q, t).astype(f32)
            if q in HIT[si]:
                x = x.reshape(8, 16, L)
                held = gate(x[:, 0:8], [deps[g * len(deps) // 8] for g in range(8)])
                x = jnp.concatenate([held, x[:, 8:]], axis=1).reshape(L, L)
            blk[q] = x
        sums = [term[1] for term in SCHEME[si] if len(term[1]) > 1]
        for i, coef in enumerate(sums):
            wsb["gud".index(n)][si][i, t * L:(t + 1) * L, :] = _lin(coef, blk.get).astype(bf16)

    def fast_lhs(x, tiles, si):
        get = lambda q: x[q[0]][:, tiles[q[1]][0] * L:(tiles[q[1]][-1] + 1) * L]
        return [_lin(term[0], get).astype(bf16) for term in SCHEME[si]]

    def fast_dot(a, n, si, ts, out, key, done=None):
        left = {q: sum(q in term[2] for term in SCHEME[si]) for term in SCHEME[si] for q in term[2]}
        i = 0
        for x, term in zip(a, SCHEME[si]):
            if len(term[1]) > 1:
                w = wsb["gud".index(n)][si][i, ts[0] * L:(ts[-1] + 1) * L, :]
                i += 1
            else:
                w = jnp.concatenate([wtile(n, si, *term[1], t) for t in ts], axis=0)
            p = jnp.dot(x, w, preferred_element_type=f32)
            for q, v in term[2].items():
                k = key(q)
                out[k] = (p if v > 0 else -p) if k not in out else (
                    out[k] + p if v > 0 else out[k] - p)
                left[q] -= 1
                if done is not None and not left[q]:
                    done(k)

    grp_fn = {"z": grp_z, "k": grp_k, "u": grp_u, "i": grp_i, "mod": grp_mod}
    job_fn = {"kv": job_kv, "mac": job_mac, "vmod": job_vmod, "setup": job_setup,
              "wsum": job_wsum}

    def run(groups, jobs, **kw):
        plan = _plan(groups, jobs, **kw)
        anchors, done = [], 0
        for g in groups + [None]:
            while done < len(jobs) and max(plan[done]) < len(anchors):
                job_fn[jobs[done][0]](*jobs[done][1:], [anchors[n] for n in plan[done]])
                done += 1
            if g is not None:
                anchors += grp_fn[g[0]](*g[1:])
        assert done == len(jobs)

    for waits, groups, jobs in SCHEDULE:
        wait(*waits)
        run(groups, jobs)

    n1, dep = [], None
    for r in range(0, H0, H0 // 2):
        x = qb0[r:r + H0 // 2, :].astype(f32)
        if dep is not None:
            x = jnp.concatenate([gate(x[:, 0:L], [dep]), x[:, L:]], axis=1)
        n1.append(_layernorm(x))
        dep = n1[-1][:, 0:L]
    n1 = jnp.concatenate(n1, axis=0)
    wait("mB")
    grp_mod("mB")
    sa, ca, ga = [modv(i) for i in range(3)]
    a1 = ga * (1.0 + ca)
    b1 = ga * sa

    def o_cp(i, c0, c1, r0=0, r1=TM):
        cols = pl.ds(c0, c1 - c0)
        if i is None:
            return pltpu.make_async_copy(ob0.at[:, cols], o_hbm.at[0, pl.ds(0, TM0), cols],
                                         osem.at[NB])
        base = TM0 + i * TM + r0
        if not isinstance(i, int):
            base = pl.multiple_of(base, 16)
        return pltpu.make_async_copy(ob.at[i, pl.ds(r0, r1 - r0), cols],
                                     o_hbm.at[0, pl.ds(base, r1 - r0), cols], osem.at[i])

    def prep_norm(q_ref, x1_ref, y0, r0, n, dep=None, n1=None):
        x = q_ref[r0:r0 + n, :].astype(f32)
        if dep is not None:
            x = jnp.concatenate([gate(x[:, 0:L], [dep]), x[:, L:]], axis=1)
        y = jnp.concatenate([yb[j, pl.ds(y0 + r0, n), :] for j in range(NT)], axis=1)
        x1 = x + ((_layernorm(x) if n1 is None else n1) * a1 + b1) * y
        x1_ref[r0:r0 + n, :] = x1
        return _layernorm(x1)

    n2 = [prep_norm(qb0, x1b0, 0, 0, H0, None, n1)]
    aff = []

    def prep_chain(i, r0, r1, pr):
        y0 = TM0 + i * TM
        if not isinstance(i, int):
            y0 = pl.multiple_of(y0, L)
        dep = None
        while r0 < r1:
            n = pr if (r1 - r0) % pr == 0 else pr + 8
            h2 = prep_norm(qb.at[i], x1b, y0, r0, n, dep if dep is None else dep[:n])
            h2 = h2 * aff[0] + aff[1]
            h2b[r0:r0 + n, :] = h2
            dep = h2[:, 0:L]
            r0 += n

    OC = (0, D)
    MH = HM // 2
    OP = [(0, D, 0, HM), (0, 3 * L, HM, TM), (3 * L, 4 * L, HM, TM),
          (4 * L, D, HM, HM + MH), (4 * L, D, HM + MH, TM)]

    def ffn_half(i, half, gb):
        r0 = half * HM
        mix = lambda x, y: (x, y - 0.5 * x)
        x = mix(h2b[r0:r0 + MH, :], h2b[r0 + MH:r0 + HM, :])
        a = [fast_lhs(x, [[t] for t in DT[si]], si) for si in range(2)]
        for par in range(2):
            gu = []
            for n in "gu":
                acc2 = {}
                for si in range(2):
                    for t in range(par, len(FT[si][0]), 2):
                        fast_dot(a[si], n, si, [t], acc2, lambda q: (q[0], FT[si][q[1]][t]))
                gu.append({(r, t): v + 0.5 * acc2[0, t] if r else v
                           for (r, t), v in acc2.items()})
            for t in range(par, F // L, 2):
                hf[0, t], hf[1, t] = mix(*[gu[0][r, t] * gu[1][r, t] for r in range(2)])
        x = [jnp.concatenate([hf[r, t] for t in range(F // L)], axis=1) for r in range(2)]
        o, ready, stored = {}, set(), set()

        def done(k):
            ready.add(k)
            for r, c in sorted(ready):
                if (0, c) in ready and (k == (r, c) or k == (0, c)):
                    v = o[r, c] + 0.5 * o[0, c] if r else o[r, c]
                    rows, cols = slice(r0 + r * MH, r0 + (r + 1) * MH), slice(c * L, (c + 1) * L)
                    ob[i, rows, cols] = (x1b[rows, cols] + gb[:, cols] * v).astype(bf16)
                    stored.add((rows.start, c * L))
            for op in OP:
                need = {(s, c) for s in range(op[2], op[3], MH) for c in range(op[0], op[1], L)}
                if need <= stored:
                    stored.difference_update(need)
                    o_cp(i, *op).start()

        for si in range(2):
            fast_dot(fast_lhs(x, FT[si], si), "d", si, range(len(FT[si][0])), o,
                     lambda q: (q[0], DT[si][q[1]]), done)

    acc, hcache, parts = {}, {}, {}

    def grp_g(p, n, f, half=None):
        if (p, half) not in hcache:
            if len(n2) == 1 and half != 0:
                n2.append(prep_norm(qb0, x1b0, 0, H0, TM0 - H0))
            x = jnp.concatenate(n2, axis=0) if half is None else n2[half]
            hcache[p, half] = (x[:, p * L:(p + 1) * L] * (1.0 + mod[4 * NT + p])
                               + mod[3 * NT + p]).astype(bf16)
        rows = {None: slice(0, TM0), 0: slice(0, H0), 1: slice(H0, TM0)}[half]
        cols = slice(f * 4 * L, (f + 1) * 4 * L)
        d = jnp.dot(hcache[p, half], wts[n][p * L:(p + 1) * L, cols],
                    preferred_element_type=f32)
        ref = gub.at["gu".index(n), rows, cols]
        if p < NT - 1:
            ref[...] = d if p == 0 else ref[...] + d
        elif n == "g":
            acc[f] = ref[...] + d
        else:
            h = acc.pop(f) * (ref[...] + d)
            for t in range(4):
                x, y = h[:TM0 // 2, t * L:(t + 1) * L], h[TM0 // 2:, t * L:(t + 1) * L]
                hf0[0, 4 * f + t], hf0[1, 4 * f + t] = x, y - 0.5 * x
        return [d[s:s + 8, 0:L] for s in range(0, d.shape[0], 16)]

    left = {(q[0], DT[si][q[1]]): sum(q in t[2] for t in SCHEME[si])
            for si in range(2) for term in SCHEME[si] for q in term[2]}
    m0 = TM0 // 2

    def grp_f(si, i):
        term = SCHEME[si][i]
        k = sum(len(t[1]) > 1 for t in SCHEME[si][:i])
        ps = []
        for ts in (range(4), range(4, len(FT[si][0]))):
            if not len(ts):
                continue
            x = _lin(term[0], lambda q: jnp.concatenate(
                [hf0[q[0], FT[si][q[1]][t]] for t in ts], axis=1)).astype(bf16)
            if len(term[1]) > 1:
                w = wsb[2][si][k, ts[0] * L:(ts[-1] + 1) * L, :]
            else:
                w = jnp.concatenate([wtile("d", si, *term[1], t) for t in ts], axis=0)
            ps.append(jnp.dot(x, w, preferred_element_type=f32))
        p = ps[0] if len(ps) == 1 else ps[0] + ps[1]
        for q, v in term[2].items():
            key = (q[0], DT[si][q[1]])
            parts[key] = (p if v > 0 else -p) if key not in parts else (
                parts[key] + p if v > 0 else parts[key] - p)
            left[key] -= 1
        for c in DT[si]:
            if (0, c) in parts and not left[0, c] and not left[1, c]:
                top, bot = parts.pop((0, c)), parts.pop((1, c))
                o = jnp.concatenate([top, bot + 0.5 * top], axis=0)
                cols = slice(c * L, (c + 1) * L)
                ob0[:, cols] = (x1b0[:, cols] + mod[5 * NT + c] * o).astype(bf16)
        return ([ps[0][s:s + 8] for s in range(0, m0, 16)]
                + [x[s:s + 8] for x in ps[1:] for s in range(0, m0, 32)])

    grp_fn.update(g=grp_g, f=grp_f)
    region = lambda r, c: dpart.at[r * m0:(r + 1) * m0, c * L:(c + 1) * L]
    for waits, rows, groups, jobs in FIRST:
        wait(*waits)
        for n in parts:
            parts[n] = region(*n)[...]
        run(groups, jobs, lead=LEAD, floor=(0.0, 0.0))
        if rows:
            aff += [1.0 + modv(4), modv(3)]
            prep_chain(0, *rows, PR)
        for n in parts:
            region(*n)[...] = parts[n]
    for c0, c1 in zip(OC[:-1], OC[1:]):
        o_cp(None, c0, c1).start()
    gb = modv(5)
    wait("q1c", *[f"q{i + 1}" for i in range(1, NB)])

    def ffn(i, carry):
        prep_chain(i, HM, TM, PL)
        ffn_half(i, 0, gb)
        prep_chain(jnp.minimum(i + 1, NB - 1), 0, HM, PL)
        ffn_half(i, 1, gb)
        return carry

    lax.fori_loop(0, NB, ffn, 0)

    for c0, c1 in zip(OC[:-1], OC[1:]):
        o_cp(None, c0, c1).wait()
    for i in range(NB):
        for op in OP:
            o_cp(i, *op).wait()


@jax.jit
def pallas_adaLN_cond__ssm_conv_h3__glu_gated_bilinear__prompt_kernel(
    A_q: jax.Array,
    A_k: jax.Array,
    A_v: jax.Array,
    A_shift_k: jax.Array,
    A_ssm_k: jax.Array,
    A_ssm_D: jax.Array,
    B_x: jax.Array,
    B_w_gate: jax.Array,
    B_w_up: jax.Array,
    B_w_down: jax.Array,
    c: jax.Array,
    w_mod: jax.Array,
):
    del B_x
    tiles = lambda x: x.reshape(S // 8, 8, NT, L).transpose(0, 2, 1, 3).reshape(S * NT, L)
    any_spec = pl.BlockSpec(memory_space=pl.ANY)
    return pl.pallas_call(
        _kernel,
        in_specs=[any_spec] * 11,
        out_specs=any_spec,
        out_shape=jax.ShapeDtypeStruct((1, S, D), bf16),
        scratch_shapes=[
            pltpu.VMEM((TM0, D), bf16),
            pltpu.VMEM((NB, TM, D), bf16),
            [pltpu.VMEM((4 * PAD + C * NT, L), bf16)] * NC,
            [pltpu.VMEM((2 * PAD + C * NT, L), bf16)] * NC,
            pltpu.VMEM((NT, L, S), bf16),
            pltpu.VMEM((D, F), bf16),
            pltpu.VMEM((D, F), bf16),
            pltpu.VMEM((F, D), bf16),
            [[pltpu.VMEM((NSUM[si], len(FT[si][0]) * L, L), bf16) for si in range(2)]] * 3,
            pltpu.VMEM((D, 6 * D), bf16),
            pltpu.VMEM((NT, NC, R, L, L), bf16),
            pltpu.VMEM((NT, NC, R, 16, 16, L), f32),
            pltpu.VMEM((NT, NC, R, 16, 16, L), f32),
            pltpu.VMEM((NT, NC, R, 16, 16, L), f32),
            pltpu.VMEM((NT, NC, 2 * R, L, L), bf16),
            pltpu.VMEM((NT, S + 32, L), f32),
            pltpu.VMEM((TM0, D), f32),
            pltpu.VMEM((TM, D), f32),
            pltpu.VMEM((TM, D), f32),
            pltpu.VMEM((2, F // L, HM // 2, L), f32),
            pltpu.VMEM((2, TM0, F), f32),
            pltpu.VMEM((TM0, D), f32),
            pltpu.VMEM((2, F // L, TM0 // 2, L), f32),
            pltpu.VMEM((TM0, D), bf16),
            pltpu.VMEM((NB, TM, D), bf16),
            pltpu.VMEM((32, 8 * VM, L), f32),
            pltpu.VMEM((KS, D), bf16),
            pltpu.VMEM((D,), bf16),
            pltpu.VMEM((1, D), bf16),
            pltpu.SemaphoreType.DMA((len(DMA_ORDER),)),
            pltpu.SemaphoreType.DMA((NB + 1,)),
        ],
        compiler_params=pltpu.CompilerParams(
            vmem_limit_bytes=120 * 1024 * 1024,
            disable_bounds_checks=True, disable_semaphore_checks=True),
        name="adaln_h3_glu",
    )(A_q, tiles(A_k), tiles(A_v), A_shift_k.T, A_ssm_k, A_ssm_D,
      B_w_gate, B_w_up, B_w_down, c, w_mod)
```

```python
import jax
import jax.numpy as jnp
from jax import lax
import jax.experimental.pallas as pl
import jax.experimental.pallas.tpu as pltpu

S = 2048
D = 640
F = 1536
KS = 4
L = 128
NT = D // L
R = 4
C = R * L
NC = S // C
EPS = 1e-5
RSQ2 = 0.7071067811865476

WPT = 4 * NT
PAD = 32

TM0 = 512
H0 = 352
TM = 512
NB = (S - TM0) // TM
HM = 256
PL = 16
PR = 24
WM = {"mA": (0, 12), "c0": (20, 21), "mB": (12, 16), "s1": (16, 17), "c1": (21, 22),
      "s2": (17, 19), "c2": (22, 24), "s4": (19, 20), "c4": (24, 25), "mG": (25, 30)}
VM = 5
RATE = 1.05
LEAD = 24
FREE = {"i": 56, "z": 56, "k": 47, "u": 46}
FREE_FFN = {"i": 20, "u": 36, "f": 36, "g": 50}

f32 = jnp.float32
bf16 = jnp.bfloat16
u32 = jnp.uint32


def _cos_turns(t):
    x = jnp.abs(t - jnp.floor(t) - 0.5) - 0.25
    x2 = x * x
    return x * (6.283164024 + x2 * (-41.33713150 + x2 * (81.34038544 + x2 * -70.98993683)))


def _tables(inverse, hold=None):
    shape = (L // 2, L) if inverse else (2 * L, L)
    rho = lax.broadcasted_iota(jnp.int32, shape, 1 if inverse else 0)
    j = lax.broadcasted_iota(jnp.int32, shape, 0 if inverse else 1)
    if inverse:
        g, rad = 8 * (rho >> 4) + (rho & 7), 2 * R
    else:
        g, rad, j = 8 * (rho >> 5) + (rho & 7) + 64 * ((rho >> 4) & 1), R, _perm(j)
    a = (4 * g + 1).astype(f32) * (1.0 / (4 * C))
    off = ((rho >> 3) & 1).astype(f32) * 0.25
    ns = [(rad * j + r).astype(f32) for r in range(rad)]
    if hold is not None:
        ns = [hold(r, n) for r, n in enumerate(ns)]
    ts = [_cos_turns(a * n + off) for n in ns]
    return [(t * (1.0 / C) if inverse else t).astype(bf16) for t in ts]


def _perm(c):
    return 16 * (c >> 4) + 2 * (c & 7) + ((c >> 3) & 1)


def _layernorm(x):
    m = jnp.mean(x, axis=-1, keepdims=True)
    xc = x - m
    v = jnp.mean(xc * xc, axis=-1, keepdims=True)
    return xc * lax.rsqrt(v + EPS)


def _split(t):
    t = t.reshape(16, 16, L)
    return t[:, :8, :], t[:, 8:, :]


def _radix4(x, sgn):
    (ar, ai), (br, bi), (cr, ci), (dr, di) = x
    s0r, s0i, d0r, d0i = ar + cr, ai + ci, ar - cr, ai - ci
    s1r, s1i, d1r, d1i = br + dr, bi + di, br - dr, bi - di
    o0 = (s0r + s1r, s0i + s1i)
    o2 = (s0r - s1r, s0i - s1i)
    pl_ = (d0r - d1i, d0i + d1r)
    mi_ = (d0r + d1i, d0i - d1r)
    return [o0, pl_, o2, mi_] if sgn > 0 else [o0, mi_, o2, pl_]


S222 = (
    ({(1, 1): 1, (0, 0): -1}, {(0, 0): 1, (1, 1): 1}, {(0, 0): -1, (1, 1): 1}),
    ({(0, 1): 1, (1, 1): 1}, {(1, 0): 1, (1, 1): 1}, {(0, 0): 1}),
    ({(0, 0): 1, (0, 1): 1}, {(1, 1): 1}, {(0, 0): -1, (0, 1): 1}),
    ({(1, 1): 1}, {(1, 0): 1, (0, 0): -1}, {(0, 0): -1, (1, 0): 1}),
    ({(1, 0): 1, (1, 1): 1}, {(0, 0): 1}, {(1, 0): 1, (1, 1): -1}),
    ({(0, 0): 1}, {(0, 1): 1, (1, 1): -1}, {(0, 1): 1, (1, 1): -1}),
    ({(0, 0): 1, (1, 0): 1}, {(0, 0): 1, (0, 1): 1}, {(1, 1): 1}),
)
S233 = (
    ({(0, 0): 1, (1, 0): 1, (1, 2): -1}, {(0, 0): 1, (2, 2): -1},
     {(0, 0): 1, (0, 2): -1, (1, 2): 1}),
    ({(1, 0): 1, (1, 2): -1}, {(0, 0): 1}, {(0, 0): -1, (0, 2): 1, (1, 0): 1, (1, 2): -1}),
    ({(0, 0): 1, (1, 0): 1, (1, 2): -1, (0, 2): -1}, {(2, 2): 1}, {(0, 0): 1, (0, 2): -1}),
    ({(0, 2): 1}, {(1, 0): 1, (2, 0): 1, (2, 2): 1}, {(0, 0): 1}),
    ({(0, 1): 1, (0, 2): -1, (1, 1): 1}, {(1, 0): 1, (2, 1): 1},
     {(0, 1): -1, (1, 0): 1, (1, 1): 1}),
    ({(0, 1): 1, (0, 2): -1}, {(1, 0): 1}, {(0, 0): 1, (0, 1): 1, (1, 0): -1, (1, 1): -1}),
    ({(0, 1): 1, (0, 2): -1, (1, 1): 1, (1, 2): -1}, {(2, 1): 1}, {(1, 0): -1, (1, 1): -1}),
    ({(1, 2): 1}, {(0, 0): 1, (2, 0): 1, (2, 1): -1}, {(1, 0): 1}),
    ({(0, 0): 1, (1, 1): 1}, {(0, 1): 1, (1, 2): -1}, {(0, 1): 1, (1, 2): -1}),
    ({(1, 0): 1, (1, 1): -1}, {(0, 1): 1}, {(1, 1): 1, (1, 2): -1}),
    ({(0, 0): 1, (0, 1): -1}, {(1, 2): 1}, {(0, 1): 1, (0, 2): -1}),
    ({(0, 0): 1}, {(0, 0): 1, (0, 2): 1, (1, 2): 1}, {(0, 2): 1, (1, 2): -1}),
    ({(0, 0): 1, (1, 0): 1}, {(0, 1): 1, (0, 2): 1, (2, 2): 1}, {(1, 2): 1}),
    ({(1, 1): 1}, {(0, 1): 1, (1, 1): 1, (1, 0): -1}, {(0, 1): -1, (1, 1): 1}),
    ({(0, 1): 1, (1, 1): 1}, {(1, 1): 1, (1, 2): 1, (2, 1): 1}, {(0, 1): 1}),
)
SCHEME = (S233, S222)
HIT = (((0, 0), (0, 1), (1, 0), (2, 1)), ((0, 0), (1, 1)))
NSUM = [sum(len(t[1]) > 1 for t in s) for s in SCHEME]
DT = ((0, 1, 2), (3, 4))
FT = ([range(0, 4), range(4, 8), range(8, 12)], [range(0, 6), range(6, 12)])


def _lin(coef, get):
    r = None
    for q, v in coef.items():
        x = get(q)
        r = (x if v > 0 else -x) if r is None else (r + x if v > 0 else r - x)
    return r


T = range(NT)
_z = lambda j: [("z", j, a) for a in range(NC)]
_k = lambda j, al: [("k", j, a) for a in al]
_u = lambda a: [("u", j, a) for j in T]
_iv = lambda jl, al: [("i", j, a) for j in jl for a in al]
_kv = lambda a: [("kv", j, a) for j in T]
_m = lambda jl, us, outs: [("mac", j, us, outs) for j in jl]

A3 = (0, 1, 2)
SCHEDULE = [
    (["ssm0"], _z(0) + _k(0, range(NC)), [("setup", None)]),
    (["ssm1"], _z(1) + _k(1, range(NC)), []),
    (["ssm2"], _z(2) + _k(2, [0, 1]), []),
    (["k0", "v0"], _k(2, [2, 3]) + _u(0), _kv(0) + _m([0], (0,), (0,))),
    (["ssm3"], _iv([0], [0]) + _z(3) + _k(3, [0, 1]), _m([1, 2], (0,), A3)),
    (["k1", "v1"], _k(3, [2, 3]) + _u(1), _kv(1) + _m([3], (0,), (0,))),
    (["ssm4"], _iv([1], [0]) + _z(4) + _k(4, range(NC)),
     _m([0], (0, 1), (1, 2)) + _m([1, 2], (1,), (1, 2))),
    (["k2", "v2"], _iv([2, 3], [0]) + _iv([0], [1]) + _u(2) + _iv([1, 2], [1]) + _iv([4], [0, 1])
     + _iv([0, 1, 2, 4], [2]),
     _kv(2) + _m([4], (0, 1), A3) + _m([0, 1, 2, 4], (2,), (2,)) + _m([3], A3, (1, 2))),
    (["q0", "mA", "c0"], [("mod", "mA", "c0")] + _iv([3], [1, 2]), []),
]
_g = lambda p: [("g", p, n, f) for f in range(3) for n in "gu"]
_v = lambda *names: [("vmod", n) for n in names]
_w = lambda names, si: [("wsum", n, si, t) for n in names for t in range(len(FT[si][0]))]
_f = lambda si, *ids: [("f", si, i) for i in ids]
FIRST = [
    (["wg0", "qh"], None, [("g", 0, "g", f, h) for h in (0, 1) for f in range(3)], []),
    (["wu0", "s1", "c1"], None, [("g", 0, "u", f) for f in range(3)],
     _v("s1", "c1") + _m([0], A3, (3,))),
    (["wg1", "wu1"], None, _g(1)[:-1], _m([1, 2, 3], A3, (3,))),
    (["wg2", "wu2", "s2", "c2"], None, _g(1)[-1:] + _g(2),
     _v("s2", "c2") + _m([4], A3, (3,)) + _w("gu", 0)),
    (["wg3", "wu3", "wg4", "wu4", "s4", "c4", "q1"], (0, HM), _g(3) + _g(4),
     _v("s4", "c4") + _w("gu", 1)),
    (["wd", "k3", "v3"], None, _f(0, 1, 2, 5, 6, 9, 10) + _f(1, 2, 4) + _u(3) + _f(0, 0, 4, 8),
     _w("d", 0) + _kv(3) + _w("d", 1) + _m([0], (3,), (3,))),
    (["mG"], None, _f(0, 3, 11, 13, 7, 12, 14) + _f(1, 0, 1, 3, 5, 6) + _iv(T, [3]),
     _v("mG") + _m([1, 2, 3, 4], (3,), (3,))),
]

DMA_ORDER = (["sk", "sd", "c", "ssm0", "ssm1", "ssm2", "k0", "v0", "ssm3", "k1", "v1", "ssm4",
              "k2", "v2", "q0", "c0", "mA", "mB", "wg0", "qh", "wu0", "s1", "c1", "wg1", "wu1",
              "s2", "c2", "wg2", "wu2", "s4", "c4", "wg3", "wu3", "wg4", "wu4", "q1", "wd", "k3",
              "v3", "mG", "q1c"] + [f"q{i + 1}" for i in range(1, NB)])


def _costs(job):
    if job[0] == "kv":
        return [48, 42] * (C // 64)
    if job[0] == "wsum":
        return [61] * 8 if job[2] == 0 else [50] * 4
    if job[0] == "setup":
        return [100] * (4 * R)
    if job[0] == "vmod":
        return [3 * D // VM // 8] * (VM * (WM[job[1]][1] - WM[job[1]][0]))
    us, outs = job[2], job[3]
    pairs = [(a, n) for a in outs for n in us if n <= a]
    mac = (2 * len({a - n for a, n in pairs if a > n}) + 8 * len(pairs)
           - (2 * len(outs) if us[0] == 0 else 0))
    fin = sum(a <= us[-1] for a in outs)
    if mac < 12 and outs[-1] <= us[-1] < NC - 1:
        return [1 + R * mac + 16 * fin, 1 + R * mac + 48 * fin] * 8
    return ([1 + mac] * 3 + [1 + mac + 16 * fin] + [1 + mac] * 3 + [1 + mac + 48 * fin]) * 8


def _plan(groups, jobs, lead=0, floor=(1.0, 0.8)):
    free = FREE_FFN if lead else FREE
    nstep = {"i": 8, "z": 8, "k": 16, "u": 16, "mod": 0, "g": TM0 // 16}
    steps = lambda g: (16, 24)[g[1]] if g[0] == "f" else nstep[g[0]]
    slots = [free[g[0]] for g in groups for _ in range(steps(g))]
    lo, hi = [], []
    for job in jobs:
        begin, limit, first = 0, len(slots), 0
        for g in groups:
            kind = (g[0], job[0])
            if (kind == ("u", "kv") and g[1:] == job[1:]
                    or kind == ("i", "mac") and g[1] == job[1] and g[2] in job[3]
                    and g[2] <= job[2][-1]):
                limit = min(limit, first - lead)
            if (kind == ("f", "wsum") and g[1] == job[2] and len(SCHEME[g[1]][g[2]][1]) > 1
                    or kind == ("f", "vmod") and g[1:] == (0, 7)):
                limit = min(limit, first - lead)
            if kind == ("g", "vmod") and job[1][1] == str(g[1]):
                limit = min(limit, first - 11)
            first += steps(g)
            if kind == ("u", "mac") and g[1] == job[1] and g[2] in job[2]:
                begin = first
        lo.append(begin)
        hi.append(limit)
    plan, credit, n = [], (slots or [0])[0], 0
    for k, job in enumerate(jobs):
        if n < lo[k]:
            n, credit = lo[k], min(credit, 0) + slots[lo[k]]
        work = [sum(_costs(j)) for j in jobs]
        if lead:
            rate = max(RATE * sum(work[k:m + 1]) / max(sum(slots[n:hi[m]]), 1)
                       for m in range(k, len(jobs)))
        else:
            rate = RATE * sum(work[k:]) / sum(slots[n:])
        rate = max(rate, floor[0] if job[0] == "kv" else floor[1])
        idx = []
        for c in _costs(job):
            while credit <= 0 and n + 1 < hi[k]:
                n += 1
                credit += slots[n] * rate
            credit -= c
            idx.append(n)
        assert n < hi[k]
        plan.append(idx)
    return plan


def _kernel(q_hbm, k_hbm, v_hbm, sk_hbm, ssm_hbm, sd_hbm, wg_hbm, wu_hbm, wd_hbm,
            c_hbm, wm_hbm, o_hbm,
            qb0, qb, kbs, vbs, ssmb, wgb, wub, wdb, wsb, wmb, uwb, ub, kpb, yp, pb, yb,
            x1b0, x1b, h2b, hf, gub, dpart, hf0, ob0, ob, mv, skb, sdb, cb_, sem, osem):
    cps = {"sk": (sk_hbm, skb), "sd": (sd_hbm, sdb), "c": (c_hbm, cb_), "wd": (wd_hbm, wdb)}
    for j in range(NT):
        cps[f"ssm{j}"] = (ssm_hbm.at[pl.ds(j * L, L), :], ssmb.at[j])
    for a in range(NC):
        n, h = C * NT, 2 * PAD
        if a == 0:
            cps["k0"] = (k_hbm.at[pl.ds(0, n), :], kbs[0].at[pl.ds(h, n), :])
        else:
            e = 48
            cps[f"k{a}"] = (k_hbm.at[pl.ds(a * n - e, n + e), :],
                            kbs[a].at[pl.ds(h - e, n + e), :])
        cps[f"v{a}"] = (v_hbm.at[pl.ds(a * n, n), :], vbs[a].at[pl.ds(0, n), :])
    for n, (c0, c1) in WM.items():
        cols = pl.ds(c0 * L, (c1 - c0) * L)
        cps[n] = (wm_hbm.at[:, cols], wmb.at[:, cols])
    cps["q0"] = (q_hbm.at[0, pl.ds(0, H0), :], qb0.at[pl.ds(0, H0), :])
    cps["qh"] = (q_hbm.at[0, pl.ds(H0, TM0 - H0), :], qb0.at[pl.ds(H0, TM0 - H0), :])
    cps["q1"] = (q_hbm.at[0, pl.ds(TM0, HM), :], qb.at[0, pl.ds(0, HM), :])
    cps["q1c"] = (q_hbm.at[0, pl.ds(TM0 + HM, TM - HM), :], qb.at[0, pl.ds(HM, TM - HM), :])
    for i in range(1, NB):
        cps[f"q{i + 1}"] = (q_hbm.at[0, pl.ds(TM0 + i * TM, TM), :], qb.at[i])
    for p in range(NT):
        rows = pl.ds(p * L, L)
        cps[f"wg{p}"] = (wg_hbm.at[rows, :], wgb.at[rows, :])
        cps[f"wu{p}"] = (wu_hbm.at[rows, :], wub.at[rows, :])
    assert sorted(cps) == sorted(DMA_ORDER)

    def cp(name):
        src, dst = cps[name]
        return pltpu.make_async_copy(src, dst, sem.at[DMA_ORDER.index(name)])

    def wait(*names):
        for n in names:
            cp(n).wait()

    kbs[0][0:2 * PAD, :] = jnp.zeros((2 * PAD, L), bf16)
    for n in DMA_ORDER:
        cp(n).start()

    tabs, ginv, ccol = _tables(False), [], []
    for ref in (ub, kpb, yp):
        ref[0, 0, 0, 0, pl.ds(0, 8, stride=2), :] = jnp.zeros((8, L), f32)
    mv[0, pl.ds(0, 8, stride=2), :] = jnp.zeros((8, L), f32)
    for ref in (hf, hf0):
        ref[0, 0, pl.ds(0, 8, stride=2), :] = jnp.zeros((8, L), f32)
    ri = lax.broadcasted_iota(jnp.int32, (L, L), 0)
    ci = lax.broadcasted_iota(jnp.int32, (L, L), 1)
    sel = jnp.where(ci == R * _perm(ri & 31) + (ri >> 5), 1.0, 0.0).astype(bf16)

    wait("sk", "sd", "c")
    skt = skb[...].astype(f32)
    sdv = sdb[...].astype(f32).reshape(1, D)
    cv = cb_[...].astype(f32)
    sig = jax.nn.sigmoid(cv)
    cs = jnp.broadcast_to((cv * sig).astype(bf16), (16, D))
    one = sig[:, 0:L]

    def gate(x, deps):
        dep = jnp.concatenate(deps, axis=0).reshape(x.shape)
        return jnp.where(jnp.broadcast_to(one, x.shape) > 2.0, dep, x)

    def put(dst, j, a, xs):
        for qi in range(R):
            dst[j, a, qi] = jnp.concatenate(xs[qi], axis=1)

    zs = {}
    mod = {}

    def grp_z(j, a):
        z = [lax.dot_general(sel, ssmb[j, :, t * L:(t + 1) * L], (((1,), (1,)), ((), ())),
                             preferred_element_type=f32) for t in range(R * a, R * a + R)]
        zs[j, a] = [jnp.concatenate([z[p][32 * r:32 * (r + 1)] for p in range(R)],
                                    axis=0).astype(bf16) for r in range(R)]
        return [z[0][16 * t:16 * t + 8] for t in range(8)]

    def grp_fwd(ws, dst, j, a, dvec=None):
        t = [jnp.dot(tabs[r], ws[r], preferred_element_type=f32) for r in range(R)]
        x = [_split(v) for v in t]
        if dvec is not None:
            x[0] = (x[0][0] + dvec[None], x[0][1])
        put(dst, j, a, _radix4(x, -1))
        return [t[0][16 * s:16 * s + 8] for s in range(16)]

    def grp_k(j, a):
        return grp_fwd(zs.pop((j, a)), kpb, j, a,
                       sdv[:, j * L:(j + 1) * L] if a == 0 else None)

    def grp_u(j, a):
        uw = [uwb[j, a, r] for r in range(R)]
        return grp_fwd(uw, ub, j, a)

    def grp_i(j, a):
        ys = []
        for r in range(2 * R):
            y = jnp.dot(ginv[r], pb[j, a, r], preferred_element_type=f32)
            yb[j, pl.ds(a * C + r, L // 2, stride=2 * R), :] = y
            ys.append(y)
        return [ys[r][16 * s:16 * s + 8] for r in (0, R) for s in range(4)]

    def grp_mod(*names):
        for name in names:
            c0, c1 = WM[name]
            m = jnp.dot(cs, wmb[:, c0 * L:c1 * L], preferred_element_type=f32)
            for c in range(c0, c1):
                mod[c] = m[0:1, (c - c0) * L:(c - c0 + 1) * L]
        return []

    def modv(i):
        return jnp.concatenate([mod[i * NT + n] for n in range(NT)], axis=1)

    def job_kv(j, a, deps):
        lo = lambda x: lax.bitcast_convert_type(x << 16, f32)
        hi = lambda x: lax.bitcast_convert_type(x & jnp.uint32(0xFFFF0000), f32)
        n = C // 8
        kw, vw = kbs[a].bitcast(u32), vbs[a].bitcast(u32)
        ld = lambda ref, o: ref[pl.ds(4 * j + o, n, stride=WPT), :]
        k = {}
        for m in range(4):
            x = ld(kw, PAD + m)
            k[2 * m], k[2 * m + 1] = lo(x), hi(x)
        k[-3] = hi(ld(kw, PAD - WPT + 2))
        x = ld(kw, PAD - WPT + 3)
        k[-2], k[-1] = lo(x), hi(x)
        w = [skt[t:t + 1, j * L:(j + 1) * L] for t in range(KS)]
        w0 = [gate(jnp.broadcast_to(w[0], (n, L)), deps[e::2]) for e in (0, 1)]
        kv = {}
        for m in range(4):
            x = ld(vw, m)
            for ph, v in ((2 * m, lo(x)), (2 * m + 1, hi(x))):
                ks = k[ph] * w0[m % 2]
                for t in range(1, KS):
                    ks = ks + k[ph - t] * w[t]
                kv[ph] = (ks * v).reshape(n // 8, 8, L)
        for r in range(R):
            uwb[j, a, r] = jnp.concatenate([kv[r], kv[r + R]], axis=1).reshape(L, L).astype(bf16)

    def job_mac(j, us, outs, deps):
        ld = lambda ref, a: (ref[j, a, :, :, 0:8, :], ref[j, a, :, :, 8:16, :])
        lo, hi = us[0], us[-1]
        u = {a: ld(ub, a) for a in us}
        if len(deps) == 16:
            ur = jnp.concatenate([gate(u[lo][0][0:1], deps), u[lo][0][1:]], axis=0)
        else:
            ur = gate(u[lo][0], [deps[R * i + qi] for qi in range(R) for i in range(16)])
        u[lo] = (ur, u[lo][1])
        ms = sorted({a - n for a in outs for n in us if n <= a})
        k = {m: ld(kpb, m) for m in sorted(set(ms) | {m - 1 for m in ms if m > 0})}
        kp = {m: k[m] if m == 0 else (k[m][0] - k[m - 1][1], k[m][1] + k[m - 1][0]) for m in ms}
        for a in outs:
            yr, yi = ld(yp, a) if lo > 0 else (None, None)
            for n in us:
                if n > a:
                    continue
                (kr, ki), (ur, ui) = kp[a - n], u[n]
                tr = kr * ur - ki * ui
                ti = kr * ui + ki * ur
                yr = tr if yr is None else yr + tr
                yi = ti if yi is None else yi + ti
            if a > hi:
                yp[j, a] = jnp.concatenate([yr, yi], axis=2)
                continue
            ps = _radix4([(yr[qi], yi[qi]) for qi in range(R)], +1)
            for r in range(R):
                pr, pi = [p.reshape(8, 2, 8, L) for p in ps[r]]
                lr, li, hr, hi_ = pr[:, 0], pi[:, 0], pr[:, 1], pi[:, 1]
                if r % 2:
                    hr, hi_ = (hr - hi_) * RSQ2, (hr + hi_) * RSQ2
                if r < 2:
                    outs2 = (lr + hr, li + hi_), (lr - hr, li - hi_)
                else:
                    outs2 = (lr - hi_, li + hr), (lr + hi_, li - hr)
                for e in range(2):
                    pb[j, a, r + R * e] = jnp.concatenate(
                        outs2[e], axis=1).reshape(L, L).astype(bf16)

    def job_setup(_, deps):
        def hold(r, n):
            return gate(n, [deps[2 * r + s // 4] for s in range(8)])

        ginv.extend(_tables(True, hold))
        csf = cs[0:1].astype(f32)
        ccol.append(jnp.concatenate([jnp.broadcast_to(csf[:, t * L:(t + 1) * L], (L, L)).T
                                     for t in range(NT)], axis=0))

    def job_vmod(name, deps):
        c0, c1 = WM[name]
        n = D // VM
        for c in range(c0, c1):
            for i in range(VM):
                cc = ccol[0][i * n:(i + 1) * n]
                cc = jnp.concatenate([gate(cc[0:8], [deps[(c - c0) * VM + i]]), cc[8:]], axis=0)
                p = wmb[i * n:(i + 1) * n, c * L:(c + 1) * L].astype(f32) * cc
                mv[c, 8 * i:8 * i + 8, :] = jnp.sum(p.reshape(n // 8, 8, L), axis=0)
            mod[c] = jnp.sum(mv[c], axis=0, keepdims=True)

    wts = {"g": wgb, "u": wub, "d": wdb}

    def wtile(n, si, q, t):
        r, c = (FT[si][q[0]][t], DT[si][q[1]]) if n == "d" else (DT[si][q[0]], FT[si][q[1]][t])
        return wts[n][r * L:(r + 1) * L, c * L:(c + 1) * L]

    def job_wsum(n, si, t, deps):
        blk = {}
        for q in sorted({q for term in SCHEME[si] for q in term[1]}):
            x = wtile(n, si, q, t).astype(f32)
            if q in HIT[si]:
                x = x.reshape(8, 16, L)
                held = gate(x[:, 0:8], [deps[g * len(deps) // 8] for g in range(8)])
                x = jnp.concatenate([held, x[:, 8:]], axis=1).reshape(L, L)
            blk[q] = x
        sums = [term[1] for term in SCHEME[si] if len(term[1]) > 1]
        for i, coef in enumerate(sums):
            wsb["gud".index(n)][si][i, t * L:(t + 1) * L, :] = _lin(coef, blk.get).astype(bf16)

    def fast_lhs(x, tiles, si):
        get = lambda q: x[q[0]][:, tiles[q[1]][0] * L:(tiles[q[1]][-1] + 1) * L]
        return [_lin(term[0], get).astype(bf16) for term in SCHEME[si]]

    def fast_dot(a, n, si, ts, out, key, done=None):
        left = {q: sum(q in term[2] for term in SCHEME[si]) for term in SCHEME[si] for q in term[2]}
        i = 0
        for x, term in zip(a, SCHEME[si]):
            if len(term[1]) > 1:
                w = wsb["gud".index(n)][si][i, ts[0] * L:(ts[-1] + 1) * L, :]
                i += 1
            else:
                w = jnp.concatenate([wtile(n, si, *term[1], t) for t in ts], axis=0)
            p = jnp.dot(x, w, preferred_element_type=f32)
            for q, v in term[2].items():
                k = key(q)
                out[k] = (p if v > 0 else -p) if k not in out else (
                    out[k] + p if v > 0 else out[k] - p)
                left[q] -= 1
                if done is not None and not left[q]:
                    done(k)

    grp_fn = {"z": grp_z, "k": grp_k, "u": grp_u, "i": grp_i, "mod": grp_mod}
    job_fn = {"kv": job_kv, "mac": job_mac, "vmod": job_vmod, "setup": job_setup,
              "wsum": job_wsum}

    def run(groups, jobs, **kw):
        plan = _plan(groups, jobs, **kw)
        anchors, done = [], 0
        for g in groups + [None]:
            while done < len(jobs) and max(plan[done]) < len(anchors):
                job_fn[jobs[done][0]](*jobs[done][1:], [anchors[n] for n in plan[done]])
                done += 1
            if g is not None:
                anchors += grp_fn[g[0]](*g[1:])
        assert done == len(jobs)

    for waits, groups, jobs in SCHEDULE:
        wait(*waits)
        run(groups, jobs)

    n1, dep = [], None
    for r in range(0, H0, H0 // 2):
        x = qb0[r:r + H0 // 2, :].astype(f32)
        if dep is not None:
            x = jnp.concatenate([gate(x[:, 0:L], [dep]), x[:, L:]], axis=1)
        n1.append(_layernorm(x))
        dep = n1[-1][:, 0:L]
    n1 = jnp.concatenate(n1, axis=0)
    wait("mB")
    grp_mod("mB")
    sa, ca, ga = [modv(i) for i in range(3)]
    a1 = ga * (1.0 + ca)
    b1 = ga * sa

    def o_cp(i, c0, c1, r0=0, r1=TM):
        cols = pl.ds(c0, c1 - c0)
        if i is None:
            return pltpu.make_async_copy(ob0.at[:, cols], o_hbm.at[0, pl.ds(0, TM0), cols],
                                         osem.at[NB])
        base = TM0 + i * TM + r0
        if not isinstance(i, int):
            base = pl.multiple_of(base, 16)
        return pltpu.make_async_copy(ob.at[i, pl.ds(r0, r1 - r0), cols],
                                     o_hbm.at[0, pl.ds(base, r1 - r0), cols], osem.at[i])

    def prep_norm(q_ref, x1_ref, y0, r0, n, dep=None, n1=None, skew=False):
        x = q_ref[r0:r0 + n, :].astype(f32)
        if dep is not None:
            x = jnp.concatenate([gate(x[:, 0:L], [dep]), x[:, L:]], axis=1)
        if skew:
            gs = [x[0:8]]
            for s in range(8, n, 8):
                lag = jnp.broadcast_to(jnp.mean(gs[-1], axis=-1, keepdims=True), (8, L))
                g = x[s:s + 8]
                gs.append(jnp.concatenate([g[:, :L], gate(g[:, L:2 * L], [lag]), g[:, 2 * L:]],
                                          axis=1))
            x = jnp.concatenate(gs, axis=0)
        y = jnp.concatenate([yb[j, pl.ds(y0 + r0, n), :] for j in range(NT)], axis=1)
        x1 = x + ((_layernorm(x) if n1 is None else n1) * a1 + b1) * y
        x1_ref[r0:r0 + n, :] = x1
        return _layernorm(x1)

    n2 = [prep_norm(qb0, x1b0, 0, 0, H0, None, n1)]
    aff = []

    def prep_chain(i, r0, r1, pr):
        y0 = TM0 + i * TM
        if not isinstance(i, int):
            y0 = pl.multiple_of(y0, L)
        dep = None
        while r0 < r1:
            n = pr if (r1 - r0) % pr == 0 else pr + 8
            h2 = prep_norm(qb.at[i], x1b, y0, r0, n, dep if dep is None else dep[:n], None, True)
            h2 = h2 * aff[0] + aff[1]
            h2b[r0:r0 + n, :] = h2
            dep = h2[:, 0:L]
            r0 += n

    OC = (0, D)
    MH = HM // 2
    OP = [(0, D, 0, HM), (0, 3 * L, HM, TM), (3 * L, 4 * L, HM, TM),
          (4 * L, D, HM, HM + MH), (4 * L, D, HM + MH, TM)]

    def ffn_half(i, half, gb):
        r0 = half * HM
        mix = lambda x, y: (x, y - 0.5 * x)
        x = mix(h2b[r0:r0 + MH, :], h2b[r0 + MH:r0 + HM, :])
        a = [fast_lhs(x, [[t] for t in DT[si]], si) for si in range(2)]
        for par in range(2):
            accs = {"g": {}, "u": {}}
            for si in range(2):
                for t in range(par, len(FT[si][0]), 2):
                    for n in "gu":
                        fast_dot(a[si], n, si, [t], accs[n], lambda q: (q[0], FT[si][q[1]][t]))
            gu = [{(r, t): v + 0.5 * c[0, t] if r else v for (r, t), v in c.items()}
                  for c in accs.values()]
            for t in range(par, F // L, 2):
                hf[0, t], hf[1, t] = mix(*[gu[0][r, t] * gu[1][r, t] for r in range(2)])
        x = [jnp.concatenate([hf[r, t] for t in range(F // L)], axis=1) for r in range(2)]
        o, ready, stored = {}, set(), set()

        def done(k):
            ready.add(k)
            for r, c in sorted(ready):
                if (0, c) in ready and (k == (r, c) or k == (0, c)):
                    v = o[r, c] + 0.5 * o[0, c] if r else o[r, c]
                    rows, cols = slice(r0 + r * MH, r0 + (r + 1) * MH), slice(c * L, (c + 1) * L)
                    ob[i, rows, cols] = (x1b[rows, cols] + gb[:, cols] * v).astype(bf16)
                    stored.add((rows.start, c * L))
            for op in OP:
                need = {(s, c) for s in range(op[2], op[3], MH) for c in range(op[0], op[1], L)}
                if need <= stored:
                    stored.difference_update(need)
                    o_cp(i, *op).start()

        for si in range(2):
            fast_dot(fast_lhs(x, FT[si], si), "d", si, range(len(FT[si][0])), o,
                     lambda q: (q[0], DT[si][q[1]]), done)

    acc, hcache, parts = {}, {}, {}

    def grp_g(p, n, f, half=None):
        if (p, half) not in hcache:
            if len(n2) == 1 and half != 0:
                n2.append(prep_norm(qb0, x1b0, 0, H0, TM0 - H0))
            x = jnp.concatenate(n2, axis=0) if half is None else n2[half]
            hcache[p, half] = (x[:, p * L:(p + 1) * L] * (1.0 + mod[4 * NT + p])
                               + mod[3 * NT + p]).astype(bf16)
        rows = {None: slice(0, TM0), 0: slice(0, H0), 1: slice(H0, TM0)}[half]
        cols = slice(f * 4 * L, (f + 1) * 4 * L)
        d = jnp.dot(hcache[p, half], wts[n][p * L:(p + 1) * L, cols],
                    preferred_element_type=f32)
        ref = gub.at["gu".index(n), rows, cols]
        if p < NT - 1:
            ref[...] = d if p == 0 else ref[...] + d
        elif n == "g":
            acc[f] = ref[...] + d
        else:
            h = acc.pop(f) * (ref[...] + d)
            for t in range(4):
                x, y = h[:TM0 // 2, t * L:(t + 1) * L], h[TM0 // 2:, t * L:(t + 1) * L]
                hf0[0, 4 * f + t], hf0[1, 4 * f + t] = x, y - 0.5 * x
        return [d[s:s + 8, 0:L] for s in range(0, d.shape[0], 16)]

    left = {(q[0], DT[si][q[1]]): sum(q in t[2] for t in SCHEME[si])
            for si in range(2) for term in SCHEME[si] for q in term[2]}
    m0 = TM0 // 2

    def grp_f(si, i):
        term = SCHEME[si][i]
        k = sum(len(t[1]) > 1 for t in SCHEME[si][:i])
        ps = []
        for ts in (range(4), range(4, len(FT[si][0]))):
            if not len(ts):
                continue
            x = _lin(term[0], lambda q: jnp.concatenate(
                [hf0[q[0], FT[si][q[1]][t]] for t in ts], axis=1)).astype(bf16)
            if len(term[1]) > 1:
                w = wsb[2][si][k, ts[0] * L:(ts[-1] + 1) * L, :]
            else:
                w = jnp.concatenate([wtile("d", si, *term[1], t) for t in ts], axis=0)
            ps.append(jnp.dot(x, w, preferred_element_type=f32))
        p = ps[0] if len(ps) == 1 else ps[0] + ps[1]
        for q, v in term[2].items():
            key = (q[0], DT[si][q[1]])
            parts[key] = (p if v > 0 else -p) if key not in parts else (
                parts[key] + p if v > 0 else parts[key] - p)
            left[key] -= 1
        for c in DT[si]:
            if (0, c) in parts and not left[0, c] and not left[1, c]:
                top, bot = parts.pop((0, c)), parts.pop((1, c))
                o = jnp.concatenate([top, bot + 0.5 * top], axis=0)
                cols = slice(c * L, (c + 1) * L)
                ob0[:, cols] = (x1b0[:, cols] + mod[5 * NT + c] * o).astype(bf16)
        return ([ps[0][s:s + 8] for s in range(0, m0, 16)]
                + [x[s:s + 8] for x in ps[1:] for s in range(0, m0, 32)])

    grp_fn.update(g=grp_g, f=grp_f)
    region = lambda r, c: dpart.at[r * m0:(r + 1) * m0, c * L:(c + 1) * L]
    for waits, rows, groups, jobs in FIRST:
        wait(*waits)
        for n in parts:
            parts[n] = region(*n)[...]
        run(groups, jobs, lead=LEAD, floor=(0.0, 0.0))
        if rows:
            aff += [1.0 + modv(4), modv(3)]
            prep_chain(0, *rows, PR)
        for n in parts:
            region(*n)[...] = parts[n]
    for c0, c1 in zip(OC[:-1], OC[1:]):
        o_cp(None, c0, c1).start()
    gb = modv(5)
    wait("q1c", *[f"q{i + 1}" for i in range(1, NB)])

    def ffn(i, carry):
        prep_chain(i, HM, TM, PL)
        ffn_half(i, 0, gb)
        prep_chain(jnp.minimum(i + 1, NB - 1), 0, HM, PL)
        ffn_half(i, 1, gb)
        return carry

    lax.fori_loop(0, NB, ffn, 0)

    for c0, c1 in zip(OC[:-1], OC[1:]):
        o_cp(None, c0, c1).wait()
    for i in range(NB):
        for op in OP:
            o_cp(i, *op).wait()


@jax.jit
def pallas_adaLN_cond__ssm_conv_h3__glu_gated_bilinear__prompt_kernel(
    A_q: jax.Array,
    A_k: jax.Array,
    A_v: jax.Array,
    A_shift_k: jax.Array,
    A_ssm_k: jax.Array,
    A_ssm_D: jax.Array,
    B_x: jax.Array,
    B_w_gate: jax.Array,
    B_w_up: jax.Array,
    B_w_down: jax.Array,
    c: jax.Array,
    w_mod: jax.Array,
):
    del B_x
    tiles = lambda x: x.reshape(S // 8, 8, NT, L).transpose(0, 2, 1, 3).reshape(S * NT, L)
    any_spec = pl.BlockSpec(memory_space=pl.ANY)
    return pl.pallas_call(
        _kernel,
        in_specs=[any_spec] * 11,
        out_specs=any_spec,
        out_shape=jax.ShapeDtypeStruct((1, S, D), bf16),
        scratch_shapes=[
            pltpu.VMEM((TM0, D), bf16),
            pltpu.VMEM((NB, TM, D), bf16),
            [pltpu.VMEM((4 * PAD + C * NT, L), bf16)] * NC,
            [pltpu.VMEM((2 * PAD + C * NT, L), bf16)] * NC,
            pltpu.VMEM((NT, L, S), bf16),
            pltpu.VMEM((D, F), bf16),
            pltpu.VMEM((D, F), bf16),
            pltpu.VMEM((F, D), bf16),
            [[pltpu.VMEM((NSUM[si], len(FT[si][0]) * L, L), bf16) for si in range(2)]] * 3,
            pltpu.VMEM((D, 6 * D), bf16),
            pltpu.VMEM((NT, NC, R, L, L), bf16),
            pltpu.VMEM((NT, NC, R, 16, 16, L), f32),
            pltpu.VMEM((NT, NC, R, 16, 16, L), f32),
            pltpu.VMEM((NT, NC, R, 16, 16, L), f32),
            pltpu.VMEM((NT, NC, 2 * R, L, L), bf16),
            pltpu.VMEM((NT, S + 32, L), f32),
            pltpu.VMEM((TM0, D), f32),
            pltpu.VMEM((TM, D), f32),
            pltpu.VMEM((TM, D), f32),
            pltpu.VMEM((2, F // L, HM // 2, L), f32),
            pltpu.VMEM((2, TM0, F), f32),
            pltpu.VMEM((TM0, D), f32),
            pltpu.VMEM((2, F // L, TM0 // 2, L), f32),
            pltpu.VMEM((TM0, D), bf16),
            pltpu.VMEM((NB, TM, D), bf16),
            pltpu.VMEM((32, 8 * VM, L), f32),
            pltpu.VMEM((KS, D), bf16),
            pltpu.VMEM((D,), bf16),
            pltpu.VMEM((1, D), bf16),
            pltpu.SemaphoreType.DMA((len(DMA_ORDER),)),
            pltpu.SemaphoreType.DMA((NB + 1,)),
        ],
        compiler_params=pltpu.CompilerParams(
            vmem_limit_bytes=120 * 1024 * 1024,
            disable_bounds_checks=True, disable_semaphore_checks=True),
        name="adaln_h3_glu",
    )(A_q, tiles(A_k), tiles(A_v), A_shift_k.T, A_ssm_k, A_ssm_D,
      B_w_gate, B_w_up, B_w_down, c, w_mod)
```

```python
import jax
import jax.numpy as jnp
from jax import lax
import jax.experimental.pallas as pl
import jax.experimental.pallas.tpu as pltpu

S = 2048
D = 640
F = 1536
KS = 4
L = 128
NT = D // L
R = 4
C = R * L
NC = S // C
EPS = 1e-5
RSQ2 = 0.7071067811865476

WPT = 4 * NT
PAD = 32

TM0 = 512
H0 = 352
TM = 512
NB = (S - TM0) // TM
HM = 256
PL = 16
PR = 24
WM = {"mA": (0, 12), "c0": (20, 21), "mB": (12, 16), "s1": (16, 17), "c1": (21, 22),
      "s2": (17, 19), "c2": (22, 24), "s4": (19, 20), "c4": (24, 25), "mG": (25, 30)}
VM = 5
RATE = 1.05
LEAD = 24
FREE = {"i": 56, "z": 56, "k": 47, "u": 46}
FREE_FFN = {"i": 20, "u": 36, "f": 36, "g": 50}

f32 = jnp.float32
bf16 = jnp.bfloat16
u32 = jnp.uint32


def _cos_turns(t):
    x = jnp.abs(t - jnp.floor(t) - 0.5) - 0.25
    x2 = x * x
    return x * (6.283164024 + x2 * (-41.33713150 + x2 * (81.34038544 + x2 * -70.98993683)))


def _tables(inverse, rs, hold=None):
    shape = (L // 2, L) if inverse else (2 * L, L)
    rho = lax.broadcasted_iota(jnp.int32, shape, 1 if inverse else 0)
    j = lax.broadcasted_iota(jnp.int32, shape, 0 if inverse else 1)
    if inverse:
        g, rad = 8 * (rho >> 4) + (rho & 7), 2 * R
    else:
        g, rad, j = 8 * (rho >> 5) + (rho & 7) + 64 * ((rho >> 4) & 1), R, _perm(j)
    a = (4 * g + 1).astype(f32) * (1.0 / (4 * C))
    off = ((rho >> 3) & 1).astype(f32) * 0.25
    ns = [(rad * j + r).astype(f32) for r in rs]
    if hold is not None:
        ns = [hold(r, n) for r, n in enumerate(ns)]
    ts = [_cos_turns(a * n + off) for n in ns]
    return [t * (1.0 / C) if inverse else t for t in ts]


def _perm(c):
    return 16 * (c >> 4) + 2 * (c & 7) + ((c >> 3) & 1)


def _layernorm(x):
    m = jnp.mean(x, axis=-1, keepdims=True)
    xc = x - m
    v = jnp.mean(xc * xc, axis=-1, keepdims=True)
    return xc * lax.rsqrt(v + EPS)


def _split(t):
    t = t.reshape(16, 16, L)
    return t[:, :8, :], t[:, 8:, :]


def _radix4(x, sgn):
    (ar, ai), (br, bi), (cr, ci), (dr, di) = x
    s0r, s0i, d0r, d0i = ar + cr, ai + ci, ar - cr, ai - ci
    s1r, s1i, d1r, d1i = br + dr, bi + di, br - dr, bi - di
    o0 = (s0r + s1r, s0i + s1i)
    o2 = (s0r - s1r, s0i - s1i)
    pl_ = (d0r - d1i, d0i + d1r)
    mi_ = (d0r + d1i, d0i - d1r)
    return [o0, pl_, o2, mi_] if sgn > 0 else [o0, mi_, o2, pl_]


S222 = (
    ({(1, 1): 1, (0, 0): -1}, {(0, 0): 1, (1, 1): 1}, {(0, 0): -1, (1, 1): 1}),
    ({(0, 1): 1, (1, 1): 1}, {(1, 0): 1, (1, 1): 1}, {(0, 0): 1}),
    ({(0, 0): 1, (0, 1): 1}, {(1, 1): 1}, {(0, 0): -1, (0, 1): 1}),
    ({(1, 1): 1}, {(1, 0): 1, (0, 0): -1}, {(0, 0): -1, (1, 0): 1}),
    ({(1, 0): 1, (1, 1): 1}, {(0, 0): 1}, {(1, 0): 1, (1, 1): -1}),
    ({(0, 0): 1}, {(0, 1): 1, (1, 1): -1}, {(0, 1): 1, (1, 1): -1}),
    ({(0, 0): 1, (1, 0): 1}, {(0, 0): 1, (0, 1): 1}, {(1, 1): 1}),
)
S233 = (
    ({(0, 0): 1, (1, 0): 1, (1, 2): -1}, {(0, 0): 1, (2, 2): -1},
     {(0, 0): 1, (0, 2): -1, (1, 2): 1}),
    ({(1, 0): 1, (1, 2): -1}, {(0, 0): 1}, {(0, 0): -1, (0, 2): 1, (1, 0): 1, (1, 2): -1}),
    ({(0, 0): 1, (1, 0): 1, (1, 2): -1, (0, 2): -1}, {(2, 2): 1}, {(0, 0): 1, (0, 2): -1}),
    ({(0, 2): 1}, {(1, 0): 1, (2, 0): 1, (2, 2): 1}, {(0, 0): 1}),
    ({(0, 1): 1, (0, 2): -1, (1, 1): 1}, {(1, 0): 1, (2, 1): 1},
     {(0, 1): -1, (1, 0): 1, (1, 1): 1}),
    ({(0, 1): 1, (0, 2): -1}, {(1, 0): 1}, {(0, 0): 1, (0, 1): 1, (1, 0): -1, (1, 1): -1}),
    ({(0, 1): 1, (0, 2): -1, (1, 1): 1, (1, 2): -1}, {(2, 1): 1}, {(1, 0): -1, (1, 1): -1}),
    ({(1, 2): 1}, {(0, 0): 1, (2, 0): 1, (2, 1): -1}, {(1, 0): 1}),
    ({(0, 0): 1, (1, 1): 1}, {(0, 1): 1, (1, 2): -1}, {(0, 1): 1, (1, 2): -1}),
    ({(1, 0): 1, (1, 1): -1}, {(0, 1): 1}, {(1, 1): 1, (1, 2): -1}),
    ({(0, 0): 1, (0, 1): -1}, {(1, 2): 1}, {(0, 1): 1, (0, 2): -1}),
    ({(0, 0): 1}, {(0, 0): 1, (0, 2): 1, (1, 2): 1}, {(0, 2): 1, (1, 2): -1}),
    ({(0, 0): 1, (1, 0): 1}, {(0, 1): 1, (0, 2): 1, (2, 2): 1}, {(1, 2): 1}),
    ({(1, 1): 1}, {(0, 1): 1, (1, 1): 1, (1, 0): -1}, {(0, 1): -1, (1, 1): 1}),
    ({(0, 1): 1, (1, 1): 1}, {(1, 1): 1, (1, 2): 1, (2, 1): 1}, {(0, 1): 1}),
)
SCHEME = (S233, S222)
HIT = (((0, 0), (0, 1), (1, 0), (2, 1)), ((0, 0), (1, 1)))
NSUM = [sum(len(t[1]) > 1 for t in s) for s in SCHEME]
DT = ((0, 1, 2), (3, 4))
FT = ([range(0, 4), range(4, 8), range(8, 12)], [range(0, 6), range(6, 12)])


def _lin(coef, get):
    r = None
    for q, v in coef.items():
        x = get(q)
        r = (x if v > 0 else -x) if r is None else (r + x if v > 0 else r - x)
    return r


T = range(NT)
_z = lambda j: [("z", j, a) for a in range(NC)]
_k = lambda j, al: [("k", j, a) for a in al]
_u = lambda a: [("u", j, a) for j in T]
_iv = lambda jl, al: [("i", j, a) for j in jl for a in al]
_kv = lambda a: [("kv", j, a) for j in T]
_m = lambda jl, us, outs: [("mac", j, us, outs) for j in jl]

A3 = (0, 1, 2)
SCHEDULE = [
    (["ssm0"], _z(0) + _k(0, range(NC)), [("setup", None)]),
    (["ssm1"], _z(1) + _k(1, range(NC)), []),
    (["ssm2"], _z(2) + _k(2, [0, 1]), []),
    (["k0", "v0"], _k(2, [2, 3]) + _u(0), _kv(0) + _m([0], (0,), (0,))),
    (["ssm3"], _iv([0], [0]) + _z(3) + _k(3, [0, 1]), _m([1, 2], (0,), A3)),
    (["k1", "v1"], _k(3, [2, 3]) + _u(1), _kv(1) + _m([3], (0,), (0,))),
    (["ssm4"], _iv([1], [0]) + _z(4) + _k(4, range(NC)),
     _m([0], (0, 1), (1, 2)) + _m([1, 2], (1,), (1, 2))),
    (["k2", "v2"], _iv([2, 3], [0]) + _iv([0], [1]) + _u(2) + _iv([1, 2], [1]) + _iv([4], [0, 1])
     + _iv([0, 1, 2, 4], [2]),
     _kv(2) + _m([4], (0, 1), A3) + _m([0, 1, 2, 4], (2,), (2,)) + _m([3], A3, (1, 2))),
    (["q0", "mA", "c0"], [("mod", "mA", "c0")] + _iv([3], [1, 2]), []),
]
_g = lambda p: [("g", p, n, f) for f in range(3) for n in "gu"]
_v = lambda *names: [("vmod", n) for n in names]
_w = lambda names, si: [("wsum", n, si, t) for n in names for t in range(len(FT[si][0]))]
_f = lambda si, *ids: [("f", si, i) for i in ids]
FIRST = [
    (["wg0", "qh"], None, [("g", 0, "g", f, h) for h in (0, 1) for f in range(3)], []),
    (["wu0", "s1", "c1"], None, [("g", 0, "u", f) for f in range(3)],
     _v("s1", "c1") + _m([0], A3, (3,))),
    (["wg1", "wu1"], None, _g(1)[:-1], _m([1, 2, 3], A3, (3,))),
    (["wg2", "wu2", "s2", "c2"], None, _g(1)[-1:] + _g(2),
     _v("s2", "c2") + _m([4], A3, (3,)) + _w("gu", 0)),
    (["wg3", "wu3", "wg4", "wu4", "s4", "c4", "q1"], (0, HM), _g(3) + _g(4),
     _v("s4", "c4") + _w("gu", 1)),
    (["wd", "k3", "v3"], None, _f(0, 1, 2, 5, 6, 9, 10) + _f(1, 2, 4) + _u(3) + _f(0, 0, 4, 8),
     _w("d", 0) + _kv(3) + _w("d", 1) + _m([0], (3,), (3,))),
    (["mG"], None, _f(0, 3, 11, 13, 7, 12, 14) + _f(1, 0, 1, 3, 5, 6) + _iv(T, [3]),
     _v("mG") + _m([1, 2, 3, 4], (3,), (3,))),
]

DMA_ORDER = (["sk", "sd", "c", "ssm0", "ssm1", "ssm2", "k0", "v0", "ssm3", "k1", "v1", "ssm4",
              "k2", "v2", "q0", "c0", "mA", "mB", "wg0", "qh", "wu0", "s1", "c1", "wg1", "wu1",
              "s2", "c2", "wg2", "wu2", "s4", "c4", "wg3", "wu3", "wg4", "wu4", "q1", "wd", "k3",
              "v3", "mG", "q1c"] + [f"q{i + 1}" for i in range(1, NB)])


def _costs(job):
    if job[0] == "kv":
        return [48, 42] * (C // 64)
    if job[0] == "wsum":
        return [61] * 8 if job[2] == 0 else [50] * 4
    if job[0] == "setup":
        return [100] * (4 * R)
    if job[0] == "vmod":
        return [3 * D // VM // 8] * (VM * (WM[job[1]][1] - WM[job[1]][0]))
    us, outs = job[2], job[3]
    pairs = [(a, n) for a in outs for n in us if n <= a]
    mac = (2 * len({a - n for a, n in pairs if a > n}) + 8 * len(pairs)
           - (2 * len(outs) if us[0] == 0 else 0))
    fin = sum(a <= us[-1] for a in outs)
    if mac < 12 and outs[-1] <= us[-1] < NC - 1:
        return [1 + R * mac + 16 * fin, 1 + R * mac + 48 * fin] * 8
    return ([1 + mac] * 3 + [1 + mac + 16 * fin] + [1 + mac] * 3 + [1 + mac + 48 * fin]) * 8


def _plan(groups, jobs, lead=0, floor=(1.0, 0.8)):
    free = FREE_FFN if lead else FREE
    nstep = {"i": 8, "z": 8, "k": 16, "u": 16, "mod": 0, "g": TM0 // 16}
    steps = lambda g: (16, 24)[g[1]] if g[0] == "f" else nstep[g[0]]
    slots = [free[g[0]] for g in groups for _ in range(steps(g))]
    lo, hi = [], []
    for job in jobs:
        begin, limit, first = 0, len(slots), 0
        for g in groups:
            kind = (g[0], job[0])
            if (kind == ("u", "kv") and g[1:] == job[1:]
                    or kind == ("i", "mac") and g[1] == job[1] and g[2] in job[3]
                    and g[2] <= job[2][-1]):
                limit = min(limit, first - lead)
            if (kind == ("f", "wsum") and g[1] == job[2] and len(SCHEME[g[1]][g[2]][1]) > 1
                    or kind == ("f", "vmod") and g[1:] == (0, 7)):
                limit = min(limit, first - lead)
            if kind == ("g", "vmod") and job[1][1] == str(g[1]):
                limit = min(limit, first - 11)
            first += steps(g)
            if kind == ("u", "mac") and g[1] == job[1] and g[2] in job[2]:
                begin = first
        lo.append(begin)
        hi.append(limit)
    plan, credit, n = [], (slots or [0])[0], 0
    for k, job in enumerate(jobs):
        if n < lo[k]:
            n, credit = lo[k], min(credit, 0) + slots[lo[k]]
        work = [sum(_costs(j)) for j in jobs]
        if lead:
            rate = max(RATE * sum(work[k:m + 1]) / max(sum(slots[n:hi[m]]), 1)
                       for m in range(k, len(jobs)))
        else:
            rate = RATE * sum(work[k:]) / sum(slots[n:])
        rate = max(rate, floor[0] if job[0] == "kv" else floor[1])
        idx = []
        for c in _costs(job):
            while credit <= 0 and n + 1 < hi[k]:
                n += 1
                credit += slots[n] * rate
            credit -= c
            idx.append(n)
        assert n < hi[k]
        plan.append(idx)
    return plan


def _kernel(q_hbm, k_hbm, v_hbm, sk_hbm, ssm_hbm, sd_hbm, wg_hbm, wu_hbm, wd_hbm,
            c_hbm, wm_hbm, o_hbm,
            qb0, qb, kbs, vbs, ssmb, wgb, wub, wdb, wsb, wmb, uwb, ub, kpb, yp, pb, yb,
            x1b0, x1b, h2b, hf, gub, dpart, hf0, ob0, ob, mv, skb, sdb, cb_, sem, osem):
    cps = {"sk": (sk_hbm, skb), "sd": (sd_hbm, sdb), "c": (c_hbm, cb_), "wd": (wd_hbm, wdb)}
    for j in range(NT):
        cps[f"ssm{j}"] = (ssm_hbm.at[pl.ds(j * L, L), :], ssmb.at[j])
    for a in range(NC):
        n, h = C * NT, 2 * PAD
        if a == 0:
            cps["k0"] = (k_hbm.at[pl.ds(0, n), :], kbs[0].at[pl.ds(h, n), :])
        else:
            e = 48
            cps[f"k{a}"] = (k_hbm.at[pl.ds(a * n - e, n + e), :],
                            kbs[a].at[pl.ds(h - e, n + e), :])
        cps[f"v{a}"] = (v_hbm.at[pl.ds(a * n, n), :], vbs[a].at[pl.ds(0, n), :])
    for n, (c0, c1) in WM.items():
        cols = pl.ds(c0 * L, (c1 - c0) * L)
        cps[n] = (wm_hbm.at[:, cols], wmb.at[:, cols])
    cps["q0"] = (q_hbm.at[0, pl.ds(0, H0), :], qb0.at[pl.ds(0, H0), :])
    cps["qh"] = (q_hbm.at[0, pl.ds(H0, TM0 - H0), :], qb0.at[pl.ds(H0, TM0 - H0), :])
    cps["q1"] = (q_hbm.at[0, pl.ds(TM0, HM), :], qb.at[0, pl.ds(0, HM), :])
    cps["q1c"] = (q_hbm.at[0, pl.ds(TM0 + HM, TM - HM), :], qb.at[0, pl.ds(HM, TM - HM), :])
    for i in range(1, NB):
        cps[f"q{i + 1}"] = (q_hbm.at[0, pl.ds(TM0 + i * TM, TM), :], qb.at[i])
    for p in range(NT):
        rows = pl.ds(p * L, L)
        cps[f"wg{p}"] = (wg_hbm.at[rows, :], wgb.at[rows, :])
        cps[f"wu{p}"] = (wu_hbm.at[rows, :], wub.at[rows, :])
    assert sorted(cps) == sorted(DMA_ORDER)

    def cp(name):
        src, dst = cps[name]
        return pltpu.make_async_copy(src, dst, sem.at[DMA_ORDER.index(name)])

    def wait(*names):
        for n in names:
            cp(n).wait()

    kbs[0][0:2 * PAD, :] = jnp.zeros((2 * PAD, L), bf16)
    for n in DMA_ORDER:
        cp(n).start()

    def table(r, carry):
        hf0[1, r] = _tables(False, [r])[0]
        return carry

    lax.fori_loop(0, R, table, 0)
    tabs, ginv, ccol = [hf0[1, r].astype(bf16) for r in range(R)], [], []
    for ref in (ub, kpb, yp):
        ref[0, 0, 0, 0, pl.ds(0, 8, stride=2), :] = jnp.zeros((8, L), f32)
    mv[0, pl.ds(0, 8, stride=2), :] = jnp.zeros((8, L), f32)
    for ref in (hf, hf0):
        ref[0, 0, pl.ds(0, 8, stride=2), :] = jnp.zeros((8, L), f32)
    ri = lax.broadcasted_iota(jnp.int32, (L, L), 0)
    ci = lax.broadcasted_iota(jnp.int32, (L, L), 1)
    sel = jnp.where(ci == R * _perm(ri & 31) + (ri >> 5), 1.0, 0.0).astype(bf16)

    wait("sk", "sd", "c")
    skt = skb[...].astype(f32)
    sdv = sdb[...].astype(f32).reshape(1, D)
    cv = cb_[...].astype(f32)
    sig = jax.nn.sigmoid(cv)
    cs = jnp.broadcast_to((cv * sig).astype(bf16), (16, D))
    one = sig[:, 0:L]

    def gate(x, deps):
        dep = jnp.concatenate(deps, axis=0).reshape(x.shape)
        return jnp.where(jnp.broadcast_to(one, x.shape) > 2.0, dep, x)

    def put(dst, j, a, xs):
        for qi in range(R):
            dst[j, a, qi] = jnp.concatenate(xs[qi], axis=1)

    zs = {}
    mod = {}

    def grp_z(j, a):
        z = [lax.dot_general(sel, ssmb[j, :, t * L:(t + 1) * L], (((1,), (1,)), ((), ())),
                             preferred_element_type=f32) for t in range(R * a, R * a + R)]
        zs[j, a] = [jnp.concatenate([z[p][32 * r:32 * (r + 1)] for p in range(R)],
                                    axis=0).astype(bf16) for r in range(R)]
        return [z[0][16 * t:16 * t + 8] for t in range(8)]

    def grp_fwd(ws, dst, j, a, dvec=None):
        t = [jnp.dot(tabs[r], ws[r], preferred_element_type=f32) for r in range(R)]
        x = [_split(v) for v in t]
        if dvec is not None:
            x[0] = (x[0][0] + dvec[None], x[0][1])
        put(dst, j, a, _radix4(x, -1))
        return [t[0][16 * s:16 * s + 8] for s in range(16)]

    def grp_k(j, a):
        return grp_fwd(zs.pop((j, a)), kpb, j, a,
                       sdv[:, j * L:(j + 1) * L] if a == 0 else None)

    def grp_u(j, a):
        uw = [uwb[j, a, r] for r in range(R)]
        return grp_fwd(uw, ub, j, a)

    def grp_i(j, a):
        ys = []
        for r in range(2 * R):
            y = jnp.dot(ginv[r], pb[j, a, r], preferred_element_type=f32)
            yb[j, pl.ds(a * C + r, L // 2, stride=2 * R), :] = y
            ys.append(y)
        return [ys[r][16 * s:16 * s + 8] for r in (0, R) for s in range(4)]

    def grp_mod(*names):
        for name in names:
            c0, c1 = WM[name]
            m = jnp.dot(cs, wmb[:, c0 * L:c1 * L], preferred_element_type=f32)
            for c in range(c0, c1):
                mod[c] = m[0:1, (c - c0) * L:(c - c0 + 1) * L]
        return []

    def modv(i):
        return jnp.concatenate([mod[i * NT + n] for n in range(NT)], axis=1)

    def job_kv(j, a, deps):
        lo = lambda x: lax.bitcast_convert_type(x << 16, f32)
        hi = lambda x: lax.bitcast_convert_type(x & jnp.uint32(0xFFFF0000), f32)
        n = C // 8
        kw, vw = kbs[a].bitcast(u32), vbs[a].bitcast(u32)
        ld = lambda ref, o: ref[pl.ds(4 * j + o, n, stride=WPT), :]
        k = {}
        for m in range(4):
            x = ld(kw, PAD + m)
            k[2 * m], k[2 * m + 1] = lo(x), hi(x)
        k[-3] = hi(ld(kw, PAD - WPT + 2))
        x = ld(kw, PAD - WPT + 3)
        k[-2], k[-1] = lo(x), hi(x)
        w = [skt[t:t + 1, j * L:(j + 1) * L] for t in range(KS)]
        w0 = [gate(jnp.broadcast_to(w[0], (n, L)), deps[e::2]) for e in (0, 1)]
        kv = {}
        for m in range(4):
            x = ld(vw, m)
            for ph, v in ((2 * m, lo(x)), (2 * m + 1, hi(x))):
                ks = k[ph] * w0[m % 2]
                for t in range(1, KS):
                    ks = ks + k[ph - t] * w[t]
                kv[ph] = (ks * v).reshape(n // 8, 8, L)
        for r in range(R):
            uwb[j, a, r] = jnp.concatenate([kv[r], kv[r + R]], axis=1).reshape(L, L).astype(bf16)

    def job_mac(j, us, outs, deps):
        ld = lambda ref, a: (ref[j, a, :, :, 0:8, :], ref[j, a, :, :, 8:16, :])
        lo, hi = us[0], us[-1]
        u = {a: ld(ub, a) for a in us}
        if len(deps) == 16:
            ur = jnp.concatenate([gate(u[lo][0][0:1], deps), u[lo][0][1:]], axis=0)
        else:
            ur = gate(u[lo][0], [deps[R * i + qi] for qi in range(R) for i in range(16)])
        u[lo] = (ur, u[lo][1])
        ms = sorted({a - n for a in outs for n in us if n <= a})
        k = {m: ld(kpb, m) for m in sorted(set(ms) | {m - 1 for m in ms if m > 0})}
        kp = {m: k[m] if m == 0 else (k[m][0] - k[m - 1][1], k[m][1] + k[m - 1][0]) for m in ms}
        for a in outs:
            yr, yi = ld(yp, a) if lo > 0 else (None, None)
            for n in us:
                if n > a:
                    continue
                (kr, ki), (ur, ui) = kp[a - n], u[n]
                tr = kr * ur - ki * ui
                ti = kr * ui + ki * ur
                yr = tr if yr is None else yr + tr
                yi = ti if yi is None else yi + ti
            if a > hi:
                yp[j, a] = jnp.concatenate([yr, yi], axis=2)
                continue
            ps = _radix4([(yr[qi], yi[qi]) for qi in range(R)], +1)
            for r in range(R):
                pr, pi = [p.reshape(8, 2, 8, L) for p in ps[r]]
                lr, li, hr, hi_ = pr[:, 0], pi[:, 0], pr[:, 1], pi[:, 1]
                if r % 2:
                    hr, hi_ = (hr - hi_) * RSQ2, (hr + hi_) * RSQ2
                if r < 2:
                    outs2 = (lr + hr, li + hi_), (lr - hr, li - hi_)
                else:
                    outs2 = (lr - hi_, li + hr), (lr + hi_, li - hr)
                for e in range(2):
                    pb[j, a, r + R * e] = jnp.concatenate(
                        outs2[e], axis=1).reshape(L, L).astype(bf16)

    def job_setup(_, deps):
        def hold(r, n):
            return gate(n, [deps[2 * r + s // 4] for s in range(8)])

        ginv.extend(t.astype(bf16) for t in _tables(True, range(2 * R), hold))
        csf = cs[0:1].astype(f32)
        ccol.append(jnp.concatenate([jnp.broadcast_to(csf[:, t * L:(t + 1) * L], (L, L)).T
                                     for t in range(NT)], axis=0))

    def job_vmod(name, deps):
        c0, c1 = WM[name]
        n = D // VM
        for c in range(c0, c1):
            for i in range(VM):
                cc = ccol[0][i * n:(i + 1) * n]
                cc = jnp.concatenate([gate(cc[0:8], [deps[(c - c0) * VM + i]]), cc[8:]], axis=0)
                p = wmb[i * n:(i + 1) * n, c * L:(c + 1) * L].astype(f32) * cc
                mv[c, 8 * i:8 * i + 8, :] = jnp.sum(p.reshape(n // 8, 8, L), axis=0)
            mod[c] = jnp.sum(mv[c], axis=0, keepdims=True)

    wts = {"g": wgb, "u": wub, "d": wdb}

    def wtile(n, si, q, t):
        r, c = (FT[si][q[0]][t], DT[si][q[1]]) if n == "d" else (DT[si][q[0]], FT[si][q[1]][t])
        return wts[n][r * L:(r + 1) * L, c * L:(c + 1) * L]

    def job_wsum(n, si, t, deps):
        blk = {}
        for q in sorted({q for term in SCHEME[si] for q in term[1]}):
            x = wtile(n, si, q, t).astype(f32)
            if q in HIT[si]:
                x = x.reshape(8, 16, L)
                held = gate(x[:, 0:8], [deps[g * len(deps) // 8] for g in range(8)])
                x = jnp.concatenate([held, x[:, 8:]], axis=1).reshape(L, L)
            blk[q] = x
        sums = [term[1] for term in SCHEME[si] if len(term[1]) > 1]
        for i, coef in enumerate(sums):
            wsb["gud".index(n)][si][i, t * L:(t + 1) * L, :] = _lin(coef, blk.get).astype(bf16)

    def fast_lhs(x, tiles, si):
        get = lambda q: x[q[0]][:, tiles[q[1]][0] * L:(tiles[q[1]][-1] + 1) * L]
        return [_lin(term[0], get).astype(bf16) for term in SCHEME[si]]

    def fast_dot(a, n, si, ts, out, key, done=None):
        left = {q: sum(q in term[2] for term in SCHEME[si]) for term in SCHEME[si] for q in term[2]}
        i = 0
        for x, term in zip(a, SCHEME[si]):
            if len(term[1]) > 1:
                w = wsb["gud".index(n)][si][i, ts[0] * L:(ts[-1] + 1) * L, :]
                i += 1
            else:
                w = jnp.concatenate([wtile(n, si, *term[1], t) for t in ts], axis=0)
            p = jnp.dot(x, w, preferred_element_type=f32)
            for q, v in term[2].items():
                k = key(q)
                out[k] = (p if v > 0 else -p) if k not in out else (
                    out[k] + p if v > 0 else out[k] - p)
                left[q] -= 1
                if done is not None and not left[q]:
                    done(k)

    grp_fn = {"z": grp_z, "k": grp_k, "u": grp_u, "i": grp_i, "mod": grp_mod}
    job_fn = {"kv": job_kv, "mac": job_mac, "vmod": job_vmod, "setup": job_setup,
              "wsum": job_wsum}

    def run(groups, jobs, **kw):
        plan = _plan(groups, jobs, **kw)
        anchors, done = [], 0
        for g in groups + [None]:
            while done < len(jobs) and max(plan[done]) < len(anchors):
                job_fn[jobs[done][0]](*jobs[done][1:], [anchors[n] for n in plan[done]])
                done += 1
            if g is not None:
                anchors += grp_fn[g[0]](*g[1:])
        assert done == len(jobs)

    for waits, groups, jobs in SCHEDULE:
        wait(*waits)
        run(groups, jobs)

    n1, dep = [], None
    for r in range(0, H0, H0 // 2):
        x = qb0[r:r + H0 // 2, :].astype(f32)
        if dep is not None:
            x = jnp.concatenate([gate(x[:, 0:L], [dep]), x[:, L:]], axis=1)
        n1.append(_layernorm(x))
        dep = n1[-1][:, 0:L]
    n1 = jnp.concatenate(n1, axis=0)
    wait("mB")
    grp_mod("mB")
    sa, ca, ga = [modv(i) for i in range(3)]
    a1 = ga * (1.0 + ca)
    b1 = ga * sa

    def o_cp(i, c0, c1, r0=0, r1=TM):
        cols = pl.ds(c0, c1 - c0)
        if i is None:
            return pltpu.make_async_copy(ob0.at[:, cols], o_hbm.at[0, pl.ds(0, TM0), cols],
                                         osem.at[NB])
        base = TM0 + i * TM + r0
        if not isinstance(i, int):
            base = pl.multiple_of(base, 16)
        return pltpu.make_async_copy(ob.at[i, pl.ds(r0, r1 - r0), cols],
                                     o_hbm.at[0, pl.ds(base, r1 - r0), cols], osem.at[i])

    def prep_norm(q_ref, x1_ref, y0, r0, n, dep=None, n1=None, skew=False):
        x = q_ref[r0:r0 + n, :].astype(f32)
        if dep is not None:
            x = jnp.concatenate([gate(x[:, 0:L], [dep]), x[:, L:]], axis=1)
        if skew:
            gs = [x[0:8]]
            for s in range(8, n, 8):
                lag = jnp.broadcast_to(jnp.mean(gs[-1], axis=-1, keepdims=True), (8, L))
                g = x[s:s + 8]
                gs.append(jnp.concatenate([g[:, :L], gate(g[:, L:2 * L], [lag]), g[:, 2 * L:]],
                                          axis=1))
            x = jnp.concatenate(gs, axis=0)
        y = jnp.concatenate([yb[j, pl.ds(y0 + r0, n), :] for j in range(NT)], axis=1)
        x1 = x + ((_layernorm(x) if n1 is None else n1) * a1 + b1) * y
        x1_ref[r0:r0 + n, :] = x1
        return _layernorm(x1)

    n2 = [prep_norm(qb0, x1b0, 0, 0, H0, None, n1)]
    aff = []

    def prep_chain(i, r0, r1, pr):
        y0 = TM0 + i * TM
        if not isinstance(i, int):
            y0 = pl.multiple_of(y0, L)
        dep = None
        while r0 < r1:
            n = pr if (r1 - r0) % pr == 0 else pr + 8
            h2 = prep_norm(qb.at[i], x1b, y0, r0, n, dep if dep is None else dep[:n], None, True)
            h2 = h2 * aff[0] + aff[1]
            h2b[r0:r0 + n, :] = h2
            dep = h2[:, 0:L]
            r0 += n

    OC = (0, D)
    MH = HM // 2
    OP = [(0, D, 0, HM), (0, 3 * L, HM, TM), (3 * L, 4 * L, HM, TM),
          (4 * L, D, HM, HM + MH), (4 * L, D, HM + MH, TM)]

    def ffn_half(i, half, gb):
        r0 = half * HM
        mix = lambda x, y: (x, y - 0.5 * x)
        x = mix(h2b[r0:r0 + MH, :], h2b[r0 + MH:r0 + HM, :])
        a = [fast_lhs(x, [[t] for t in DT[si]], si) for si in range(2)]
        for par in range(2):
            accs = {"g": {}, "u": {}}
            for si in range(2):
                for t in range(par, len(FT[si][0]), 2):
                    for n in "gu":
                        fast_dot(a[si], n, si, [t], accs[n], lambda q: (q[0], FT[si][q[1]][t]))
            gu = [{(r, t): v + 0.5 * c[0, t] if r else v for (r, t), v in c.items()}
                  for c in accs.values()]
            for t in range(par, F // L, 2):
                hf[0, t], hf[1, t] = mix(*[gu[0][r, t] * gu[1][r, t] for r in range(2)])
        x = [jnp.concatenate([hf[r, t] for t in range(F // L)], axis=1) for r in range(2)]
        o, ready, stored = {}, set(), set()

        def done(k):
            ready.add(k)
            for r, c in sorted(ready):
                if (0, c) in ready and (k == (r, c) or k == (0, c)):
                    v = o[r, c] + 0.5 * o[0, c] if r else o[r, c]
                    rows, cols = slice(r0 + r * MH, r0 + (r + 1) * MH), slice(c * L, (c + 1) * L)
                    ob[i, rows, cols] = (x1b[rows, cols] + gb[:, cols] * v).astype(bf16)
                    stored.add((rows.start, c * L))
            for op in OP:
                need = {(s, c) for s in range(op[2], op[3], MH) for c in range(op[0], op[1], L)}
                if need <= stored:
                    stored.difference_update(need)
                    o_cp(i, *op).start()

        for si in range(2):
            fast_dot(fast_lhs(x, FT[si], si), "d", si, range(len(FT[si][0])), o,
                     lambda q: (q[0], DT[si][q[1]]), done)

    acc, hcache, parts = {}, {}, {}

    def grp_g(p, n, f, half=None):
        if (p, half) not in hcache:
            if len(n2) == 1 and half != 0:
                n2.append(prep_norm(qb0, x1b0, 0, H0, TM0 - H0))
            x = jnp.concatenate(n2, axis=0) if half is None else n2[half]
            hcache[p, half] = (x[:, p * L:(p + 1) * L] * (1.0 + mod[4 * NT + p])
                               + mod[3 * NT + p]).astype(bf16)
        rows = {None: slice(0, TM0), 0: slice(0, H0), 1: slice(H0, TM0)}[half]
        cols = slice(f * 4 * L, (f + 1) * 4 * L)
        d = jnp.dot(hcache[p, half], wts[n][p * L:(p + 1) * L, cols],
                    preferred_element_type=f32)
        ref = gub.at["gu".index(n), rows, cols]
        if p < NT - 1:
            ref[...] = d if p == 0 else ref[...] + d
        elif n == "g":
            acc[f] = ref[...] + d
        else:
            h = acc.pop(f) * (ref[...] + d)
            for t in range(4):
                x, y = h[:TM0 // 2, t * L:(t + 1) * L], h[TM0 // 2:, t * L:(t + 1) * L]
                hf0[0, 4 * f + t], hf0[1, 4 * f + t] = x, y - 0.5 * x
        return [d[s:s + 8, 0:L] for s in range(0, d.shape[0], 16)]

    left = {(q[0], DT[si][q[1]]): sum(q in t[2] for t in SCHEME[si])
            for si in range(2) for term in SCHEME[si] for q in term[2]}
    m0 = TM0 // 2

    def grp_f(si, i):
        term = SCHEME[si][i]
        k = sum(len(t[1]) > 1 for t in SCHEME[si][:i])
        ps = []
        for ts in (range(4), range(4, len(FT[si][0]))):
            if not len(ts):
                continue
            x = _lin(term[0], lambda q: jnp.concatenate(
                [hf0[q[0], FT[si][q[1]][t]] for t in ts], axis=1)).astype(bf16)
            if len(term[1]) > 1:
                w = wsb[2][si][k, ts[0] * L:(ts[-1] + 1) * L, :]
            else:
                w = jnp.concatenate([wtile("d", si, *term[1], t) for t in ts], axis=0)
            ps.append(jnp.dot(x, w, preferred_element_type=f32))
        p = ps[0] if len(ps) == 1 else ps[0] + ps[1]
        for q, v in term[2].items():
            key = (q[0], DT[si][q[1]])
            parts[key] = (p if v > 0 else -p) if key not in parts else (
                parts[key] + p if v > 0 else parts[key] - p)
            left[key] -= 1
        for c in DT[si]:
            if (0, c) in parts and not left[0, c] and not left[1, c]:
                top, bot = parts.pop((0, c)), parts.pop((1, c))
                o = jnp.concatenate([top, bot + 0.5 * top], axis=0)
                cols = slice(c * L, (c + 1) * L)
                ob0[:, cols] = (x1b0[:, cols] + mod[5 * NT + c] * o).astype(bf16)
        return ([ps[0][s:s + 8] for s in range(0, m0, 16)]
                + [x[s:s + 8] for x in ps[1:] for s in range(0, m0, 32)])

    grp_fn.update(g=grp_g, f=grp_f)
    region = lambda r, c: dpart.at[r * m0:(r + 1) * m0, c * L:(c + 1) * L]
    for waits, rows, groups, jobs in FIRST:
        wait(*waits)
        for n in parts:
            parts[n] = region(*n)[...]
        run(groups, jobs, lead=LEAD, floor=(0.0, 0.0))
        if rows:
            aff += [1.0 + modv(4), modv(3)]
            prep_chain(0, *rows, PR)
        for n in parts:
            region(*n)[...] = parts[n]
    for c0, c1 in zip(OC[:-1], OC[1:]):
        o_cp(None, c0, c1).start()
    gb = modv(5)
    wait("q1c", *[f"q{i + 1}" for i in range(1, NB)])

    def ffn(i, carry):
        prep_chain(i, HM, TM, PL)
        ffn_half(i, 0, gb)
        prep_chain(jnp.minimum(i + 1, NB - 1), 0, HM, PL)
        ffn_half(i, 1, gb)
        return carry

    lax.fori_loop(0, NB, ffn, 0)

    for c0, c1 in zip(OC[:-1], OC[1:]):
        o_cp(None, c0, c1).wait()
    for i in range(NB):
        for op in OP:
            o_cp(i, *op).wait()


@jax.jit
def pallas_adaLN_cond__ssm_conv_h3__glu_gated_bilinear__prompt_kernel(
    A_q: jax.Array,
    A_k: jax.Array,
    A_v: jax.Array,
    A_shift_k: jax.Array,
    A_ssm_k: jax.Array,
    A_ssm_D: jax.Array,
    B_x: jax.Array,
    B_w_gate: jax.Array,
    B_w_up: jax.Array,
    B_w_down: jax.Array,
    c: jax.Array,
    w_mod: jax.Array,
):
    del B_x
    tiles = lambda x: x.reshape(S // 8, 8, NT, L).transpose(0, 2, 1, 3).reshape(S * NT, L)
    any_spec = pl.BlockSpec(memory_space=pl.ANY)
    return pl.pallas_call(
        _kernel,
        in_specs=[any_spec] * 11,
        out_specs=any_spec,
        out_shape=jax.ShapeDtypeStruct((1, S, D), bf16),
        scratch_shapes=[
            pltpu.VMEM((TM0, D), bf16),
            pltpu.VMEM((NB, TM, D), bf16),
            [pltpu.VMEM((4 * PAD + C * NT, L), bf16)] * NC,
            [pltpu.VMEM((2 * PAD + C * NT, L), bf16)] * NC,
            pltpu.VMEM((NT, L, S), bf16),
            pltpu.VMEM((D, F), bf16),
            pltpu.VMEM((D, F), bf16),
            pltpu.VMEM((F, D), bf16),
            [[pltpu.VMEM((NSUM[si], len(FT[si][0]) * L, L), bf16) for si in range(2)]] * 3,
            pltpu.VMEM((D, 6 * D), bf16),
            pltpu.VMEM((NT, NC, R, L, L), bf16),
            pltpu.VMEM((NT, NC, R, 16, 16, L), f32),
            pltpu.VMEM((NT, NC, R, 16, 16, L), f32),
            pltpu.VMEM((NT, NC, R, 16, 16, L), f32),
            pltpu.VMEM((NT, NC, 2 * R, L, L), bf16),
            pltpu.VMEM((NT, S + 32, L), f32),
            pltpu.VMEM((TM0, D), f32),
            pltpu.VMEM((TM, D), f32),
            pltpu.VMEM((TM, D), f32),
            pltpu.VMEM((2, F // L, HM // 2, L), f32),
            pltpu.VMEM((2, TM0, F), f32),
            pltpu.VMEM((TM0, D), f32),
            pltpu.VMEM((2, F // L, TM0 // 2, L), f32),
            pltpu.VMEM((TM0, D), bf16),
            pltpu.VMEM((NB, TM, D), bf16),
            pltpu.VMEM((32, 8 * VM, L), f32),
            pltpu.VMEM((KS, D), bf16),
            pltpu.VMEM((D,), bf16),
            pltpu.VMEM((1, D), bf16),
            pltpu.SemaphoreType.DMA((len(DMA_ORDER),)),
            pltpu.SemaphoreType.DMA((NB + 1,)),
        ],
        compiler_params=pltpu.CompilerParams(
            vmem_limit_bytes=120 * 1024 * 1024,
            disable_bounds_checks=True, disable_semaphore_checks=True),
        name="adaln_h3_glu",
    )(A_q, tiles(A_k), tiles(A_v), A_shift_k.T, A_ssm_k, A_ssm_D,
      B_w_gate, B_w_up, B_w_down, c, w_mod)
```

```python
import jax
import jax.numpy as jnp
from jax import lax
import jax.experimental.pallas as pl
import jax.experimental.pallas.tpu as pltpu

S = 2048
D = 640
F = 1536
KS = 4
L = 128
NT = D // L
R = 4
C = R * L
NC = S // C
EPS = 1e-5
RSQ2 = 0.7071067811865476

WPT = 4 * NT
PAD = 32

TM0 = 512
H0 = 352
TM = 512
NB = (S - TM0) // TM
HM = 256
PL = 16
PR = 24
WM = {"mA": (0, 12), "c0": (20, 21), "mB": (12, 16), "s1": (16, 17), "c1": (21, 22),
      "s2": (17, 19), "c2": (22, 24), "s4": (19, 20), "c4": (24, 25), "mG": (25, 30)}
VM = 5
RATE = 1.05
LEAD = 24
FREE = {"i": 56, "z": 56, "k": 47, "u": 46}
FREE_FFN = {"i": 20, "u": 36, "f": 36, "g": 50}

f32 = jnp.float32
bf16 = jnp.bfloat16
u32 = jnp.uint32


def _cos_turns(t):
    x = jnp.abs(t - jnp.floor(t) - 0.5) - 0.25
    x2 = x * x
    return x * (6.283164024 + x2 * (-41.33713150 + x2 * (81.34038544 + x2 * -70.98993683)))


def _tables(inverse, rs, hold=None):
    shape = (L // 2, L) if inverse else (2 * L, L)
    rho = lax.broadcasted_iota(jnp.int32, shape, 1 if inverse else 0)
    j = lax.broadcasted_iota(jnp.int32, shape, 0 if inverse else 1)
    if inverse:
        g, rad = 8 * (rho >> 4) + (rho & 7), 2 * R
    else:
        g, rad, j = 8 * (rho >> 5) + (rho & 7) + 64 * ((rho >> 4) & 1), R, _perm(j)
    a = (4 * g + 1).astype(f32) * (1.0 / (4 * C))
    off = ((rho >> 3) & 1).astype(f32) * 0.25
    ns = [(rad * j + r).astype(f32) for r in rs]
    if hold is not None:
        ns = [hold(r, n) for r, n in enumerate(ns)]
    ts = [_cos_turns(a * n + off) for n in ns]
    return [t * (1.0 / C) if inverse else t for t in ts]


def _perm(c):
    return 16 * (c >> 4) + 2 * (c & 7) + ((c >> 3) & 1)


def _layernorm(x):
    m = jnp.mean(x, axis=-1, keepdims=True)
    xc = x - m
    v = jnp.mean(xc * xc, axis=-1, keepdims=True)
    return xc * lax.rsqrt(v + EPS)


def _split(t):
    t = t.reshape(16, 16, L)
    return t[:, :8, :], t[:, 8:, :]


def _radix4(x, sgn):
    (ar, ai), (br, bi), (cr, ci), (dr, di) = x
    s0r, s0i, d0r, d0i = ar + cr, ai + ci, ar - cr, ai - ci
    s1r, s1i, d1r, d1i = br + dr, bi + di, br - dr, bi - di
    o0 = (s0r + s1r, s0i + s1i)
    o2 = (s0r - s1r, s0i - s1i)
    pl_ = (d0r - d1i, d0i + d1r)
    mi_ = (d0r + d1i, d0i - d1r)
    return [o0, pl_, o2, mi_] if sgn > 0 else [o0, mi_, o2, pl_]


S222 = (
    ({(1, 1): 1, (0, 0): -1}, {(0, 0): 1, (1, 1): 1}, {(0, 0): -1, (1, 1): 1}),
    ({(0, 1): 1, (1, 1): 1}, {(1, 0): 1, (1, 1): 1}, {(0, 0): 1}),
    ({(0, 0): 1, (0, 1): 1}, {(1, 1): 1}, {(0, 0): -1, (0, 1): 1}),
    ({(1, 1): 1}, {(1, 0): 1, (0, 0): -1}, {(0, 0): -1, (1, 0): 1}),
    ({(1, 0): 1, (1, 1): 1}, {(0, 0): 1}, {(1, 0): 1, (1, 1): -1}),
    ({(0, 0): 1}, {(0, 1): 1, (1, 1): -1}, {(0, 1): 1, (1, 1): -1}),
    ({(0, 0): 1, (1, 0): 1}, {(0, 0): 1, (0, 1): 1}, {(1, 1): 1}),
)
S233 = (
    ({(0, 0): 1, (1, 0): 1, (1, 2): -1}, {(0, 0): 1, (2, 2): -1},
     {(0, 0): 1, (0, 2): -1, (1, 2): 1}),
    ({(1, 0): 1, (1, 2): -1}, {(0, 0): 1}, {(0, 0): -1, (0, 2): 1, (1, 0): 1, (1, 2): -1}),
    ({(0, 0): 1, (1, 0): 1, (1, 2): -1, (0, 2): -1}, {(2, 2): 1}, {(0, 0): 1, (0, 2): -1}),
    ({(0, 2): 1}, {(1, 0): 1, (2, 0): 1, (2, 2): 1}, {(0, 0): 1}),
    ({(0, 1): 1, (0, 2): -1, (1, 1): 1}, {(1, 0): 1, (2, 1): 1},
     {(0, 1): -1, (1, 0): 1, (1, 1): 1}),
    ({(0, 1): 1, (0, 2): -1}, {(1, 0): 1}, {(0, 0): 1, (0, 1): 1, (1, 0): -1, (1, 1): -1}),
    ({(0, 1): 1, (0, 2): -1, (1, 1): 1, (1, 2): -1}, {(2, 1): 1}, {(1, 0): -1, (1, 1): -1}),
    ({(1, 2): 1}, {(0, 0): 1, (2, 0): 1, (2, 1): -1}, {(1, 0): 1}),
    ({(0, 0): 1, (1, 1): 1}, {(0, 1): 1, (1, 2): -1}, {(0, 1): 1, (1, 2): -1}),
    ({(1, 0): 1, (1, 1): -1}, {(0, 1): 1}, {(1, 1): 1, (1, 2): -1}),
    ({(0, 0): 1, (0, 1): -1}, {(1, 2): 1}, {(0, 1): 1, (0, 2): -1}),
    ({(0, 0): 1}, {(0, 0): 1, (0, 2): 1, (1, 2): 1}, {(0, 2): 1, (1, 2): -1}),
    ({(0, 0): 1, (1, 0): 1}, {(0, 1): 1, (0, 2): 1, (2, 2): 1}, {(1, 2): 1}),
    ({(1, 1): 1}, {(0, 1): 1, (1, 1): 1, (1, 0): -1}, {(0, 1): -1, (1, 1): 1}),
    ({(0, 1): 1, (1, 1): 1}, {(1, 1): 1, (1, 2): 1, (2, 1): 1}, {(0, 1): 1}),
)
SCHEME = (S233, S222)
HIT = (((0, 0), (0, 1), (1, 0), (2, 1)), ((0, 0), (1, 1)))
NSUM = [sum(len(t[1]) > 1 for t in s) for s in SCHEME]
DT = ((0, 1, 2), (3, 4))
FT = ([range(0, 4), range(4, 8), range(8, 12)], [range(0, 6), range(6, 12)])


def _lin(coef, get):
    r = None
    for q, v in coef.items():
        x = get(q)
        r = (x if v > 0 else -x) if r is None else (r + x if v > 0 else r - x)
    return r


T = range(NT)
_z = lambda j: [("z", j, a) for a in range(NC)]
_k = lambda j, al: [("k", j, a) for a in al]
_u = lambda a: [("u", j, a) for j in T]
_iv = lambda jl, al: [("i", j, a) for j in jl for a in al]
_kv = lambda a: [("kv", j, a) for j in T]
_m = lambda jl, us, outs: [("mac", j, us, outs) for j in jl]

A3 = (0, 1, 2)
SCHEDULE = [
    (["ssm0"], _z(0) + _k(0, range(NC)), [("setup", None)]),
    (["ssm1"], _z(1) + _k(1, range(NC)), []),
    (["ssm2"], _z(2) + _k(2, [0, 1]), []),
    (["k0", "v0"], _k(2, [2, 3]) + _u(0), _kv(0) + _m([0], (0,), (0,))),
    (["ssm3"], _iv([0], [0]) + _z(3) + _k(3, [0, 1]), _m([1, 2], (0,), A3)),
    (["k1", "v1"], _k(3, [2, 3]) + _u(1), _kv(1) + _m([3], (0,), (0,))),
    (["ssm4"], _iv([1], [0]) + _z(4) + _k(4, range(NC)),
     _m([0], (0, 1), (1, 2)) + _m([1, 2], (1,), (1, 2))),
    (["k2", "v2"], _iv([2, 3], [0]) + _iv([0], [1]) + _u(2) + _iv([1, 2], [1]) + _iv([4], [0, 1])
     + _iv([0, 1, 2, 4], [2]),
     _kv(2) + _m([4], (0, 1), A3) + _m([0, 1, 2, 4], (2,), (2,)) + _m([3], A3, (1, 2))),
    (["q0", "mA", "c0"], [("mod", "mA", "c0")] + _iv([3], [1, 2]), []),
]
_g = lambda p: [("g", p, n, f) for f in range(3) for n in "gu"]
_v = lambda *names: [("vmod", n) for n in names]
_w = lambda names, si: [("wsum", n, si, t) for n in names for t in range(len(FT[si][0]))]
_f = lambda si, *ids: [("f", si, i) for i in ids]
FIRST = [
    (["wg0", "qh"], None, [("g", 0, "g", f, h) for h in (0, 1) for f in range(3)], []),
    (["wu0", "s1", "c1"], None, [("g", 0, "u", f) for f in range(3)],
     _v("s1", "c1") + _m([0], A3, (3,))),
    (["wg1", "wu1"], None, _g(1)[:-1], _m([1, 2, 3], A3, (3,))),
    (["wg2", "wu2", "s2", "c2"], None, _g(1)[-1:] + _g(2),
     _v("s2", "c2") + _m([4], A3, (3,)) + _w("gu", 0)),
    (["wg3", "wu3", "wg4", "wu4", "s4", "c4", "q1"], (0, HM), _g(3) + _g(4),
     _v("s4", "c4") + _w("gu", 1)),
    (["wd", "k3", "v3"], None, _f(0, 1, 2, 5, 6, 9, 10) + _f(1, 2, 4) + _u(3) + _f(0, 0, 4, 8),
     _w("d", 0) + _kv(3) + _w("d", 1) + _m([0], (3,), (3,))),
    (["mG"], None, _f(0, 3, 11, 13, 7, 12, 14) + _f(1, 0, 1, 3, 5, 6) + _iv(T, [3]),
     _v("mG") + _m([1, 2, 3, 4], (3,), (3,))),
]

DMA_ORDER = (["sk", "sd", "c", "ssm0", "ssm1", "ssm2", "k0", "v0", "ssm3", "k1", "v1", "ssm4",
              "k2", "v2", "q0", "c0", "mA", "mB", "wg0", "qh", "wu0", "s1", "c1", "wg1", "wu1",
              "s2", "c2", "wg2", "wu2", "s4", "c4", "wg3", "wu3", "wg4", "wu4", "q1", "wd", "k3",
              "v3", "mG", "q1c"] + [f"q{i + 1}" for i in range(1, NB)])


def _costs(job):
    if job[0] == "kv":
        return [48, 42] * (C // 64)
    if job[0] == "wsum":
        return [61] * 8 if job[2] == 0 else [50] * 4
    if job[0] == "setup":
        return [100] * (4 * R)
    if job[0] == "vmod":
        return [3 * D // VM // 8] * (VM * (WM[job[1]][1] - WM[job[1]][0]))
    us, outs = job[2], job[3]
    pairs = [(a, n) for a in outs for n in us if n <= a]
    mac = (2 * len({a - n for a, n in pairs if a > n}) + 8 * len(pairs)
           - (2 * len(outs) if us[0] == 0 else 0))
    fin = sum(a <= us[-1] for a in outs)
    if mac < 12 and outs[-1] <= us[-1] < NC - 1:
        return [1 + R * mac + 16 * fin, 1 + R * mac + 48 * fin] * 8
    return ([1 + mac] * 3 + [1 + mac + 16 * fin] + [1 + mac] * 3 + [1 + mac + 48 * fin]) * 8


def _plan(groups, jobs, lead=0, floor=(1.0, 0.8)):
    free = FREE_FFN if lead else FREE
    nstep = {"i": 8, "z": 8, "k": 16, "u": 16, "mod": 0, "g": TM0 // 16}
    steps = lambda g: (16, 24)[g[1]] if g[0] == "f" else nstep[g[0]]
    slots = [free[g[0]] for g in groups for _ in range(steps(g))]
    lo, hi = [], []
    for job in jobs:
        begin, limit, first = 0, len(slots), 0
        for g in groups:
            kind = (g[0], job[0])
            if (kind == ("u", "kv") and g[1:] == job[1:]
                    or kind == ("i", "mac") and g[1] == job[1] and g[2] in job[3]
                    and g[2] <= job[2][-1]):
                limit = min(limit, first - lead)
            if (kind == ("f", "wsum") and g[1] == job[2] and len(SCHEME[g[1]][g[2]][1]) > 1
                    or kind == ("f", "vmod") and g[1:] == (0, 7)):
                limit = min(limit, first - lead)
            if kind == ("g", "vmod") and job[1][1] == str(g[1]):
                limit = min(limit, first - 11)
            first += steps(g)
            if kind == ("u", "mac") and g[1] == job[1] and g[2] in job[2]:
                begin = first
        lo.append(begin)
        hi.append(limit)
    plan, credit, n = [], (slots or [0])[0], 0
    for k, job in enumerate(jobs):
        if n < lo[k]:
            n, credit = lo[k], min(credit, 0) + slots[lo[k]]
        work = [sum(_costs(j)) for j in jobs]
        if lead:
            rate = max(RATE * sum(work[k:m + 1]) / max(sum(slots[n:hi[m]]), 1)
                       for m in range(k, len(jobs)))
        else:
            rate = RATE * sum(work[k:]) / sum(slots[n:])
        rate = max(rate, floor[0] if job[0] == "kv" else floor[1])
        idx = []
        for c in _costs(job):
            while credit <= 0 and n + 1 < hi[k]:
                n += 1
                credit += slots[n] * rate
            credit -= c
            idx.append(n)
        assert n < hi[k]
        plan.append(idx)
    return plan


def _kernel(q_hbm, k_hbm, v_hbm, sk_hbm, ssm_hbm, sd_hbm, wg_hbm, wu_hbm, wd_hbm,
            c_hbm, wm_hbm, o_hbm,
            qb0, qb, kbs, vbs, ssmb, wgb, wub, wdb, wsb, wmb, uwb, ub, kpb, yp, pb, yb,
            x1b0, x1b, h2b, hf, gub, dpart, hf0, ob0, ob, mv, skb, sdb, cb_, sem, osem):
    cps = {"sk": (sk_hbm, skb), "sd": (sd_hbm, sdb), "c": (c_hbm, cb_), "wd": (wd_hbm, wdb)}
    for j in range(NT):
        cps[f"ssm{j}"] = (ssm_hbm.at[pl.ds(j * L, L), :], ssmb.at[j])
    for a in range(NC):
        n, h = C * NT, 2 * PAD
        if a == 0:
            cps["k0"] = (k_hbm.at[pl.ds(0, n), :], kbs[0].at[pl.ds(h, n), :])
        else:
            e = 48
            cps[f"k{a}"] = (k_hbm.at[pl.ds(a * n - e, n + e), :],
                            kbs[a].at[pl.ds(h - e, n + e), :])
        cps[f"v{a}"] = (v_hbm.at[pl.ds(a * n, n), :], vbs[a].at[pl.ds(0, n), :])
    for n, (c0, c1) in WM.items():
        cols = pl.ds(c0 * L, (c1 - c0) * L)
        cps[n] = (wm_hbm.at[:, cols], wmb.at[:, cols])
    cps["q0"] = (q_hbm.at[0, pl.ds(0, H0), :], qb0.at[pl.ds(0, H0), :])
    cps["qh"] = (q_hbm.at[0, pl.ds(H0, TM0 - H0), :], qb0.at[pl.ds(H0, TM0 - H0), :])
    cps["q1"] = (q_hbm.at[0, pl.ds(TM0, HM), :], qb.at[0, pl.ds(0, HM), :])
    cps["q1c"] = (q_hbm.at[0, pl.ds(TM0 + HM, TM - HM), :], qb.at[0, pl.ds(HM, TM - HM), :])
    for i in range(1, NB):
        cps[f"q{i + 1}"] = (q_hbm.at[0, pl.ds(TM0 + i * TM, TM), :], qb.at[i])
    for p in range(NT):
        rows = pl.ds(p * L, L)
        cps[f"wg{p}"] = (wg_hbm.at[rows, :], wgb.at[rows, :])
        cps[f"wu{p}"] = (wu_hbm.at[rows, :], wub.at[rows, :])
    assert sorted(cps) == sorted(DMA_ORDER)

    def cp(name):
        src, dst = cps[name]
        return pltpu.make_async_copy(src, dst, sem.at[DMA_ORDER.index(name)])

    def wait(*names):
        for n in names:
            cp(n).wait()

    kbs[0][0:2 * PAD, :] = jnp.zeros((2 * PAD, L), bf16)
    for n in DMA_ORDER:
        cp(n).start()

    for a in range(NC):
        for ref in (kbs[a], vbs[a]):
            n = ref.shape[0] - 2 * PAD
            ref[n:, :] = jnp.zeros((2 * PAD, L), ref.dtype)
        if a:
            kbs[a][0:16, :] = jnp.zeros((16, L), kbs[a].dtype)

    def table(r, carry):
        hf0[1, r] = _tables(False, [r])[0]
        return carry

    lax.fori_loop(0, R, table, 0)
    tabs, ginv, ccol = [hf0[1, r].astype(bf16) for r in range(R)], [], []
    for ref in (ub, kpb, yp):
        ref[0, 0, 0, 0, pl.ds(0, 8, stride=2), :] = jnp.zeros((8, L), f32)
    mv[0, pl.ds(0, 8, stride=2), :] = jnp.zeros((8, L), f32)
    for ref in (hf, hf0):
        ref[0, 0, pl.ds(0, 8, stride=2), :] = jnp.zeros((8, L), f32)
    ri = lax.broadcasted_iota(jnp.int32, (L, L), 0)
    ci = lax.broadcasted_iota(jnp.int32, (L, L), 1)
    sel = jnp.where(ci == R * _perm(ri & 31) + (ri >> 5), 1.0, 0.0).astype(bf16)

    wait("sk", "sd", "c")
    skt = skb[...].astype(f32)
    sdv = sdb[...].astype(f32).reshape(1, D)
    cv = cb_[...].astype(f32)
    sig = jax.nn.sigmoid(cv)
    cs = jnp.broadcast_to((cv * sig).astype(bf16), (16, D))
    one = sig[:, 0:L]

    def gate(x, deps):
        dep = jnp.concatenate(deps, axis=0).reshape(x.shape)
        return jnp.where(jnp.broadcast_to(one, x.shape) > 2.0, dep, x)

    def put(dst, j, a, xs):
        for qi in range(R):
            dst[j, a, qi] = jnp.concatenate(xs[qi], axis=1)

    zs = {}
    mod = {}

    def grp_z(j, a):
        z = [lax.dot_general(sel, ssmb[j, :, t * L:(t + 1) * L], (((1,), (1,)), ((), ())),
                             preferred_element_type=f32) for t in range(R * a, R * a + R)]
        zs[j, a] = [jnp.concatenate([z[p][32 * r:32 * (r + 1)] for p in range(R)],
                                    axis=0).astype(bf16) for r in range(R)]
        return [z[0][16 * t:16 * t + 8] for t in range(8)]

    def grp_fwd(ws, dst, j, a, dvec=None):
        t = [jnp.dot(tabs[r], ws[r], preferred_element_type=f32) for r in range(R)]
        x = [_split(v) for v in t]
        if dvec is not None:
            x[0] = (x[0][0] + dvec[None], x[0][1])
        put(dst, j, a, _radix4(x, -1))
        return [t[0][16 * s:16 * s + 8] for s in range(16)]

    def grp_k(j, a):
        return grp_fwd(zs.pop((j, a)), kpb, j, a,
                       sdv[:, j * L:(j + 1) * L] if a == 0 else None)

    def grp_u(j, a):
        uw = [uwb[j, a, r] for r in range(R)]
        return grp_fwd(uw, ub, j, a)

    def grp_i(j, a):
        ys = []
        for r in range(2 * R):
            y = jnp.dot(ginv[r], pb[j, a, r], preferred_element_type=f32)
            yb[j, pl.ds(a * C + r, L // 2, stride=2 * R), :] = y
            ys.append(y)
        return [ys[r][16 * s:16 * s + 8] for r in (0, R) for s in range(4)]

    def grp_mod(*names):
        for name in names:
            c0, c1 = WM[name]
            m = jnp.dot(cs, wmb[:, c0 * L:c1 * L], preferred_element_type=f32)
            for c in range(c0, c1):
                mod[c] = m[0:1, (c - c0) * L:(c - c0 + 1) * L]
        return []

    def modv(i):
        return jnp.concatenate([mod[i * NT + n] for n in range(NT)], axis=1)

    def job_kv(j, a, deps):
        lo = lambda x: lax.bitcast_convert_type(x << 16, f32)
        hi = lambda x: lax.bitcast_convert_type(x & jnp.uint32(0xFFFF0000), f32)
        n = C // 8
        kw, vw = kbs[a].bitcast(u32), vbs[a].bitcast(u32)
        ld = lambda ref, o: ref[pl.ds(4 * j + o, n, stride=WPT), :]
        k = {}
        for m in range(4):
            x = ld(kw, PAD + m)
            k[2 * m], k[2 * m + 1] = lo(x), hi(x)
        k[-3] = hi(ld(kw, PAD - WPT + 2))
        x = ld(kw, PAD - WPT + 3)
        k[-2], k[-1] = lo(x), hi(x)
        w = [skt[t:t + 1, j * L:(j + 1) * L] for t in range(KS)]
        w0 = [gate(jnp.broadcast_to(w[0], (n, L)), deps[e::2]) for e in (0, 1)]
        kv = {}
        for m in range(4):
            x = ld(vw, m)
            for ph, v in ((2 * m, lo(x)), (2 * m + 1, hi(x))):
                ks = k[ph] * w0[m % 2]
                for t in range(1, KS):
                    ks = ks + k[ph - t] * w[t]
                kv[ph] = (ks * v).reshape(n // 8, 8, L)
        for r in range(R):
            uwb[j, a, r] = jnp.concatenate([kv[r], kv[r + R]], axis=1).reshape(L, L).astype(bf16)

    def job_mac(j, us, outs, deps):
        ld = lambda ref, a: (ref[j, a, :, :, 0:8, :], ref[j, a, :, :, 8:16, :])
        lo, hi = us[0], us[-1]
        u = {a: ld(ub, a) for a in us}
        if len(deps) == 16:
            ur = jnp.concatenate([gate(u[lo][0][0:1], deps), u[lo][0][1:]], axis=0)
        else:
            ur = gate(u[lo][0], [deps[R * i + qi] for qi in range(R) for i in range(16)])
        u[lo] = (ur, u[lo][1])
        ms = sorted({a - n for a in outs for n in us if n <= a})
        k = {m: ld(kpb, m) for m in sorted(set(ms) | {m - 1 for m in ms if m > 0})}
        kp = {m: k[m] if m == 0 else (k[m][0] - k[m - 1][1], k[m][1] + k[m - 1][0]) for m in ms}
        for a in outs:
            yr, yi = ld(yp, a) if lo > 0 else (None, None)
            for n in us:
                if n > a:
                    continue
                (kr, ki), (ur, ui) = kp[a - n], u[n]
                tr = kr * ur - ki * ui
                ti = kr * ui + ki * ur
                yr = tr if yr is None else yr + tr
                yi = ti if yi is None else yi + ti
            if a > hi:
                yp[j, a] = jnp.concatenate([yr, yi], axis=2)
                continue
            ps = _radix4([(yr[qi], yi[qi]) for qi in range(R)], +1)
            for r in range(R):
                pr, pi = [p.reshape(8, 2, 8, L) for p in ps[r]]
                lr, li, hr, hi_ = pr[:, 0], pi[:, 0], pr[:, 1], pi[:, 1]
                if r % 2:
                    hr, hi_ = (hr - hi_) * RSQ2, (hr + hi_) * RSQ2
                if r < 2:
                    outs2 = (lr + hr, li + hi_), (lr - hr, li - hi_)
                else:
                    outs2 = (lr - hi_, li + hr), (lr + hi_, li - hr)
                for e in range(2):
                    pb[j, a, r + R * e] = jnp.concatenate(
                        outs2[e], axis=1).reshape(L, L).astype(bf16)

    def job_setup(_, deps):
        def hold(r, n):
            return gate(n, [deps[2 * r + s // 4] for s in range(8)])

        ginv.extend(t.astype(bf16) for t in _tables(True, range(2 * R), hold))
        csf = cs[0:1].astype(f32)
        ccol.append(jnp.concatenate([jnp.broadcast_to(csf[:, t * L:(t + 1) * L], (L, L)).T
                                     for t in range(NT)], axis=0))

    def job_vmod(name, deps):
        c0, c1 = WM[name]
        n = D // VM
        for c in range(c0, c1):
            for i in range(VM):
                cc = ccol[0][i * n:(i + 1) * n]
                cc = jnp.concatenate([gate(cc[0:8], [deps[(c - c0) * VM + i]]), cc[8:]], axis=0)
                p = wmb[i * n:(i + 1) * n, c * L:(c + 1) * L].astype(f32) * cc
                mv[c, 8 * i:8 * i + 8, :] = jnp.sum(p.reshape(n // 8, 8, L), axis=0)
            mod[c] = jnp.sum(mv[c], axis=0, keepdims=True)

    wts = {"g": wgb, "u": wub, "d": wdb}

    def wtile(n, si, q, t):
        r, c = (FT[si][q[0]][t], DT[si][q[1]]) if n == "d" else (DT[si][q[0]], FT[si][q[1]][t])
        return wts[n][r * L:(r + 1) * L, c * L:(c + 1) * L]

    def job_wsum(n, si, t, deps):
        blk = {}
        for q in sorted({q for term in SCHEME[si] for q in term[1]}):
            x = wtile(n, si, q, t).astype(f32)
            if q in HIT[si]:
                x = x.reshape(8, 16, L)
                held = gate(x[:, 0:8], [deps[g * len(deps) // 8] for g in range(8)])
                x = jnp.concatenate([held, x[:, 8:]], axis=1).reshape(L, L)
            blk[q] = x
        sums = [term[1] for term in SCHEME[si] if len(term[1]) > 1]
        for i, coef in enumerate(sums):
            wsb["gud".index(n)][si][i, t * L:(t + 1) * L, :] = _lin(coef, blk.get).astype(bf16)

    def fast_lhs(x, tiles, si):
        get = lambda q: x[q[0]][:, tiles[q[1]][0] * L:(tiles[q[1]][-1] + 1) * L]
        return [_lin(term[0], get).astype(bf16) for term in SCHEME[si]]

    def fast_dot(a, n, si, ts, out, key, done=None):
        left = {q: sum(q in term[2] for term in SCHEME[si]) for term in SCHEME[si] for q in term[2]}
        i = 0
        for x, term in zip(a, SCHEME[si]):
            if len(term[1]) > 1:
                w = wsb["gud".index(n)][si][i, ts[0] * L:(ts[-1] + 1) * L, :]
                i += 1
            else:
                w = jnp.concatenate([wtile(n, si, *term[1], t) for t in ts], axis=0)
            p = jnp.dot(x, w, preferred_element_type=f32)
            for q, v in term[2].items():
                k = key(q)
                out[k] = (p if v > 0 else -p) if k not in out else (
                    out[k] + p if v > 0 else out[k] - p)
                left[q] -= 1
                if done is not None and not left[q]:
                    done(k)

    grp_fn = {"z": grp_z, "k": grp_k, "u": grp_u, "i": grp_i, "mod": grp_mod}
    job_fn = {"kv": job_kv, "mac": job_mac, "vmod": job_vmod, "setup": job_setup,
              "wsum": job_wsum}

    def run(groups, jobs, **kw):
        plan = _plan(groups, jobs, **kw)
        anchors, done = [], 0
        for g in groups + [None]:
            while done < len(jobs) and max(plan[done]) < len(anchors):
                job_fn[jobs[done][0]](*jobs[done][1:], [anchors[n] for n in plan[done]])
                done += 1
            if g is not None:
                anchors += grp_fn[g[0]](*g[1:])
        assert done == len(jobs)

    for waits, groups, jobs in SCHEDULE:
        wait(*waits)
        run(groups, jobs)

    n1, dep = [], None
    for r in range(0, H0, H0 // 2):
        x = qb0[r:r + H0 // 2, :].astype(f32)
        if dep is not None:
            x = jnp.concatenate([gate(x[:, 0:L], [dep]), x[:, L:]], axis=1)
        n1.append(_layernorm(x))
        dep = n1[-1][:, 0:L]
    n1 = jnp.concatenate(n1, axis=0)
    wait("mB")
    grp_mod("mB")
    sa, ca, ga = [modv(i) for i in range(3)]
    a1 = ga * (1.0 + ca)
    b1 = ga * sa

    def o_cp(i, c0, c1, r0=0, r1=TM):
        cols = pl.ds(c0, c1 - c0)
        if i is None:
            return pltpu.make_async_copy(ob0.at[:, cols], o_hbm.at[0, pl.ds(0, TM0), cols],
                                         osem.at[NB])
        base = TM0 + i * TM + r0
        if not isinstance(i, int):
            base = pl.multiple_of(base, 16)
        return pltpu.make_async_copy(ob.at[i, pl.ds(r0, r1 - r0), cols],
                                     o_hbm.at[0, pl.ds(base, r1 - r0), cols], osem.at[i])

    def prep_norm(q_ref, x1_ref, y0, r0, n, dep=None, n1=None, skew=False):
        x = q_ref[r0:r0 + n, :].astype(f32)
        if dep is not None:
            x = jnp.concatenate([gate(x[:, 0:L], [dep]), x[:, L:]], axis=1)
        if skew:
            gs = [x[0:8]]
            for s in range(8, n, 8):
                lag = jnp.broadcast_to(jnp.mean(gs[-1], axis=-1, keepdims=True), (8, L))
                g = x[s:s + 8]
                gs.append(jnp.concatenate([g[:, :L], gate(g[:, L:2 * L], [lag]), g[:, 2 * L:]],
                                          axis=1))
            x = jnp.concatenate(gs, axis=0)
        y = jnp.concatenate([yb[j, pl.ds(y0 + r0, n), :] for j in range(NT)], axis=1)
        x1 = x + ((_layernorm(x) if n1 is None else n1) * a1 + b1) * y
        x1_ref[r0:r0 + n, :] = x1
        return _layernorm(x1)

    n2 = [prep_norm(qb0, x1b0, 0, 0, H0, None, n1)]
    aff = []

    def prep_chain(i, r0, r1, pr):
        y0 = TM0 + i * TM
        if not isinstance(i, int):
            y0 = pl.multiple_of(y0, L)
        dep = None
        while r0 < r1:
            n = pr if (r1 - r0) % pr == 0 else pr + 8
            h2 = prep_norm(qb.at[i], x1b, y0, r0, n, dep if dep is None else dep[:n], None, True)
            h2 = h2 * aff[0] + aff[1]
            h2b[r0:r0 + n, :] = h2
            dep = h2[:, 0:L]
            r0 += n

    OC = (0, D)
    MH = HM // 2
    OP = [(0, D, 0, HM), (0, 3 * L, HM, TM), (3 * L, 4 * L, HM, TM),
          (4 * L, D, HM, HM + MH), (4 * L, D, HM + MH, TM)]

    def ffn_half(i, half, gb):
        r0 = half * HM
        mix = lambda x, y: (x, y - 0.5 * x)
        x = mix(h2b[r0:r0 + MH, :], h2b[r0 + MH:r0 + HM, :])
        a = [fast_lhs(x, [[t] for t in DT[si]], si) for si in range(2)]
        for par in range(2):
            accs = {"g": {}, "u": {}}
            for si in range(2):
                for t in range(par, len(FT[si][0]), 2):
                    for n in "gu":
                        fast_dot(a[si], n, si, [t], accs[n], lambda q: (q[0], FT[si][q[1]][t]))
            gu = [{(r, t): v + 0.5 * c[0, t] if r else v for (r, t), v in c.items()}
                  for c in accs.values()]
            for t in range(par, F // L, 2):
                hf[0, t], hf[1, t] = mix(*[gu[0][r, t] * gu[1][r, t] for r in range(2)])
        x = [jnp.concatenate([hf[r, t] for t in range(F // L)], axis=1) for r in range(2)]
        o, ready, stored = {}, set(), set()

        def done(k):
            ready.add(k)
            for r, c in sorted(ready):
                if (0, c) in ready and (k == (r, c) or k == (0, c)):
                    v = o[r, c] + 0.5 * o[0, c] if r else o[r, c]
                    rows, cols = slice(r0 + r * MH, r0 + (r + 1) * MH), slice(c * L, (c + 1) * L)
                    ob[i, rows, cols] = (x1b[rows, cols] + gb[:, cols] * v).astype(bf16)
                    stored.add((rows.start, c * L))
            for op in OP:
                need = {(s, c) for s in range(op[2], op[3], MH) for c in range(op[0], op[1], L)}
                if need <= stored:
                    stored.difference_update(need)
                    o_cp(i, *op).start()

        for si in range(2):
            fast_dot(fast_lhs(x, FT[si], si), "d", si, range(len(FT[si][0])), o,
                     lambda q: (q[0], DT[si][q[1]]), done)

    acc, hcache, parts = {}, {}, {}

    def grp_g(p, n, f, half=None):
        if (p, half) not in hcache:
            if len(n2) == 1 and half != 0:
                n2.append(prep_norm(qb0, x1b0, 0, H0, TM0 - H0))
            x = jnp.concatenate(n2, axis=0) if half is None else n2[half]
            hcache[p, half] = (x[:, p * L:(p + 1) * L] * (1.0 + mod[4 * NT + p])
                               + mod[3 * NT + p]).astype(bf16)
        rows = {None: slice(0, TM0), 0: slice(0, H0), 1: slice(H0, TM0)}[half]
        cols = slice(f * 4 * L, (f + 1) * 4 * L)
        d = jnp.dot(hcache[p, half], wts[n][p * L:(p + 1) * L, cols],
                    preferred_element_type=f32)
        ref = gub.at["gu".index(n), rows, cols]
        if p < NT - 1:
            ref[...] = d if p == 0 else ref[...] + d
        elif n == "g":
            acc[f] = ref[...] + d
        else:
            h = acc.pop(f) * (ref[...] + d)
            for t in range(4):
                x, y = h[:TM0 // 2, t * L:(t + 1) * L], h[TM0 // 2:, t * L:(t + 1) * L]
                hf0[0, 4 * f + t], hf0[1, 4 * f + t] = x, y - 0.5 * x
        return [d[s:s + 8, 0:L] for s in range(0, d.shape[0], 16)]

    left = {(q[0], DT[si][q[1]]): sum(q in t[2] for t in SCHEME[si])
            for si in range(2) for term in SCHEME[si] for q in term[2]}
    m0 = TM0 // 2

    def grp_f(si, i):
        term = SCHEME[si][i]
        k = sum(len(t[1]) > 1 for t in SCHEME[si][:i])
        ps = []
        for ts in (range(4), range(4, len(FT[si][0]))):
            if not len(ts):
                continue
            x = _lin(term[0], lambda q: jnp.concatenate(
                [hf0[q[0], FT[si][q[1]][t]] for t in ts], axis=1)).astype(bf16)
            if len(term[1]) > 1:
                w = wsb[2][si][k, ts[0] * L:(ts[-1] + 1) * L, :]
            else:
                w = jnp.concatenate([wtile("d", si, *term[1], t) for t in ts], axis=0)
            ps.append(jnp.dot(x, w, preferred_element_type=f32))
        p = ps[0] if len(ps) == 1 else ps[0] + ps[1]
        for q, v in term[2].items():
            key = (q[0], DT[si][q[1]])
            parts[key] = (p if v > 0 else -p) if key not in parts else (
                parts[key] + p if v > 0 else parts[key] - p)
            left[key] -= 1
        for c in DT[si]:
            if (0, c) in parts and not left[0, c] and not left[1, c]:
                top, bot = parts.pop((0, c)), parts.pop((1, c))
                o = jnp.concatenate([top, bot + 0.5 * top], axis=0)
                cols = slice(c * L, (c + 1) * L)
                ob0[:, cols] = (x1b0[:, cols] + mod[5 * NT + c] * o).astype(bf16)
        return ([ps[0][s:s + 8] for s in range(0, m0, 16)]
                + [x[s:s + 8] for x in ps[1:] for s in range(0, m0, 32)])

    grp_fn.update(g=grp_g, f=grp_f)
    region = lambda r, c: dpart.at[r * m0:(r + 1) * m0, c * L:(c + 1) * L]
    for waits, rows, groups, jobs in FIRST:
        wait(*waits)
        for n in parts:
            parts[n] = region(*n)[...]
        run(groups, jobs, lead=LEAD, floor=(0.0, 0.0))
        if rows:
            aff += [1.0 + modv(4), modv(3)]
            prep_chain(0, *rows, PR)
        for n in parts:
            region(*n)[...] = parts[n]
    for c0, c1 in zip(OC[:-1], OC[1:]):
        o_cp(None, c0, c1).start()
    gb = modv(5)
    wait("q1c", *[f"q{i + 1}" for i in range(1, NB)])

    def ffn(i, carry):
        prep_chain(i, HM, TM, PL)
        ffn_half(i, 0, gb)
        prep_chain(jnp.minimum(i + 1, NB - 1), 0, HM, PL)
        ffn_half(i, 1, gb)
        return carry

    lax.fori_loop(0, NB, ffn, 0)

    for c0, c1 in zip(OC[:-1], OC[1:]):
        o_cp(None, c0, c1).wait()
    for i in range(NB):
        for op in OP:
            o_cp(i, *op).wait()


@jax.jit
def pallas_adaLN_cond__ssm_conv_h3__glu_gated_bilinear__prompt_kernel(
    A_q: jax.Array,
    A_k: jax.Array,
    A_v: jax.Array,
    A_shift_k: jax.Array,
    A_ssm_k: jax.Array,
    A_ssm_D: jax.Array,
    B_x: jax.Array,
    B_w_gate: jax.Array,
    B_w_up: jax.Array,
    B_w_down: jax.Array,
    c: jax.Array,
    w_mod: jax.Array,
):
    del B_x
    tiles = lambda x: x.reshape(S // 8, 8, NT, L).transpose(0, 2, 1, 3).reshape(S * NT, L)
    any_spec = pl.BlockSpec(memory_space=pl.ANY)
    return pl.pallas_call(
        _kernel,
        in_specs=[any_spec] * 11,
        out_specs=any_spec,
        out_shape=jax.ShapeDtypeStruct((1, S, D), bf16),
        scratch_shapes=[
            pltpu.VMEM((TM0, D), bf16),
            pltpu.VMEM((NB, TM, D), bf16),
            [pltpu.VMEM((4 * PAD + C * NT, L), bf16)] * NC,
            [pltpu.VMEM((2 * PAD + C * NT, L), bf16)] * NC,
            pltpu.VMEM((NT, L, S), bf16),
            pltpu.VMEM((D, F), bf16),
            pltpu.VMEM((D, F), bf16),
            pltpu.VMEM((F, D), bf16),
            [[pltpu.VMEM((NSUM[si], len(FT[si][0]) * L, L), bf16) for si in range(2)]] * 3,
            pltpu.VMEM((D, 6 * D), bf16),
            pltpu.VMEM((NT, NC, R, L, L), bf16),
            pltpu.VMEM((NT, NC, R, 16, 16, L), f32),
            pltpu.VMEM((NT, NC, R, 16, 16, L), f32),
            pltpu.VMEM((NT, NC, R, 16, 16, L), f32),
            pltpu.VMEM((NT, NC, 2 * R, L, L), bf16),
            pltpu.VMEM((NT, S + 32, L), f32),
            pltpu.VMEM((TM0, D), f32),
            pltpu.VMEM((TM, D), f32),
            pltpu.VMEM((TM, D), f32),
            pltpu.VMEM((2, F // L, HM // 2, L), f32),
            pltpu.VMEM((2, TM0, F), f32),
            pltpu.VMEM((TM0, D), f32),
            pltpu.VMEM((2, F // L, TM0 // 2, L), f32),
            pltpu.VMEM((TM0, D), bf16),
            pltpu.VMEM((NB, TM, D), bf16),
            pltpu.VMEM((32, 8 * VM, L), f32),
            pltpu.VMEM((KS, D), bf16),
            pltpu.VMEM((D,), bf16),
            pltpu.VMEM((1, D), bf16),
            pltpu.SemaphoreType.DMA((len(DMA_ORDER),)),
            pltpu.SemaphoreType.DMA((NB + 1,)),
        ],
        compiler_params=pltpu.CompilerParams(
            vmem_limit_bytes=120 * 1024 * 1024,
            disable_bounds_checks=True, disable_semaphore_checks=True),
        name="adaln_h3_glu",
    )(A_q, tiles(A_k), tiles(A_v), A_shift_k.T, A_ssm_k, A_ssm_D,
      B_w_gate, B_w_up, B_w_down, c, w_mod)
```

```python
import jax
import jax.numpy as jnp
from jax import lax
import jax.experimental.pallas as pl
import jax.experimental.pallas.tpu as pltpu

S = 2048
D = 640
F = 1536
KS = 4
L = 128
NT = D // L
R = 4
C = R * L
NC = S // C
EPS = 1e-5
RSQ2 = 0.7071067811865476

PAD = 64

TM0 = 512
H0 = 352
TM = 512
NB = (S - TM0) // TM
HM = 256
PL = 16
PR = 24
WM = {"mA": (0, 12), "c0": (20, 21), "mB": (12, 16), "s1": (16, 17), "c1": (21, 22),
      "s2": (17, 19), "c2": (22, 24), "s4": (19, 20), "c4": (24, 25), "mG": (25, 30)}
VM = 5
RATE = 1.05
LEAD = 24
FREE = {"i": 56, "z": 56, "k": 47, "u": 46}
FREE_FFN = {"i": 20, "u": 44, "f": 36, "g": 50}

f32 = jnp.float32
bf16 = jnp.bfloat16


def _cos_turns(t):
    x = jnp.abs(t - jnp.floor(t) - 0.5) - 0.25
    x2 = x * x
    return x * (6.283164024 + x2 * (-41.33713150 + x2 * (81.34038544 + x2 * -70.98993683)))


def _tables(inverse, rs, hold=None):
    shape = (L // 2, L) if inverse else (2 * L, L)
    rho = lax.broadcasted_iota(jnp.int32, shape, 1 if inverse else 0)
    j = lax.broadcasted_iota(jnp.int32, shape, 0 if inverse else 1)
    if inverse:
        g, rad = 8 * (rho >> 4) + (rho & 7), 2 * R
    else:
        g, rad = 8 * (rho >> 5) + (rho & 7) + 64 * ((rho >> 4) & 1), R
    a = (4 * g + 1).astype(f32) * (1.0 / (4 * C))
    off = ((rho >> 3) & 1).astype(f32) * 0.25
    ns = [(rad * j + r).astype(f32) for r in rs]
    if hold is not None:
        ns = [hold(r, n) for r, n in enumerate(ns)]
    ts = [_cos_turns(a * n + off) for n in ns]
    return [t * (1.0 / C) if inverse else t for t in ts]


def _layernorm(x):
    m = jnp.mean(x, axis=-1, keepdims=True)
    xc = x - m
    v = jnp.mean(xc * xc, axis=-1, keepdims=True)
    return xc * lax.rsqrt(v + EPS)


def _split(t):
    t = t.reshape(16, 16, L)
    return t[:, :8, :], t[:, 8:, :]


def _radix4(x, sgn):
    (ar, ai), (br, bi), (cr, ci), (dr, di) = x
    s0r, s0i, d0r, d0i = ar + cr, ai + ci, ar - cr, ai - ci
    s1r, s1i, d1r, d1i = br + dr, bi + di, br - dr, bi - di
    o0 = (s0r + s1r, s0i + s1i)
    o2 = (s0r - s1r, s0i - s1i)
    pl_ = (d0r - d1i, d0i + d1r)
    mi_ = (d0r + d1i, d0i - d1r)
    return [o0, pl_, o2, mi_] if sgn > 0 else [o0, mi_, o2, pl_]


S222 = (
    ({(1, 1): 1, (0, 0): -1}, {(0, 0): 1, (1, 1): 1}, {(0, 0): -1, (1, 1): 1}),
    ({(0, 1): 1, (1, 1): 1}, {(1, 0): 1, (1, 1): 1}, {(0, 0): 1}),
    ({(0, 0): 1, (0, 1): 1}, {(1, 1): 1}, {(0, 0): -1, (0, 1): 1}),
    ({(1, 1): 1}, {(1, 0): 1, (0, 0): -1}, {(0, 0): -1, (1, 0): 1}),
    ({(1, 0): 1, (1, 1): 1}, {(0, 0): 1}, {(1, 0): 1, (1, 1): -1}),
    ({(0, 0): 1}, {(0, 1): 1, (1, 1): -1}, {(0, 1): 1, (1, 1): -1}),
    ({(0, 0): 1, (1, 0): 1}, {(0, 0): 1, (0, 1): 1}, {(1, 1): 1}),
)
S233 = (
    ({(0, 0): 1, (1, 0): 1, (1, 2): -1}, {(0, 0): 1, (2, 2): -1},
     {(0, 0): 1, (0, 2): -1, (1, 2): 1}),
    ({(1, 0): 1, (1, 2): -1}, {(0, 0): 1}, {(0, 0): -1, (0, 2): 1, (1, 0): 1, (1, 2): -1}),
    ({(0, 0): 1, (1, 0): 1, (1, 2): -1, (0, 2): -1}, {(2, 2): 1}, {(0, 0): 1, (0, 2): -1}),
    ({(0, 2): 1}, {(1, 0): 1, (2, 0): 1, (2, 2): 1}, {(0, 0): 1}),
    ({(0, 1): 1, (0, 2): -1, (1, 1): 1}, {(1, 0): 1, (2, 1): 1},
     {(0, 1): -1, (1, 0): 1, (1, 1): 1}),
    ({(0, 1): 1, (0, 2): -1}, {(1, 0): 1}, {(0, 0): 1, (0, 1): 1, (1, 0): -1, (1, 1): -1}),
    ({(0, 1): 1, (0, 2): -1, (1, 1): 1, (1, 2): -1}, {(2, 1): 1}, {(1, 0): -1, (1, 1): -1}),
    ({(1, 2): 1}, {(0, 0): 1, (2, 0): 1, (2, 1): -1}, {(1, 0): 1}),
    ({(0, 0): 1, (1, 1): 1}, {(0, 1): 1, (1, 2): -1}, {(0, 1): 1, (1, 2): -1}),
    ({(1, 0): 1, (1, 1): -1}, {(0, 1): 1}, {(1, 1): 1, (1, 2): -1}),
    ({(0, 0): 1, (0, 1): -1}, {(1, 2): 1}, {(0, 1): 1, (0, 2): -1}),
    ({(0, 0): 1}, {(0, 0): 1, (0, 2): 1, (1, 2): 1}, {(0, 2): 1, (1, 2): -1}),
    ({(0, 0): 1, (1, 0): 1}, {(0, 1): 1, (0, 2): 1, (2, 2): 1}, {(1, 2): 1}),
    ({(1, 1): 1}, {(0, 1): 1, (1, 1): 1, (1, 0): -1}, {(0, 1): -1, (1, 1): 1}),
    ({(0, 1): 1, (1, 1): 1}, {(1, 1): 1, (1, 2): 1, (2, 1): 1}, {(0, 1): 1}),
)
SCHEME = (S233, S222)
HIT = (((0, 0), (0, 1), (1, 0), (2, 1)), ((0, 0), (1, 1)))
NSUM = [sum(len(t[1]) > 1 for t in s) for s in SCHEME]
DT = ((0, 1, 2), (3, 4))
FT = ([range(0, 4), range(4, 8), range(8, 12)], [range(0, 6), range(6, 12)])


def _lin(coef, get):
    r = None
    for q, v in coef.items():
        x = get(q)
        r = (x if v > 0 else -x) if r is None else (r + x if v > 0 else r - x)
    return r


T = range(NT)
_z = lambda j: [("z", j, a) for a in range(NC)]
_k = lambda j, al: [("k", j, a) for a in al]
_u = lambda a: [("u", j, a) for j in T]
_iv = lambda jl, al: [("i", j, a) for j in jl for a in al]
_kv = lambda a: [("kv", j, a) for j in T]
_m = lambda jl, us, outs: [("mac", j, us, outs) for j in jl]

A3 = (0, 1, 2)
SCHEDULE = [
    (["ssm0"], _z(0) + _k(0, range(NC)), [("setup", None)]),
    (["ssm1"], _z(1) + _k(1, range(NC)), []),
    (["ssm2"], _z(2) + _k(2, [0, 1]), []),
    (["k0", "v0"], _k(2, [2, 3]) + _u(0), _kv(0)),
    (["ssm3"], _z(3) + _k(3, [0, 1]), _m([0, 1], (0,), (0,)) + _m([2], (0,), A3)),
    (["k1", "v1"], _k(3, [2, 3]) + _u(1), _kv(1) + _m([3], (0,), (0,))),
    (["ssm4"], _iv([0, 1], [0]) + _z(4) + _k(4, range(NC)),
     _m([0, 1], (0, 1), (1, 2)) + _m([2], (1,), (1, 2))),
    (["k2", "v2"], _iv([2, 3], [0]) + _iv([0], [1]) + _u(2) + _iv([1, 2], [1]) + _iv([4], [0, 1])
     + _iv([0, 1, 2, 4], [2]),
     _kv(2) + _m([4], (0, 1), A3) + _m([0, 1, 2, 4], (2,), (2,)) + _m([3], (0, 1), (1,))),
    (["q0", "mA", "c0"], [("mod", "mA", "c0")] + _iv([3], [1]), []),
]
_g = lambda p: [("g", p, n, f) for f in range(3) for n in "gu"]
_v = lambda *names: [("vmod", n) for n in names]
_w = lambda names, si: [("wsum", n, si, t) for n in names for t in range(len(FT[si][0]))]
_f = lambda si, *ids: [("f", si, i) for i in ids]
FIRST = [
    (["wg0", "qh"], None, [("g", 0, "g", f, h) for h in (0, 1) for f in range(3)], []),
    (["wu0", "s1", "c1"], None, [("g", 0, "u", f) for f in range(3)],
     _v("s1", "c1") + _m([3], A3, (2,))),
    (["wg1", "wu1"], None, _g(1)[:-1] + _iv([3], [2]), _m([0, 1, 2], A3, (3,))),
    (["wg2", "wu2", "s2", "c2"], None, _g(1)[-1:] + _g(2),
     _v("s2", "c2") + _m([3, 4], A3, (3,)) + _w("gu", 0)),
    (["wg3", "wu3", "wg4", "wu4", "s4", "c4", "q1"], (0, HM), _g(3) + _g(4),
     _v("s4", "c4") + _w("gu", 1)),
    (["wd", "k3", "v3"], None, _f(0, 1, 2, 5, 6, 9, 10) + _f(1, 2, 4) + _u(3) + _f(0, 0, 4, 8),
     _w("d", 0) + _kv(3) + _w("d", 1) + _m([0], (3,), (3,))),
    (["mG"], None, _f(0, 3, 11, 13, 7, 12, 14) + _f(1, 0, 1, 3, 5, 6) + _iv(T, [3]),
     _v("mG") + _m([1, 2, 3, 4], (3,), (3,))),
]

DMA_ORDER = (["sk", "sd", "c", "ssm0", "ssm1", "ssm2", "k0", "v0", "ssm3", "k1", "v1", "ssm4",
              "k2", "v2", "q0", "c0", "mA", "mB", "wg0", "qh", "wu0", "s1", "c1", "wg1", "wu1",
              "s2", "c2", "wg2", "wu2", "s4", "c4", "wg3", "wu3", "wg4", "wu4", "q1", "wd", "k3",
              "v3", "mG", "q1c"] + [f"q{i + 1}" for i in range(1, NB)])


def _costs(job):
    if job[0] == "kv":
        return [57] * (C // 32)
    if job[0] == "wsum":
        return [61] * 8 if job[2] == 0 else [50] * 4
    if job[0] == "setup":
        return [100] * (4 * R)
    if job[0] == "vmod":
        return [3 * D // VM // 8] * (VM * (WM[job[1]][1] - WM[job[1]][0]))
    us, outs = job[2], job[3]
    pairs = [(a, n) for a in outs for n in us if n <= a]
    mac = (2 * len({a - n for a, n in pairs if a > n}) + 8 * len(pairs)
           - (2 * len(outs) if us[0] == 0 else 0))
    fin = sum(a <= us[-1] for a in outs)
    if mac < 12 and outs[-1] <= us[-1] < NC - 1:
        return [1 + R * mac + 16 * fin, 1 + R * mac + 48 * fin] * 8
    return ([1 + mac] * 3 + [1 + mac + 16 * fin] + [1 + mac] * 3 + [1 + mac + 48 * fin]) * 8


def _plan(groups, jobs, lead=0, floor=(1.15, 0.8)):
    free = FREE_FFN if lead else FREE
    nstep = {"i": 8, "z": 8, "k": 16, "u": 16, "mod": 0, "g": TM0 // 16}
    steps = lambda g: (16, 24)[g[1]] if g[0] == "f" else nstep[g[0]]
    slots = [free[g[0]] for g in groups for _ in range(steps(g))]
    lo, hi = [], []
    for job in jobs:
        begin, limit, first = 0, len(slots), 0
        for g in groups:
            kind = (g[0], job[0])
            if (kind == ("u", "kv") and g[1:] == job[1:]
                    or kind == ("i", "mac") and g[1] == job[1] and g[2] in job[3]
                    and g[2] <= job[2][-1]):
                limit = min(limit, first - lead)
            if (kind == ("f", "wsum") and g[1] == job[2] and len(SCHEME[g[1]][g[2]][1]) > 1
                    or kind == ("f", "vmod") and g[1:] == (0, 7)):
                limit = min(limit, first - lead)
            if kind == ("g", "vmod") and job[1][1] == str(g[1]):
                limit = min(limit, first - 11)
            first += steps(g)
            if kind == ("u", "mac") and g[1] == job[1] and g[2] in job[2]:
                begin = first
        lo.append(begin)
        hi.append(limit)
    plan, credit, n = [], (slots or [0])[0], 0
    for k, job in enumerate(jobs):
        if n < lo[k]:
            n, credit = lo[k], min(credit, 0) + slots[lo[k]]
        work = [sum(_costs(j)) for j in jobs]
        if lead:
            rate = max(RATE * sum(work[k:m + 1]) / max(sum(slots[n:hi[m]]), 1)
                       for m in range(k, len(jobs)))
        else:
            rate = RATE * sum(work[k:]) / sum(slots[n:])
        rate = max(rate, floor[0] if job[0] == "kv" else floor[1])
        idx = []
        for c in _costs(job):
            while credit <= 0 and n + 1 < hi[k]:
                n += 1
                credit += slots[n] * rate
            credit -= c
            idx.append(n)
        assert n < hi[k]
        plan.append(idx)
    return plan


def _kernel(q_hbm, k_hbm, v_hbm, sk_hbm, ssm_hbm, sd_hbm, wg_hbm, wu_hbm, wd_hbm,
            c_hbm, wm_hbm, o_hbm,
            qb0, qb, kb, vb, ssmb, wgb, wub, wdb, wsb, wmb, kvf, ub, kpb, yp, pb, yb,
            x1b0, x1b, h2b, hf, gub, dpart, hf0, ob0, ob, mv, skb, sdb, cb_, sem, osem):
    cps = {"sk": (sk_hbm, skb), "sd": (sd_hbm, sdb), "c": (c_hbm, cb_), "wd": (wd_hbm, wdb)}
    for j in range(NT):
        cps[f"ssm{j}"] = (ssm_hbm.at[pl.ds(j * L, L), :], ssmb.at[j])
    for a in range(NC):
        cps[f"k{a}"] = (k_hbm.at[0, pl.ds(a * C, C), :], kb.at[pl.ds(PAD + a * C, C), :])
        cps[f"v{a}"] = (v_hbm.at[0, pl.ds(a * C, C), :], vb.at[pl.ds(a * C, C), :])
    for n, (c0, c1) in WM.items():
        cols = pl.ds(c0 * L, (c1 - c0) * L)
        cps[n] = (wm_hbm.at[:, cols], wmb.at[:, cols])
    cps["q0"] = (q_hbm.at[0, pl.ds(0, H0), :], qb0.at[pl.ds(0, H0), :])
    cps["qh"] = (q_hbm.at[0, pl.ds(H0, TM0 - H0), :], qb0.at[pl.ds(H0, TM0 - H0), :])
    cps["q1"] = (q_hbm.at[0, pl.ds(TM0, HM), :], qb.at[0, pl.ds(0, HM), :])
    cps["q1c"] = (q_hbm.at[0, pl.ds(TM0 + HM, TM - HM), :], qb.at[0, pl.ds(HM, TM - HM), :])
    for i in range(1, NB):
        cps[f"q{i + 1}"] = (q_hbm.at[0, pl.ds(TM0 + i * TM, TM), :], qb.at[i])
    for p in range(NT):
        rows = pl.ds(p * L, L)
        cps[f"wg{p}"] = (wg_hbm.at[rows, :], wgb.at[rows, :])
        cps[f"wu{p}"] = (wu_hbm.at[rows, :], wub.at[rows, :])
    assert sorted(cps) == sorted(DMA_ORDER)

    def cp(name):
        src, dst = cps[name]
        return pltpu.make_async_copy(src, dst, sem.at[DMA_ORDER.index(name)])

    def wait(*names):
        for n in names:
            cp(n).wait()

    kb[0:PAD, :] = jnp.zeros((PAD, D), bf16)
    for n in DMA_ORDER:
        cp(n).start()

    def table(r, carry):
        hf0[1, r] = _tables(False, [r])[0]
        return carry

    lax.fori_loop(0, R, table, 0)
    tabs, ginv, ccol = [hf0[1, r].astype(bf16) for r in range(R)], [], []
    for ref in (ub, kpb, yp):
        ref[0, 0, 0, 0, pl.ds(0, 8, stride=2), :] = jnp.zeros((8, L), f32)
    mv[0, pl.ds(0, 8, stride=2), :] = jnp.zeros((8, L), f32)
    for ref in (hf, hf0):
        ref[0, 0, pl.ds(0, 8, stride=2), :] = jnp.zeros((8, L), f32)
    ri = lax.broadcasted_iota(jnp.int32, (L, L), 0)
    ci = lax.broadcasted_iota(jnp.int32, (L, L), 1)
    sel = jnp.where(ci == R * (ri & 31) + (ri >> 5), 1.0, 0.0).astype(bf16)

    wait("sk", "sd", "c")
    skt = skb[...].astype(f32)
    sdv = sdb[...].astype(f32).reshape(1, D)
    cv = cb_[...].astype(f32)
    sig = jax.nn.sigmoid(cv)
    cs = jnp.broadcast_to((cv * sig).astype(bf16), (16, D))
    one = sig[:, 0:L]

    def gate(x, deps):
        dep = jnp.concatenate(deps, axis=0).reshape(x.shape)
        return jnp.where(jnp.broadcast_to(one, x.shape) > 2.0, dep, x)

    def put(dst, j, a, xs):
        for qi in range(R):
            dst[j, a, qi] = jnp.concatenate(xs[qi], axis=1)

    zs = {}
    mod = {}

    def grp_z(j, a):
        z = [lax.dot_general(sel, ssmb[j, :, t * L:(t + 1) * L], (((1,), (1,)), ((), ())),
                             preferred_element_type=f32) for t in range(R * a, R * a + R)]
        zs[j, a] = [jnp.concatenate([z[p][32 * r:32 * (r + 1)] for p in range(R)],
                                    axis=0).astype(bf16) for r in range(R)]
        return [z[0][16 * t:16 * t + 8] for t in range(8)]

    def grp_fwd(ws, dst, j, a, dvec=None):
        t = [jnp.dot(tabs[r], ws[r], preferred_element_type=f32) for r in range(R)]
        x = [_split(v) for v in t]
        if dvec is not None:
            x[0] = (x[0][0] + dvec[None], x[0][1])
        put(dst, j, a, _radix4(x, -1))
        return [t[0][16 * s:16 * s + 8] for s in range(16)]

    def grp_k(j, a):
        return grp_fwd(zs.pop((j, a)), kpb, j, a,
                       sdv[:, j * L:(j + 1) * L] if a == 0 else None)

    def grp_u(j, a):
        uw = [kvf[j, pl.ds(a * C + r, L, stride=R), :].astype(bf16) for r in range(R)]
        return grp_fwd(uw, ub, j, a)

    def grp_i(j, a):
        ys = []
        for r in range(2 * R):
            y = jnp.dot(ginv[r], pb[j, a, r], preferred_element_type=f32)
            yb[j, pl.ds(a * C + r, L // 2, stride=2 * R), :] = y
            ys.append(y)
        return [ys[r][16 * s:16 * s + 8] for r in (0, R) for s in range(4)]

    def grp_mod(*names):
        for name in names:
            c0, c1 = WM[name]
            m = jnp.dot(cs, wmb[:, c0 * L:c1 * L], preferred_element_type=f32)
            for c in range(c0, c1):
                mod[c] = m[0:1, (c - c0) * L:(c - c0 + 1) * L]
        return []

    def modv(i):
        return jnp.concatenate([mod[i * NT + n] for n in range(NT)], axis=1)

    def job_kv(j, a, deps):
        cols = slice(j * L, (j + 1) * L)
        w = [skt[t:t + 1, cols] for t in range(KS)]
        k = kb[PAD + a * C - 16:PAD + (a + 1) * C, cols].astype(f32)
        k0, k1 = k[8:], jnp.concatenate([k[7:8], k[8:C + 15]], axis=0)
        late = k0 * w[2] + k1 * w[3]
        rep = C // 8 // len(deps)
        w0 = gate(jnp.broadcast_to(w[0], (8 * len(deps), L)), deps).reshape(len(deps), 1, 8, L)
        w0 = jnp.broadcast_to(w0, (len(deps), rep, 8, L)).reshape(C, L)
        ks = k0[8:] * w0 + k1[8:] * w[1] + late[6:C + 6]
        kvf[j, a * C:(a + 1) * C, :] = ks * vb[a * C:(a + 1) * C, cols].astype(f32)

    def job_mac(j, us, outs, deps):
        ld = lambda ref, a: (ref[j, a, :, :, 0:8, :], ref[j, a, :, :, 8:16, :])
        lo, hi = us[0], us[-1]
        u = {a: ld(ub, a) for a in us}
        if len(deps) == 16:
            ur = jnp.concatenate([gate(u[lo][0][0:1], deps), u[lo][0][1:]], axis=0)
        else:
            ur = gate(u[lo][0], [deps[R * i + qi] for qi in range(R) for i in range(16)])
        u[lo] = (ur, u[lo][1])
        ms = sorted({a - n for a in outs for n in us if n <= a})
        k = {m: ld(kpb, m) for m in sorted(set(ms) | {m - 1 for m in ms if m > 0})}
        kp = {m: k[m] if m == 0 else (k[m][0] - k[m - 1][1], k[m][1] + k[m - 1][0]) for m in ms}
        for a in outs:
            yr, yi = ld(yp, a) if lo > 0 else (None, None)
            for n in us:
                if n > a:
                    continue
                (kr, ki), (ur, ui) = kp[a - n], u[n]
                tr = kr * ur - ki * ui
                ti = kr * ui + ki * ur
                yr = tr if yr is None else yr + tr
                yi = ti if yi is None else yi + ti
            if a > hi:
                yp[j, a] = jnp.concatenate([yr, yi], axis=2)
                continue
            ps = _radix4([(yr[qi], yi[qi]) for qi in range(R)], +1)
            for r in range(R):
                pr, pi = [p.reshape(8, 2, 8, L) for p in ps[r]]
                lr, li, hr, hi_ = pr[:, 0], pi[:, 0], pr[:, 1], pi[:, 1]
                if r % 2:
                    hr, hi_ = (hr - hi_) * RSQ2, (hr + hi_) * RSQ2
                if r < 2:
                    outs2 = (lr + hr, li + hi_), (lr - hr, li - hi_)
                else:
                    outs2 = (lr - hi_, li + hr), (lr + hi_, li - hr)
                for e in range(2):
                    pb[j, a, r + R * e] = jnp.concatenate(
                        outs2[e], axis=1).reshape(L, L).astype(bf16)

    def job_setup(_, deps):
        def hold(r, n):
            return gate(n, [deps[2 * r + s // 4] for s in range(8)])

        ginv.extend(t.astype(bf16) for t in _tables(True, range(2 * R), hold))
        csf = cs[0:1].astype(f32)
        ccol.append(jnp.concatenate([jnp.broadcast_to(csf[:, t * L:(t + 1) * L], (L, L)).T
                                     for t in range(NT)], axis=0))

    def job_vmod(name, deps):
        c0, c1 = WM[name]
        n = D // VM
        for c in range(c0, c1):
            for i in range(VM):
                cc = ccol[0][i * n:(i + 1) * n]
                cc = jnp.concatenate([gate(cc[0:8], [deps[(c - c0) * VM + i]]), cc[8:]], axis=0)
                p = wmb[i * n:(i + 1) * n, c * L:(c + 1) * L].astype(f32) * cc
                mv[c, 8 * i:8 * i + 8, :] = jnp.sum(p.reshape(n // 8, 8, L), axis=0)
            mod[c] = jnp.sum(mv[c], axis=0, keepdims=True)

    wts = {"g": wgb, "u": wub, "d": wdb}

    def wtile(n, si, q, t):
        r, c = (FT[si][q[0]][t], DT[si][q[1]]) if n == "d" else (DT[si][q[0]], FT[si][q[1]][t])
        return wts[n][r * L:(r + 1) * L, c * L:(c + 1) * L]

    def job_wsum(n, si, t, deps):
        blk = {}
        for q in sorted({q for term in SCHEME[si] for q in term[1]}):
            x = wtile(n, si, q, t).astype(f32)
            if q in HIT[si]:
                x = x.reshape(8, 16, L)
                held = gate(x[:, 0:8], [deps[g * len(deps) // 8] for g in range(8)])
                x = jnp.concatenate([held, x[:, 8:]], axis=1).reshape(L, L)
            blk[q] = x
        sums = [term[1] for term in SCHEME[si] if len(term[1]) > 1]
        for i, coef in enumerate(sums):
            wsb["gud".index(n)][si][i, t * L:(t + 1) * L, :] = _lin(coef, blk.get).astype(bf16)

    def fast_lhs(x, tiles, si):
        get = lambda q: x[q[0]][:, tiles[q[1]][0] * L:(tiles[q[1]][-1] + 1) * L]
        return [_lin(term[0], get).astype(bf16) for term in SCHEME[si]]

    def fast_dot(a, n, si, ts, out, key, done=None):
        left = {q: sum(q in term[2] for term in SCHEME[si]) for term in SCHEME[si] for q in term[2]}
        i = 0
        for x, term in zip(a, SCHEME[si]):
            if len(term[1]) > 1:
                w = wsb["gud".index(n)][si][i, ts[0] * L:(ts[-1] + 1) * L, :]
                i += 1
            else:
                w = jnp.concatenate([wtile(n, si, *term[1], t) for t in ts], axis=0)
            p = jnp.dot(x, w, preferred_element_type=f32)
            for q, v in term[2].items():
                k = key(q)
                out[k] = (p if v > 0 else -p) if k not in out else (
                    out[k] + p if v > 0 else out[k] - p)
                left[q] -= 1
                if done is not None and not left[q]:
                    done(k)

    grp_fn = {"z": grp_z, "k": grp_k, "u": grp_u, "i": grp_i, "mod": grp_mod}
    job_fn = {"kv": job_kv, "mac": job_mac, "vmod": job_vmod, "setup": job_setup,
              "wsum": job_wsum}

    def run(groups, jobs, **kw):
        plan = _plan(groups, jobs, **kw)
        anchors, done = [], 0
        for g in groups + [None]:
            while done < len(jobs) and max(plan[done]) < len(anchors):
                job_fn[jobs[done][0]](*jobs[done][1:], [anchors[n] for n in plan[done]])
                done += 1
            if g is not None:
                anchors += grp_fn[g[0]](*g[1:])
        assert done == len(jobs)

    for waits, groups, jobs in SCHEDULE:
        wait(*waits)
        run(groups, jobs)

    n1, dep = [], None
    for r in range(0, H0, H0 // 2):
        x = qb0[r:r + H0 // 2, :].astype(f32)
        if dep is not None:
            x = jnp.concatenate([gate(x[:, 0:L], [dep]), x[:, L:]], axis=1)
        n1.append(_layernorm(x))
        dep = n1[-1][:, 0:L]
    n1 = jnp.concatenate(n1, axis=0)
    wait("mB")
    grp_mod("mB")
    sa, ca, ga = [modv(i) for i in range(3)]
    a1 = ga * (1.0 + ca)
    b1 = ga * sa

    def o_cp(i, c0, c1, r0=0, r1=TM):
        cols = pl.ds(c0, c1 - c0)
        if i is None:
            return pltpu.make_async_copy(ob0.at[:, cols], o_hbm.at[0, pl.ds(0, TM0), cols],
                                         osem.at[NB])
        base = TM0 + i * TM + r0
        if not isinstance(i, int):
            base = pl.multiple_of(base, 16)
        return pltpu.make_async_copy(ob.at[i, pl.ds(r0, r1 - r0), cols],
                                     o_hbm.at[0, pl.ds(base, r1 - r0), cols], osem.at[i])

    def prep_norm(q_ref, x1_ref, y0, r0, n, dep=None, n1=None, skew=False):
        x = q_ref[r0:r0 + n, :].astype(f32)
        if dep is not None:
            x = jnp.concatenate([gate(x[:, 0:L], [dep]), x[:, L:]], axis=1)
        if skew:
            gs = [x[0:8]]
            for s in range(8, n, 8):
                lag = jnp.broadcast_to(jnp.mean(gs[-1], axis=-1, keepdims=True), (8, L))
                g = x[s:s + 8]
                gs.append(jnp.concatenate([g[:, :L], gate(g[:, L:2 * L], [lag]), g[:, 2 * L:]],
                                          axis=1))
            x = jnp.concatenate(gs, axis=0)
        y = jnp.concatenate([yb[j, pl.ds(y0 + r0, n), :] for j in range(NT)], axis=1)
        x1 = x + ((_layernorm(x) if n1 is None else n1) * a1 + b1) * y
        x1_ref[r0:r0 + n, :] = x1
        return _layernorm(x1)

    n2 = [prep_norm(qb0, x1b0, 0, 0, H0, None, n1)]
    aff = []

    def prep_chain(i, r0, r1, pr):
        y0 = TM0 + i * TM
        if not isinstance(i, int):
            y0 = pl.multiple_of(y0, L)
        dep = None
        while r0 < r1:
            n = pr if (r1 - r0) % pr == 0 else pr + 8
            h2 = prep_norm(qb.at[i], x1b, y0, r0, n, dep if dep is None else dep[:n], None, True)
            h2 = h2 * aff[0] + aff[1]
            h2b[r0:r0 + n, :] = h2
            dep = h2[:, 0:L]
            r0 += n

    OC = (0, D)
    MH = HM // 2
    OP = [(0, D, 0, HM), (0, 3 * L, HM, TM), (3 * L, 4 * L, HM, TM),
          (4 * L, D, HM, HM + MH), (4 * L, D, HM + MH, TM)]

    def ffn_half(i, half, gb):
        r0 = half * HM
        mix = lambda x, y: (x, y - 0.5 * x)
        x = mix(h2b[r0:r0 + MH, :], h2b[r0 + MH:r0 + HM, :])
        a = [fast_lhs(x, [[t] for t in DT[si]], si) for si in range(2)]
        for par in range(2):
            accs = {"g": {}, "u": {}}
            for si in range(2):
                for t in range(par, len(FT[si][0]), 2):
                    for n in "gu":
                        fast_dot(a[si], n, si, [t], accs[n], lambda q: (q[0], FT[si][q[1]][t]))
            gu = [{(r, t): v + 0.5 * c[0, t] if r else v for (r, t), v in c.items()}
                  for c in accs.values()]
            for t in range(par, F // L, 2):
                hf[0, t], hf[1, t] = mix(*[gu[0][r, t] * gu[1][r, t] for r in range(2)])
        x = [jnp.concatenate([hf[r, t] for t in range(F // L)], axis=1) for r in range(2)]
        o, ready, stored = {}, set(), set()

        def done(k):
            ready.add(k)
            for r, c in sorted(ready):
                if (0, c) in ready and (k == (r, c) or k == (0, c)):
                    v = o[r, c] + 0.5 * o[0, c] if r else o[r, c]
                    rows, cols = slice(r0 + r * MH, r0 + (r + 1) * MH), slice(c * L, (c + 1) * L)
                    ob[i, rows, cols] = (x1b[rows, cols] + gb[:, cols] * v).astype(bf16)
                    stored.add((rows.start, c * L))
            for op in OP:
                need = {(s, c) for s in range(op[2], op[3], MH) for c in range(op[0], op[1], L)}
                if need <= stored:
                    stored.difference_update(need)
                    o_cp(i, *op).start()

        for si in range(2):
            fast_dot(fast_lhs(x, FT[si], si), "d", si, range(len(FT[si][0])), o,
                     lambda q: (q[0], DT[si][q[1]]), done)

    acc, hcache, parts = {}, {}, {}

    def grp_g(p, n, f, half=None):
        if (p, half) not in hcache:
            if len(n2) == 1 and half != 0:
                n2.append(prep_norm(qb0, x1b0, 0, H0, TM0 - H0))
            x = jnp.concatenate(n2, axis=0) if half is None else n2[half]
            hcache[p, half] = (x[:, p * L:(p + 1) * L] * (1.0 + mod[4 * NT + p])
                               + mod[3 * NT + p]).astype(bf16)
        rows = {None: slice(0, TM0), 0: slice(0, H0), 1: slice(H0, TM0)}[half]
        cols = slice(f * 4 * L, (f + 1) * 4 * L)
        d = jnp.dot(hcache[p, half], wts[n][p * L:(p + 1) * L, cols],
                    preferred_element_type=f32)
        ref = gub.at["gu".index(n), rows, cols]
        if p < NT - 1:
            ref[...] = d if p == 0 else ref[...] + d
        elif n == "g":
            acc[f] = ref[...] + d
        else:
            h = acc.pop(f) * (ref[...] + d)
            for t in range(4):
                x, y = h[:TM0 // 2, t * L:(t + 1) * L], h[TM0 // 2:, t * L:(t + 1) * L]
                hf0[0, 4 * f + t], hf0[1, 4 * f + t] = x, y - 0.5 * x
        return [d[s:s + 8, 0:L] for s in range(0, d.shape[0], 16)]

    left = {(q[0], DT[si][q[1]]): sum(q in t[2] for t in SCHEME[si])
            for si in range(2) for term in SCHEME[si] for q in term[2]}
    m0 = TM0 // 2

    def grp_f(si, i):
        term = SCHEME[si][i]
        k = sum(len(t[1]) > 1 for t in SCHEME[si][:i])
        ps = []
        for ts in (range(4), range(4, len(FT[si][0]))):
            if not len(ts):
                continue
            x = _lin(term[0], lambda q: jnp.concatenate(
                [hf0[q[0], FT[si][q[1]][t]] for t in ts], axis=1)).astype(bf16)
            if len(term[1]) > 1:
                w = wsb[2][si][k, ts[0] * L:(ts[-1] + 1) * L, :]
            else:
                w = jnp.concatenate([wtile("d", si, *term[1], t) for t in ts], axis=0)
            ps.append(jnp.dot(x, w, preferred_element_type=f32))
        p = ps[0] if len(ps) == 1 else ps[0] + ps[1]
        for q, v in term[2].items():
            key = (q[0], DT[si][q[1]])
            parts[key] = (p if v > 0 else -p) if key not in parts else (
                parts[key] + p if v > 0 else parts[key] - p)
            left[key] -= 1
        for c in DT[si]:
            if (0, c) in parts and not left[0, c] and not left[1, c]:
                top, bot = parts.pop((0, c)), parts.pop((1, c))
                o = jnp.concatenate([top, bot + 0.5 * top], axis=0)
                cols = slice(c * L, (c + 1) * L)
                ob0[:, cols] = (x1b0[:, cols] + mod[5 * NT + c] * o).astype(bf16)
        return ([ps[0][s:s + 8] for s in range(0, m0, 16)]
                + [x[s:s + 8] for x in ps[1:] for s in range(0, m0, 32)])

    grp_fn.update(g=grp_g, f=grp_f)
    region = lambda r, c: dpart.at[r * m0:(r + 1) * m0, c * L:(c + 1) * L]
    for waits, rows, groups, jobs in FIRST:
        wait(*waits)
        for n in parts:
            parts[n] = region(*n)[...]
        run(groups, jobs, lead=LEAD, floor=(0.0, 0.0))
        if rows:
            aff += [1.0 + modv(4), modv(3)]
            prep_chain(0, *rows, PR)
        for n in parts:
            region(*n)[...] = parts[n]
    for c0, c1 in zip(OC[:-1], OC[1:]):
        o_cp(None, c0, c1).start()
    gb = modv(5)
    wait("q1c", *[f"q{i + 1}" for i in range(1, NB)])

    def ffn(i, carry):
        prep_chain(i, HM, TM, PL)
        ffn_half(i, 0, gb)
        prep_chain(jnp.minimum(i + 1, NB - 1), 0, HM, PL)
        ffn_half(i, 1, gb)
        return carry

    lax.fori_loop(0, NB, ffn, 0)

    for c0, c1 in zip(OC[:-1], OC[1:]):
        o_cp(None, c0, c1).wait()
    for i in range(NB):
        for op in OP:
            o_cp(i, *op).wait()


@jax.jit
def pallas_adaLN_cond__ssm_conv_h3__glu_gated_bilinear__prompt_kernel(
    A_q: jax.Array,
    A_k: jax.Array,
    A_v: jax.Array,
    A_shift_k: jax.Array,
    A_ssm_k: jax.Array,
    A_ssm_D: jax.Array,
    B_x: jax.Array,
    B_w_gate: jax.Array,
    B_w_up: jax.Array,
    B_w_down: jax.Array,
    c: jax.Array,
    w_mod: jax.Array,
):
    del B_x
    any_spec = pl.BlockSpec(memory_space=pl.ANY)
    return pl.pallas_call(
        _kernel,
        in_specs=[any_spec] * 11,
        out_specs=any_spec,
        out_shape=jax.ShapeDtypeStruct((1, S, D), bf16),
        scratch_shapes=[
            pltpu.VMEM((TM0, D), bf16),
            pltpu.VMEM((NB, TM, D), bf16),
            pltpu.VMEM((PAD + S, D), bf16),
            pltpu.VMEM((S, D), bf16),
            pltpu.VMEM((NT, L, S), bf16),
            pltpu.VMEM((D, F), bf16),
            pltpu.VMEM((D, F), bf16),
            pltpu.VMEM((F, D), bf16),
            [[pltpu.VMEM((NSUM[si], len(FT[si][0]) * L, L), bf16) for si in range(2)]] * 3,
            pltpu.VMEM((D, 6 * D), bf16),
            pltpu.VMEM((NT, S + 32, L), f32),
            pltpu.VMEM((NT, NC, R, 16, 16, L), f32),
            pltpu.VMEM((NT, NC, R, 16, 16, L), f32),
            pltpu.VMEM((NT, NC, R, 16, 16, L), f32),
            pltpu.VMEM((NT, NC, 2 * R, L, L), bf16),
            pltpu.VMEM((NT, S + 32, L), f32),
            pltpu.VMEM((TM0, D), f32),
            pltpu.VMEM((TM, D), f32),
            pltpu.VMEM((TM, D), f32),
            pltpu.VMEM((2, F // L, HM // 2, L), f32),
            pltpu.VMEM((2, TM0, F), f32),
            pltpu.VMEM((TM0, D), f32),
            pltpu.VMEM((2, F // L, TM0 // 2, L), f32),
            pltpu.VMEM((TM0, D), bf16),
            pltpu.VMEM((NB, TM, D), bf16),
            pltpu.VMEM((32, 8 * VM, L), f32),
            pltpu.VMEM((KS, D), bf16),
            pltpu.VMEM((D,), bf16),
            pltpu.VMEM((1, D), bf16),
            pltpu.SemaphoreType.DMA((len(DMA_ORDER),)),
            pltpu.SemaphoreType.DMA((NB + 1,)),
        ],
        compiler_params=pltpu.CompilerParams(
            vmem_limit_bytes=120 * 1024 * 1024,
            disable_bounds_checks=True, disable_semaphore_checks=True),
        name="adaln_h3_glu",
    )(A_q, A_k, A_v, A_shift_k.T, A_ssm_k, A_ssm_D,
      B_w_gate, B_w_up, B_w_down, c, w_mod)
```
